```python
import jax
import jax.numpy as jnp

def _softmax(x, axis=-1):
    return jax.nn.softmax(x, axis=axis)

def _gelu(x):
    return jax.nn.gelu(x, approximate=True)

def _silu(x):
    return jax.nn.silu(x)

def _sigmoid(x):
    return jax.nn.sigmoid(x)

def _layernorm(x, axis=-1, eps=1e-05):
    m = jnp.mean(x, axis=axis, keepdims=True)
    v = jnp.var(x, axis=axis, keepdims=True)
    return (x - m) / jnp.sqrt(v + eps)

def _scatter_add(tgt, idx, src, axis=0):
    return tgt.at[idx].add(src)

def _segment_sum(src, seg, n):
    return jax.ops.segment_sum(src, seg, n)

class _Rng:

    def __init__(self, key):
        self._k = key

    def _next(self):
        self._k, sub = jax.random.split(self._k)
        return sub

    def normal(self, shape):
        return jax.random.normal(self._next(), shape, dtype=jnp.bfloat16)

    def randint(self, lo, hi, shape):
        return jax.random.randint(self._next(), shape, lo, hi, dtype=jnp.int32)

    def uniform(self, shape, lo=0.0, hi=1.0):
        return jax.random.uniform(self._next(), shape, jnp.bfloat16, lo, hi)

    def permutation(self, n):
        return jax.random.permutation(self._next(), n)
kernel_name = 'interleave_layers__memory_aug_recurrent_mem_tr__moe_arch_mod__prompt'

def setup_inputs():
    _rng = _Rng(jax.random.key(int.from_bytes(__import__("os").urandom(4), "little")))
    _w = lambda a: (lambda t: t.astype(jnp.bfloat16) if jnp.issubdtype(t.dtype, jnp.floating) else t)(jnp.asarray(a))

    def _A_setup():
        B, S, Dm = (1, 2048, 512)
        H, Dh = (32, 128)
        M, seg = (8, 32)
        seg = min(seg, S)
        S = S // seg * seg
        return {'x': _w((lambda *s: _rng.normal(s) * 0.05)(B, S, Dm)), 'mem0': _w((lambda *s: _rng.normal(s) * 0.05)(B, M, Dm)), 'Wq': _w((lambda *s: _rng.normal(s) * 0.05)(Dm, H, Dh) * Dm ** (-0.5)), 'Wk': _w((lambda *s: _rng.normal(s) * 0.05)(Dm, H, Dh) * Dm ** (-0.5)), 'Wv': _w((lambda *s: _rng.normal(s) * 0.05)(Dm, H, Dh) * Dm ** (-0.5)), 'Wo': _w((lambda *s: _rng.normal(s) * 0.05)(H, Dh, Dm) * (H * Dh) ** (-0.5)), 'seg_len': seg}
    _A_in = _A_setup()

    def _B_setup():
        B, S, D, F, C = (1, 2048, 512, 1792, 1)
        return {'x': _w((lambda *s: _rng.normal(s) * 0.05)(B, S, D)), 'w_r': _w((lambda *s: _rng.normal(s) * 0.05)(D)), 'w_gate': _w((lambda *s: _rng.normal(s) * 0.05)(D, F)), 'w_up': _w((lambda *s: _rng.normal(s) * 0.05)(D, F)), 'w_down': _w((lambda *s: _rng.normal(s) * 0.05)(F, D))}
    _B_in = _B_setup()
    return {'A_x': _A_in['x'], 'A_mem0': _A_in['mem0'], 'A_Wq': _A_in['Wq'], 'A_Wk': _A_in['Wk'], 'A_Wv': _A_in['Wv'], 'A_Wo': _A_in['Wo'], 'A_seg_len': _A_in['seg_len'], 'B_x': _B_in['x'], 'B_w_r': _B_in['w_r'], 'B_w_gate': _B_in['w_gate'], 'B_w_up': _B_in['w_up'], 'B_w_down': _B_in['w_down']}

def reference(A_x, A_mem0, A_Wq, A_Wk, A_Wv, A_Wo, A_seg_len, B_x, B_w_r, B_w_gate, B_w_up, B_w_down):

    def _A_ref(x, mem0, Wq, Wk, Wv, Wo, seg_len):
        B, S, Dm = x.shape
        H, Dh = (Wq.shape[1], Wq.shape[2])
        M = mem0.shape[1]
        scale = Dh ** (-0.5)
        n_seg = S // seg_len
        L = M + seg_len
        idx = jnp.arange(L)
        mask = (idx[:, None] < M) | (idx[:, None] >= idx[None, :])
        mem = mem0
        outs = []
        for s in range(n_seg):
            xs = x[:, s * seg_len:(s + 1) * seg_len, :].copy()
            h = jnp.concatenate([mem, xs], axis=1)
            q = jnp.einsum('btd,dhe->bhte', h, Wq)
            k = jnp.einsum('btd,dhe->bhte', h, Wk)
            v = jnp.einsum('btd,dhe->bhte', h, Wv)
            scores = jnp.einsum('bhqe,bhke->bhqk', q, k) * scale
            scores = jnp.where(mask[None, None], scores, -1000000000.0)
            p = _softmax(scores, axis=-1)
            o = jnp.einsum('bhqk,bhke->bhqe', p, v)
            o = jnp.einsum('bhte,hed->btd', o, Wo)
            mem = o[:, :M, :].copy()
            outs.append(o[:, M:, :])
        return jnp.concatenate(outs, axis=1)

    def _B_ref(x, w_r, w_gate, w_up, w_down):
        B, S, D = x.shape
        C = 1
        r = x @ w_r
        idx = jnp.argsort(-r, axis=-1)[:, :C]
        idx_e = jnp.repeat(idx.reshape(B, C, 1), D, axis=2)
        x_sel = jnp.take_along_axis(x, idx_e, axis=1)
        g = _silu(x_sel @ w_gate)
        u = x_sel @ w_up
        y = g * u @ w_down
        r_sel = _sigmoid(jnp.take_along_axis(r, idx, axis=1))
        y = y * r_sel.reshape(B, C, 1)
        b_off = (jnp.arange(B) * S).reshape(B, 1)
        flat_idx = (idx + b_off).reshape(B * C)
        zero = (x * 0.0).reshape(B * S, D)
        upd = _scatter_add(zero, flat_idx, y.reshape(B * C, D), axis=0)
        return x + upd.reshape(B, S, D)
    x = A_x
    x = x + _A_ref(_layernorm(x, axis=-1), A_mem0, A_Wq, A_Wk, A_Wv, A_Wo, A_seg_len)
    x = x + _B_ref(_layernorm(x, axis=-1), B_w_r, B_w_gate, B_w_up, B_w_down)
    x = x + _A_ref(_layernorm(x, axis=-1), A_mem0, A_Wq, A_Wk, A_Wv, A_Wo, A_seg_len)
    x = x + _B_ref(_layernorm(x, axis=-1), B_w_r, B_w_gate, B_w_up, B_w_down)
    return x
```

```python
import functools

import jax
import jax.numpy as jnp
import jax.experimental.pallas as pl
import jax.experimental.pallas.tpu as pltpu

S = 2048
D = 512
H = 32
E = 128
M = 8
SEG = 32
F = 1792
NPAIR = H // 2
NU = S // (2 * SEG)
W = 2 * SEG
L2 = 2 * (M + SEG)
EPS = 1e-05
SCALE = float(E) ** -0.5
LOG2E = 1.4426950408889634
F32 = jnp.float32
BF16 = jnp.bfloat16
U32 = jnp.uint32


def _rb(x):
    return x.astype(BF16).astype(F32)


def _ln(x):
    mu = jnp.sum(x, axis=-1, keepdims=True) * (1.0 / D)
    xc0 = x - mu
    var = jnp.sum(xc0 * xc0, axis=-1, keepdims=True) * (1.0 / D)
    sd = _rb(jnp.sqrt(_rb(_rb(var) + EPS)))
    xc = _rb(x - _rb(mu))
    return _rb(xc * (1.0 / sd))


def _dot(a, b):
    return jnp.dot(a, b, preferred_element_type=F32)


def _w(ref_slab):
    return pltpu.bitcast(ref_slab, BF16)


def _kernel(x_hbm, mem0_ref, wq_hbm, wk_hbm, wv_hbm, wo_hbm, wr_ref, wg_hbm, wu_hbm, wd_hbm,
            out_hbm,
            xs, x1buf, hbuf, raw, wqkv, wo_raw, wo, wg, wu, wd,
            ring, oring, abuf, maskv, best, sems):
    cp_x = pltpu.make_async_copy(x_hbm, xs.at[pl.ds(0, S)], sems.at[0])
    cp_x.start()
    cp_w = [pltpu.make_async_copy(w, raw.at[i], sems.at[1 + i])
            for i, w in enumerate((wq_hbm, wk_hbm, wv_hbm))]
    for c in cp_w:
        c.start()
    cp_wo = [pltpu.make_async_copy(wo_hbm.at[:, pl.ds(n * 128, 128)], wo_raw.at[n], sems.at[4 + n])
             for n in range(4)]
    for c in cp_wo:
        c.start()
    cp_f = [pltpu.make_async_copy(wg_hbm, wg, sems.at[8]),
            pltpu.make_async_copy(wu_hbm, wu, sems.at[9]),
            pltpu.make_async_copy(wd_hbm, wd, sems.at[10])]
    for c in cp_f:
        c.start()

    oring[...] = jnp.zeros(oring.shape, F32)
    abuf[...] = jnp.zeros(abuf.shape, F32)
    xs[pl.ds(S, 2 * W), :] = jnp.zeros((2 * W, D), BF16)
    hbuf[pl.ds(2 * S, 2 * W), :] = jnp.zeros((2 * W, D), F32)

    ri = jax.lax.broadcasted_iota(jnp.int32, (L2, L2), 0)
    ci = jax.lax.broadcasted_iota(jnp.int32, (L2, L2), 1)

    def head_of(i):
        return jnp.where(i < 2 * M, i // M, (i - 2 * M) // SEG)

    def pos_of(i):
        return jnp.where(i < 2 * M, i % M, M + (i - 2 * M) % SEG)

    same = head_of(ri) == head_of(ci)
    ok = (pos_of(ri) < M) | (pos_of(ri) >= pos_of(ci))
    maskv[...] = jnp.where(same, jnp.where(ok, 0.0, -1e9 / SCALE), -jnp.inf).astype(F32)

    cp_x.wait()

    def ln0(i, c):
        r0 = pl.multiple_of(i * 32, 32)
        hbuf[pl.ds(r0, 32), :] = _ln(xs[pl.ds(r0, 32), :].astype(F32))
        return c

    jax.lax.fori_loop(0, S // 32, ln0, 0)

    for i in range(3):
        cp_w[i].wait()

        def relay(db, c, i=i):
            d0 = pl.multiple_of(db * 16, 16)
            a = jnp.swapaxes(raw[i, pl.ds(d0, 16)], 0, 1)
            p0 = pl.multiple_of(db * 8, 8)
            for h in range(H):
                t = (h // 2) * 6 + 2 * i + (h % 2)
                wqkv[t, pl.ds(p0, 8), :] = pltpu.bitcast(a[h], U32)
            return c

        jax.lax.fori_loop(0, D // 16, relay, 0)

    def qkv_window(hrow0, ring0):
        lhs = hbuf[pl.ds(hrow0, W), :].astype(BF16)

        def body(t, c):
            ring[t, pl.ds(ring0, W), :] = _dot(lhs, _w(wqkv[t]))
            return c

        jax.lax.fori_loop(0, 6 * NPAIR, body, 0, unroll=4)

    qkv_window(0, 0)

    for n in range(4):
        cp_wo[n].wait()

        def cpwo(k, c, n=n):
            k0 = pl.multiple_of(k * 256, 256)
            p0 = pl.multiple_of(k * 128, 128)
            wo[n, pl.ds(p0, 128), :] = pltpu.bitcast(wo_raw[n, pl.ds(k0, 256), :], U32)
            return c

        jax.lax.fori_loop(0, H * E // 256, cpwo, 0)

    def post(row0, arow0, hrow0, valid, n):
        a = _rb(abuf[pl.ds(arow0, n), :])
        x1 = _rb(xs[pl.ds(row0, n), :].astype(F32) + a)
        x1buf[pl.ds(row0, n), :] = x1.astype(BF16)
        hb = _ln(x1)
        r = _rb(jnp.sum(hb * wr_ref[...].astype(F32), axis=-1, keepdims=True))
        x2 = _rb(x1 + hb)
        xs[pl.ds(row0, n), :] = x2.astype(BF16)
        hbuf[pl.ds(hrow0, n), :] = _ln(x2)
        if valid is not True:
            r = jnp.where(valid, r, -jnp.inf)
        bv = best[0]
        bi = best[1]
        sub = jax.lax.broadcasted_iota(jnp.int32, (8, 128), 0).astype(F32)
        for g in range(n // 8):
            rg = jnp.broadcast_to(r[8 * g:8 * g + 8], (8, 128))
            ig = sub + (float(row0 + 8 * g) if isinstance(row0, int) else (row0 + 8 * g).astype(F32))
            gt = rg > bv
            bv = jnp.where(gt, rg, bv)
            bi = jnp.where(gt, ig, bi)
        best[0] = bv
        best[1] = bi

    def wo_pair(g, half):
        return jnp.concatenate(
            [_w(wo[2 * half + c, pl.ds(g * 128, 128), :]) for c in range(2)], axis=1)

    def step(par, layer, u, mem):
        hw = pl.multiple_of(layer * S + W * (u + 1), W)
        rw = pl.multiple_of(((u + 1) % 2) * W, W)
        rr = pl.multiple_of((u % 2) * W + par * SEG, SEG)
        if par == 0:
            rows = ((0, 40), (0, 24))
        else:
            rows = ((40, 64), (24, 64))
        lhs = [jnp.concatenate([mem, hbuf[pl.ds(hw + lo, hi - lo), :]], axis=0).astype(BF16)
               for lo, hi in rows]

        def qkv(g):
            half = g // (NPAIR // 2)
            lo, hi = rows[half]
            res = []
            for t in range(6):
                y = _dot(lhs[half], _w(wqkv[6 * g + t]))
                ring[6 * g + t, pl.ds(rw + lo, hi - lo), :] = y[M:]
                res.append(y[:M])
            return res

        def attn(g, mres):
            def stack(i):
                return jnp.concatenate(
                    [mres[2 * i], mres[2 * i + 1],
                     ring[6 * g + 2 * i, pl.ds(rr, SEG), :],
                     ring[6 * g + 2 * i + 1, pl.ds(rr, SEG), :]], axis=0).astype(BF16)

            q2, k2, v2 = stack(0), stack(1), stack(2)
            s = jax.lax.dot_general(q2, k2, (((1,), (1,)), ((), ())), preferred_element_type=F32)
            mk = maskv[...]
            s = jnp.where(mk == 0.0, s, mk)
            mx = jnp.max(s, axis=-1, keepdims=True)
            p = jnp.exp2((s - mx) * (SCALE * LOG2E))
            l = jnp.sum(p, axis=-1, keepdims=True)
            o = _dot(p.astype(BF16), v2)
            r0 = pl.reciprocal(l, approx=True)
            r = r0 * (2.0 - l * r0)
            o = o * r
            oring[2 * g, pl.ds(rr, SEG), :] = o[2 * M:2 * M + SEG]
            oring[2 * g + 1, pl.ds(rr, SEG), :] = o[2 * M + SEG:]
            return o[:M], o[M:2 * M]

        def oproj(g, om, acc):
            out = []
            for half in range(2):
                lo, hi = rows[half]
                l = jnp.concatenate(
                    [jnp.concatenate([om[c], oring[2 * g + c, pl.ds(rw + lo, hi - lo), :]], axis=0)
                     for c in range(2)], axis=1).astype(BF16)
                y = _dot(l, wo_pair(g, half))
                out.append(y if acc is None else acc[half] + y)
            return out

        oms = []
        for g in range(NPAIR):
            mres = qkv(g)
            oms.append(attn(g, mres))
        acc = None
        for g in range(NPAIR):
            acc = oproj(g, oms[g], acc)
        for half in range(2):
            lo, hi = rows[half]
            abuf[pl.ds(rw + lo, hi - lo), pl.ds(half * 256, 256)] = acc[half][M:]

        valid = u >= 2
        prow = W * (u - 2) + par * SEG
        row0 = pl.multiple_of(jnp.where(valid, prow, S + par * SEG), SEG)
        hrow0 = pl.multiple_of(
            jnp.where(valid & (layer == 0), S + prow, 2 * S + W + par * SEG), SEG)
        post(row0, rr, hrow0, valid, SEG)

        return jnp.concatenate([acc[0][:M], acc[1][:M]], axis=1)

    def layer_body(layer, carry):
        best[0] = jnp.full((8, 128), -jnp.inf, F32)
        best[1] = jnp.zeros((8, 128), F32)

        def dstep(u, mem):
            mem = step(0, layer, u, mem)
            mem = step(1, layer, u, mem)
            return mem

        jax.lax.fori_loop(0, NU, dstep, mem0_ref[...].astype(F32))

        acc = None
        for g in range(NPAIR):
            l = jnp.concatenate([oring[2 * g + c, pl.ds(W, W), :] for c in range(2)],
                                axis=1).astype(BF16)
            y = _dot(l, jnp.concatenate([wo_pair(g, 0), wo_pair(g, 1)], axis=1))
            acc = y if acc is None else acc + y
        abuf[pl.ds(W, W), :] = acc
        hlast = pl.multiple_of(jnp.where(layer == 0, 2 * S - 2 * W, 2 * S + W), W)
        hlast2 = pl.multiple_of(jnp.where(layer == 0, 2 * S - W, 2 * S + W), W)
        post(S - 2 * W, 0, hlast, True, W)
        post(S - W, W, hlast2, True, W)

        @pl.when(layer == 0)
        def _():
            for c in cp_f:
                c.wait()

        bv = best[0]
        bi = best[1]
        vmax = jnp.max(bv, axis=0, keepdims=True)
        imin = jnp.min(jnp.where(bv == vmax, bi, float(S)), axis=0, keepdims=True)
        idx = jnp.clip(jnp.min(imin).astype(jnp.int32), 0, S - 1)
        g0 = pl.multiple_of((idx // 16) * 16, 16)
        x1 = x1buf[pl.ds(g0, 16), :].astype(F32)
        hb = _ln(x1)
        hbb = hb.astype(BF16)
        gpre = _rb(_dot(hbb, wg[...]))
        gs = _rb(gpre * _rb(jax.nn.sigmoid(gpre)))
        up = _rb(_dot(hbb, wu[...]))
        y = _rb(_dot((gs * up).astype(BF16), wd[...]))
        rsel = _rb(jax.nn.sigmoid(vmax))[:, :1]
        y = _rb(y * rsel)
        x2 = _rb(x1 + _rb(hb + y))
        rowi = jax.lax.broadcasted_iota(jnp.int32, (16, D), 0) + g0
        x2 = jnp.where(rowi == idx, x2, xs[pl.ds(g0, 16), :].astype(F32))
        xs[pl.ds(g0, 16), :] = x2.astype(BF16)

        @pl.when(layer == 0)
        def _():
            hbuf[pl.ds(S + g0, 16), :] = _ln(x2)

            @pl.when(idx < W)
            def _():
                qkv_window(S, 0)

        return carry

    jax.lax.fori_loop(0, 2, layer_body, 0)

    cp_o = pltpu.make_async_copy(xs.at[pl.ds(0, S)], out_hbm, sems.at[0])
    cp_o.start()
    cp_o.wait()


@functools.partial(jax.jit, static_argnames=("A_seg_len",))
def pallas_interleave_layers__memory_aug_recurrent_mem_tr__moe_arch_mod__prompt_kernel(
    A_x: jax.Array,
    A_mem0: jax.Array,
    A_Wq: jax.Array,
    A_Wk: jax.Array,
    A_Wv: jax.Array,
    A_Wo: jax.Array,
    A_seg_len,
    B_x: jax.Array,
    B_w_r: jax.Array,
    B_w_gate: jax.Array,
    B_w_up: jax.Array,
    B_w_down: jax.Array,
):
    assert A_seg_len == SEG
    assert A_x.shape == (1, S, D) and A_Wq.shape == (D, H, E) and A_mem0.shape == (1, M, D)
    any_spec = pl.BlockSpec(memory_space=pl.ANY)
    vmem_spec = pl.BlockSpec(memory_space=pltpu.VMEM)
    out = pl.pallas_call(
        _kernel,
        out_shape=jax.ShapeDtypeStruct((S, D), BF16),
        in_specs=[any_spec, vmem_spec, any_spec, any_spec, any_spec, any_spec,
                  vmem_spec, any_spec, any_spec, any_spec],
        out_specs=any_spec,
        scratch_shapes=[
            pltpu.VMEM((S + 2 * W, D), BF16),
            pltpu.VMEM((S + 2 * W, D), BF16),
            pltpu.VMEM((2 * S + 2 * W, D), F32),
            pltpu.VMEM((3, D, H, E), BF16),
            pltpu.VMEM((6 * NPAIR, D // 2, E), U32),
            pltpu.VMEM((4, H * E, 128), BF16),
            pltpu.VMEM((4, H * E // 2, 128), U32),
            pltpu.VMEM((D, F), BF16),
            pltpu.VMEM((D, F), BF16),
            pltpu.VMEM((F, D), BF16),
            pltpu.VMEM((6 * NPAIR, 2 * W, E), F32),
            pltpu.VMEM((H, 2 * W, E), F32),
            pltpu.VMEM((2 * W, D), F32),
            pltpu.VMEM((L2, L2), F32),
            pltpu.VMEM((2, 8, 128), F32),
            pltpu.SemaphoreType.DMA((11,)),
        ],
        compiler_params=pltpu.CompilerParams(vmem_limit_bytes=110 * 1024 * 1024),
        name="rmt_mod",
    )(A_x.reshape(S, D), A_mem0.reshape(M, D), A_Wq, A_Wk, A_Wv, A_Wo.reshape(H * E, D),
      B_w_r.reshape(1, D), B_w_gate, B_w_up, B_w_down)
    return out.reshape(1, S, D)
```

```python
import functools

import jax
import jax.numpy as jnp
import jax.experimental.pallas as pl
import jax.experimental.pallas.tpu as pltpu

S = 2048
D = 512
H = 32
E = 128
M = 8
SEG = 32
F = 1792
NPAIR = H // 2
NU = S // (2 * SEG)
W = 2 * SEG
L2 = 2 * (M + SEG)
EPS = 1e-05
SCALE = float(E) ** -0.5
LOG2E = 1.4426950408889634
F32 = jnp.float32
BF16 = jnp.bfloat16
U32 = jnp.uint32


def _rb(x):
    return x.astype(BF16).astype(F32)


def _ln(x):
    mu = jnp.sum(x, axis=-1, keepdims=True) * (1.0 / D)
    xc0 = x - mu
    var = jnp.sum(xc0 * xc0, axis=-1, keepdims=True) * (1.0 / D)
    sd = _rb(jnp.sqrt(_rb(_rb(var) + EPS)))
    xc = _rb(x - _rb(mu))
    return _rb(xc * (1.0 / sd))


def _dot(a, b):
    return jnp.dot(a, b, preferred_element_type=F32)


def _w(ref_slab):
    return pltpu.bitcast(ref_slab, BF16)


def _kernel(x_hbm, mem0_ref, wq_hbm, wk_hbm, wv_hbm, wo_hbm, wr_ref, wg_hbm, wu_hbm, wd_hbm,
            out_hbm,
            xs, x1buf, hbuf, raw, wqkv, wo_raw, wo, wg, wu, wd,
            ring, oring, abuf, maskv, best, sems):
    cp_x = pltpu.make_async_copy(x_hbm, xs.at[pl.ds(0, S)], sems.at[0])
    cp_x.start()
    cp_w = [pltpu.make_async_copy(w, raw.at[i], sems.at[1 + i])
            for i, w in enumerate((wq_hbm, wk_hbm, wv_hbm))]
    for c in cp_w:
        c.start()
    cp_wo = [pltpu.make_async_copy(wo_hbm.at[:, pl.ds(n * 128, 128)], wo_raw.at[n], sems.at[4 + n])
             for n in range(4)]
    for c in cp_wo:
        c.start()
    cp_f = [pltpu.make_async_copy(wg_hbm, wg, sems.at[8]),
            pltpu.make_async_copy(wu_hbm, wu, sems.at[9]),
            pltpu.make_async_copy(wd_hbm, wd, sems.at[10])]
    for c in cp_f:
        c.start()

    oring[...] = jnp.zeros(oring.shape, F32)
    abuf[...] = jnp.zeros(abuf.shape, F32)
    xs[pl.ds(S, 2 * W), :] = jnp.zeros((2 * W, D), BF16)
    hbuf[pl.ds(2 * S, 2 * W), :] = jnp.zeros((2 * W, D), F32)

    ri = jax.lax.broadcasted_iota(jnp.int32, (L2, L2), 0)
    ci = jax.lax.broadcasted_iota(jnp.int32, (L2, L2), 1)

    def head_of(i):
        return jnp.where(i < 2 * M, i // M, (i - 2 * M) // SEG)

    def pos_of(i):
        return jnp.where(i < 2 * M, i % M, M + (i - 2 * M) % SEG)

    same = head_of(ri) == head_of(ci)
    ok = (pos_of(ri) < M) | (pos_of(ri) >= pos_of(ci))
    maskv[...] = jnp.where(same, jnp.where(ok, 0.0, -1e9 / SCALE), -jnp.inf).astype(F32)

    cp_x.wait()

    def ln0(i, c):
        r0 = pl.multiple_of(i * 32, 32)
        hbuf[pl.ds(r0, 32), :] = _ln(xs[pl.ds(r0, 32), :].astype(F32))
        return c

    jax.lax.fori_loop(0, S // 32, ln0, 0)

    for i in range(3):
        cp_w[i].wait()

        def relay(db, c, i=i):
            d0 = pl.multiple_of(db * 16, 16)
            a = jnp.swapaxes(raw[i, pl.ds(d0, 16)], 0, 1)
            p0 = pl.multiple_of(db * 8, 8)
            for h in range(H):
                t = (h // 2) * 6 + 2 * i + (h % 2)
                wqkv[t, pl.ds(p0, 8), :] = pltpu.bitcast(a[h], U32)
            return c

        jax.lax.fori_loop(0, D // 16, relay, 0)

    def qkv_window(hrow0, ring0):
        lhs = hbuf[pl.ds(hrow0, W), :].astype(BF16)

        def body(t, c):
            ring[t, pl.ds(ring0, W), :] = _dot(lhs, _w(wqkv[t]))
            return c

        jax.lax.fori_loop(0, 6 * NPAIR, body, 0, unroll=4)

    qkv_window(0, 0)

    for n in range(4):
        cp_wo[n].wait()

        def cpwo(k, c, n=n):
            k0 = pl.multiple_of(k * 256, 256)
            p0 = pl.multiple_of(k * 128, 128)
            wo[n, pl.ds(p0, 128), :] = pltpu.bitcast(wo_raw[n, pl.ds(k0, 256), :], U32)
            return c

        jax.lax.fori_loop(0, H * E // 256, cpwo, 0)

    def post(row0, arow0, hrow0, valid, n):
        a = _rb(abuf[pl.ds(arow0, n), :])
        x1 = _rb(xs[pl.ds(row0, n), :].astype(F32) + a)
        x1buf[pl.ds(row0, n), :] = x1.astype(BF16)
        hb = _ln(x1)
        r = _rb(jnp.sum(hb * wr_ref[...].astype(F32), axis=-1, keepdims=True))
        x2 = _rb(x1 + hb)
        xs[pl.ds(row0, n), :] = x2.astype(BF16)
        hbuf[pl.ds(hrow0, n), :] = _ln(x2)
        if valid is not True:
            r = jnp.where(valid, r, -jnp.inf)
        bv = best[0]
        bi = best[1]
        sub = jax.lax.broadcasted_iota(jnp.int32, (8, 128), 0).astype(F32)
        for g in range(n // 8):
            rg = jnp.broadcast_to(r[8 * g:8 * g + 8], (8, 128))
            ig = sub + (float(row0 + 8 * g) if isinstance(row0, int) else (row0 + 8 * g).astype(F32))
            gt = rg > bv
            bv = jnp.where(gt, rg, bv)
            bi = jnp.where(gt, ig, bi)
        best[0] = bv
        best[1] = bi

    def wo_pair(g, half):
        return jnp.concatenate(
            [_w(wo[2 * half + c, pl.ds(g * 128, 128), :]) for c in range(2)], axis=1)

    def step(par, layer, u, mem):
        hw = pl.multiple_of(layer * S + W * (u + 1), W)
        rw = pl.multiple_of(((u + 1) % 2) * W, W)
        rr = pl.multiple_of((u % 2) * W + par * SEG, SEG)
        if par == 0:
            rows = ((0, 40), (0, 24))
        else:
            rows = ((40, 64), (24, 64))
        lhs = [jnp.concatenate([mem, hbuf[pl.ds(hw + lo, hi - lo), :]], axis=0).astype(BF16)
               for lo, hi in rows]

        def qkv(g):
            half = g // (NPAIR // 2)
            lo, hi = rows[half]
            res = []
            for t in range(6):
                y = _dot(lhs[half], _w(wqkv[6 * g + t]))
                ring[6 * g + t, pl.ds(rw + lo, hi - lo), :] = y[M:]
                res.append(y[:M])
            return res

        def stack(g, mres, i):
            return jnp.concatenate(
                [mres[2 * i], mres[2 * i + 1],
                 ring[6 * g + 2 * i, pl.ds(rr, SEG), :],
                 ring[6 * g + 2 * i + 1, pl.ds(rr, SEG), :]], axis=0).astype(BF16)

        def qk(g, mres):
            q2, k2 = stack(g, mres, 0), stack(g, mres, 1)
            s = jax.lax.dot_general(q2, k2, (((1,), (1,)), ((), ())), preferred_element_type=F32)
            mk = maskv[...]
            s = jnp.where(mk == 0.0, s, mk)
            mx = jnp.max(s, axis=-1, keepdims=True)
            p = jnp.exp2((s - mx) * (SCALE * LOG2E))
            l = jnp.sum(p, axis=-1, keepdims=True)
            r0 = pl.reciprocal(l, approx=True)
            r = r0 * (2.0 - l * r0)
            return p.astype(BF16), r

        def pv(g, mres, pr):
            p, r = pr
            o = _dot(p, stack(g, mres, 2)) * r
            oring[2 * g, pl.ds(rr, SEG), :] = o[2 * M:2 * M + SEG]
            oring[2 * g + 1, pl.ds(rr, SEG), :] = o[2 * M + SEG:]
            return o[:M], o[M:2 * M]

        def oproj(g, om, acc):
            out = []
            for half in range(2):
                lo, hi = rows[half]
                l = jnp.concatenate(
                    [jnp.concatenate([om[c], oring[2 * g + c, pl.ds(rw + lo, hi - lo), :]], axis=0)
                     for c in range(2)], axis=1).astype(BF16)
                y = _dot(l, wo_pair(g, half))
                out.append(y if acc is None else acc[half] + y)
            return out

        valid = u >= 2
        prow = W * (u - 2) + par * SEG
        row0 = pl.multiple_of(jnp.where(valid, prow, S + par * SEG), SEG)
        hrow0 = pl.multiple_of(
            jnp.where(valid & (layer == 0), S + prow, 2 * S + W + par * SEG), SEG)
        post(row0, rr, hrow0, valid, SEG)

        NST = NPAIR // 2
        st = [(i, i + NST) for i in range(NST)]
        mres, prs, oms = {}, {}, {}
        acc = None
        order = []
        for i in range(NST):
            order += [("qkv", g) for g in st[i]]
            if i >= 1:
                order += [("qk", g) for g in st[i - 1]]
            if i >= 2:
                order += [("pv", g) for g in st[i - 2]]
        oq = [g for i in range(NST) for g in st[i]]
        order += [("o", g) for g in oq[0:2]]
        order += [("qk", g) for g in st[NST - 1]] + [("pv", g) for g in st[NST - 2]]
        order += [("o", g) for g in oq[2:8]]
        order += [("pv", g) for g in st[NST - 1]]
        order += [("o", g) for g in oq[8:]]
        for kind, g in order:
            if kind == "qkv":
                mres[g] = qkv(g)
            elif kind == "qk":
                prs[g] = qk(g, mres[g])
            elif kind == "pv":
                oms[g] = pv(g, mres[g], prs[g])
            else:
                acc = oproj(g, oms[g], acc)
        for half in range(2):
            lo, hi = rows[half]
            abuf[pl.ds(rw + lo, hi - lo), pl.ds(half * 256, 256)] = acc[half][M:]

        return jnp.concatenate([acc[0][:M], acc[1][:M]], axis=1)

    def layer_body(layer, carry):
        best[0] = jnp.full((8, 128), -jnp.inf, F32)
        best[1] = jnp.zeros((8, 128), F32)

        def dstep(u, mem):
            mem = step(0, layer, u, mem)
            mem = step(1, layer, u, mem)
            return mem

        jax.lax.fori_loop(0, NU, dstep, mem0_ref[...].astype(F32))

        acc = None
        for g in range(NPAIR):
            l = jnp.concatenate([oring[2 * g + c, pl.ds(W, W), :] for c in range(2)],
                                axis=1).astype(BF16)
            y = _dot(l, jnp.concatenate([wo_pair(g, 0), wo_pair(g, 1)], axis=1))
            acc = y if acc is None else acc + y
        abuf[pl.ds(W, W), :] = acc
        hlast = pl.multiple_of(jnp.where(layer == 0, 2 * S - 2 * W, 2 * S + W), W)
        hlast2 = pl.multiple_of(jnp.where(layer == 0, 2 * S - W, 2 * S + W), W)
        post(S - 2 * W, 0, hlast, True, W)
        post(S - W, W, hlast2, True, W)

        @pl.when(layer == 0)
        def _():
            for c in cp_f:
                c.wait()

        bv = best[0]
        bi = best[1]
        vmax = jnp.max(bv, axis=0, keepdims=True)
        imin = jnp.min(jnp.where(bv == vmax, bi, float(S)), axis=0, keepdims=True)
        idx = jnp.clip(jnp.min(imin).astype(jnp.int32), 0, S - 1)
        g0 = pl.multiple_of((idx // 16) * 16, 16)
        x1 = x1buf[pl.ds(g0, 16), :].astype(F32)
        hb = _ln(x1)
        hbb = hb.astype(BF16)
        gpre = _rb(_dot(hbb, wg[...]))
        gs = _rb(gpre * _rb(jax.nn.sigmoid(gpre)))
        up = _rb(_dot(hbb, wu[...]))
        y = _rb(_dot((gs * up).astype(BF16), wd[...]))
        rsel = _rb(jax.nn.sigmoid(vmax))[:, :1]
        y = _rb(y * rsel)
        x2 = _rb(x1 + _rb(hb + y))
        rowi = jax.lax.broadcasted_iota(jnp.int32, (16, D), 0) + g0
        x2 = jnp.where(rowi == idx, x2, xs[pl.ds(g0, 16), :].astype(F32))
        xs[pl.ds(g0, 16), :] = x2.astype(BF16)

        @pl.when(layer == 0)
        def _():
            hbuf[pl.ds(S + g0, 16), :] = _ln(x2)

            @pl.when(idx < W)
            def _():
                qkv_window(S, 0)

        return carry

    jax.lax.fori_loop(0, 2, layer_body, 0)

    cp_o = pltpu.make_async_copy(xs.at[pl.ds(0, S)], out_hbm, sems.at[0])
    cp_o.start()
    cp_o.wait()


@functools.partial(jax.jit, static_argnames=("A_seg_len",))
def pallas_interleave_layers__memory_aug_recurrent_mem_tr__moe_arch_mod__prompt_kernel(
    A_x: jax.Array,
    A_mem0: jax.Array,
    A_Wq: jax.Array,
    A_Wk: jax.Array,
    A_Wv: jax.Array,
    A_Wo: jax.Array,
    A_seg_len,
    B_x: jax.Array,
    B_w_r: jax.Array,
    B_w_gate: jax.Array,
    B_w_up: jax.Array,
    B_w_down: jax.Array,
):
    assert A_seg_len == SEG
    assert A_x.shape == (1, S, D) and A_Wq.shape == (D, H, E) and A_mem0.shape == (1, M, D)
    any_spec = pl.BlockSpec(memory_space=pl.ANY)
    vmem_spec = pl.BlockSpec(memory_space=pltpu.VMEM)
    out = pl.pallas_call(
        _kernel,
        out_shape=jax.ShapeDtypeStruct((S, D), BF16),
        in_specs=[any_spec, vmem_spec, any_spec, any_spec, any_spec, any_spec,
                  vmem_spec, any_spec, any_spec, any_spec],
        out_specs=any_spec,
        scratch_shapes=[
            pltpu.VMEM((S + 2 * W, D), BF16),
            pltpu.VMEM((S + 2 * W, D), BF16),
            pltpu.VMEM((2 * S + 2 * W, D), F32),
            pltpu.VMEM((3, D, H, E), BF16),
            pltpu.VMEM((6 * NPAIR, D // 2, E), U32),
            pltpu.VMEM((4, H * E, 128), BF16),
            pltpu.VMEM((4, H * E // 2, 128), U32),
            pltpu.VMEM((D, F), BF16),
            pltpu.VMEM((D, F), BF16),
            pltpu.VMEM((F, D), BF16),
            pltpu.VMEM((6 * NPAIR, 2 * W, E), F32),
            pltpu.VMEM((H, 2 * W, E), F32),
            pltpu.VMEM((2 * W, D), F32),
            pltpu.VMEM((L2, L2), F32),
            pltpu.VMEM((2, 8, 128), F32),
            pltpu.SemaphoreType.DMA((11,)),
        ],
        compiler_params=pltpu.CompilerParams(vmem_limit_bytes=110 * 1024 * 1024),
        name="rmt_mod",
    )(A_x.reshape(S, D), A_mem0.reshape(M, D), A_Wq, A_Wk, A_Wv, A_Wo.reshape(H * E, D),
      B_w_r.reshape(1, D), B_w_gate, B_w_up, B_w_down)
    return out.reshape(1, S, D)
```

```python
import functools

import jax
import jax.numpy as jnp
import jax.experimental.pallas as pl
import jax.experimental.pallas.tpu as pltpu

S = 2048
D = 512
H = 32
E = 128
M = 8
SEG = 32
F = 1792
NPAIR = H // 2
NU = S // (2 * SEG)
W = 2 * SEG
L2 = 2 * (M + SEG)
EPS = 1e-05
SCALE = float(E) ** -0.5
LOG2E = 1.4426950408889634
F32 = jnp.float32
BF16 = jnp.bfloat16
U32 = jnp.uint32


def _rb(x):
    return x.astype(BF16).astype(F32)


def _ln(x):
    mu = jnp.sum(x, axis=-1, keepdims=True) * (1.0 / D)
    xc0 = x - mu
    var = jnp.sum(xc0 * xc0, axis=-1, keepdims=True) * (1.0 / D)
    sd = _rb(jnp.sqrt(_rb(_rb(var) + EPS)))
    xc = _rb(x - _rb(mu))
    return _rb(xc * (1.0 / sd))


def _dot(a, b):
    return jnp.dot(a, b, preferred_element_type=F32)


def _w(ref_slab):
    return pltpu.bitcast(ref_slab, BF16)


def _kernel(x_hbm, mem0_ref, wq_hbm, wk_hbm, wv_hbm, wo_hbm, wr_ref, wg_hbm, wu_hbm, wd_hbm,
            out_hbm,
            xs, x1buf, hbuf, raw, wqkv, wo_raw, wo, wg, wu, wd,
            ring, oring, abuf, maskv, best, sems):
    cp_x = pltpu.make_async_copy(x_hbm, xs.at[pl.ds(0, S)], sems.at[0])
    cp_x.start()
    cp_w = [pltpu.make_async_copy(w, raw.at[i], sems.at[1 + i])
            for i, w in enumerate((wq_hbm, wk_hbm, wv_hbm))]
    for c in cp_w:
        c.start()
    cp_wo = [pltpu.make_async_copy(wo_hbm.at[:, pl.ds(n * 128, 128)], wo_raw.at[n], sems.at[4 + n])
             for n in range(4)]
    for c in cp_wo:
        c.start()
    cp_f = [pltpu.make_async_copy(wg_hbm, wg, sems.at[8]),
            pltpu.make_async_copy(wu_hbm, wu, sems.at[9]),
            pltpu.make_async_copy(wd_hbm, wd, sems.at[10])]
    for c in cp_f:
        c.start()

    oring[...] = jnp.zeros(oring.shape, F32)
    abuf[...] = jnp.zeros(abuf.shape, F32)
    xs[pl.ds(S, 2 * W), :] = jnp.zeros((2 * W, D), BF16)
    hbuf[pl.ds(2 * S, 2 * W), :] = jnp.zeros((2 * W, D), F32)

    ri = jax.lax.broadcasted_iota(jnp.int32, (L2, L2), 0)
    ci = jax.lax.broadcasted_iota(jnp.int32, (L2, L2), 1)

    def head_of(i):
        return jnp.where(i < 2 * M, i // M, (i - 2 * M) // SEG)

    def pos_of(i):
        return jnp.where(i < 2 * M, i % M, M + (i - 2 * M) % SEG)

    same = head_of(ri) == head_of(ci)
    ok = (pos_of(ri) < M) | (pos_of(ri) >= pos_of(ci))
    maskv[...] = jnp.where(same, jnp.where(ok, 0.0, -1e9 / SCALE), -jnp.inf).astype(F32)

    cp_x.wait()

    def ln0(i, c):
        r0 = pl.multiple_of(i * 32, 32)
        hbuf[pl.ds(r0, 32), :] = _ln(xs[pl.ds(r0, 32), :].astype(F32))
        return c

    jax.lax.fori_loop(0, S // 32, ln0, 0)

    for i in range(3):
        cp_w[i].wait()

        def relay(db, c, i=i):
            d0 = pl.multiple_of(db * 16, 16)
            a = jnp.swapaxes(raw[i, pl.ds(d0, 16)], 0, 1)
            p0 = pl.multiple_of(db * 8, 8)
            for h in range(H):
                t = (h // 2) * 6 + 2 * i + (h % 2)
                wqkv[t, pl.ds(p0, 8), :] = pltpu.bitcast(a[h], U32)
            return c

        jax.lax.fori_loop(0, D // 16, relay, 0)

    def qkv_window(hrow0, ring0):
        lhs = hbuf[pl.ds(hrow0, W), :].astype(BF16)

        def body(t, c):
            ring[t, pl.ds(ring0, W), :] = _dot(lhs, _w(wqkv[t]))
            return c

        jax.lax.fori_loop(0, 6 * NPAIR, body, 0, unroll=4)

    qkv_window(0, 0)

    for n in range(4):
        cp_wo[n].wait()

        def cpwo(k, c, n=n):
            k0 = pl.multiple_of(k * 256, 256)
            p0 = pl.multiple_of(k * 128, 128)
            wo[n, pl.ds(p0, 128), :] = pltpu.bitcast(wo_raw[n, pl.ds(k0, 256), :], U32)
            return c

        jax.lax.fori_loop(0, H * E // 256, cpwo, 0)

    def post(row0, arow0, hrow0, valid, n):
        a = _rb(abuf[pl.ds(arow0, n), :])
        x1 = _rb(xs[pl.ds(row0, n), :].astype(F32) + a)
        x1buf[pl.ds(row0, n), :] = x1.astype(BF16)
        hb = _ln(x1)
        r = _rb(jnp.sum(hb * wr_ref[...].astype(F32), axis=-1, keepdims=True))
        x2 = _rb(x1 + hb)
        xs[pl.ds(row0, n), :] = x2.astype(BF16)
        hbuf[pl.ds(hrow0, n), :] = _ln(x2)
        if valid is not True:
            r = jnp.where(valid, r, -jnp.inf)
        bv = best[0]
        bi = best[1]
        sub = jax.lax.broadcasted_iota(jnp.int32, (8, 128), 0).astype(F32)
        for g in range(n // 8):
            rg = jnp.broadcast_to(r[8 * g:8 * g + 8], (8, 128))
            ig = sub + (float(row0 + 8 * g) if isinstance(row0, int) else (row0 + 8 * g).astype(F32))
            gt = rg > bv
            bv = jnp.where(gt, rg, bv)
            bi = jnp.where(gt, ig, bi)
        best[0] = bv
        best[1] = bi

    def wo_pair(g, half):
        return jnp.concatenate(
            [_w(wo[2 * half + c, pl.ds(g * 128, 128), :]) for c in range(2)], axis=1)

    def step(par, layer, u, mem, korder):
        hw = pl.multiple_of(layer * S + W * (u + 1), W)
        rw = pl.multiple_of(((u + 1) % 2) * W, W)
        rr = pl.multiple_of((u % 2) * W + par * SEG, SEG)
        if par == 0:
            rows = ((0, 40), (0, 24))
        else:
            rows = ((40, 64), (24, 64))
        lhs = [jnp.concatenate([mem, hbuf[pl.ds(hw + lo, hi - lo), :]], axis=0).astype(BF16)
               for lo, hi in rows]

        def qkv(g, korder=None):
            half = g // (NPAIR // 2)
            lo, hi = rows[half]
            res = []
            ys = {}
            if korder is not None:
                part = None
                for k in korder:
                    wk = jnp.concatenate([_w(wqkv[6 * g + t, pl.ds(64 * k, 64), :])
                                          for t in range(4)], axis=1)
                    y = jnp.dot(lhs[half][:, 128 * k:128 * (k + 1)], wk,
                                preferred_element_type=F32)
                    part = y if part is None else part + y
                for t in range(4):
                    ys[t] = part[:, 128 * t:128 * (t + 1)]
            for t in range(6):
                if t in ys:
                    y = ys[t]
                else:
                    y = jnp.dot(lhs[half], _w(wqkv[6 * g + t]), preferred_element_type=F32)
                ring[6 * g + t, pl.ds(rw + lo, hi - lo), :] = y[M:]
                res.append(y[:M])
            return res

        def stack(g, mres, i):
            return jnp.concatenate(
                [mres[2 * i], mres[2 * i + 1],
                 ring[6 * g + 2 * i, pl.ds(rr, SEG), :],
                 ring[6 * g + 2 * i + 1, pl.ds(rr, SEG), :]], axis=0).astype(BF16)

        def qk(g, mres, prenorm):
            q2, k2 = stack(g, mres, 0), stack(g, mres, 1)
            s = jax.lax.dot_general(q2, k2, (((1,), (1,)), ((), ())), preferred_element_type=F32)
            mk = maskv[...]
            s = jnp.where(mk == 0.0, s, mk)
            mx = jnp.max(s, axis=-1, keepdims=True)
            p = jnp.exp2((s - mx) * (SCALE * LOG2E))
            l = jnp.sum(p, axis=-1, keepdims=True)
            r0 = pl.reciprocal(l, approx=True)
            r = r0 * (2.0 - l * r0)
            if prenorm:
                return (p * r).astype(BF16), None
            return p.astype(BF16), r

        def pv(g, mres, pr):
            p, r = pr
            o = jnp.dot(p, stack(g, mres, 2), preferred_element_type=F32)
            if r is not None:
                o = o * r
            oring[2 * g, pl.ds(rr, SEG), :] = o[2 * M:2 * M + SEG]
            oring[2 * g + 1, pl.ds(rr, SEG), :] = o[2 * M + SEG:]
            return o[:M], o[M:2 * M]

        def olhs(g, om, half):
            lo, hi = rows[half]
            return jnp.concatenate(
                [jnp.concatenate([om[c], oring[2 * g + c, pl.ds(rw + lo, hi - lo), :]], axis=0)
                 for c in range(2)], axis=1).astype(BF16)

        valid = u >= 2
        prow = W * (u - 2) + par * SEG
        row0 = pl.multiple_of(jnp.where(valid, prow, S + par * SEG), SEG)
        hrow0 = pl.multiple_of(
            jnp.where(valid & (layer == 0), S + prow, 2 * S + W + par * SEG), SEG)
        post(row0, rr, hrow0, valid, SEG)

        NST = NPAIR // 2
        st = [(i, i + NST) if par == 0 else (i + NST, i) for i in range(NST)]
        mres, prs, oms = {}, {}, {}
        acc = [None] * 4
        order = []
        for i in range(NST):
            order += [("qkv", g) for g in st[i]]
            if i >= 1:
                order += [("qk", g) for g in st[i - 1]]
            if i >= 2:
                order += [("pv", g) for g in st[i - 2]]
        oq = [g for i in range(NST) for g in st[i]]
        NE = 8
        order += [("o", g) for g in oq[0:3]]
        order += [("qk", g) for g in st[NST - 1]] + [("pv", g) for g in st[NST - 2]]
        order += [("o", g) for g in oq[3:7]]
        order += [("pv", g) for g in st[NST - 1]]
        order += [("o", g) for g in oq[7:NE]]
        norder = (2, 3, 0, 1) if par == 0 else (0, 1, 2, 3)
        order += [("on", n) for n in norder]
        for kind, g in order:
            if kind == "qkv":
                mres[g] = qkv(g, korder if g == st[0][0] else None)
            elif kind == "qk":
                prs[g] = qk(g, mres[g], g not in st[NST - 1] + st[NST - 2])
            elif kind == "pv":
                oms[g] = pv(g, mres[g], prs[g])
            elif kind == "o":
                for half in range(2):
                    y = jnp.dot(olhs(g, oms[g], half), wo_pair(g, half), preferred_element_type=F32)
                    for c in range(2):
                        yc = y[:, 128 * c:128 * (c + 1)]
                        n = 2 * half + c
                        acc[n] = yc if acc[n] is None else acc[n] + yc
            else:
                n = g
                l = jnp.concatenate([olhs(g2, oms[g2], n // 2) for g2 in oq[NE:]], axis=1)
                wn = jnp.concatenate([_w(wo[n, pl.ds(g2 * 128, 128), :]) for g2 in oq[NE:]], axis=0)
                acc[n] = acc[n] + jnp.dot(l, wn, preferred_element_type=F32)
        for n in range(4):
            lo, hi = rows[n // 2]
            abuf[pl.ds(rw + lo, hi - lo), pl.ds(n * 128, 128)] = acc[n][M:]

        return jnp.concatenate([acc[n][:M] for n in range(4)], axis=1), norder

    def layer_body(layer, carry):
        best[0] = jnp.full((8, 128), -jnp.inf, F32)
        best[1] = jnp.zeros((8, 128), F32)

        def dstep(u, mem):
            mem, lk_ = step(0, layer, u, mem, None)
            mem, _ = step(1, layer, u, mem, lk_)
            return mem

        jax.lax.fori_loop(0, NU, dstep, mem0_ref[...].astype(F32))

        acc = None
        for g in range(NPAIR):
            l = jnp.concatenate([oring[2 * g + c, pl.ds(W, W), :] for c in range(2)],
                                axis=1).astype(BF16)
            y = _dot(l, jnp.concatenate([wo_pair(g, 0), wo_pair(g, 1)], axis=1))
            acc = y if acc is None else acc + y
        abuf[pl.ds(W, W), :] = acc
        hlast = pl.multiple_of(jnp.where(layer == 0, 2 * S - 2 * W, 2 * S + W), W)
        hlast2 = pl.multiple_of(jnp.where(layer == 0, 2 * S - W, 2 * S + W), W)
        post(S - 2 * W, 0, hlast, True, W)
        post(S - W, W, hlast2, True, W)

        @pl.when(layer == 0)
        def _():
            for c in cp_f:
                c.wait()

        bv = best[0]
        bi = best[1]
        vmax = jnp.max(bv, axis=0, keepdims=True)
        imin = jnp.min(jnp.where(bv == vmax, bi, float(S)), axis=0, keepdims=True)
        idx = jnp.clip(jnp.min(imin).astype(jnp.int32), 0, S - 1)
        g0 = pl.multiple_of((idx // 16) * 16, 16)
        x1 = x1buf[pl.ds(g0, 16), :].astype(F32)
        hb = _ln(x1)
        hbb = hb.astype(BF16)
        gpre = _rb(_dot(hbb, wg[...]))
        gs = _rb(gpre * _rb(jax.nn.sigmoid(gpre)))
        up = _rb(_dot(hbb, wu[...]))
        y = _rb(_dot((gs * up).astype(BF16), wd[...]))
        rsel = _rb(jax.nn.sigmoid(vmax))[:, :1]
        y = _rb(y * rsel)
        x2 = _rb(x1 + _rb(hb + y))
        rowi = jax.lax.broadcasted_iota(jnp.int32, (16, D), 0) + g0
        x2 = jnp.where(rowi == idx, x2, xs[pl.ds(g0, 16), :].astype(F32))
        xs[pl.ds(g0, 16), :] = x2.astype(BF16)

        @pl.when(layer == 0)
        def _():
            hbuf[pl.ds(S + g0, 16), :] = _ln(x2)

            @pl.when(idx < W)
            def _():
                qkv_window(S, 0)

        return carry

    jax.lax.fori_loop(0, 2, layer_body, 0)

    cp_o = pltpu.make_async_copy(xs.at[pl.ds(0, S)], out_hbm, sems.at[0])
    cp_o.start()
    cp_o.wait()


@functools.partial(jax.jit, static_argnames=("A_seg_len",))
def pallas_interleave_layers__memory_aug_recurrent_mem_tr__moe_arch_mod__prompt_kernel(
    A_x: jax.Array,
    A_mem0: jax.Array,
    A_Wq: jax.Array,
    A_Wk: jax.Array,
    A_Wv: jax.Array,
    A_Wo: jax.Array,
    A_seg_len,
    B_x: jax.Array,
    B_w_r: jax.Array,
    B_w_gate: jax.Array,
    B_w_up: jax.Array,
    B_w_down: jax.Array,
):
    assert A_seg_len == SEG
    assert A_x.shape == (1, S, D) and A_Wq.shape == (D, H, E) and A_mem0.shape == (1, M, D)
    any_spec = pl.BlockSpec(memory_space=pl.ANY)
    vmem_spec = pl.BlockSpec(memory_space=pltpu.VMEM)
    out = pl.pallas_call(
        _kernel,
        out_shape=jax.ShapeDtypeStruct((S, D), BF16),
        in_specs=[any_spec, vmem_spec, any_spec, any_spec, any_spec, any_spec,
                  vmem_spec, any_spec, any_spec, any_spec],
        out_specs=any_spec,
        scratch_shapes=[
            pltpu.VMEM((S + 2 * W, D), BF16),
            pltpu.VMEM((S + 2 * W, D), BF16),
            pltpu.VMEM((2 * S + 2 * W, D), F32),
            pltpu.VMEM((3, D, H, E), BF16),
            pltpu.VMEM((6 * NPAIR, D // 2, E), U32),
            pltpu.VMEM((4, H * E, 128), BF16),
            pltpu.VMEM((4, H * E // 2, 128), U32),
            pltpu.VMEM((D, F), BF16),
            pltpu.VMEM((D, F), BF16),
            pltpu.VMEM((F, D), BF16),
            pltpu.VMEM((6 * NPAIR, 2 * W, E), F32),
            pltpu.VMEM((H, 2 * W, E), F32),
            pltpu.VMEM((2 * W, D), F32),
            pltpu.VMEM((L2, L2), F32),
            pltpu.VMEM((2, 8, 128), F32),
            pltpu.SemaphoreType.DMA((11,)),
        ],
        compiler_params=pltpu.CompilerParams(vmem_limit_bytes=110 * 1024 * 1024),
        name="rmt_mod",
    )(A_x.reshape(S, D), A_mem0.reshape(M, D), A_Wq, A_Wk, A_Wv, A_Wo.reshape(H * E, D),
      B_w_r.reshape(1, D), B_w_gate, B_w_up, B_w_down)
    return out.reshape(1, S, D)
```

```python
import functools

import jax
import jax.numpy as jnp
import jax.experimental.pallas as pl
import jax.experimental.pallas.tpu as pltpu

S = 2048
D = 512
H = 32
E = 128
M = 8
SEG = 32
F = 1792
NPAIR = H // 2
NU = S // (2 * SEG)
W = 2 * SEG
L2 = 2 * (M + SEG)
EPS = 1e-05
SCALE = float(E) ** -0.5
LOG2E = 1.4426950408889634
F32 = jnp.float32
BF16 = jnp.bfloat16
U32 = jnp.uint32


def _rb(x):
    return x.astype(BF16).astype(F32)


def _ln(x):
    mu = jnp.sum(x, axis=-1, keepdims=True) * (1.0 / D)
    xc0 = x - mu
    var = jnp.sum(xc0 * xc0, axis=-1, keepdims=True) * (1.0 / D)
    sd = _rb(jnp.sqrt(_rb(_rb(var) + EPS)))
    xc = _rb(x - _rb(mu))
    return _rb(xc * (1.0 / sd))


def _dot(a, b):
    return jnp.dot(a, b, preferred_element_type=F32)


def _w(ref_slab):
    return pltpu.bitcast(ref_slab, BF16)


XA = 4 * W
OB = 2 * W


def _kernel(x_hbm, mem0_ref, wq_hbm, wk_hbm, wv_hbm, wo_hbm, wr_ref, wg_hbm, wu_hbm, wd_hbm,
            out_hbm,
            xs, x1buf, raw, wqkv, wo_raw, wo, wg, wu, wd,
            ring0, ring1, oring0, oring1, abuf0, abuf1, hwin0, hwin1, maskv, best, sems):
    ring, oring, abuf, hwin = (ring0, ring1), (oring0, oring1), (abuf0, abuf1), (hwin0, hwin1)
    cp_xa = pltpu.make_async_copy(x_hbm.at[pl.ds(0, XA)], xs.at[pl.ds(0, XA)], sems.at[0])
    cp_xa.start()
    NCH = 4
    HC = H // NCH
    cp_w = {}
    for c in range(NCH):
        for i, w in enumerate((wq_hbm, wk_hbm, wv_hbm)):
            cp_w[c, i] = pltpu.make_async_copy(
                w.at[:, pl.ds(c * HC, HC), :], raw.at[i, c], sems.at[11 + 3 * c + i])
            cp_w[c, i].start()
    cp_wo = [pltpu.make_async_copy(wo_hbm.at[:, pl.ds(n * 128, 128)], wo_raw.at[n], sems.at[4 + n])
             for n in range(4)]
    for c in cp_wo:
        c.start()
    cp_xb = pltpu.make_async_copy(x_hbm.at[pl.ds(XA, S - XA)], xs.at[pl.ds(XA, S - XA)], sems.at[1])
    cp_xb.start()
    cp_f = [pltpu.make_async_copy(wg_hbm, wg, sems.at[8]),
            pltpu.make_async_copy(wu_hbm, wu, sems.at[9]),
            pltpu.make_async_copy(wd_hbm, wd, sems.at[10])]
    for c in cp_f:
        c.start()

    def out_copy(row0, n):
        return pltpu.make_async_copy(xs.at[pl.ds(row0, n)], out_hbm.at[pl.ds(row0, n)], sems.at[2])

    oring1[...] = jnp.zeros(oring1.shape, F32)
    abuf0[...] = jnp.zeros(abuf0.shape, F32)
    xs[pl.ds(S, W), :] = jnp.zeros((W, D), BF16)

    ri = jax.lax.broadcasted_iota(jnp.int32, (L2, L2), 0)
    ci = jax.lax.broadcasted_iota(jnp.int32, (L2, L2), 1)

    def head_of(i):
        return jnp.where(i < 2 * M, i // M, (i - 2 * M) // SEG)

    def pos_of(i):
        return jnp.where(i < 2 * M, i % M, M + (i - 2 * M) % SEG)

    same = head_of(ri) == head_of(ci)
    ok = (pos_of(ri) < M) | (pos_of(ri) >= pos_of(ci))
    maskv[...] = jnp.where(same, jnp.where(ok, 0.0, -1e9 / SCALE), -jnp.inf).astype(F32)

    cp_xa.wait()
    hwin0[...] = _ln(xs[pl.ds(0, W), :].astype(F32))
    hwin1[...] = _ln(xs[pl.ds(W, W), :].astype(F32))

    for c in range(NCH):
        for i in range(3):
            cp_w[c, i].wait()

            def relay(db, carry, i=i, c=c):
                d0 = pl.multiple_of(db * 64, 64)
                for sb in range(4):
                    a = jnp.swapaxes(raw[i, c, pl.ds(d0 + 16 * sb, 16)], 0, 1)
                    p0 = pl.multiple_of(db * 32 + 8 * sb, 8)
                    for hh in range(HC):
                        h = c * HC + hh
                        t = (h // 2) * 6 + 2 * i + (h % 2)
                        wqkv[t, pl.ds(p0, 8), :] = pltpu.bitcast(a[hh], U32)
                return carry

            jax.lax.fori_loop(0, D // 64, relay, 0)
            lhs0 = hwin0[...].astype(BF16)
            for hh in range(HC):
                h = c * HC + hh
                t = (h // 2) * 6 + 2 * i + (h % 2)
                ring0[t] = _dot(lhs0, _w(wqkv[t]))

    for n in range(4):
        cp_wo[n].wait()

        def cpwo(k, c, n=n):
            k0 = pl.multiple_of(k * 512, 512)
            p0 = pl.multiple_of(k * 256, 256)
            wo[n, pl.ds(p0, 256), :] = pltpu.bitcast(wo_raw[n, pl.ds(k0, 512), :], U32)
            return c

        jax.lax.fori_loop(0, H * E // 512, cpwo, 0)

    def post(row0, a, valid):
        n = a.shape[0]
        x1 = _rb(xs[pl.ds(row0, n), :].astype(F32) + _rb(a))
        x1buf[pl.ds(row0, n), :] = x1.astype(BF16)
        hb = _ln(x1)
        r = _rb(jnp.sum(hb * wr_ref[...].astype(F32), axis=-1, keepdims=True))
        xs[pl.ds(row0, n), :] = (x1 + hb).astype(BF16)
        if valid is not True:
            r = jnp.where(valid, r, -jnp.inf)
        bv = best[0]
        bi = best[1]
        sub = jax.lax.broadcasted_iota(jnp.int32, (8, 128), 0).astype(F32)
        for g in range(n // 8):
            rg = jnp.broadcast_to(r[8 * g:8 * g + 8], (8, 128))
            ig = sub + (float(row0 + 8 * g) if isinstance(row0, int) else (row0 + 8 * g).astype(F32))
            gt = rg > bv
            bv = jnp.where(gt, rg, bv)
            bi = jnp.where(gt, ig, bi)
        best[0] = bv
        best[1] = bi

    def wo_pair(g, half):
        return jnp.concatenate(
            [_w(wo[2 * half + c, pl.ds(g * 128, 128), :]) for c in range(2)], axis=1)

    def step(q, par, u, mem, korder):
        rr = par * SEG
        if par == 0:
            rows = ((0, 40), (0, 24))
        else:
            rows = ((40, 64), (24, 64))
        lhs = [jnp.concatenate([mem, hwin[1 - q][lo:hi, :]], axis=0).astype(BF16)
               for lo, hi in rows]

        def qkv(g, korder=None):
            half = g // (NPAIR // 2)
            lo, hi = rows[half]
            res = []
            ys = {}
            if korder is not None:
                part = None
                for k in korder:
                    wk = jnp.concatenate([_w(wqkv[6 * g + t, pl.ds(64 * k, 64), :])
                                          for t in range(4)], axis=1)
                    y = jnp.dot(lhs[half][:, 128 * k:128 * (k + 1)], wk,
                                preferred_element_type=F32)
                    part = y if part is None else part + y
                for t in range(4):
                    ys[t] = part[:, 128 * t:128 * (t + 1)]
            for t in range(6):
                if t in ys:
                    y = ys[t]
                else:
                    y = jnp.dot(lhs[half], _w(wqkv[6 * g + t]), preferred_element_type=F32)
                ring[1 - q][6 * g + t, lo:hi, :] = y[M:]
                res.append(y[:M])
            return res

        def stack(g, mres, i):
            return jnp.concatenate(
                [mres[2 * i], mres[2 * i + 1],
                 ring[q][6 * g + 2 * i, rr:rr + SEG, :],
                 ring[q][6 * g + 2 * i + 1, rr:rr + SEG, :]], axis=0).astype(BF16)

        def qk(g, mres, prenorm):
            q2, k2 = stack(g, mres, 0), stack(g, mres, 1)
            s = jax.lax.dot_general(q2, k2, (((1,), (1,)), ((), ())), preferred_element_type=F32)
            mk = maskv[...]
            s = jnp.where(mk == 0.0, s, mk)
            mx = jnp.max(s, axis=-1, keepdims=True)
            p = jnp.exp2((s - mx) * (SCALE * LOG2E))
            l = jnp.sum(p, axis=-1, keepdims=True)
            r0 = pl.reciprocal(l, approx=True)
            r = r0 * (2.0 - l * r0)
            if prenorm:
                return (p * r).astype(BF16), None
            return p.astype(BF16), r

        def pv(g, mres, pr):
            p, r = pr
            o = jnp.dot(p, stack(g, mres, 2), preferred_element_type=F32)
            if r is not None:
                o = o * r
            oring[q][2 * g, rr:rr + SEG, :] = o[2 * M:2 * M + SEG]
            oring[q][2 * g + 1, rr:rr + SEG, :] = o[2 * M + SEG:]
            return o[:M], o[M:2 * M]

        def olhs(g, om, half):
            lo, hi = rows[half]
            return jnp.concatenate(
                [jnp.concatenate([om[c], oring[1 - q][2 * g + c, lo:hi, :]], axis=0)
                 for c in range(2)], axis=1).astype(BF16)

        prow = pl.multiple_of(((u + 2) % NU) * W + rr, SEG)
        hwin[q][rr:rr + SEG, :] = _ln(xs[pl.ds(prow, SEG), :].astype(F32))
        valid = u >= 2
        row0 = pl.multiple_of(jnp.where(valid, W * (u - 2), S) + rr, SEG)
        post(row0, abuf[q][rr:rr + SEG, :], valid)

        NST = NPAIR // 2
        st = [(i, i + NST) if par == 0 else (i + NST, i) for i in range(NST)]
        mres, prs, oms = {}, {}, {}
        acc = [None] * 4
        order = []
        for i in range(NST):
            order += [("qkv", g) for g in st[i]]
            if i >= 1:
                order += [("qk", g) for g in st[i - 1]]
            if i >= 2:
                order += [("pv", g) for g in st[i - 2]]
        oq = [g for i in range(NST) for g in st[i]]
        NE = 8
        order += [("o", g) for g in oq[0:3]]
        order += [("qk", g) for g in st[NST - 1]] + [("pv", g) for g in st[NST - 2]]
        order += [("o", g) for g in oq[3:7]]
        order += [("pv", g) for g in st[NST - 1]]
        order += [("o", g) for g in oq[7:NE]]
        norder = (2, 3, 0, 1) if par == 0 else (0, 1, 2, 3)
        order += [("on", n) for n in norder]
        for kind, g in order:
            if kind == "qkv":
                mres[g] = qkv(g, korder if g == st[0][0] else None)
            elif kind == "qk":
                prs[g] = qk(g, mres[g], g not in st[NST - 1] + st[NST - 2])
            elif kind == "pv":
                oms[g] = pv(g, mres[g], prs[g])
            elif kind == "o":
                for half in range(2):
                    y = jnp.dot(olhs(g, oms[g], half), wo_pair(g, half), preferred_element_type=F32)
                    for c in range(2):
                        yc = y[:, 128 * c:128 * (c + 1)]
                        n = 2 * half + c
                        acc[n] = yc if acc[n] is None else acc[n] + yc
            else:
                n = g
                l = jnp.concatenate([olhs(g2, oms[g2], n // 2) for g2 in oq[NE:]], axis=1)
                wn = jnp.concatenate([_w(wo[n, pl.ds(g2 * 128, 128), :]) for g2 in oq[NE:]], axis=0)
                acc[n] = acc[n] + jnp.dot(l, wn, preferred_element_type=F32)
        for n in range(4):
            lo, hi = rows[n // 2]
            abuf[1 - q][lo:hi, n * 128:(n + 1) * 128] = acc[n][M:]

        return jnp.concatenate([acc[n][:M] for n in range(4)], axis=1), norder

    def layer_body(layer, carry):
        best[0] = jnp.full((8, 128), -jnp.inf, F32)
        best[1] = jnp.zeros((8, 128), F32)

        def qstep(j, mem):
            @pl.when((layer == 0) & (j == 1))
            def _():
                cp_xb.wait()

            @pl.when((layer == 1) & (j >= 2))
            def _():
                out_copy(pl.multiple_of((j - 2) * OB, OB), OB).start()

            ko = None
            for q in range(2):
                for par in range(2):
                    mem, ko = step(q, par, 2 * j + q, mem, ko)
            return mem

        jax.lax.fori_loop(0, NU // 2, qstep, mem0_ref[...].astype(F32))

        @pl.when(layer == 1)
        def _():
            out_copy(S - 2 * OB, OB).start()

        post(S - 2 * W, abuf0[...], True)
        acc = None
        for g in range(NPAIR):
            l = jnp.concatenate([oring1[2 * g + c] for c in range(2)], axis=1).astype(BF16)
            y = _dot(l, jnp.concatenate([wo_pair(g, 0), wo_pair(g, 1)], axis=1))
            acc = y if acc is None else acc + y
        post(S - W, acc, True)

        @pl.when(layer == 0)
        def _():
            for c in cp_f:
                c.wait()

        bv = best[0]
        bi = best[1]
        vmax = jnp.max(bv, axis=0, keepdims=True)
        imin = jnp.min(jnp.where(bv == vmax, bi, float(S)), axis=0, keepdims=True)
        idx = jnp.clip(jnp.min(imin).astype(jnp.int32), 0, S - 1)
        g0 = pl.multiple_of((idx // 16) * 16, 16)
        x1 = x1buf[pl.ds(g0, 16), :].astype(F32)
        hb = _ln(x1)
        hbb = hb.astype(BF16)
        gpre = _rb(_dot(hbb, wg[...]))
        gs = _rb(gpre * _rb(jax.nn.sigmoid(gpre)))
        up = _rb(_dot(hbb, wu[...]))
        y = _rb(_dot((gs * up).astype(BF16), wd[...]))
        rsel = _rb(jax.nn.sigmoid(vmax))[:, :1]
        y = _rb(y * rsel)
        x2 = _rb(x1 + _rb(hb + y))
        rowi = jax.lax.broadcasted_iota(jnp.int32, (16, D), 0) + g0

        @pl.when(layer == 1)
        def _():
            for _i in range(S // OB - 1):
                out_copy(0, OB).wait()

        xs[pl.ds(g0, 16), :] = jnp.where(
            rowi == idx, x2, xs[pl.ds(g0, 16), :].astype(F32)).astype(BF16)

        @pl.when(layer == 0)
        def _():
            @pl.when(idx < 2 * W)
            def _():
                hwin1[...] = _ln(xs[pl.ds(W, W), :].astype(F32))
                lhs = _ln(xs[pl.ds(0, W), :].astype(F32)).astype(BF16)

                def body(t, c):
                    ring0[t] = _dot(lhs, _w(wqkv[t]))
                    return c

                jax.lax.fori_loop(0, 6 * NPAIR, body, 0, unroll=4)

        @pl.when(layer == 1)
        def _():
            last = out_copy(S - OB, OB)
            last.start()

            @pl.when(g0 < S - OB)
            def _():
                fix = pltpu.make_async_copy(xs.at[pl.ds(g0, 16)], out_hbm.at[pl.ds(g0, 16)],
                                            sems.at[3])
                fix.start()
                fix.wait()

            last.wait()

        return carry

    jax.lax.fori_loop(0, 2, layer_body, 0)


@functools.partial(jax.jit, static_argnames=("A_seg_len",))
def pallas_interleave_layers__memory_aug_recurrent_mem_tr__moe_arch_mod__prompt_kernel(
    A_x: jax.Array,
    A_mem0: jax.Array,
    A_Wq: jax.Array,
    A_Wk: jax.Array,
    A_Wv: jax.Array,
    A_Wo: jax.Array,
    A_seg_len,
    B_x: jax.Array,
    B_w_r: jax.Array,
    B_w_gate: jax.Array,
    B_w_up: jax.Array,
    B_w_down: jax.Array,
):
    assert A_seg_len == SEG
    assert A_x.shape == (1, S, D) and A_Wq.shape == (D, H, E) and A_mem0.shape == (1, M, D)
    any_spec = pl.BlockSpec(memory_space=pl.ANY)
    vmem_spec = pl.BlockSpec(memory_space=pltpu.VMEM)
    out = pl.pallas_call(
        _kernel,
        out_shape=jax.ShapeDtypeStruct((S, D), BF16),
        in_specs=[any_spec, vmem_spec, any_spec, any_spec, any_spec, any_spec,
                  vmem_spec, any_spec, any_spec, any_spec],
        out_specs=any_spec,
        scratch_shapes=[
            pltpu.VMEM((S + W, D), BF16),
            pltpu.VMEM((S + W, D), BF16),
            pltpu.VMEM((3, 4, D, H // 4, E), BF16),
            pltpu.VMEM((6 * NPAIR, D // 2, E), U32),
            pltpu.VMEM((4, H * E, 128), BF16),
            pltpu.VMEM((4, H * E // 2, 128), U32),
            pltpu.VMEM((D, F), BF16),
            pltpu.VMEM((D, F), BF16),
            pltpu.VMEM((F, D), BF16),
            pltpu.VMEM((6 * NPAIR, W, E), F32),
            pltpu.VMEM((6 * NPAIR, W, E), F32),
            pltpu.VMEM((H, W, E), F32),
            pltpu.VMEM((H, W, E), F32),
            pltpu.VMEM((W, D), F32),
            pltpu.VMEM((W, D), F32),
            pltpu.VMEM((W, D), F32),
            pltpu.VMEM((W, D), F32),
            pltpu.VMEM((L2, L2), F32),
            pltpu.VMEM((2, 8, 128), F32),
            pltpu.SemaphoreType.DMA((23,)),
        ],
        compiler_params=pltpu.CompilerParams(vmem_limit_bytes=110 * 1024 * 1024),
        name="rmt_mod",
    )(A_x.reshape(S, D), A_mem0.reshape(M, D), A_Wq, A_Wk, A_Wv, A_Wo.reshape(H * E, D),
      B_w_r.reshape(1, D), B_w_gate, B_w_up, B_w_down)
    return out.reshape(1, S, D)
```

```python
import functools

import jax
import jax.numpy as jnp
import jax.experimental.pallas as pl
import jax.experimental.pallas.tpu as pltpu

S = 2048
D = 512
H = 32
E = 128
M = 8
SEG = 32
F = 1792
NPAIR = H // 2
NU = S // (2 * SEG)
W = 2 * SEG
L2 = 2 * (M + SEG)
EPS = 1e-05
SCALE = float(E) ** -0.5
LOG2E = 1.4426950408889634
F32 = jnp.float32
BF16 = jnp.bfloat16
U32 = jnp.uint32


def _rb(x):
    return x.astype(BF16).astype(F32)


def _ln(x):
    mu = jnp.sum(x, axis=-1, keepdims=True) * (1.0 / D)
    xc0 = x - mu
    var = jnp.sum(xc0 * xc0, axis=-1, keepdims=True) * (1.0 / D)
    sd = _rb(jnp.sqrt(_rb(_rb(var) + EPS)))
    xc = _rb(x - _rb(mu))
    return _rb(xc * (1.0 / sd))


def _dot(a, b):
    return jnp.dot(a, b, preferred_element_type=F32)


def _w(ref_slab):
    return pltpu.bitcast(ref_slab, BF16)


XA = 4 * W
OB = 2 * W


def _tok(*vals):
    parts = []
    for v in vals:
        if v.shape[1] < 128:
            v = jnp.broadcast_to(v[:, :1], (v.shape[0], 128))
        for i in range(v.shape[0] // 8):
            for j in range(v.shape[1] // 128):
                parts.append(v[8 * i:8 * i + 8, 128 * j:128 * j + 128])
    while len(parts) > 1:
        parts = [jnp.maximum(parts[i], parts[i + 1]) if i + 1 < len(parts) else parts[i]
                 for i in range(0, len(parts), 2)]
    return parts[0]


def _kernel(x_hbm, mem0_ref, wq_hbm, wk_hbm, wv_hbm, wo_hbm, wr_ref, wg_hbm, wu_hbm, wd_hbm,
            out_hbm,
            xs, x1buf, raw, wqkv, wo_raw, wo, wg, wu, wd,
            ring0, ring1, oring0, oring1, abuf0, abuf1, hwin0, hwin1, maskv, best, zflag, sems):
    ring, oring, abuf, hwin = (ring0, ring1), (oring0, oring1), (abuf0, abuf1), (hwin0, hwin1)
    cp_xa = pltpu.make_async_copy(x_hbm.at[pl.ds(0, XA)], xs.at[pl.ds(0, XA)], sems.at[0])
    cp_xa.start()
    NCH = 4
    HC = H // NCH
    cp_w = {}
    for c in range(NCH):
        for i, w in enumerate((wq_hbm, wk_hbm, wv_hbm)):
            cp_w[c, i] = pltpu.make_async_copy(
                w.at[:, pl.ds(c * HC, HC), :], raw.at[i, c], sems.at[11 + 3 * c + i])
            cp_w[c, i].start()
    cp_wo = [pltpu.make_async_copy(wo_hbm.at[:, pl.ds(n * 128, 128)], wo_raw.at[n], sems.at[4 + n])
             for n in range(4)]
    for c in cp_wo:
        c.start()
    cp_xb = pltpu.make_async_copy(x_hbm.at[pl.ds(XA, S - XA)], xs.at[pl.ds(XA, S - XA)], sems.at[1])
    cp_xb.start()
    cp_f = [pltpu.make_async_copy(wg_hbm, wg, sems.at[8]),
            pltpu.make_async_copy(wu_hbm, wu, sems.at[9]),
            pltpu.make_async_copy(wd_hbm, wd, sems.at[10])]
    for c in cp_f:
        c.start()

    def out_copy(row0, n):
        return pltpu.make_async_copy(xs.at[pl.ds(row0, n)], out_hbm.at[pl.ds(row0, n)], sems.at[2])

    oring1[...] = jnp.zeros(oring1.shape, F32)
    abuf0[...] = jnp.zeros(abuf0.shape, F32)
    xs[pl.ds(S, W), :] = jnp.zeros((W, D), BF16)
    zflag[...] = jnp.zeros(zflag.shape, jnp.int32)

    ri = jax.lax.broadcasted_iota(jnp.int32, (L2, L2), 0)
    ci = jax.lax.broadcasted_iota(jnp.int32, (L2, L2), 1)

    def head_of(i):
        return jnp.where(i < 2 * M, i // M, (i - 2 * M) // SEG)

    def pos_of(i):
        return jnp.where(i < 2 * M, i % M, M + (i - 2 * M) % SEG)

    same = head_of(ri) == head_of(ci)
    ok = (pos_of(ri) < M) | (pos_of(ri) >= pos_of(ci))
    maskv[...] = jnp.where(same, jnp.where(ok, 0.0, -1e9 / SCALE), -jnp.inf).astype(F32)

    cp_xa.wait()
    hwin0[...] = _ln(xs[pl.ds(0, W), :].astype(F32))
    hwin1[...] = _ln(xs[pl.ds(W, W), :].astype(F32))

    for c in range(NCH):
        for i in range(3):
            cp_w[c, i].wait()

            def relay(db, carry, i=i, c=c):
                d0 = pl.multiple_of(db * 64, 64)
                for sb in range(4):
                    a = jnp.swapaxes(raw[i, c, pl.ds(d0 + 16 * sb, 16)], 0, 1)
                    p0 = pl.multiple_of(db * 32 + 8 * sb, 8)
                    for hh in range(HC):
                        h = c * HC + hh
                        t = (h // 2) * 6 + 2 * i + (h % 2)
                        wqkv[t, pl.ds(p0, 8), :] = pltpu.bitcast(a[hh], U32)
                return carry

            jax.lax.fori_loop(0, D // 64, relay, 0)
            lhs0 = hwin0[...].astype(BF16)
            for hh in range(HC):
                h = c * HC + hh
                t = (h // 2) * 6 + 2 * i + (h % 2)
                ring0[t] = _dot(lhs0, _w(wqkv[t]))

    for n in range(4):
        cp_wo[n].wait()

        def cpwo(k, c, n=n):
            k0 = pl.multiple_of(k * 512, 512)
            p0 = pl.multiple_of(k * 256, 256)
            wo[n, pl.ds(p0, 256), :] = pltpu.bitcast(wo_raw[n, pl.ds(k0, 512), :], U32)
            return c

        jax.lax.fori_loop(0, H * E // 512, cpwo, 0)

    def post(row0, a, valid):
        n = a.shape[0]
        x1 = _rb(xs[pl.ds(row0, n), :].astype(F32) + _rb(a))
        x1buf[pl.ds(row0, n), :] = x1.astype(BF16)
        hb = _ln(x1)
        r = _rb(jnp.sum(hb * wr_ref[...].astype(F32), axis=-1, keepdims=True))
        x2 = x1 + hb
        xs[pl.ds(row0, n), :] = x2.astype(BF16)
        if valid is not True:
            r = jnp.where(valid, r, -jnp.inf)
        bv = best[0]
        bi = best[1]
        sub = jax.lax.broadcasted_iota(jnp.int32, (8, 128), 0).astype(F32)
        for g in range(n // 8):
            rg = jnp.broadcast_to(r[8 * g:8 * g + 8], (8, 128))
            ig = sub + (float(row0 + 8 * g) if isinstance(row0, int) else (row0 + 8 * g).astype(F32))
            gt = rg > bv
            bv = jnp.where(gt, rg, bv)
            bi = jnp.where(gt, ig, bi)
        best[0] = bv
        best[1] = bi
        return _tok(x2, bv, bi)

    def anchor(val, tok):
        return jnp.where(zflag[...] != 0, tok, val)

    def wo_pair(g, half):
        return jnp.concatenate(
            [_w(wo[2 * half + c, pl.ds(g * 128, 128), :]) for c in range(2)], axis=1)

    def step(q, par, u, mem, korder):
        rr = par * SEG
        if par == 0:
            rows = ((0, 40), (0, 24))
        else:
            rows = ((40, 64), (24, 64))
        lhs = [jnp.concatenate([mem, hwin[1 - q][lo:hi, :]], axis=0).astype(BF16)
               for lo, hi in rows]

        def qkv(g, korder=None):
            half = g // (NPAIR // 2)
            lo, hi = rows[half]
            res = []
            ys = {}
            if korder is not None:
                part = None
                for k in korder:
                    wk = jnp.concatenate([_w(wqkv[6 * g + t, pl.ds(64 * k, 64), :])
                                          for t in range(4)], axis=1)
                    y = jnp.dot(lhs[half][:, 128 * k:128 * (k + 1)], wk,
                                preferred_element_type=F32)
                    part = y if part is None else part + y
                for t in range(4):
                    ys[t] = part[:, 128 * t:128 * (t + 1)]
            for t in range(6):
                if t in ys:
                    y = ys[t]
                else:
                    y = jnp.dot(lhs[half], _w(wqkv[6 * g + t]), preferred_element_type=F32)
                ring[1 - q][6 * g + t, lo:hi, :] = y[M:]
                res.append(y[:M])
            return res

        def stack(g, mres, i):
            return jnp.concatenate(
                [mres[2 * i], mres[2 * i + 1],
                 ring[q][6 * g + 2 * i, rr:rr + SEG, :],
                 ring[q][6 * g + 2 * i + 1, rr:rr + SEG, :]], axis=0).astype(BF16)

        def qk(g, mres, prenorm):
            q2, k2 = stack(g, mres, 0), stack(g, mres, 1)
            s = jax.lax.dot_general(q2, k2, (((1,), (1,)), ((), ())), preferred_element_type=F32)
            mk = maskv[...]
            s = jnp.where(mk == 0.0, s, mk)
            mx = jnp.max(s, axis=-1, keepdims=True)
            p = jnp.exp2((s - mx) * (SCALE * LOG2E))
            l = jnp.sum(p, axis=-1, keepdims=True)
            r0 = pl.reciprocal(l, approx=True)
            r = r0 * (2.0 - l * r0)
            if prenorm:
                return (p * r).astype(BF16), None
            return p.astype(BF16), r

        def pv(g, mres, pr):
            p, r = pr
            o = jnp.dot(p, stack(g, mres, 2), preferred_element_type=F32)
            if r is not None:
                o = o * r
            oring[q][2 * g, rr:rr + SEG, :] = o[2 * M:2 * M + SEG]
            oring[q][2 * g + 1, rr:rr + SEG, :] = o[2 * M + SEG:]
            return o[:M], o[M:2 * M]

        def olhs(g, om, half):
            lo, hi = rows[half]
            return jnp.concatenate(
                [jnp.concatenate([om[c], oring[1 - q][2 * g + c, lo:hi, :]], axis=0)
                 for c in range(2)], axis=1).astype(BF16)

        prow = pl.multiple_of(((u + 2) % NU) * W + rr, SEG)
        hpre = _ln(xs[pl.ds(prow, SEG), :].astype(F32))
        hwin[q][rr:rr + SEG, :] = hpre
        tok_pre = _tok(hpre)
        valid = u >= 2
        row0 = pl.multiple_of(jnp.where(valid, W * (u - 2), S) + rr, SEG)
        tok_post = post(row0, abuf[q][rr:rr + SEG, :], valid)

        NST = NPAIR // 2
        st = [(i, i + NST) if par == 0 else (i + NST, i) for i in range(NST)]
        mres, prs, oms = {}, {}, {}
        acc = [None] * 4
        order = []
        for i in range(NST):
            order += [("qkv", g) for g in st[i]]
            if i >= 1:
                order += [("qk", g) for g in st[i - 1]]
            if i >= 2:
                order += [("pv", g) for g in st[i - 2]]
        oq = [g for i in range(NST) for g in st[i]]
        NE = 8
        order += [("o", g) for g in oq[0:3]]
        order += [("qk", g) for g in st[NST - 1]] + [("pv", g) for g in st[NST - 2]]
        order += [("o", g) for g in oq[3:7]]
        order += [("pv", g) for g in st[NST - 1]]
        order += [("o", g) for g in oq[7:NE]]
        norder = (2, 3, 0, 1) if par == 0 else (0, 1, 2, 3)
        order += [("on", n) for n in norder]
        for kind, g in order:
            if kind == "qkv":
                mres[g] = qkv(g, korder if g == st[0][0] else None)
                if g == st[2][0]:
                    mres[g][0] = anchor(mres[g][0], tok_pre)
                if g == st[4][0]:
                    mres[g][0] = anchor(mres[g][0], tok_post)
            elif kind == "qk":
                prs[g] = qk(g, mres[g], g not in st[NST - 1] + st[NST - 2])
            elif kind == "pv":
                oms[g] = pv(g, mres[g], prs[g])
                if prs[g][1] is not None:
                    oms[g] = (anchor(oms[g][0], _tok(prs[g][1][2 * M:])), oms[g][1])
            elif kind == "o":
                for half in range(2):
                    y = jnp.dot(olhs(g, oms[g], half), wo_pair(g, half), preferred_element_type=F32)
                    for c in range(2):
                        yc = y[:, 128 * c:128 * (c + 1)]
                        n = 2 * half + c
                        acc[n] = yc if acc[n] is None else acc[n] + yc
            else:
                n = g
                l = jnp.concatenate([olhs(g2, oms[g2], n // 2) for g2 in oq[NE:]], axis=1)
                wn = jnp.concatenate([_w(wo[n, pl.ds(g2 * 128, 128), :]) for g2 in oq[NE:]], axis=0)
                acc[n] = acc[n] + jnp.dot(l, wn, preferred_element_type=F32)
        for n in range(4):
            lo, hi = rows[n // 2]
            abuf[1 - q][lo:hi, n * 128:(n + 1) * 128] = acc[n][M:]

        return jnp.concatenate([acc[n][:M] for n in range(4)], axis=1), norder

    def layer_body(layer, carry):
        best[0] = jnp.full((8, 128), -jnp.inf, F32)
        best[1] = jnp.zeros((8, 128), F32)

        def qstep(j, mem):
            @pl.when((layer == 0) & (j == 1))
            def _():
                cp_xb.wait()

            @pl.when((layer == 1) & (j >= 2))
            def _():
                out_copy(pl.multiple_of((j - 2) * OB, OB), OB).start()

            ko = None
            for q in range(2):
                for par in range(2):
                    mem, ko = step(q, par, 2 * j + q, mem, ko)
            return mem

        jax.lax.fori_loop(0, NU // 2, qstep, mem0_ref[...].astype(F32))

        @pl.when(layer == 1)
        def _():
            out_copy(S - 2 * OB, OB).start()

        post(S - 2 * W, abuf0[...], True)
        acc = None
        for g in range(NPAIR):
            l = jnp.concatenate([oring1[2 * g + c] for c in range(2)], axis=1).astype(BF16)
            y = _dot(l, jnp.concatenate([wo_pair(g, 0), wo_pair(g, 1)], axis=1))
            acc = y if acc is None else acc + y
        post(S - W, acc, True)

        @pl.when(layer == 0)
        def _():
            for c in cp_f:
                c.wait()

        bv = best[0]
        bi = best[1]
        vmax = jnp.max(bv, axis=0, keepdims=True)
        imin = jnp.min(jnp.where(bv == vmax, bi, float(S)), axis=0, keepdims=True)
        idx = jnp.clip(jnp.min(imin).astype(jnp.int32), 0, S - 1)
        g0 = pl.multiple_of((idx // 16) * 16, 16)
        x1 = x1buf[pl.ds(g0, 16), :].astype(F32)
        hb = _ln(x1)
        hbb = hb.astype(BF16)
        gpre = _rb(_dot(hbb, wg[...]))
        gs = _rb(gpre * _rb(jax.nn.sigmoid(gpre)))
        up = _rb(_dot(hbb, wu[...]))
        y = _rb(_dot((gs * up).astype(BF16), wd[...]))
        rsel = _rb(jax.nn.sigmoid(vmax))[:, :1]
        y = _rb(y * rsel)
        x2 = _rb(x1 + _rb(hb + y))
        rowi = jax.lax.broadcasted_iota(jnp.int32, (16, D), 0) + g0

        @pl.when(layer == 1)
        def _():
            for _i in range(S // OB - 1):
                out_copy(0, OB).wait()

        xs[pl.ds(g0, 16), :] = jnp.where(
            rowi == idx, x2, xs[pl.ds(g0, 16), :].astype(F32)).astype(BF16)

        @pl.when(layer == 0)
        def _():
            @pl.when(idx < 2 * W)
            def _():
                hwin1[...] = _ln(xs[pl.ds(W, W), :].astype(F32))
                lhs = _ln(xs[pl.ds(0, W), :].astype(F32)).astype(BF16)

                def body(t, c):
                    ring0[t] = _dot(lhs, _w(wqkv[t]))
                    return c

                jax.lax.fori_loop(0, 6 * NPAIR, body, 0, unroll=4)

        @pl.when(layer == 1)
        def _():
            last = out_copy(S - OB, OB)
            last.start()

            @pl.when(g0 < S - OB)
            def _():
                fix = pltpu.make_async_copy(xs.at[pl.ds(g0, 16)], out_hbm.at[pl.ds(g0, 16)],
                                            sems.at[3])
                fix.start()
                fix.wait()

            last.wait()

        return carry

    jax.lax.fori_loop(0, 2, layer_body, 0)


@functools.partial(jax.jit, static_argnames=("A_seg_len",))
def pallas_interleave_layers__memory_aug_recurrent_mem_tr__moe_arch_mod__prompt_kernel(
    A_x: jax.Array,
    A_mem0: jax.Array,
    A_Wq: jax.Array,
    A_Wk: jax.Array,
    A_Wv: jax.Array,
    A_Wo: jax.Array,
    A_seg_len,
    B_x: jax.Array,
    B_w_r: jax.Array,
    B_w_gate: jax.Array,
    B_w_up: jax.Array,
    B_w_down: jax.Array,
):
    assert A_seg_len == SEG
    assert A_x.shape == (1, S, D) and A_Wq.shape == (D, H, E) and A_mem0.shape == (1, M, D)
    any_spec = pl.BlockSpec(memory_space=pl.ANY)
    vmem_spec = pl.BlockSpec(memory_space=pltpu.VMEM)
    out = pl.pallas_call(
        _kernel,
        out_shape=jax.ShapeDtypeStruct((S, D), BF16),
        in_specs=[any_spec, vmem_spec, any_spec, any_spec, any_spec, any_spec,
                  vmem_spec, any_spec, any_spec, any_spec],
        out_specs=any_spec,
        scratch_shapes=[
            pltpu.VMEM((S + W, D), BF16),
            pltpu.VMEM((S + W, D), BF16),
            pltpu.VMEM((3, 4, D, H // 4, E), BF16),
            pltpu.VMEM((6 * NPAIR, D // 2, E), U32),
            pltpu.VMEM((4, H * E, 128), BF16),
            pltpu.VMEM((4, H * E // 2, 128), U32),
            pltpu.VMEM((D, F), BF16),
            pltpu.VMEM((D, F), BF16),
            pltpu.VMEM((F, D), BF16),
            pltpu.VMEM((6 * NPAIR, W, E), F32),
            pltpu.VMEM((6 * NPAIR, W, E), F32),
            pltpu.VMEM((H, W, E), F32),
            pltpu.VMEM((H, W, E), F32),
            pltpu.VMEM((W, D), F32),
            pltpu.VMEM((W, D), F32),
            pltpu.VMEM((W, D), F32),
            pltpu.VMEM((W, D), F32),
            pltpu.VMEM((L2, L2), F32),
            pltpu.VMEM((2, 8, 128), F32),
            pltpu.VMEM((8, 128), jnp.int32),
            pltpu.SemaphoreType.DMA((23,)),
        ],
        compiler_params=pltpu.CompilerParams(vmem_limit_bytes=110 * 1024 * 1024),
        name="rmt_mod",
    )(A_x.reshape(S, D), A_mem0.reshape(M, D), A_Wq, A_Wk, A_Wv, A_Wo.reshape(H * E, D),
      B_w_r.reshape(1, D), B_w_gate, B_w_up, B_w_down)
    return out.reshape(1, S, D)
```

```python
import functools

import jax
import jax.numpy as jnp
import jax.experimental.pallas as pl
import jax.experimental.pallas.tpu as pltpu

S = 2048
D = 512
H = 32
E = 128
M = 8
SEG = 32
F = 1792
NPAIR = H // 2
NU = S // (2 * SEG)
W = 2 * SEG
L2 = 2 * (M + SEG)
EPS = 1e-05
SCALE = float(E) ** -0.5
LOG2E = 1.4426950408889634
F32 = jnp.float32
BF16 = jnp.bfloat16
U32 = jnp.uint32


def _rb(x):
    return x.astype(BF16).astype(F32)


def _ln(x):
    mu = jnp.sum(x, axis=-1, keepdims=True) * (1.0 / D)
    xc0 = x - mu
    var = jnp.sum(xc0 * xc0, axis=-1, keepdims=True) * (1.0 / D)
    sd = _rb(jnp.sqrt(_rb(_rb(var) + EPS)))
    xc = _rb(x - _rb(mu))
    return _rb(xc * (1.0 / sd))


def _dot(a, b):
    return jnp.dot(a, b, preferred_element_type=F32)


def _w(ref_slab):
    return pltpu.bitcast(ref_slab, BF16)


NLP = 12
P0 = 1072
LR = 24
XC = 384
XLN = 3 * XC
XA = XLN + W
FD = P0 + LR * 2 * NU - S
OB = 2 * W


def _tok(*vals):
    parts = []
    for v in vals:
        if v.shape[1] < 128:
            v = jnp.broadcast_to(v[:, :1], (v.shape[0], 128))
        for i in range(v.shape[0] // 8):
            for j in range(v.shape[1] // 128):
                parts.append(v[8 * i:8 * i + 8, 128 * j:128 * j + 128])
    while len(parts) > 1:
        parts = [jnp.maximum(parts[i], parts[i + 1]) if i + 1 < len(parts) else parts[i]
                 for i in range(0, len(parts), 2)]
    return parts[0]


def _kernel(x_hbm, mem0_ref, wq_hbm, wk_hbm, wv_hbm, wo_hbm, wr_ref, wg_hbm, wu_hbm, wd_hbm,
            out_hbm,
            xs, x1buf, hbuf, hpack, raw, wqkv, wo_raw, wo, wg, wu, wd,
            ring0, ring1, qbig, oring0, oring1, abuf0, abuf1, maskv, best, zflag, sems):
    ring, oring, abuf = (ring0, ring1), (oring0, oring1), (abuf0, abuf1)

    def x_copy(row0, n, sem):
        return pltpu.make_async_copy(x_hbm.at[pl.ds(row0, n)], xs.at[pl.ds(row0, n)], sems.at[sem])

    for c in range(3):
        x_copy(c * XC, XC, 23 + c).start()
    cp_xa = x_copy(XLN, XA - XLN, 0)
    cp_xa.start()
    HC = H // 4

    def w_copy(ph, src=None):
        if src is None:
            src = wq_hbm.at[:, pl.ds(0, HC), :]
        return pltpu.make_async_copy(src, raw.at[ph], sems.at[11 + ph])

    for i, w in enumerate((wq_hbm, wk_hbm, wv_hbm)):
        for c in range(4):
            w_copy(4 * i + c, w.at[:, pl.ds(c * HC, HC), :]).start()
    cp_wo = [pltpu.make_async_copy(wo_hbm.at[:, pl.ds(n * 128, 128)], wo_raw.at[n], sems.at[4 + n])
             for n in range(4)]
    for c in cp_wo:
        c.start()
    cp_xb = x_copy(XA, S - XA, 1)
    cp_xb.start()
    cp_f = [pltpu.make_async_copy(wg_hbm, wg, sems.at[8]),
            pltpu.make_async_copy(wu_hbm, wu, sems.at[9]),
            pltpu.make_async_copy(wd_hbm, wd, sems.at[10])]
    for c in cp_f:
        c.start()

    def out_copy(row0, n):
        return pltpu.make_async_copy(xs.at[pl.ds(row0, n)], out_hbm.at[pl.ds(row0, n)], sems.at[2])

    oring1[...] = jnp.zeros(oring1.shape, F32)
    abuf0[...] = jnp.zeros(abuf0.shape, F32)
    xs[pl.ds(S, W), :] = jnp.zeros((W, D), BF16)
    hbuf[pl.ds(2 * S, 2 * W), :] = jnp.zeros((2 * W, D), F32)
    zflag[...] = jnp.zeros(zflag.shape, jnp.int32)

    ri = jax.lax.broadcasted_iota(jnp.int32, (L2, L2), 0)
    ci = jax.lax.broadcasted_iota(jnp.int32, (L2, L2), 1)

    def head_of(i):
        return jnp.where(i < 2 * M, i // M, (i - 2 * M) // SEG)

    def pos_of(i):
        return jnp.where(i < 2 * M, i % M, M + (i - 2 * M) % SEG)

    same = head_of(ri) == head_of(ci)
    ok = (pos_of(ri) < M) | (pos_of(ri) >= pos_of(ci))
    maskv[...] = jnp.where(same, jnp.where(ok, 0.0, -1e9 / SCALE), -jnp.inf).astype(F32)

    def ln0(c, carry):
        r0 = pl.multiple_of(c * XC, XC)
        x_copy(r0, XC, 23 + c).wait()
        for k in range(XC // 64):
            h = _ln(xs[pl.ds(r0 + 64 * k, 64), :].astype(F32))
            hbuf[pl.ds(r0 + 64 * k, 64), :] = h
            hpack[pl.ds(pl.multiple_of(c * (XC // 2), XC // 2) + 32 * k, 32), :] = (
                pltpu.bitcast(h.astype(BF16), U32))
        return carry

    jax.lax.fori_loop(0, 3, ln0, 0)

    def tile_base(ph):
        return (ph % 4) * 24 + (ph // 4) * 2

    def relay(ph):
        tb = tile_base(ph)
        for db in range(D // 16):
            a = jnp.swapaxes(raw[ph, pl.ds(16 * db, 16)], 0, 1)
            for hh in range(HC):
                wqkv[tb + (hh // 2) * 6 + hh % 2, pl.ds(8 * db, 8), :] = pltpu.bitcast(a[hh], U32)

    def light(g):
        lhs = _w(hpack[pl.ds(0, P0 // 2), :])
        for c in range(2):
            qbig[2 * g + c, pl.ds(0, P0), :] = _dot(lhs, _w(wqkv[6 * g + c]))

    def win0(ph):
        tb = tile_base(ph)
        lhs = _w(hpack[pl.ds(0, W // 2), :])
        for hh in range(HC):
            t = tb + (hh // 2) * 6 + hh % 2
            ring0[t] = _dot(lhs, _w(wqkv[t]))

    w_copy(0).wait()
    relay(0)

    def phase_a(ph, carry):
        w_copy(ph).wait()
        light(ph - 1)
        relay(ph)
        return carry

    def phase_b(ph, carry):
        w_copy(ph).wait()
        win0(ph - 1)
        light(ph - 1)
        relay(ph)
        return carry

    jax.lax.fori_loop(1, 4, phase_a, 0)
    jax.lax.fori_loop(4, 12, phase_b, 0)
    for c in cp_wo:
        c.wait()
    cp_xa.wait()
    win0(11)
    light(11)
    for n in range(4):
        wo[n] = pltpu.bitcast(wo_raw[n], U32)
    for g in range(NLP):
        for c in range(2):
            ring0[6 * g + c, 0:SEG, :] = qbig[2 * g + c, 0:SEG, :]

    def post(row0, a, valid):
        n = a.shape[0]
        x1 = _rb(xs[pl.ds(row0, n), :].astype(F32) + _rb(a))
        x1buf[pl.ds(row0, n), :] = x1.astype(BF16)
        hb = _ln(x1)
        r = _rb(jnp.sum(hb * wr_ref[...].astype(F32), axis=-1, keepdims=True))
        x2 = x1 + hb
        xs[pl.ds(row0, n), :] = x2.astype(BF16)
        if valid is not True:
            r = jnp.where(valid, r, -jnp.inf)
        bv = best[0]
        bi = best[1]
        sub = jax.lax.broadcasted_iota(jnp.int32, (8, 128), 0).astype(F32)
        for g in range(n // 8):
            rg = jnp.broadcast_to(r[8 * g:8 * g + 8], (8, 128))
            ig = sub + (float(row0 + 8 * g) if isinstance(row0, int) else (row0 + 8 * g).astype(F32))
            gt = rg > bv
            bv = jnp.where(gt, rg, bv)
            bi = jnp.where(gt, ig, bi)
        best[0] = bv
        best[1] = bi
        return _tok(x2, bv, bi)

    def anchor(val, tok):
        return jnp.where(zflag[...] != 0, tok, val)

    def wo_pair(g, half):
        return jnp.concatenate(
            [_w(wo[2 * half + c, pl.ds(g * 128, 128), :]) for c in range(2)], axis=1)

    def step(q, par, layer, u, mem, korder):
        rr = par * SEG
        if par == 0:
            rows = ((0, 40), (0, 24))
        else:
            rows = ((40, 64), (24, 64))
        sg = layer * (2 * NU) + 2 * u + par
        hw = pl.multiple_of(layer * S + W * (u + 1), W)
        pl0 = pl.multiple_of(P0 + LR * sg, 8)
        lhs = [jnp.concatenate([mem, hbuf[pl.ds(hw + lo, hi - lo), :]], axis=0).astype(BF16)
               for lo, hi in rows]
        lhsl = jnp.concatenate([mem, hbuf[pl.ds(pl0, LR), :]], axis=0).astype(BF16)
        qrow = [pl.multiple_of((pl0 + 8 * i) % S, 8) for i in range(LR // 8)]

        def qkv(g, korder=None):
            half = g // (NPAIR // 2)
            lo, hi = rows[half]
            res = []
            ys = {}
            if korder is not None:
                part = None
                for k in korder:
                    wk = jnp.concatenate([_w(wqkv[6 * g + t, pl.ds(64 * k, 64), :])
                                          for t in range(2, 6)], axis=1)
                    y = jnp.dot(lhs[half][:, 128 * k:128 * (k + 1)], wk,
                                preferred_element_type=F32)
                    part = y if part is None else part + y
                for t in range(4):
                    ys[t + 2] = part[:, 128 * t:128 * (t + 1)]
            for t in range(6):
                if g < NLP and t < 2:
                    y = jnp.dot(lhsl, _w(wqkv[6 * g + t]), preferred_element_type=F32)
                    for i in range(LR // 8):
                        qbig[2 * g + t, pl.ds(qrow[i], 8), :] = y[M + 8 * i:M + 8 * i + 8]
                    res.append(y[:M])
                    continue
                if t in ys:
                    y = ys[t]
                else:
                    y = jnp.dot(lhs[half], _w(wqkv[6 * g + t]), preferred_element_type=F32)
                ring[1 - q][6 * g + t, lo:hi, :] = y[M:]
                res.append(y[:M])
            return res

        def stack(g, mres, i):
            return jnp.concatenate(
                [mres[2 * i], mres[2 * i + 1],
                 ring[q][6 * g + 2 * i, rr:rr + SEG, :],
                 ring[q][6 * g + 2 * i + 1, rr:rr + SEG, :]], axis=0).astype(BF16)

        def qk(g, mres, prenorm):
            q2, k2 = stack(g, mres, 0), stack(g, mres, 1)
            s = jax.lax.dot_general(q2, k2, (((1,), (1,)), ((), ())), preferred_element_type=F32)
            mk = maskv[...]
            s = jnp.where(mk == 0.0, s, mk)
            mx = jnp.max(s, axis=-1, keepdims=True)
            p = jnp.exp2((s - mx) * (SCALE * LOG2E))
            l = jnp.sum(p, axis=-1, keepdims=True)
            r0 = pl.reciprocal(l, approx=True)
            r = r0 * (2.0 - l * r0)
            if prenorm:
                return (p * r).astype(BF16), None
            return p.astype(BF16), r

        def pv(g, mres, pr):
            p, r = pr
            o = jnp.dot(p, stack(g, mres, 2), preferred_element_type=F32)
            if r is not None:
                o = o * r
            oring[q][2 * g, rr:rr + SEG, :] = o[2 * M:2 * M + SEG]
            oring[q][2 * g + 1, rr:rr + SEG, :] = o[2 * M + SEG:]
            return o[:M], o[M:2 * M]

        def olhs(g, om, half):
            lo, hi = rows[half]
            return jnp.concatenate(
                [jnp.concatenate([om[c], oring[1 - q][2 * g + c, lo:hi, :]], axis=0)
                 for c in range(2)], axis=1).astype(BF16)

        crow = pl.multiple_of((SEG * (sg + 1)) % S, SEG)
        dst = ring[q] if par == 0 else ring[1 - q]
        cvals = []
        for g in range(NLP):
            for c in range(2):
                v = qbig[2 * g + c, pl.ds(crow, SEG), :]
                dst[6 * g + c, SEG - rr:2 * SEG - rr, :] = v
                cvals.append(v)
        tok_cp = _tok(*cvals)
        xr = jnp.concatenate(
            [xs[pl.ds(pl.multiple_of((pl0 + LR + 8 * i) % S, 8), 8), :].astype(F32)
             for i in range(LR // 8)], axis=0)
        hpre = _ln(xr)
        hbuf[pl.ds(pl0 + LR, LR), :] = hpre
        tok_pre = _tok(hpre)
        valid = u >= 2
        row0 = pl.multiple_of(jnp.where(valid, W * (u - 2), S) + rr, SEG)
        tok_post = post(row0, abuf[q][rr:rr + SEG, :], valid)

        NST = NPAIR // 2
        st = [(i, i + NST) if par == 0 else (i + NST, i) for i in range(NST)]
        mres, prs, oms = {}, {}, {}
        acc = [None] * 4
        order = []
        for i in range(NST):
            order += [("qkv", g) for g in st[i]]
            if i >= 1:
                order += [("qk", g) for g in st[i - 1]]
            if i >= 2:
                order += [("pv", g) for g in st[i - 2]]
        oq = [g for i in range(NST) for g in st[i]]
        NE = 8
        order += [("o", g) for g in oq[0:3]]
        order += [("qk", g) for g in st[NST - 1]] + [("pv", g) for g in st[NST - 2]]
        order += [("o", g) for g in oq[3:7]]
        order += [("pv", g) for g in st[NST - 1]]
        order += [("o", g) for g in oq[7:NE]]
        norder = (2, 3, 0, 1) if par == 0 else (0, 1, 2, 3)
        order += [("on", n) for n in norder]
        for kind, g in order:
            if kind == "qkv":
                mres[g] = qkv(g, korder if g == st[0][0] else None)
                if g == st[0][0]:
                    mres[g][0] = anchor(mres[g][0], tok_cp)
                if g == st[2][0]:
                    mres[g][0] = anchor(mres[g][0], tok_pre)
                if g == st[4][0]:
                    mres[g][0] = anchor(mres[g][0], tok_post)
            elif kind == "qk":
                prs[g] = qk(g, mres[g], g not in st[NST - 1] + st[NST - 2])
            elif kind == "pv":
                oms[g] = pv(g, mres[g], prs[g])
                if prs[g][1] is not None:
                    oms[g] = (anchor(oms[g][0], _tok(prs[g][1][2 * M:])), oms[g][1])
            elif kind == "o":
                for half in range(2):
                    y = jnp.dot(olhs(g, oms[g], half), wo_pair(g, half), preferred_element_type=F32)
                    for c in range(2):
                        yc = y[:, 128 * c:128 * (c + 1)]
                        n = 2 * half + c
                        acc[n] = yc if acc[n] is None else acc[n] + yc
            else:
                n = g
                l = jnp.concatenate([olhs(g2, oms[g2], n // 2) for g2 in oq[NE:]], axis=1)
                wn = jnp.concatenate([_w(wo[n, pl.ds(g2 * 128, 128), :]) for g2 in oq[NE:]], axis=0)
                acc[n] = acc[n] + jnp.dot(l, wn, preferred_element_type=F32)
        for n in range(4):
            lo, hi = rows[n // 2]
            abuf[1 - q][lo:hi, n * 128:(n + 1) * 128] = acc[n][M:]

        return jnp.concatenate([acc[n][:M] for n in range(4)], axis=1), norder

    def layer_body(layer, carry):
        best[0] = jnp.full((8, 128), -jnp.inf, F32)
        best[1] = jnp.zeros((8, 128), F32)

        def qstep(j, mem):
            @pl.when((layer == 0) & (j == 1))
            def _():
                cp_xb.wait()

            @pl.when((layer == 1) & (j >= 2))
            def _():
                out_copy(pl.multiple_of((j - 2) * OB, OB), OB).start()

            ko = None
            for q in range(2):
                for par in range(2):
                    mem, ko = step(q, par, layer, 2 * j + q, mem, ko)
            return mem

        jax.lax.fori_loop(0, NU // 2, qstep, mem0_ref[...].astype(F32))

        @pl.when(layer == 1)
        def _():
            out_copy(S - 2 * OB, OB).start()

        post(S - 2 * W, abuf0[...], True)
        acc = None
        for g in range(NPAIR):
            l = jnp.concatenate([oring1[2 * g + c] for c in range(2)], axis=1).astype(BF16)
            y = _dot(l, jnp.concatenate([wo_pair(g, 0), wo_pair(g, 1)], axis=1))
            acc = y if acc is None else acc + y
        post(S - W, acc, True)

        @pl.when(layer == 0)
        def _():
            for c in cp_f:
                c.wait()

        bv = best[0]
        bi = best[1]
        vmax = jnp.max(bv, axis=0, keepdims=True)
        imin = jnp.min(jnp.where(bv == vmax, bi, float(S)), axis=0, keepdims=True)
        idx = jnp.clip(jnp.min(imin).astype(jnp.int32), 0, S - 1)
        g0 = pl.multiple_of((idx // 16) * 16, 16)
        x1 = x1buf[pl.ds(g0, 16), :].astype(F32)
        hb = _ln(x1)
        hbb = hb.astype(BF16)
        gpre = _rb(_dot(hbb, wg[...]))
        gs = _rb(gpre * _rb(jax.nn.sigmoid(gpre)))
        up = _rb(_dot(hbb, wu[...]))
        y = _rb(_dot((gs * up).astype(BF16), wd[...]))
        rsel = _rb(jax.nn.sigmoid(vmax))[:, :1]
        y = _rb(y * rsel)
        x2 = _rb(x1 + _rb(hb + y))
        rowi = jax.lax.broadcasted_iota(jnp.int32, (16, D), 0) + g0

        @pl.when(layer == 1)
        def _():
            for _i in range(S // OB - 1):
                out_copy(0, OB).wait()

        x2 = jnp.where(rowi == idx, x2, xs[pl.ds(g0, 16), :].astype(F32))
        xs[pl.ds(g0, 16), :] = x2.astype(BF16)

        @pl.when(layer == 0)
        def _():
            h16 = _ln(x2)
            hbuf[pl.ds(S + g0, 16), :] = h16

            @pl.when(idx < FD)
            def _():
                def body(g, c):
                    for t in range(2):
                        qbig[2 * g + t, pl.ds(g0, 16), :] = _dot(h16.astype(BF16), _w(wqkv[6 * g + t]))
                    return c

                jax.lax.fori_loop(0, NLP, body, 0, unroll=2)

            @pl.when(idx < W)
            def _():
                gw = pl.multiple_of(jnp.minimum(g0, W - 16), 16)

                def body(t, c):
                    ring0[t, pl.ds(gw, 16), :] = _dot(h16.astype(BF16), _w(wqkv[t]))
                    return c

                jax.lax.fori_loop(0, 6 * NPAIR, body, 0, unroll=4)

        @pl.when(layer == 1)
        def _():
            last = out_copy(S - OB, OB)
            last.start()

            @pl.when(g0 < S - OB)
            def _():
                fix = pltpu.make_async_copy(xs.at[pl.ds(g0, 16)], out_hbm.at[pl.ds(g0, 16)],
                                            sems.at[3])
                fix.start()
                fix.wait()

            last.wait()

        return carry

    jax.lax.fori_loop(0, 2, layer_body, 0)


@functools.partial(jax.jit, static_argnames=("A_seg_len",))
def pallas_interleave_layers__memory_aug_recurrent_mem_tr__moe_arch_mod__prompt_kernel(
    A_x: jax.Array,
    A_mem0: jax.Array,
    A_Wq: jax.Array,
    A_Wk: jax.Array,
    A_Wv: jax.Array,
    A_Wo: jax.Array,
    A_seg_len,
    B_x: jax.Array,
    B_w_r: jax.Array,
    B_w_gate: jax.Array,
    B_w_up: jax.Array,
    B_w_down: jax.Array,
):
    assert A_seg_len == SEG
    assert A_x.shape == (1, S, D) and A_Wq.shape == (D, H, E) and A_mem0.shape == (1, M, D)
    any_spec = pl.BlockSpec(memory_space=pl.ANY)
    vmem_spec = pl.BlockSpec(memory_space=pltpu.VMEM)
    out = pl.pallas_call(
        _kernel,
        out_shape=jax.ShapeDtypeStruct((S, D), BF16),
        in_specs=[any_spec, vmem_spec, any_spec, any_spec, any_spec, any_spec,
                  vmem_spec, any_spec, any_spec, any_spec],
        out_specs=any_spec,
        scratch_shapes=[
            pltpu.VMEM((S + W, D), BF16),
            pltpu.VMEM((S + W, D), BF16),
            pltpu.VMEM((2 * S + 2 * W, D), F32),
            pltpu.VMEM((XLN // 2, D), U32),
            pltpu.VMEM((12, D, H // 4, E), BF16),
            pltpu.VMEM((6 * NPAIR, D // 2, E), U32),
            pltpu.VMEM((4, H * E, 128), BF16),
            pltpu.VMEM((4, H * E // 2, 128), U32),
            pltpu.VMEM((D, F), BF16),
            pltpu.VMEM((D, F), BF16),
            pltpu.VMEM((F, D), BF16),
            pltpu.VMEM((6 * NPAIR, W, E), F32),
            pltpu.VMEM((6 * NPAIR, W, E), F32),
            pltpu.VMEM((2 * NLP, S, E), F32),
            pltpu.VMEM((H, W, E), F32),
            pltpu.VMEM((H, W, E), F32),
            pltpu.VMEM((W, D), F32),
            pltpu.VMEM((W, D), F32),
            pltpu.VMEM((L2, L2), F32),
            pltpu.VMEM((2, 8, 128), F32),
            pltpu.VMEM((8, 128), jnp.int32),
            pltpu.SemaphoreType.DMA((26,)),
        ],
        compiler_params=pltpu.CompilerParams(vmem_limit_bytes=110 * 1024 * 1024),
        name="rmt_mod",
    )(A_x.reshape(S, D), A_mem0.reshape(M, D), A_Wq, A_Wk, A_Wv, A_Wo.reshape(H * E, D),
      B_w_r.reshape(1, D), B_w_gate, B_w_up, B_w_down)
    return out.reshape(1, S, D)
```

```python
import functools

import jax
import jax.numpy as jnp
import jax.experimental.pallas as pl
import jax.experimental.pallas.tpu as pltpu

S = 2048
D = 512
H = 32
E = 128
M = 8
SEG = 32
F = 1792
NPAIR = H // 2
NU = S // (2 * SEG)
W = 2 * SEG
L2 = 2 * (M + SEG)
EPS = 1e-05
SCALE = float(E) ** -0.5
LOG2E = 1.4426950408889634
F32 = jnp.float32
BF16 = jnp.bfloat16
U32 = jnp.uint32


def _rb(x):
    return x.astype(BF16).astype(F32)


def _ln(x):
    mu = jnp.sum(x, axis=-1, keepdims=True) * (1.0 / D)
    xc0 = x - mu
    var = jnp.sum(xc0 * xc0, axis=-1, keepdims=True) * (1.0 / D)
    sd = _rb(jnp.sqrt(_rb(_rb(var) + EPS)))
    xc = _rb(x - _rb(mu))
    return _rb(xc * (1.0 / sd))


def _dot(a, b):
    return jnp.dot(a, b, preferred_element_type=F32)


def _w(ref_slab):
    return pltpu.bitcast(ref_slab, BF16)


NLP = 12
P0 = 1024
PLN = 1096
LR = 24
XC = 384
XLN = 3 * XC
XA = XLN + W
FD = P0 + LR * 2 * NU - S
OB = 2 * W


def _tok(*vals):
    parts = []
    for v in vals:
        if v.shape[1] < 128:
            v = jnp.broadcast_to(v[:, :1], (v.shape[0], 128))
        for i in range(v.shape[0] // 8):
            for j in range(v.shape[1] // 128):
                parts.append(v[8 * i:8 * i + 8, 128 * j:128 * j + 128])
    while len(parts) > 1:
        parts = [jnp.maximum(parts[i], parts[i + 1]) if i + 1 < len(parts) else parts[i]
                 for i in range(0, len(parts), 2)]
    return parts[0]


def _kernel(x_hbm, mem0_ref, wq_hbm, wk_hbm, wv_hbm, wo_hbm, wr_ref, wg_hbm, wu_hbm, wd_hbm,
            out_hbm,
            xs, x1buf, hbuf, hpack, raw, wql, wqkv, wo_raw, wo, wg, wu, wd,
            ring0, ring1, qbig, oring0, oring1, abuf0, abuf1, maskv, best, zflag, sems):
    ring, oring, abuf = (ring0, ring1), (oring0, oring1), (abuf0, abuf1)

    def x_copy(row0, n, sem):
        return pltpu.make_async_copy(x_hbm.at[pl.ds(row0, n)], xs.at[pl.ds(row0, n)], sems.at[sem])

    for c in range(3):
        x_copy(c * XC, XC, 23 + c).start()
    cp_xa = x_copy(XLN, XA - XLN, 0)
    cp_xa.start()
    HC = H // 4

    def w_copy(ph, src=None):
        if src is None:
            src = wq_hbm.at[:, pl.ds(0, HC), :]
        return pltpu.make_async_copy(src, raw.at[ph], sems.at[11 + ph])

    for i, w in enumerate((wq_hbm, wk_hbm, wv_hbm)):
        for c in range(4):
            w_copy(4 * i + c, w.at[:, pl.ds(c * HC, HC), :]).start()
    cp_wo = [pltpu.make_async_copy(wo_hbm.at[:, pl.ds(n * 128, 128)], wo_raw.at[n], sems.at[4 + n])
             for n in range(4)]
    for c in cp_wo:
        c.start()
    cp_xb = x_copy(XA, S - XA, 1)
    cp_xb.start()
    cp_f = [pltpu.make_async_copy(wg_hbm, wg, sems.at[8]),
            pltpu.make_async_copy(wu_hbm, wu, sems.at[9]),
            pltpu.make_async_copy(wd_hbm, wd, sems.at[10])]
    for c in cp_f:
        c.start()

    def out_copy(row0, n):
        return pltpu.make_async_copy(xs.at[pl.ds(row0, n)], out_hbm.at[pl.ds(row0, n)], sems.at[2])

    oring1[...] = jnp.zeros(oring1.shape, F32)
    abuf0[...] = jnp.zeros(abuf0.shape, F32)
    xs[pl.ds(S, W), :] = jnp.zeros((W, D), BF16)
    hbuf[pl.ds(2 * S, 2 * W), :] = jnp.zeros((2 * W, D), F32)
    zflag[...] = jnp.zeros(zflag.shape, jnp.int32)

    ri = jax.lax.broadcasted_iota(jnp.int32, (L2, L2), 0)
    ci = jax.lax.broadcasted_iota(jnp.int32, (L2, L2), 1)

    def head_of(i):
        return jnp.where(i < 2 * M, i // M, (i - 2 * M) // SEG)

    def pos_of(i):
        return jnp.where(i < 2 * M, i % M, M + (i - 2 * M) % SEG)

    same = head_of(ri) == head_of(ci)
    ok = (pos_of(ri) < M) | (pos_of(ri) >= pos_of(ci))
    maskv[...] = jnp.where(same, jnp.where(ok, 0.0, -1e9 / SCALE), -jnp.inf).astype(F32)

    def ln0(c, carry):
        r0 = pl.multiple_of(c * XC, XC)
        x_copy(r0, XC, 23 + c).wait()
        for k in range(XC // 64):
            h = _ln(xs[pl.ds(r0 + 64 * k, 64), :].astype(F32))
            hbuf[pl.ds(r0 + 64 * k, 64), :] = h
            hpack[pl.ds(pl.multiple_of(c * (XC // 2), XC // 2) + 32 * k, 32), :] = (
                pltpu.bitcast(h.astype(BF16), U32))
        return carry

    jax.lax.fori_loop(0, 3, ln0, 0)

    def tile_base(ph):
        return (ph % 4) * 24 + (ph // 4) * 2

    def relay(ph, ys=None):
        is_light = isinstance(ph, int) and ph < NLP // 4
        tb = tile_base(ph)
        for db in range(D // 16):
            d0 = 16 * db
            if ys is not None:
                tok = ys[db // 16][64 * (db % 16):64 * (db % 16) + 8]
                z = jnp.where(zflag[...] != 0, tok.astype(jnp.int32), 0)[0, 0]
                d0 = jnp.clip(d0 + z, 0, D - 16)
            a = jnp.swapaxes(raw[ph, pl.ds(d0, 16)], 0, 1)
            for hh in range(HC):
                v = pltpu.bitcast(a[hh], U32)
                if is_light:
                    wql[ph * HC + hh, pl.ds(8 * db, 8), :] = v
                else:
                    wqkv[tb + (hh // 2) * 6 + hh % 2, pl.ds(8 * db, 8), :] = v

    def light(g):
        lhs = _w(hpack[pl.ds(0, P0 // 2), :])
        ys = []
        for c in range(2):
            y = _dot(lhs, _w(wql[2 * g + c]))
            qbig[2 * g + c, pl.ds(0, P0), :] = y
            ys.append(y)
        return ys

    def win0(ph):
        tb = tile_base(ph)
        lhs = _w(hpack[pl.ds(0, W // 2), :])
        for hh in range(HC):
            t = tb + (hh // 2) * 6 + hh % 2
            ring0[t] = _dot(lhs, _w(wqkv[t]))

    w_copy(0).wait()
    relay(0)
    for ph in range(1, 4):
        w_copy(ph).wait()
        relay(ph, light(ph - 1))

    def phase_b(ph, carry):
        w_copy(ph).wait()
        win0(ph - 1)
        relay(ph, light(ph - 1))
        return carry

    jax.lax.fori_loop(4, 12, phase_b, 0)
    for c in cp_wo:
        c.wait()
    cp_xa.wait()
    win0(11)
    ys = light(NLP - 1)
    zf = zflag[...] != 0
    for k in range(32):
        tok = pltpu.bitcast(ys[k // 16][64 * (k % 16):64 * (k % 16) + 8], U32)
        n, kk = k // 8, k % 8
        v = pltpu.bitcast(wo_raw[n, pl.ds(512 * kk, 512), :], U32).reshape(32, 8, 128)
        wo[n, pl.ds(256 * kk, 256), :] = jnp.where(zf[None], tok[None], v).reshape(256, 128)
    def post(row0, a, valid):
        n = a.shape[0]
        x1 = _rb(xs[pl.ds(row0, n), :].astype(F32) + _rb(a))
        x1buf[pl.ds(row0, n), :] = x1.astype(BF16)
        hb = _ln(x1)
        r = _rb(jnp.sum(hb * wr_ref[...].astype(F32), axis=-1, keepdims=True))
        x2 = x1 + hb
        xs[pl.ds(row0, n), :] = x2.astype(BF16)
        if valid is not True:
            r = jnp.where(valid, r, -jnp.inf)
        bv = best[0]
        bi = best[1]
        sub = jax.lax.broadcasted_iota(jnp.int32, (8, 128), 0).astype(F32)
        for g in range(n // 8):
            rg = jnp.broadcast_to(r[8 * g:8 * g + 8], (8, 128))
            ig = sub + (float(row0 + 8 * g) if isinstance(row0, int) else (row0 + 8 * g).astype(F32))
            gt = rg > bv
            bv = jnp.where(gt, rg, bv)
            bi = jnp.where(gt, ig, bi)
        best[0] = bv
        best[1] = bi
        return _tok(x2, bv, bi)

    def anchor(val, tok):
        return jnp.where(zflag[...] != 0, tok, val)

    def wo_pair(g, half):
        return jnp.concatenate(
            [_w(wo[2 * half + c, pl.ds(g * 128, 128), :]) for c in range(2)], axis=1)

    def step(q, par, layer, u, mem, korder):
        rr = par * SEG
        if par == 0:
            rows = ((0, 40), (0, 24))
        else:
            rows = ((40, 64), (24, 64))
        sg = layer * (2 * NU) + 2 * u + par
        hw = pl.multiple_of(layer * S + W * (u + 1), W)
        pl0 = pl.multiple_of(P0 + LR * sg, 8)
        lhs = [jnp.concatenate([mem, hbuf[pl.ds(hw + lo, hi - lo), :]], axis=0).astype(BF16)
               for lo, hi in rows]
        lhsl = jnp.concatenate([mem, hbuf[pl.ds(pl0, LR), :]], axis=0).astype(BF16)
        qrow = [pl.multiple_of((pl0 + 8 * i) % S, 8) for i in range(LR // 8)]

        def qkv(g, korder=None):
            half = g // (NPAIR // 2)
            lo, hi = rows[half]
            res = []
            ys = {}
            if korder is not None:
                part = None
                for k in korder:
                    wk = jnp.concatenate([_w(wqkv[6 * g + t, pl.ds(64 * k, 64), :])
                                          for t in range(2, 6)], axis=1)
                    y = jnp.dot(lhs[half][:, 128 * k:128 * (k + 1)], wk,
                                preferred_element_type=F32)
                    part = y if part is None else part + y
                for t in range(4):
                    ys[t + 2] = part[:, 128 * t:128 * (t + 1)]
            for t in range(6):
                if g < NLP and t < 2:
                    y = jnp.dot(lhsl, _w(wql[2 * g + t]), preferred_element_type=F32)
                    for i in range(LR // 8):
                        qbig[2 * g + t, pl.ds(qrow[i], 8), :] = y[M + 8 * i:M + 8 * i + 8]
                    res.append(y[:M])
                    continue
                if t in ys:
                    y = ys[t]
                else:
                    y = jnp.dot(lhs[half], _w(wqkv[6 * g + t]), preferred_element_type=F32)
                ring[1 - q][6 * g + t, lo:hi, :] = y[M:]
                res.append(y[:M])
            return res

        crow = pl.multiple_of(W * u + rr, SEG)
        qx = {}

        def stack(g, mres, i):
            if i == 0 and g < NLP:
                return jnp.concatenate(
                    [jnp.concatenate([mres[0], mres[1]], axis=0).astype(BF16), qx[g]], axis=0)
            return jnp.concatenate(
                [mres[2 * i], mres[2 * i + 1],
                 ring[q][6 * g + 2 * i, rr:rr + SEG, :],
                 ring[q][6 * g + 2 * i + 1, rr:rr + SEG, :]], axis=0).astype(BF16)

        def qk(g, mres, prenorm):
            q2, k2 = stack(g, mres, 0), stack(g, mres, 1)
            s = jax.lax.dot_general(q2, k2, (((1,), (1,)), ((), ())), preferred_element_type=F32)
            mk = maskv[...]
            s = jnp.where(mk == 0.0, s, mk)
            mx = jnp.max(s, axis=-1, keepdims=True)
            p = jnp.exp2((s - mx) * (SCALE * LOG2E))
            l = jnp.sum(p, axis=-1, keepdims=True)
            r0 = pl.reciprocal(l, approx=True)
            r = r0 * (2.0 - l * r0)
            if prenorm:
                return (p * r).astype(BF16), None
            return p.astype(BF16), r

        def pv(g, mres, pr):
            p, r = pr
            o = jnp.dot(p, stack(g, mres, 2), preferred_element_type=F32)
            if r is not None:
                o = o * r
            oring[q][2 * g, rr:rr + SEG, :] = o[2 * M:2 * M + SEG]
            oring[q][2 * g + 1, rr:rr + SEG, :] = o[2 * M + SEG:]
            return o[:M], o[M:2 * M]

        def olhs(g, om, half):
            lo, hi = rows[half]
            return jnp.concatenate(
                [jnp.concatenate([om[c], oring[1 - q][2 * g + c, lo:hi, :]], axis=0)
                 for c in range(2)], axis=1).astype(BF16)

        pn0 = pl.multiple_of(PLN + LR * sg, 8)
        xr = jnp.concatenate(
            [xs[pl.ds(pl.multiple_of((pn0 + 8 * i) % S, 8), 8), :].astype(F32)
             for i in range(LR // 8)], axis=0)
        hpre = _ln(xr)
        hbuf[pl.ds(pn0, LR), :] = hpre
        tok_pre = _tok(hpre)
        valid = u >= 2
        row0 = pl.multiple_of(jnp.where(valid, W * (u - 2), S) + rr, SEG)
        tok_post = post(row0, abuf[q][rr:rr + SEG, :], valid)

        NST = NPAIR // 2
        st = [(i, i + NST) if par == 0 else (i + NST, i) for i in range(NST)]
        mres, prs, oms = {}, {}, {}
        acc = [None] * 4
        order = []
        for i in range(NST):
            order += [("qkv", g) for g in st[i]]
            if i >= 1:
                order += [("qk", g) for g in st[i - 1]]
            if i >= 2:
                order += [("pv", g) for g in st[i - 2]]
        oq = [g for i in range(NST) for g in st[i]]
        NE = 8
        order += [("o", g) for g in oq[0:3]]
        order += [("qk", g) for g in st[NST - 1]] + [("pv", g) for g in st[NST - 2]]
        order += [("o", g) for g in oq[3:7]]
        order += [("pv", g) for g in st[NST - 1]]
        order += [("o", g) for g in oq[7:NE]]
        norder = (2, 3, 0, 1) if par == 0 else (0, 1, 2, 3)
        order += [("on", n) for n in norder]
        for kind, g in order:
            if kind == "qkv":
                mres[g] = qkv(g, korder if g == st[0][0] else None)
                if g < NLP:
                    qx[g] = jnp.concatenate([qbig[2 * g + c, pl.ds(crow, SEG), :] for c in range(2)],
                                            axis=0).astype(BF16)
                if g == st[2][0]:
                    mres[g][0] = anchor(mres[g][0], tok_pre)
                if g == st[4][0]:
                    mres[g][0] = anchor(mres[g][0], tok_post)
            elif kind == "qk":
                prs[g] = qk(g, mres[g], g not in st[NST - 1] + st[NST - 2])
            elif kind == "pv":
                oms[g] = pv(g, mres[g], prs[g])
                if prs[g][1] is not None:
                    oms[g] = (anchor(oms[g][0], _tok(prs[g][1][2 * M:])), oms[g][1])
            elif kind == "o":
                for half in range(2):
                    y = jnp.dot(olhs(g, oms[g], half), wo_pair(g, half), preferred_element_type=F32)
                    for c in range(2):
                        yc = y[:, 128 * c:128 * (c + 1)]
                        n = 2 * half + c
                        acc[n] = yc if acc[n] is None else acc[n] + yc
            else:
                n = g
                l = jnp.concatenate([olhs(g2, oms[g2], n // 2) for g2 in oq[NE:]], axis=1)
                wn = jnp.concatenate([_w(wo[n, pl.ds(g2 * 128, 128), :]) for g2 in oq[NE:]], axis=0)
                acc[n] = acc[n] + jnp.dot(l, wn, preferred_element_type=F32)
        for n in range(4):
            lo, hi = rows[n // 2]
            abuf[1 - q][lo:hi, n * 128:(n + 1) * 128] = acc[n][M:]

        return jnp.concatenate([acc[n][:M] for n in range(4)], axis=1), norder

    def layer_body(layer, carry):
        best[0] = jnp.full((8, 128), -jnp.inf, F32)
        best[1] = jnp.zeros((8, 128), F32)

        def qstep(j, mem):
            @pl.when((layer == 0) & (j == 1))
            def _():
                cp_xb.wait()

            @pl.when((layer == 1) & (j >= 2))
            def _():
                out_copy(pl.multiple_of((j - 2) * OB, OB), OB).start()

            ko = None
            for q in range(2):
                for par in range(2):
                    mem, ko = step(q, par, layer, 2 * j + q, mem, ko)
            return mem

        jax.lax.fori_loop(0, NU // 2, qstep, mem0_ref[...].astype(F32))

        @pl.when(layer == 1)
        def _():
            out_copy(S - 2 * OB, OB).start()

        post(S - 2 * W, abuf0[...], True)
        acc = None
        for g in range(NPAIR):
            l = jnp.concatenate([oring1[2 * g + c] for c in range(2)], axis=1).astype(BF16)
            y = _dot(l, jnp.concatenate([wo_pair(g, 0), wo_pair(g, 1)], axis=1))
            acc = y if acc is None else acc + y
        post(S - W, acc, True)

        @pl.when(layer == 0)
        def _():
            for c in cp_f:
                c.wait()

        bv = best[0]
        bi = best[1]
        vmax = jnp.max(bv, axis=0, keepdims=True)
        imin = jnp.min(jnp.where(bv == vmax, bi, float(S)), axis=0, keepdims=True)
        idx = jnp.clip(jnp.min(imin).astype(jnp.int32), 0, S - 1)
        g0 = pl.multiple_of((idx // 16) * 16, 16)
        x1 = x1buf[pl.ds(g0, 16), :].astype(F32)
        hb = _ln(x1)
        hbb = hb.astype(BF16)
        gpre = _rb(_dot(hbb, wg[...]))
        gs = _rb(gpre * _rb(jax.nn.sigmoid(gpre)))
        up = _rb(_dot(hbb, wu[...]))
        y = _rb(_dot((gs * up).astype(BF16), wd[...]))
        rsel = _rb(jax.nn.sigmoid(vmax))[:, :1]
        y = _rb(y * rsel)
        x2 = _rb(x1 + _rb(hb + y))
        rowi = jax.lax.broadcasted_iota(jnp.int32, (16, D), 0) + g0

        @pl.when(layer == 1)
        def _():
            for _i in range(S // OB - 1):
                out_copy(0, OB).wait()

        x2 = jnp.where(rowi == idx, x2, xs[pl.ds(g0, 16), :].astype(F32))
        xs[pl.ds(g0, 16), :] = x2.astype(BF16)

        @pl.when(layer == 0)
        def _():
            h16 = _ln(x2)
            hbuf[pl.ds(S + g0, 16), :] = h16

            @pl.when(idx < FD)
            def _():
                def body(g, c):
                    for t in range(2):
                        qbig[2 * g + t, pl.ds(g0, 16), :] = _dot(h16.astype(BF16), _w(wql[2 * g + t]))
                    return c

                jax.lax.fori_loop(0, NLP, body, 0, unroll=2)

            @pl.when(idx < W)
            def _():
                gw = pl.multiple_of(jnp.minimum(g0, W - 16), 16)

                def body(g, c):
                    for t in range(2, 6):
                        ring0[6 * g + t, pl.ds(gw, 16), :] = _dot(h16.astype(BF16), _w(wqkv[6 * g + t]))
                    return c

                jax.lax.fori_loop(0, NPAIR, body, 0)
                for g in range(NLP, NPAIR):
                    for t in range(2):
                        ring0[6 * g + t, pl.ds(gw, 16), :] = _dot(h16.astype(BF16),
                                                                  _w(wqkv[6 * g + t]))

        @pl.when(layer == 1)
        def _():
            last = out_copy(S - OB, OB)
            last.start()

            @pl.when(g0 < S - OB)
            def _():
                fix = pltpu.make_async_copy(xs.at[pl.ds(g0, 16)], out_hbm.at[pl.ds(g0, 16)],
                                            sems.at[3])
                fix.start()
                fix.wait()

            last.wait()

        return carry

    jax.lax.fori_loop(0, 2, layer_body, 0)


@functools.partial(jax.jit, static_argnames=("A_seg_len",))
def pallas_interleave_layers__memory_aug_recurrent_mem_tr__moe_arch_mod__prompt_kernel(
    A_x: jax.Array,
    A_mem0: jax.Array,
    A_Wq: jax.Array,
    A_Wk: jax.Array,
    A_Wv: jax.Array,
    A_Wo: jax.Array,
    A_seg_len,
    B_x: jax.Array,
    B_w_r: jax.Array,
    B_w_gate: jax.Array,
    B_w_up: jax.Array,
    B_w_down: jax.Array,
):
    assert A_seg_len == SEG
    assert A_x.shape == (1, S, D) and A_Wq.shape == (D, H, E) and A_mem0.shape == (1, M, D)
    any_spec = pl.BlockSpec(memory_space=pl.ANY)
    vmem_spec = pl.BlockSpec(memory_space=pltpu.VMEM)
    out = pl.pallas_call(
        _kernel,
        out_shape=jax.ShapeDtypeStruct((S, D), BF16),
        in_specs=[any_spec, vmem_spec, any_spec, any_spec, any_spec, any_spec,
                  vmem_spec, any_spec, any_spec, any_spec],
        out_specs=any_spec,
        scratch_shapes=[
            pltpu.VMEM((S + W, D), BF16),
            pltpu.VMEM((S + W, D), BF16),
            pltpu.VMEM((2 * S + 2 * W, D), F32),
            pltpu.VMEM((XLN // 2, D), U32),
            pltpu.VMEM((12, D, H // 4, E), BF16),
            pltpu.VMEM((2 * NLP, D // 2, E), U32),
            pltpu.VMEM((6 * NPAIR, D // 2, E), U32),
            pltpu.VMEM((4, H * E, 128), BF16),
            pltpu.VMEM((4, H * E // 2, 128), U32),
            pltpu.VMEM((D, F), BF16),
            pltpu.VMEM((D, F), BF16),
            pltpu.VMEM((F, D), BF16),
            pltpu.VMEM((6 * NPAIR, W, E), F32),
            pltpu.VMEM((6 * NPAIR, W, E), F32),
            pltpu.VMEM((2 * NLP, S, E), F32),
            pltpu.VMEM((H, W, E), F32),
            pltpu.VMEM((H, W, E), F32),
            pltpu.VMEM((W, D), F32),
            pltpu.VMEM((W, D), F32),
            pltpu.VMEM((L2, L2), F32),
            pltpu.VMEM((2, 8, 128), F32),
            pltpu.VMEM((8, 128), jnp.int32),
            pltpu.SemaphoreType.DMA((26,)),
        ],
        compiler_params=pltpu.CompilerParams(vmem_limit_bytes=110 * 1024 * 1024),
        name="rmt_mod",
    )(A_x.reshape(S, D), A_mem0.reshape(M, D), A_Wq, A_Wk, A_Wv, A_Wo.reshape(H * E, D),
      B_w_r.reshape(1, D), B_w_gate, B_w_up, B_w_down)
    return out.reshape(1, S, D)
```

```python
import functools

import jax
import jax.numpy as jnp
import jax.experimental.pallas as pl
import jax.experimental.pallas.tpu as pltpu

S = 2048
D = 512
H = 32
E = 128
M = 8
SEG = 32
F = 1792
NPAIR = H // 2
NU = S // (2 * SEG)
W = 2 * SEG
L2 = 2 * (M + SEG)
EPS = 1e-05
SCALE = float(E) ** -0.5
LOG2E = 1.4426950408889634
F32 = jnp.float32
BF16 = jnp.bfloat16
U32 = jnp.uint32


def _rb(x):
    return x.astype(BF16).astype(F32)


def _ln(x):
    mu = jnp.sum(x, axis=-1, keepdims=True) * (1.0 / D)
    xc0 = x - mu
    var = jnp.sum(xc0 * xc0, axis=-1, keepdims=True) * (1.0 / D)
    sd = _rb(jnp.sqrt(_rb(_rb(var) + EPS)))
    xc = _rb(x - _rb(mu))
    return _rb(xc * (1.0 / sd))


def _dot(a, b):
    return jnp.dot(a, b, preferred_element_type=F32)


def _w(ref_slab):
    return pltpu.bitcast(ref_slab, BF16)


NLP = 12
P0 = 1024
PLN = 1096
LR = 24
XC = 256
XLN = P0 + 2 * W
XA = XLN + W
FD = P0 + LR * 2 * NU - S
OB = 2 * W


def _tok(*vals):
    parts = []
    for v in vals:
        if v.shape[1] < 128:
            v = jnp.broadcast_to(v[:, :1], (v.shape[0], 128))
        for i in range(v.shape[0] // 8):
            for j in range(v.shape[1] // 128):
                parts.append(v[8 * i:8 * i + 8, 128 * j:128 * j + 128])
    while len(parts) > 1:
        parts = [jnp.maximum(parts[i], parts[i + 1]) if i + 1 < len(parts) else parts[i]
                 for i in range(0, len(parts), 2)]
    return parts[0]


def _kernel(x_hbm, mem0_ref, wq_hbm, wk_hbm, wv_hbm, wo_hbm, wr_ref, wg_hbm, wu_hbm, wd_hbm,
            out_hbm,
            xs, x1buf, hbuf, hpack, raw, wql, wqkv, wo_raw, wo, wg, wu, wd,
            ring0, ring1, qbig, oring0, oring1, abuf0, abuf1, maskv, best, zflag, sems):
    ring, oring, abuf = (ring0, ring1), (oring0, oring1), (abuf0, abuf1)

    def x_copy(row0, n, sem):
        return pltpu.make_async_copy(x_hbm.at[pl.ds(row0, n)], xs.at[pl.ds(row0, n)], sems.at[sem])

    HC = H // 4

    def w_copy(ph, src=None):
        if src is None:
            src = wq_hbm.at[:, pl.ds(0, HC), :]
        return pltpu.make_async_copy(src, raw.at[ph], sems.at[11 + ph])

    cp_x = [x_copy(c * XC, XC, 23 + c) for c in range(4)]
    cp_xa = x_copy(P0, XA - P0, 0)
    cp_x[0].start()
    cp_x[1].start()
    w_copy(0).start()
    cp_x[2].start()
    cp_x[3].start()
    cp_xa.start()
    for i, w in enumerate((wq_hbm, wk_hbm, wv_hbm)):
        for c in range(4):
            if 4 * i + c > 0:
                w_copy(4 * i + c, w.at[:, pl.ds(c * HC, HC), :]).start()
    cp_wo = [pltpu.make_async_copy(wo_hbm.at[:, pl.ds(n * 128, 128)], wo_raw.at[n], sems.at[4 + n])
             for n in range(4)]
    for c in cp_wo:
        c.start()
    cp_xb = x_copy(XA, S - XA, 1)
    cp_xb.start()
    cp_f = [pltpu.make_async_copy(wg_hbm, wg, sems.at[8]),
            pltpu.make_async_copy(wu_hbm, wu, sems.at[9]),
            pltpu.make_async_copy(wd_hbm, wd, sems.at[10])]
    for c in cp_f:
        c.start()

    def out_copy(row0, n):
        return pltpu.make_async_copy(xs.at[pl.ds(row0, n)], out_hbm.at[pl.ds(row0, n)], sems.at[2])

    oring1[...] = jnp.zeros(oring1.shape, F32)
    abuf0[...] = jnp.zeros(abuf0.shape, F32)
    xs[pl.ds(S, W), :] = jnp.zeros((W, D), BF16)
    hbuf[pl.ds(2 * S, 2 * W), :] = jnp.zeros((2 * W, D), F32)
    zflag[...] = jnp.zeros(zflag.shape, jnp.int32)

    ri = jax.lax.broadcasted_iota(jnp.int32, (L2, L2), 0)
    ci = jax.lax.broadcasted_iota(jnp.int32, (L2, L2), 1)

    def head_of(i):
        return jnp.where(i < 2 * M, i // M, (i - 2 * M) // SEG)

    def pos_of(i):
        return jnp.where(i < 2 * M, i % M, M + (i - 2 * M) % SEG)

    same = head_of(ri) == head_of(ci)
    ok = (pos_of(ri) < M) | (pos_of(ri) >= pos_of(ci))
    maskv[...] = jnp.where(same, jnp.where(ok, 0.0, -1e9 / SCALE), -jnp.inf).astype(F32)

    def gate(tok):
        return jnp.where(zflag[...] != 0, tok.astype(jnp.int32), 0)[0, 0]

    def toks(ys, n, frac=0.8):
        rows = [(y, r) for y in ys for r in range(0, y.shape[0], 8)]
        return [rows[int(len(rows) * frac * i / n)] for i in range(n)]

    def ln0(r0, tk=None):
        r = r0
        if tk is not None:
            r = pl.multiple_of(jnp.clip(r0 + gate(tk[0][tk[1]:tk[1] + 8]), 0, S - W), W)
        h = _ln(xs[pl.ds(r, W), :].astype(F32))
        hbuf[r0:r0 + W, :] = h
        if r0 < P0:
            hpack[r0 // 2:(r0 + W) // 2, :] = pltpu.bitcast(h.astype(BF16), U32)

    def tile_base(ph):
        return (ph % 4) * 24 + (ph // 4) * 2

    def relay(ph, tks=None):
        is_light = isinstance(ph, int) and ph < NLP // 4
        tb = tile_base(ph)
        for db in range(D // 16):
            d0 = 16 * db
            if tks is not None:
                y, r = tks[db]
                d0 = jnp.clip(d0 + gate(y[r:r + 8]), 0, D - 16)
            a = jnp.swapaxes(raw[ph, pl.ds(d0, 16)], 0, 1)
            for hh in range(HC):
                v = pltpu.bitcast(a[hh], U32)
                if is_light:
                    wql[ph * HC + hh, pl.ds(8 * db, 8), :] = v
                else:
                    wqkv[tb + (hh // 2) * 6 + hh % 2, pl.ds(8 * db, 8), :] = v

    def light(heads, r0=0, r1=P0):
        lhs = _w(hpack[r0 // 2:r1 // 2, :])
        ys = []
        for h in heads:
            y = _dot(lhs, _w(wql[h]))
            qbig[h, pl.ds(r0, r1 - r0), :] = y
            ys.append(y)
        return ys

    def win0(ph):
        tb = tile_base(ph)
        lhs = _w(hpack[pl.ds(0, W // 2), :])
        for hh in range(HC):
            t = tb + (hh // 2) * 6 + hh % 2
            ring0[t] = _dot(lhs, _w(wqkv[t]))

    for c in range(2):
        cp_x[c].wait()
        for k in range(XC // W):
            ln0(c * XC + k * W)
    w_copy(0).wait()
    relay(0)

    cp_x[2].wait()
    cp_x[3].wait()
    tks = toks(light(range(4), 0, 2 * XC), 2 * XC // W, 0.7)
    for k in range(2 * XC // W):
        ln0(2 * XC + k * W, tks[k])

    w_copy(1).wait()
    cp_xa.wait()
    tks = toks(light(range(4), 2 * XC, P0), 34)
    relay(1, tks[:16] + tks[17:33])
    ln0(P0, tks[16])
    ln0(P0 + W, tks[33])

    for ph in range(2, 4):
        w_copy(ph).wait()
        relay(ph, toks(light((2 * ph, 2 * ph + 1)), 32))

    def phase_b(ph, carry):
        w_copy(ph).wait()
        win0(ph - 1)
        relay(ph, toks(light((2 * ph, 2 * ph + 1)), 32))
        return carry

    jax.lax.fori_loop(4, 11, phase_b, 0)

    w_copy(11).wait()
    win0(10)
    relay(11, toks(light((22,)), 32))

    for c in cp_wo:
        c.wait()
    win0(11)
    tks = toks(light((23,)), 32, 0.9)
    zf = zflag[...] != 0
    for k in range(32):
        y, r = tks[k]
        tok = pltpu.bitcast(y[r:r + 8], U32)
        n, kk = k // 8, k % 8
        v = pltpu.bitcast(wo_raw[n, pl.ds(512 * kk, 512), :], U32).reshape(32, 8, 128)
        wo[n, pl.ds(256 * kk, 256), :] = jnp.where(zf[None], tok[None], v).reshape(256, 128)

    def post(row0, a, valid):
        n = a.shape[0]
        x1 = _rb(xs[pl.ds(row0, n), :].astype(F32) + _rb(a))
        x1buf[pl.ds(row0, n), :] = x1.astype(BF16)
        hb = _ln(x1)
        r = _rb(jnp.sum(hb * wr_ref[...].astype(F32), axis=-1, keepdims=True))
        x2 = x1 + hb
        xs[pl.ds(row0, n), :] = x2.astype(BF16)
        if valid is not True:
            r = jnp.where(valid, r, -jnp.inf)
        bv = best[0]
        bi = best[1]
        sub = jax.lax.broadcasted_iota(jnp.int32, (8, 128), 0).astype(F32)
        for g in range(n // 8):
            rg = jnp.broadcast_to(r[8 * g:8 * g + 8], (8, 128))
            ig = sub + (float(row0 + 8 * g) if isinstance(row0, int) else (row0 + 8 * g).astype(F32))
            gt = rg > bv
            bv = jnp.where(gt, rg, bv)
            bi = jnp.where(gt, ig, bi)
        best[0] = bv
        best[1] = bi
        return _tok(x2, bv, bi)

    def anchor(val, tok):
        return jnp.where(zflag[...] != 0, tok, val)

    def wo_pair(g, half):
        return jnp.concatenate(
            [_w(wo[2 * half + c, pl.ds(g * 128, 128), :]) for c in range(2)], axis=1)

    def step(q, par, layer, u, mem, korder):
        rr = par * SEG
        if par == 0:
            rows = ((0, 40), (0, 24))
        else:
            rows = ((40, 64), (24, 64))
        sg = layer * (2 * NU) + 2 * u + par
        hw = pl.multiple_of(layer * S + W * (u + 1), W)
        pl0 = pl.multiple_of(P0 + LR * sg, 8)
        lhs = [jnp.concatenate([mem, hbuf[pl.ds(hw + lo, hi - lo), :]], axis=0).astype(BF16)
               for lo, hi in rows]
        lhsl = jnp.concatenate([mem, hbuf[pl.ds(pl0, LR), :]], axis=0).astype(BF16)
        qrow = [pl.multiple_of((pl0 + 8 * i) % S, 8) for i in range(LR // 8)]

        def qkv(g, korder=None):
            half = g // (NPAIR // 2)
            lo, hi = rows[half]
            res = []
            ys = {}
            if korder is not None:
                part = None
                for k in korder:
                    wk = jnp.concatenate([_w(wqkv[6 * g + t, pl.ds(64 * k, 64), :])
                                          for t in range(2, 6)], axis=1)
                    y = jnp.dot(lhs[half][:, 128 * k:128 * (k + 1)], wk,
                                preferred_element_type=F32)
                    part = y if part is None else part + y
                for t in range(4):
                    ys[t + 2] = part[:, 128 * t:128 * (t + 1)]
            for t in range(6):
                if g < NLP and t < 2:
                    y = jnp.dot(lhsl, _w(wql[2 * g + t]), preferred_element_type=F32)
                    for i in range(LR // 8):
                        qbig[2 * g + t, pl.ds(qrow[i], 8), :] = y[M + 8 * i:M + 8 * i + 8]
                    res.append(y[:M])
                    continue
                if t in ys:
                    y = ys[t]
                else:
                    y = jnp.dot(lhs[half], _w(wqkv[6 * g + t]), preferred_element_type=F32)
                ring[1 - q][6 * g + t, lo:hi, :] = y[M:]
                res.append(y[:M])
            return res

        crow = pl.multiple_of(W * u + rr, SEG)
        qx = {}

        def stack(g, mres, i):
            if i == 0 and g < NLP:
                return jnp.concatenate(
                    [jnp.concatenate([mres[0], mres[1]], axis=0).astype(BF16), qx[g]], axis=0)
            return jnp.concatenate(
                [mres[2 * i], mres[2 * i + 1],
                 ring[q][6 * g + 2 * i, rr:rr + SEG, :],
                 ring[q][6 * g + 2 * i + 1, rr:rr + SEG, :]], axis=0).astype(BF16)

        def qk(g, mres, prenorm):
            q2, k2 = stack(g, mres, 0), stack(g, mres, 1)
            s = jax.lax.dot_general(q2, k2, (((1,), (1,)), ((), ())), preferred_element_type=F32)
            mk = maskv[...]
            s = jnp.where(mk == 0.0, s, mk)
            mx = jnp.max(s, axis=-1, keepdims=True)
            p = jnp.exp2((s - mx) * (SCALE * LOG2E))
            l = jnp.sum(p, axis=-1, keepdims=True)
            r0 = pl.reciprocal(l, approx=True)
            r = r0 * (2.0 - l * r0)
            if prenorm:
                return (p * r).astype(BF16), None
            return p.astype(BF16), r

        def pv(g, mres, pr):
            p, r = pr
            o = jnp.dot(p, stack(g, mres, 2), preferred_element_type=F32)
            if r is not None:
                o = o * r
            oring[q][2 * g, rr:rr + SEG, :] = o[2 * M:2 * M + SEG]
            oring[q][2 * g + 1, rr:rr + SEG, :] = o[2 * M + SEG:]
            return o[:M], o[M:2 * M]

        def olhs(g, om, half):
            lo, hi = rows[half]
            return jnp.concatenate(
                [jnp.concatenate([om[c], oring[1 - q][2 * g + c, lo:hi, :]], axis=0)
                 for c in range(2)], axis=1).astype(BF16)

        pn0 = pl.multiple_of(PLN + LR * sg, 8)
        xr = jnp.concatenate(
            [xs[pl.ds(pl.multiple_of((pn0 + 8 * i) % S, 8), 8), :].astype(F32)
             for i in range(LR // 8)], axis=0)
        hpre = _ln(xr)
        hbuf[pl.ds(pn0, LR), :] = hpre
        tok_pre = _tok(hpre)
        valid = u >= 2
        row0 = pl.multiple_of(jnp.where(valid, W * (u - 2), S) + rr, SEG)
        tok_post = post(row0, abuf[q][rr:rr + SEG, :], valid)

        NST = NPAIR // 2
        st = [(i, i + NST) if par == 0 else (i + NST, i) for i in range(NST)]
        mres, prs, oms = {}, {}, {}
        acc = [None] * 4
        order = []
        for i in range(NST):
            order += [("qkv", g) for g in st[i]]
            if i >= 1:
                order += [("qk", g) for g in st[i - 1]]
            if i >= 2:
                order += [("pv", g) for g in st[i - 2]]
        oq = [g for i in range(NST) for g in st[i]]
        NE = 8
        order += [("o", g) for g in oq[0:3]]
        order += [("qk", g) for g in st[NST - 1]] + [("pv", g) for g in st[NST - 2]]
        order += [("o", g) for g in oq[3:7]]
        order += [("pv", g) for g in st[NST - 1]]
        order += [("o", g) for g in oq[7:NE]]
        norder = (2, 3, 0, 1) if par == 0 else (0, 1, 2, 3)
        order += [("on", n) for n in norder]
        for kind, g in order:
            if kind == "qkv":
                mres[g] = qkv(g, korder if g == st[0][0] else None)
                if g < NLP:
                    qx[g] = jnp.concatenate([qbig[2 * g + c, pl.ds(crow, SEG), :] for c in range(2)],
                                            axis=0).astype(BF16)
                if g == st[2][0]:
                    mres[g][0] = anchor(mres[g][0], tok_pre)
                if g == st[4][0]:
                    mres[g][0] = anchor(mres[g][0], tok_post)
            elif kind == "qk":
                prs[g] = qk(g, mres[g], g not in st[NST - 1] + st[NST - 2])
            elif kind == "pv":
                oms[g] = pv(g, mres[g], prs[g])
                if prs[g][1] is not None:
                    oms[g] = (anchor(oms[g][0], _tok(prs[g][1][2 * M:])), oms[g][1])
            elif kind == "o":
                for half in range(2):
                    y = jnp.dot(olhs(g, oms[g], half), wo_pair(g, half), preferred_element_type=F32)
                    for c in range(2):
                        yc = y[:, 128 * c:128 * (c + 1)]
                        n = 2 * half + c
                        acc[n] = yc if acc[n] is None else acc[n] + yc
            else:
                n = g
                l = jnp.concatenate([olhs(g2, oms[g2], n // 2) for g2 in oq[NE:]], axis=1)
                wn = jnp.concatenate([_w(wo[n, pl.ds(g2 * 128, 128), :]) for g2 in oq[NE:]], axis=0)
                acc[n] = acc[n] + jnp.dot(l, wn, preferred_element_type=F32)
        for n in range(4):
            lo, hi = rows[n // 2]
            abuf[1 - q][lo:hi, n * 128:(n + 1) * 128] = acc[n][M:]

        return jnp.concatenate([acc[n][:M] for n in range(4)], axis=1), norder

    def layer_body(layer, carry):
        best[0] = jnp.full((8, 128), -jnp.inf, F32)
        best[1] = jnp.zeros((8, 128), F32)

        def qstep(j, mem):
            @pl.when((layer == 0) & (j == 1))
            def _():
                cp_xb.wait()

            @pl.when((layer == 1) & (j >= 2))
            def _():
                out_copy(pl.multiple_of((j - 2) * OB, OB), OB).start()

            ko = None
            for q in range(2):
                for par in range(2):
                    mem, ko = step(q, par, layer, 2 * j + q, mem, ko)
            return mem

        jax.lax.fori_loop(0, NU // 2, qstep, mem0_ref[...].astype(F32))

        @pl.when(layer == 1)
        def _():
            out_copy(S - 2 * OB, OB).start()

        post(S - 2 * W, abuf0[...], True)
        acc = None
        for g in range(NPAIR):
            l = jnp.concatenate([oring1[2 * g + c] for c in range(2)], axis=1).astype(BF16)
            y = _dot(l, jnp.concatenate([wo_pair(g, 0), wo_pair(g, 1)], axis=1))
            acc = y if acc is None else acc + y
        post(S - W, acc, True)

        @pl.when(layer == 0)
        def _():
            for c in cp_f:
                c.wait()

        bv = best[0]
        bi = best[1]
        vmax = jnp.max(bv, axis=0, keepdims=True)
        imin = jnp.min(jnp.where(bv == vmax, bi, float(S)), axis=0, keepdims=True)
        idx = jnp.clip(jnp.min(imin).astype(jnp.int32), 0, S - 1)
        g0 = pl.multiple_of((idx // 16) * 16, 16)
        x1 = x1buf[pl.ds(g0, 16), :].astype(F32)
        hb = _ln(x1)
        hbb = hb.astype(BF16)
        gpre = _rb(_dot(hbb, wg[...]))
        gs = _rb(gpre * _rb(jax.nn.sigmoid(gpre)))
        up = _rb(_dot(hbb, wu[...]))
        y = _rb(_dot((gs * up).astype(BF16), wd[...]))
        rsel = _rb(jax.nn.sigmoid(vmax))[:, :1]
        y = _rb(y * rsel)
        x2 = _rb(x1 + _rb(hb + y))
        rowi = jax.lax.broadcasted_iota(jnp.int32, (16, D), 0) + g0

        @pl.when(layer == 1)
        def _():
            for _i in range(S // OB - 1):
                out_copy(0, OB).wait()

        x2 = jnp.where(rowi == idx, x2, xs[pl.ds(g0, 16), :].astype(F32))
        xs[pl.ds(g0, 16), :] = x2.astype(BF16)

        @pl.when(layer == 0)
        def _():
            h16 = _ln(x2)
            hbuf[pl.ds(S + g0, 16), :] = h16

            @pl.when(idx < FD)
            def _():
                def body(g, c):
                    for t in range(2):
                        qbig[2 * g + t, pl.ds(g0, 16), :] = _dot(h16.astype(BF16), _w(wql[2 * g + t]))
                    return c

                jax.lax.fori_loop(0, NLP, body, 0, unroll=2)

            @pl.when(idx < W)
            def _():
                gw = pl.multiple_of(jnp.minimum(g0, W - 16), 16)

                def body(g, c):
                    for t in range(2, 6):
                        ring0[6 * g + t, pl.ds(gw, 16), :] = _dot(h16.astype(BF16), _w(wqkv[6 * g + t]))
                    return c

                jax.lax.fori_loop(0, NPAIR, body, 0)
                for g in range(NLP, NPAIR):
                    for t in range(2):
                        ring0[6 * g + t, pl.ds(gw, 16), :] = _dot(h16.astype(BF16),
                                                                  _w(wqkv[6 * g + t]))

        @pl.when(layer == 1)
        def _():
            last = out_copy(S - OB, OB)
            last.start()

            @pl.when(g0 < S - OB)
            def _():
                fix = pltpu.make_async_copy(xs.at[pl.ds(g0, 16)], out_hbm.at[pl.ds(g0, 16)],
                                            sems.at[3])
                fix.start()
                fix.wait()

            last.wait()

        return carry

    jax.lax.fori_loop(0, 2, layer_body, 0)


@functools.partial(jax.jit, static_argnames=("A_seg_len",))
def pallas_interleave_layers__memory_aug_recurrent_mem_tr__moe_arch_mod__prompt_kernel(
    A_x: jax.Array,
    A_mem0: jax.Array,
    A_Wq: jax.Array,
    A_Wk: jax.Array,
    A_Wv: jax.Array,
    A_Wo: jax.Array,
    A_seg_len,
    B_x: jax.Array,
    B_w_r: jax.Array,
    B_w_gate: jax.Array,
    B_w_up: jax.Array,
    B_w_down: jax.Array,
):
    assert A_seg_len == SEG
    assert A_x.shape == (1, S, D) and A_Wq.shape == (D, H, E) and A_mem0.shape == (1, M, D)
    any_spec = pl.BlockSpec(memory_space=pl.ANY)
    vmem_spec = pl.BlockSpec(memory_space=pltpu.VMEM)
    out = pl.pallas_call(
        _kernel,
        out_shape=jax.ShapeDtypeStruct((S, D), BF16),
        in_specs=[any_spec, vmem_spec, any_spec, any_spec, any_spec, any_spec,
                  vmem_spec, any_spec, any_spec, any_spec],
        out_specs=any_spec,
        scratch_shapes=[
            pltpu.VMEM((S + W, D), BF16),
            pltpu.VMEM((S + W, D), BF16),
            pltpu.VMEM((2 * S + 2 * W, D), F32),
            pltpu.VMEM((P0 // 2, D), U32),
            pltpu.VMEM((12, D, H // 4, E), BF16),
            pltpu.VMEM((2 * NLP, D // 2, E), U32),
            pltpu.VMEM((6 * NPAIR, D // 2, E), U32),
            pltpu.VMEM((4, H * E, 128), BF16),
            pltpu.VMEM((4, H * E // 2, 128), U32),
            pltpu.VMEM((D, F), BF16),
            pltpu.VMEM((D, F), BF16),
            pltpu.VMEM((F, D), BF16),
            pltpu.VMEM((6 * NPAIR, W, E), F32),
            pltpu.VMEM((6 * NPAIR, W, E), F32),
            pltpu.VMEM((2 * NLP, S, E), F32),
            pltpu.VMEM((H, W, E), F32),
            pltpu.VMEM((H, W, E), F32),
            pltpu.VMEM((W, D), F32),
            pltpu.VMEM((W, D), F32),
            pltpu.VMEM((L2, L2), F32),
            pltpu.VMEM((2, 8, 128), F32),
            pltpu.VMEM((8, 128), jnp.int32),
            pltpu.SemaphoreType.DMA((27,)),
        ],
        compiler_params=pltpu.CompilerParams(vmem_limit_bytes=110 * 1024 * 1024),
        name="rmt_mod",
    )(A_x.reshape(S, D), A_mem0.reshape(M, D), A_Wq, A_Wk, A_Wv, A_Wo.reshape(H * E, D),
      B_w_r.reshape(1, D), B_w_gate, B_w_up, B_w_down)
    return out.reshape(1, S, D)
```

```python
import functools

import jax
import jax.numpy as jnp
import jax.experimental.pallas as pl
import jax.experimental.pallas.tpu as pltpu

S = 2048
D = 512
H = 32
E = 128
M = 8
SEG = 32
F = 1792
NPAIR = H // 2
NU = S // (2 * SEG)
W = 2 * SEG
L2 = 2 * (M + SEG)
EPS = 1e-05
SCALE = float(E) ** -0.5
LOG2E = 1.4426950408889634
F32 = jnp.float32
BF16 = jnp.bfloat16
U32 = jnp.uint32


def _rb(x):
    return x.astype(BF16).astype(F32)


def _ln(x):
    mu = jnp.sum(x, axis=-1, keepdims=True) * (1.0 / D)
    xc0 = x - mu
    var = jnp.sum(xc0 * xc0, axis=-1, keepdims=True) * (1.0 / D)
    sd = _rb(jnp.sqrt(_rb(_rb(var) + EPS)))
    xc = _rb(x - _rb(mu))
    return _rb(xc * (1.0 / sd))


def _dot(a, b):
    return jnp.dot(a, b, preferred_element_type=F32)


def _w(ref_slab):
    return pltpu.bitcast(ref_slab, BF16)


NLP = 12
P0 = 1024
PLN = 1096
LR = 24
XC = 256
XLN = P0 + 2 * W
XA = XLN + W
FD = P0 + LR * 2 * NU - S
OB = 2 * W


def _tok(*vals):
    parts = []
    for v in vals:
        if v.shape[1] < 128:
            v = jnp.broadcast_to(v[:, :1], (v.shape[0], 128))
        for i in range(v.shape[0] // 8):
            for j in range(v.shape[1] // 128):
                parts.append(v[8 * i:8 * i + 8, 128 * j:128 * j + 128])
    while len(parts) > 1:
        parts = [jnp.maximum(parts[i], parts[i + 1]) if i + 1 < len(parts) else parts[i]
                 for i in range(0, len(parts), 2)]
    return parts[0]


def _kernel(x_hbm, mem0_hbm, wq_hbm, wk_hbm, wv_hbm, wo_hbm, wr_hbm, wg_hbm, wu_hbm, wd_hbm,
            out_hbm,
            xs, x1buf, hbuf, hpack, raw, wql, wqkv, wo_raw, wo, wg, wu, wd,
            ring0, ring1, qbig, oring0, oring1, abuf0, abuf1, maskv, best, zflag,
            mem0_ref, wr_ref, sems):
    ring, oring, abuf = (ring0, ring1), (oring0, oring1), (abuf0, abuf1)

    def x_copy(row0, n, sem):
        return pltpu.make_async_copy(x_hbm.at[pl.ds(row0, n)], xs.at[pl.ds(row0, n)], sems.at[sem])

    HC = H // 4

    def w_copy(ph, src=None):
        if src is None:
            src = wq_hbm.at[:, pl.ds(0, HC), :]
        return pltpu.make_async_copy(src, raw.at[ph], sems.at[11 + ph])

    cp_x = [x_copy(c * XC, XC, 23 + c) for c in range(4)]
    cp_xa = x_copy(P0, XA - P0, 0)
    cp_x[0].start()
    cp_x[1].start()
    w_copy(0).start()
    cp_x[2].start()
    cp_x[3].start()
    cp_xa.start()
    cp_s = [pltpu.make_async_copy(mem0_hbm, mem0_ref, sems.at[27]),
            pltpu.make_async_copy(wr_hbm, wr_ref, sems.at[28])]
    for c in cp_s:
        c.start()
    for i, w in enumerate((wq_hbm, wk_hbm, wv_hbm)):
        for c in range(4):
            if 4 * i + c > 0:
                w_copy(4 * i + c, w.at[:, pl.ds(c * HC, HC), :]).start()
    cp_wo = [pltpu.make_async_copy(wo_hbm.at[:, pl.ds(n * 128, 128)], wo_raw.at[n], sems.at[4 + n])
             for n in range(4)]
    for c in cp_wo:
        c.start()
    cp_xb = x_copy(XA, S - XA, 1)
    cp_f = [pltpu.make_async_copy(wg_hbm, wg, sems.at[8]),
            pltpu.make_async_copy(wu_hbm, wu, sems.at[9]),
            pltpu.make_async_copy(wd_hbm, wd, sems.at[10])]

    def out_copy(row0, n):
        return pltpu.make_async_copy(xs.at[pl.ds(row0, n)], out_hbm.at[pl.ds(row0, n)], sems.at[2])

    oring1[...] = jnp.zeros(oring1.shape, F32)
    abuf0[...] = jnp.zeros(abuf0.shape, F32)
    xs[pl.ds(S, W), :] = jnp.zeros((W, D), BF16)
    hbuf[pl.ds(2 * S, 2 * W), :] = jnp.zeros((2 * W, D), F32)
    zflag[...] = jnp.zeros(zflag.shape, jnp.int32)

    ri = jax.lax.broadcasted_iota(jnp.int32, (L2, L2), 0)
    ci = jax.lax.broadcasted_iota(jnp.int32, (L2, L2), 1)

    def head_of(i):
        return jnp.where(i < 2 * M, i // M, (i - 2 * M) // SEG)

    def pos_of(i):
        return jnp.where(i < 2 * M, i % M, M + (i - 2 * M) % SEG)

    same = head_of(ri) == head_of(ci)
    ok = (pos_of(ri) < M) | (pos_of(ri) >= pos_of(ci))
    maskv[...] = jnp.where(same, jnp.where(ok, 0.0, -1e9 / SCALE), -jnp.inf).astype(F32)

    def gate(v, tk):
        y, r = tk
        ns = min(v.shape[-2], 8)
        tok = pltpu.bitcast(y[r:r + 8], v.dtype)[:ns]
        zf = (zflag[...] != 0)[:ns]
        reps = (v.shape[-2] // ns, v.shape[-1] // 128)
        tok, zf = jnp.tile(tok, reps), jnp.tile(zf, reps)
        return jnp.where(zf, tok, v)

    def toks(ys, n, frac=0.8):
        rows = [(y, r) for y in ys for r in range(0, y.shape[0], 8)]
        return [rows[int(len(rows) * frac * i / n)] for i in range(n)]

    def ln0(r0, tk=None, n=W):
        x = xs[r0:r0 + n, :].astype(F32)
        if tk is not None:
            x = gate(x, tk)
        h = _ln(x)
        hbuf[r0:r0 + n, :] = h
        if r0 < P0:
            hpack[r0 // 2:(r0 + n) // 2, :] = pltpu.bitcast(h.astype(BF16), U32)

    def tile_base(ph):
        return (ph % 4) * 24 + (ph // 4) * 2

    def relay(ph, tks=None):
        is_light = isinstance(ph, int) and ph < NLP // 4
        tb = tile_base(ph)
        for db in range(D // 16):
            a = raw[ph, pl.ds(16 * db, 16)]
            if tks is not None:
                a = pltpu.bitcast(gate(pltpu.bitcast(a, U32), tks[db]), BF16)
            a = jnp.swapaxes(a, 0, 1)
            for hh in range(HC):
                v = pltpu.bitcast(a[hh], U32)
                if is_light:
                    wql[ph * HC + hh, pl.ds(8 * db, 8), :] = v
                else:
                    wqkv[tb + (hh // 2) * 6 + hh % 2, pl.ds(8 * db, 8), :] = v

    def light(heads, r0=0, r1=P0):
        lhs = _w(hpack[r0 // 2:r1 // 2, :])
        ys = []
        for h in heads:
            y = _dot(lhs, _w(wql[h]))
            qbig[h, pl.ds(r0, r1 - r0), :] = y
            ys.append(y)
        return ys

    def win0(ph):
        tb = tile_base(ph)
        lhs = _w(hpack[pl.ds(0, W // 2), :])
        ys = []
        for hh in range(HC):
            t = tb + (hh // 2) * 6 + hh % 2
            y = _dot(lhs, _w(wqkv[t]))
            ring0[t] = y
            ys.append(y)
        return ys

    for c in range(2):
        cp_x[c].wait()
        for k in range(XC // W):
            ln0(c * XC + k * W)
    w_copy(0).wait()
    relay(0)

    cp_x[2].wait()
    cp_x[3].wait()
    tks = toks(light(range(4), 0, 2 * XC), 2 * XC // SEG, 0.85)
    for k in range(2 * XC // SEG):
        ln0(2 * XC + k * SEG, tks[k], SEG)

    w_copy(1).wait()
    relay(1, toks(light(range(4), 2 * XC, P0), 32))
    w_copy(2).wait()
    cp_xa.wait()
    tks = toks(light((4, 5)), 36, 0.85)
    relay(2, tks[:32])
    for k in range(4):
        ln0(P0 + k * SEG, tks[32 + k], SEG)
    w_copy(3).wait()
    relay(3, toks(light((6, 7)), 32))

    def phase_b(ph, carry):
        w_copy(ph).wait()
        win0(ph - 1)
        relay(ph, toks(light((2 * ph, 2 * ph + 1)), 32))
        return carry

    jax.lax.fori_loop(4, 12, phase_b, 0)

    for c in cp_wo[:3] + cp_s:
        c.wait()
    tks = toks(win0(11), 24, 0.9)
    for k in range(24):
        n, kk = k // 8, k % 8
        wo[n, pl.ds(256 * kk, 256), :] = gate(
            pltpu.bitcast(wo_raw[n, pl.ds(512 * kk, 512), :], U32), tks[k])
    cp_wo[3].wait()
    cp_xb.start()
    for c in cp_f:
        c.start()
    wo[3] = pltpu.bitcast(wo_raw[3], U32)

    def post(row0, a, valid):
        n = a.shape[0]
        x1 = _rb(xs[pl.ds(row0, n), :].astype(F32) + _rb(a))
        x1buf[pl.ds(row0, n), :] = x1.astype(BF16)
        hb = _ln(x1)
        r = _rb(jnp.sum(hb * wr_ref[...].astype(F32), axis=-1, keepdims=True))
        x2 = x1 + hb
        xs[pl.ds(row0, n), :] = x2.astype(BF16)
        if valid is not True:
            r = jnp.where(valid, r, -jnp.inf)
        bv = best[0]
        bi = best[1]
        sub = jax.lax.broadcasted_iota(jnp.int32, (8, 128), 0).astype(F32)
        for g in range(n // 8):
            rg = jnp.broadcast_to(r[8 * g:8 * g + 8], (8, 128))
            ig = sub + (float(row0 + 8 * g) if isinstance(row0, int) else (row0 + 8 * g).astype(F32))
            gt = rg > bv
            bv = jnp.where(gt, rg, bv)
            bi = jnp.where(gt, ig, bi)
        best[0] = bv
        best[1] = bi
        return _tok(x2, bv, bi)

    def anchor(val, tok):
        return jnp.where(zflag[...] != 0, tok, val)

    def wo_pair(g, half):
        return jnp.concatenate(
            [_w(wo[2 * half + c, pl.ds(g * 128, 128), :]) for c in range(2)], axis=1)

    def step(q, par, layer, u, mem, korder):
        rr = par * SEG
        if par == 0:
            rows = ((0, 40), (0, 24))
        else:
            rows = ((40, 64), (24, 64))
        sg = layer * (2 * NU) + 2 * u + par
        hw = pl.multiple_of(layer * S + W * (u + 1), W)
        pl0 = pl.multiple_of(P0 + LR * sg, 8)
        lhs = [jnp.concatenate([mem, hbuf[pl.ds(hw + lo, hi - lo), :]], axis=0).astype(BF16)
               for lo, hi in rows]
        lhsl = jnp.concatenate([mem, hbuf[pl.ds(pl0, LR), :]], axis=0).astype(BF16)
        qrow = [pl.multiple_of((pl0 + 8 * i) % S, 8) for i in range(LR // 8)]

        def qkv(g, korder=None):
            half = g // (NPAIR // 2)
            lo, hi = rows[half]
            res = []
            ys = {}
            if korder is not None:
                part = None
                for k in korder:
                    wk = jnp.concatenate([_w(wqkv[6 * g + t, pl.ds(64 * k, 64), :])
                                          for t in range(2, 6)], axis=1)
                    y = jnp.dot(lhs[half][:, 128 * k:128 * (k + 1)], wk,
                                preferred_element_type=F32)
                    part = y if part is None else part + y
                for t in range(4):
                    ys[t + 2] = part[:, 128 * t:128 * (t + 1)]
            for t in range(6):
                if g < NLP and t < 2:
                    y = jnp.dot(lhsl, _w(wql[2 * g + t]), preferred_element_type=F32)
                    for i in range(LR // 8):
                        qbig[2 * g + t, pl.ds(qrow[i], 8), :] = y[M + 8 * i:M + 8 * i + 8]
                    res.append(y[:M])
                    continue
                if t in ys:
                    y = ys[t]
                else:
                    y = jnp.dot(lhs[half], _w(wqkv[6 * g + t]), preferred_element_type=F32)
                ring[1 - q][6 * g + t, lo:hi, :] = y[M:]
                res.append(y[:M])
            return res

        crow = pl.multiple_of(W * u + rr, SEG)
        qx = {}

        def stack(g, mres, i):
            if i == 0 and g < NLP:
                return jnp.concatenate(
                    [jnp.concatenate([mres[0], mres[1]], axis=0).astype(BF16), qx[g]], axis=0)
            return jnp.concatenate(
                [mres[2 * i], mres[2 * i + 1],
                 ring[q][6 * g + 2 * i, rr:rr + SEG, :],
                 ring[q][6 * g + 2 * i + 1, rr:rr + SEG, :]], axis=0).astype(BF16)

        def qk(g, mres, prenorm):
            q2, k2 = stack(g, mres, 0), stack(g, mres, 1)
            s = jax.lax.dot_general(q2, k2, (((1,), (1,)), ((), ())), preferred_element_type=F32)
            mk = maskv[...]
            s = jnp.where(mk == 0.0, s, mk)
            mx = jnp.max(s, axis=-1, keepdims=True)
            p = jnp.exp2((s - mx) * (SCALE * LOG2E))
            l = jnp.sum(p, axis=-1, keepdims=True)
            r0 = pl.reciprocal(l, approx=True)
            r = r0 * (2.0 - l * r0)
            if prenorm:
                return (p * r).astype(BF16), None
            return p.astype(BF16), r

        def pv(g, mres, pr):
            p, r = pr
            o = jnp.dot(p, stack(g, mres, 2), preferred_element_type=F32)
            if r is not None:
                o = o * r
            oring[q][2 * g, rr:rr + SEG, :] = o[2 * M:2 * M + SEG]
            oring[q][2 * g + 1, rr:rr + SEG, :] = o[2 * M + SEG:]
            return o[:M], o[M:2 * M]

        def olhs(g, om, half):
            lo, hi = rows[half]
            return jnp.concatenate(
                [jnp.concatenate([om[c], oring[1 - q][2 * g + c, lo:hi, :]], axis=0)
                 for c in range(2)], axis=1).astype(BF16)

        pn0 = pl.multiple_of(PLN + LR * sg, 8)
        xr = jnp.concatenate(
            [xs[pl.ds(pl.multiple_of((pn0 + 8 * i) % S, 8), 8), :].astype(F32)
             for i in range(LR // 8)], axis=0)
        hpre = _ln(xr)
        hbuf[pl.ds(pn0, LR), :] = hpre
        tok_pre = _tok(hpre)
        valid = u >= 2
        row0 = pl.multiple_of(jnp.where(valid, W * (u - 2), S) + rr, SEG)
        tok_post = post(row0, abuf[q][rr:rr + SEG, :], valid)

        NST = NPAIR // 2
        st = [(i, i + NST) if par == 0 else (i + NST, i) for i in range(NST)]
        mres, prs, oms = {}, {}, {}
        acc = [None] * 4
        order = []
        for i in range(NST):
            order += [("qkv", g) for g in st[i]]
            if i >= 1:
                order += [("qk", g) for g in st[i - 1]]
            if i >= 2:
                order += [("pv", g) for g in st[i - 2]]
        oq = [g for i in range(NST) for g in st[i]]
        NE = 8
        order += [("o", g) for g in oq[0:3]]
        order += [("qk", g) for g in st[NST - 1]] + [("pv", g) for g in st[NST - 2]]
        order += [("o", g) for g in oq[3:7]]
        order += [("pv", g) for g in st[NST - 1]]
        order += [("o", g) for g in oq[7:NE]]
        norder = (2, 3, 0, 1) if par == 0 else (0, 1, 2, 3)
        order += [("on", n) for n in norder]
        for kind, g in order:
            if kind == "qkv":
                mres[g] = qkv(g, korder if g == st[0][0] else None)
                if g < NLP:
                    qx[g] = jnp.concatenate([qbig[2 * g + c, pl.ds(crow, SEG), :] for c in range(2)],
                                            axis=0).astype(BF16)
                if g == st[2][0]:
                    mres[g][0] = anchor(mres[g][0], tok_pre)
                if g == st[4][0]:
                    mres[g][0] = anchor(mres[g][0], tok_post)
            elif kind == "qk":
                prs[g] = qk(g, mres[g], g not in st[NST - 1] + st[NST - 2])
            elif kind == "pv":
                oms[g] = pv(g, mres[g], prs[g])
                if prs[g][1] is not None:
                    oms[g] = (anchor(oms[g][0], _tok(prs[g][1][2 * M:])), oms[g][1])
            elif kind == "o":
                for half in range(2):
                    y = jnp.dot(olhs(g, oms[g], half), wo_pair(g, half), preferred_element_type=F32)
                    for c in range(2):
                        yc = y[:, 128 * c:128 * (c + 1)]
                        n = 2 * half + c
                        acc[n] = yc if acc[n] is None else acc[n] + yc
            else:
                n = g
                l = jnp.concatenate([olhs(g2, oms[g2], n // 2) for g2 in oq[NE:]], axis=1)
                wn = jnp.concatenate([_w(wo[n, pl.ds(g2 * 128, 128), :]) for g2 in oq[NE:]], axis=0)
                acc[n] = acc[n] + jnp.dot(l, wn, preferred_element_type=F32)
        for n in range(4):
            lo, hi = rows[n // 2]
            abuf[1 - q][lo:hi, n * 128:(n + 1) * 128] = acc[n][M:]

        return jnp.concatenate([acc[n][:M] for n in range(4)], axis=1), norder

    def layer_body(layer, carry):
        best[0] = jnp.full((8, 128), -jnp.inf, F32)
        best[1] = jnp.zeros((8, 128), F32)

        def qstep(j, mem):
            @pl.when((layer == 0) & (j == 1))
            def _():
                cp_xb.wait()

            @pl.when((layer == 1) & (j >= 2))
            def _():
                out_copy(pl.multiple_of((j - 2) * OB, OB), OB).start()

            ko = None
            for q in range(2):
                for par in range(2):
                    mem, ko = step(q, par, layer, 2 * j + q, mem, ko)
            return mem

        jax.lax.fori_loop(0, NU // 2, qstep, mem0_ref[...].astype(F32))

        @pl.when(layer == 1)
        def _():
            out_copy(S - 2 * OB, OB).start()

        post(S - 2 * W, abuf0[...], True)
        acc = None
        for g in range(NPAIR):
            l = jnp.concatenate([oring1[2 * g + c] for c in range(2)], axis=1).astype(BF16)
            y = _dot(l, jnp.concatenate([wo_pair(g, 0), wo_pair(g, 1)], axis=1))
            acc = y if acc is None else acc + y
        post(S - W, acc, True)

        @pl.when(layer == 0)
        def _():
            for c in cp_f:
                c.wait()

        bv = best[0]
        bi = best[1]
        vmax = jnp.max(bv, axis=0, keepdims=True)
        imin = jnp.min(jnp.where(bv == vmax, bi, float(S)), axis=0, keepdims=True)
        idx = jnp.clip(jnp.min(imin).astype(jnp.int32), 0, S - 1)
        g0 = pl.multiple_of((idx // 16) * 16, 16)
        x1 = x1buf[pl.ds(g0, 16), :].astype(F32)
        hb = _ln(x1)
        hbb = hb.astype(BF16)
        gpre = _rb(_dot(hbb, wg[...]))
        gs = _rb(gpre * _rb(jax.nn.sigmoid(gpre)))
        up = _rb(_dot(hbb, wu[...]))
        y = _rb(_dot((gs * up).astype(BF16), wd[...]))
        rsel = _rb(jax.nn.sigmoid(vmax))[:, :1]
        y = _rb(y * rsel)
        x2 = _rb(x1 + _rb(hb + y))
        rowi = jax.lax.broadcasted_iota(jnp.int32, (16, D), 0) + g0

        @pl.when(layer == 1)
        def _():
            for _i in range(S // OB - 1):
                out_copy(0, OB).wait()

        x2 = jnp.where(rowi == idx, x2, xs[pl.ds(g0, 16), :].astype(F32))
        xs[pl.ds(g0, 16), :] = x2.astype(BF16)

        @pl.when(layer == 0)
        def _():
            h16 = _ln(x2)
            hbuf[pl.ds(S + g0, 16), :] = h16

            @pl.when(idx < FD)
            def _():
                def body(g, c):
                    for t in range(2):
                        qbig[2 * g + t, pl.ds(g0, 16), :] = _dot(h16.astype(BF16), _w(wql[2 * g + t]))
                    return c

                jax.lax.fori_loop(0, NLP, body, 0, unroll=2)

            @pl.when(idx < W)
            def _():
                gw = pl.multiple_of(jnp.minimum(g0, W - 16), 16)

                def body(g, c):
                    for t in range(2, 6):
                        ring0[6 * g + t, pl.ds(gw, 16), :] = _dot(h16.astype(BF16), _w(wqkv[6 * g + t]))
                    return c

                jax.lax.fori_loop(0, NPAIR, body, 0)
                for g in range(NLP, NPAIR):
                    for t in range(2):
                        ring0[6 * g + t, pl.ds(gw, 16), :] = _dot(h16.astype(BF16),
                                                                  _w(wqkv[6 * g + t]))

        @pl.when(layer == 1)
        def _():
            last = out_copy(S - OB, OB)
            last.start()

            @pl.when(g0 < S - OB)
            def _():
                fix = pltpu.make_async_copy(xs.at[pl.ds(g0, 16)], out_hbm.at[pl.ds(g0, 16)],
                                            sems.at[3])
                fix.start()
                fix.wait()

            last.wait()

        return carry

    jax.lax.fori_loop(0, 2, layer_body, 0)


@functools.partial(jax.jit, static_argnames=("A_seg_len",))
def pallas_interleave_layers__memory_aug_recurrent_mem_tr__moe_arch_mod__prompt_kernel(
    A_x: jax.Array,
    A_mem0: jax.Array,
    A_Wq: jax.Array,
    A_Wk: jax.Array,
    A_Wv: jax.Array,
    A_Wo: jax.Array,
    A_seg_len,
    B_x: jax.Array,
    B_w_r: jax.Array,
    B_w_gate: jax.Array,
    B_w_up: jax.Array,
    B_w_down: jax.Array,
):
    assert A_seg_len == SEG
    assert A_x.shape == (1, S, D) and A_Wq.shape == (D, H, E) and A_mem0.shape == (1, M, D)
    any_spec = pl.BlockSpec(memory_space=pl.ANY)
    out = pl.pallas_call(
        _kernel,
        out_shape=jax.ShapeDtypeStruct((S, D), BF16),
        in_specs=[any_spec] * 10,
        out_specs=any_spec,
        scratch_shapes=[
            pltpu.VMEM((S + W, D), BF16),
            pltpu.VMEM((S + W, D), BF16),
            pltpu.VMEM((2 * S + 2 * W, D), F32),
            pltpu.VMEM((P0 // 2, D), U32),
            pltpu.VMEM((12, D, H // 4, E), BF16),
            pltpu.VMEM((2 * NLP, D // 2, E), U32),
            pltpu.VMEM((6 * NPAIR, D // 2, E), U32),
            pltpu.VMEM((4, H * E, 128), BF16),
            pltpu.VMEM((4, H * E // 2, 128), U32),
            pltpu.VMEM((D, F), BF16),
            pltpu.VMEM((D, F), BF16),
            pltpu.VMEM((F, D), BF16),
            pltpu.VMEM((6 * NPAIR, W, E), F32),
            pltpu.VMEM((6 * NPAIR, W, E), F32),
            pltpu.VMEM((2 * NLP, S, E), F32),
            pltpu.VMEM((H, W, E), F32),
            pltpu.VMEM((H, W, E), F32),
            pltpu.VMEM((W, D), F32),
            pltpu.VMEM((W, D), F32),
            pltpu.VMEM((L2, L2), F32),
            pltpu.VMEM((2, 8, 128), F32),
            pltpu.VMEM((8, 128), jnp.int32),
            pltpu.VMEM((M, D), BF16),
            pltpu.VMEM((1, D), BF16),
            pltpu.SemaphoreType.DMA((29,)),
        ],
        compiler_params=pltpu.CompilerParams(vmem_limit_bytes=110 * 1024 * 1024),
        name="rmt_mod",
    )(A_x.reshape(S, D), A_mem0.reshape(M, D), A_Wq, A_Wk, A_Wv, A_Wo.reshape(H * E, D),
      B_w_r.reshape(1, D), B_w_gate, B_w_up, B_w_down)
    return out.reshape(1, S, D)
```

```python
import functools

import jax
import jax.numpy as jnp
import jax.experimental.pallas as pl
import jax.experimental.pallas.tpu as pltpu

S = 2048
D = 512
H = 32
E = 128
M = 8
SEG = 32
F = 1792
NPAIR = H // 2
NU = S // (2 * SEG)
W = 2 * SEG
L2 = 2 * (M + SEG)
EPS = 1e-05
SCALE = float(E) ** -0.5
LOG2E = 1.4426950408889634
F32 = jnp.float32
BF16 = jnp.bfloat16
U32 = jnp.uint32


def _rb(x):
    return x.astype(BF16).astype(F32)


def _ln(x):
    mu = jnp.sum(x, axis=-1, keepdims=True) * (1.0 / D)
    xc0 = x - mu
    var = jnp.sum(xc0 * xc0, axis=-1, keepdims=True) * (1.0 / D)
    sd = _rb(jnp.sqrt(_rb(_rb(var) + EPS)))
    xc = _rb(x - _rb(mu))
    return _rb(xc * (1.0 / sd))


def _dot(a, b):
    return jnp.dot(a, b, preferred_element_type=F32)


def _w(ref_slab):
    return pltpu.bitcast(ref_slab, BF16)


P0 = S // 2
LR = 24
PLN = P0 + LR
XC = P0 // 4
XLN = P0 + SEG
XA = P0 + 4 * SEG
FD = P0 + LR * 2 * NU - S
R = 4 * SEG
HC = H // 4


def _tok(*vals):
    parts = []
    for v in vals:
        if v.shape[1] < 128:
            v = jnp.broadcast_to(v[:, :1], (v.shape[0], 128))
        for i in range(v.shape[0] // 8):
            for j in range(v.shape[1] // 128):
                parts.append(v[8 * i:8 * i + 8, 128 * j:128 * j + 128])
    while len(parts) > 1:
        parts = [jnp.maximum(parts[i], parts[i + 1]) if i + 1 < len(parts) else parts[i]
                 for i in range(0, len(parts), 2)]
    return parts[0]


def _rslices(row0, n):
    row0 %= R
    if row0 + n <= R:
        return [(row0, row0 + n, 0)]
    return [(row0, R, 0), (0, row0 + n - R, R - row0)]


def _kernel(x_hbm, mem0_hbm, wq_hbm, wk_hbm, wv_hbm, wo_hbm, wr_hbm, wg_hbm, wu_hbm, wd_hbm,
            out_hbm,
            xs, x1buf, hbbuf, hbuf, hpack, raw, wq, wkv, wo_raw, wo, wg, wu, wd,
            qbig, kvring, oring, abuf, ybuf, maskv, best, zflag, mem0_ref, wr_ref, sems):
    def x_copy(row0, n, sem):
        return pltpu.make_async_copy(x_hbm.at[pl.ds(row0, n)], xs.at[pl.ds(row0, n)], sems.at[sem])

    def w_copy(ph, src=None):
        if src is None:
            src = wq_hbm.at[:, pl.ds(0, HC), :]
        return pltpu.make_async_copy(src, raw.at[ph], sems.at[11 + ph])

    cp_x = [x_copy(c * XC, XC, 23 + c) for c in range(4)]
    cp_xa = x_copy(P0, XA - P0, 0)
    cp_x[0].start()
    cp_x[1].start()
    w_copy(0).start()
    cp_x[2].start()
    cp_x[3].start()
    cp_xa.start()
    cp_s = [pltpu.make_async_copy(mem0_hbm, mem0_ref, sems.at[27]),
            pltpu.make_async_copy(wr_hbm, wr_ref, sems.at[28])]
    for c in cp_s:
        c.start()
    for i, w in enumerate((wq_hbm, wk_hbm, wv_hbm)):
        for c in range(4):
            if 4 * i + c > 0:
                w_copy(4 * i + c, w.at[:, pl.ds(c * HC, HC), :]).start()
    cp_wo = [pltpu.make_async_copy(wo_hbm.at[:, pl.ds(n * 128, 128)], wo_raw.at[n], sems.at[4 + n])
             for n in range(4)]
    for c in cp_wo:
        c.start()
    cp_xb = x_copy(XA, S - XA, 1)
    cp_f = [pltpu.make_async_copy(wg_hbm, wg, sems.at[8]),
            pltpu.make_async_copy(wu_hbm, wu, sems.at[9]),
            pltpu.make_async_copy(wd_hbm, wd, sems.at[10])]

    def out_copy(row0, n, sem=2):
        return pltpu.make_async_copy(xs.at[pl.ds(row0, n)], out_hbm.at[pl.ds(row0, n)], sems.at[sem])

    oring[:, R - M:R, :] = jnp.zeros((H, M, E), F32)
    abuf[...] = jnp.zeros(abuf.shape, F32)
    xs[pl.ds(S, SEG), :] = jnp.zeros((SEG, D), BF16)
    hbuf[pl.ds(2 * S, SEG), :] = jnp.zeros((SEG, D), F32)
    zflag[...] = jnp.zeros(zflag.shape, jnp.int32)

    ri = jax.lax.broadcasted_iota(jnp.int32, (L2, L2), 0)
    ci = jax.lax.broadcasted_iota(jnp.int32, (L2, L2), 1)

    def head_of(i):
        return jnp.where(i < 2 * M, i // M, (i - 2 * M) // SEG)

    def pos_of(i):
        return jnp.where(i < 2 * M, i % M, M + (i - 2 * M) % SEG)

    same = head_of(ri) == head_of(ci)
    ok = (pos_of(ri) < M) | (pos_of(ri) >= pos_of(ci))
    maskv[...] = jnp.where(same, jnp.where(ok, 0.0, -1e9 / SCALE), -jnp.inf).astype(F32)

    def gate(v, tk):
        y, r = tk
        ns = min(v.shape[-2], 8)
        tok = pltpu.bitcast(y[r:r + 8], v.dtype)[:ns]
        zf = (zflag[...] != 0)[:ns]
        reps = (v.shape[-2] // ns, v.shape[-1] // 128)
        tok, zf = jnp.tile(tok, reps), jnp.tile(zf, reps)
        return jnp.where(zf, tok, v)

    def toks(ys, n, frac=0.8):
        rows = [(y, r) for y in ys for r in range(0, y.shape[0], 8)]
        return [rows[int(len(rows) * frac * i / n)] for i in range(n)]

    def ln0(r0, tk=None, n=W):
        x = xs[r0:r0 + n, :].astype(F32)
        if tk is not None:
            x = gate(x, tk)
        h = _ln(x)
        hbuf[r0:r0 + n, :] = h
        if r0 < P0:
            hpack[r0 // 2:(r0 + n) // 2, :] = pltpu.bitcast(h.astype(BF16), U32)

    def relay(ph, tks=None):
        is_q = isinstance(ph, int) and ph < 4
        for db in range(D // 16):
            a = raw[ph, pl.ds(16 * db, 16)]
            if tks is not None:
                a = pltpu.bitcast(gate(pltpu.bitcast(a, U32), tks[db]), BF16)
            a = jnp.swapaxes(a, 0, 1)
            for hh in range(HC):
                v = pltpu.bitcast(a[hh], U32)
                if is_q:
                    wq[ph * HC + hh, pl.ds(8 * db, 8), :] = v
                else:
                    tb = (ph % 4) * 16 + (ph // 4 - 1) * 2
                    wkv[tb + (hh // 2) * 4 + hh % 2, pl.ds(8 * db, 8), :] = v

    def light(heads, r0=0, r1=P0):
        lhs = _w(hpack[r0 // 2:r1 // 2, :])
        ys = []
        for h in heads:
            y = _dot(lhs, _w(wq[h]))
            qbig[h, pl.ds(r0, r1 - r0), :] = y
            ys.append(y)
        return ys

    def kv_head(lhs16):
        ys = []
        for t in range(2 * NPAIR, 4 * NPAIR):
            y = _dot(lhs16, _w(wkv[t]))
            kvring[t, 0:M, :] = y[:M]
            ys.append(y)
        return ys

    for c in range(2):
        cp_x[c].wait()
        for k in range(XC // W):
            ln0(c * XC + k * W)
    w_copy(0).wait()
    relay(0)

    cp_x[2].wait()
    cp_x[3].wait()
    tks = toks(light(range(4), 0, 2 * XC), 2 * XC // SEG, 0.85)
    for k in range(2 * XC // SEG):
        ln0(2 * XC + k * SEG, tks[k], SEG)

    w_copy(1).wait()
    relay(1, toks(light(range(4), 2 * XC, P0), 32))
    w_copy(2).wait()
    cp_xa.wait()
    tks = toks(light((4, 5)), 33, 0.85)
    relay(2, tks[:32])
    ln0(P0, tks[32], SEG)
    w_copy(3).wait()
    relay(3, toks(light((6, 7)), 32))

    def phase_b(ph, carry):
        w_copy(ph).wait()
        relay(ph, toks(light([3 * ph - 4 + i for i in range(3)]), 32))
        return carry

    jax.lax.fori_loop(4, 12, phase_b, 0)

    for c in cp_wo + cp_s:
        c.wait()
    cp_xb.start()
    for c in cp_f:
        c.start()
    tks = toks(kv_head(_w(hpack[0:8, :])), 32, 0.9)
    for k in range(32):
        n, kk = k // 8, k % 8
        wo[n, pl.ds(256 * kk, 256), :] = gate(
            pltpu.bitcast(wo_raw[n, pl.ds(512 * kk, 512), :], U32), tks[k])

    def post(row0, a, valid):
        n = a.shape[0]
        x1 = _rb(xs[pl.ds(row0, n), :].astype(F32) + _rb(a))
        x1buf[pl.ds(row0, n), :] = x1.astype(BF16)
        hb = _ln(x1)
        hbbuf[pl.ds(row0, n), :] = hb.astype(BF16)
        r = _rb(jnp.sum(hb * wr_ref[...].astype(F32), axis=-1, keepdims=True))
        x2 = x1 + hb
        xs[pl.ds(row0, n), :] = x2.astype(BF16)
        if valid is not True:
            r = jnp.where(valid, r, -jnp.inf)
        bv = best[0]
        bi = best[1]
        sub = jax.lax.broadcasted_iota(jnp.int32, (8, 128), 0).astype(F32)
        for g in range(n // 8):
            rg = jnp.broadcast_to(r[8 * g:8 * g + 8], (8, 128))
            ig = sub + (float(row0 + 8 * g) if isinstance(row0, int) else (row0 + 8 * g).astype(F32))
            gt = rg > bv
            bv = jnp.where(gt, rg, bv)
            bi = jnp.where(gt, ig, bi)
        best[0] = bv
        best[1] = bi
        return _tok(x2, bv, bi)

    def anchor(val, tok):
        return jnp.where(zflag[...] != 0, tok, val)

    def wo_pair(g, half):
        return jnp.concatenate(
            [_w(wo[2 * half + c, pl.ds(g * 128, 128), :]) for c in range(2)], axis=1)

    def rload(buf, t, row0, n):
        return [buf[t, a:b, :] for a, b, _ in _rslices(row0, n)]

    def step(ts, layer, j, mem, korder):
        q, par = ts // 2, ts % 2
        sr = ts * SEG
        if par == 0:
            kvw = ((W * q, 40), (W * q + 8, 24))
            ow = ((W * q - 8, 40), (W * q, 24))
        else:
            kvw = ((W * q + 40, 24), (W * q + 32, 40))
            ow = ((W * q + 32, 24), (W * q + 24, 40))
        sl = 4 * j + ts
        sg = layer * (2 * NU) + sl
        hb0 = pl.multiple_of(layer * S + R * j, R)
        pq0 = pl.multiple_of(P0 + LR * sg, 8)
        lhs = [jnp.concatenate([mem, hbuf[pl.ds(hb0 + r0, n), :]], axis=0).astype(BF16)
               for r0, n in kvw]
        lhsq = jnp.concatenate([mem, hbuf[pl.ds(pq0, LR), :]], axis=0).astype(BF16)
        qrow = [pl.multiple_of((pq0 + 8 * i) % S, 8) for i in range(LR // 8)]
        crow = pl.multiple_of(R * j + sr, SEG)

        def qkv(g, korder=None):
            half = g // (NPAIR // 2)
            r0, n = kvw[half]
            ys = {}
            if korder is not None:
                part = None
                for k in korder:
                    wk = jnp.concatenate([_w(wkv[4 * g + t, pl.ds(64 * k, 64), :])
                                          for t in range(4)], axis=1)
                    y = jnp.dot(lhs[half][:, 128 * k:128 * (k + 1)], wk,
                                preferred_element_type=F32)
                    part = y if part is None else part + y
                for t in range(4):
                    ys[t] = part[:, 128 * t:128 * (t + 1)]
            res = []
            for c in range(2):
                y = jnp.dot(lhsq, _w(wq[2 * g + c]), preferred_element_type=F32)
                for i in range(LR // 8):
                    qbig[2 * g + c, pl.ds(qrow[i], 8), :] = y[M + 8 * i:M + 8 * i + 8]
                res.append(y[:M])
            for t in range(4):
                if t in ys:
                    y = ys[t]
                else:
                    y = jnp.dot(lhs[half], _w(wkv[4 * g + t]), preferred_element_type=F32)
                for a, b, o in _rslices(r0, n):
                    kvring[4 * g + t, a:b, :] = y[M + o:M + o + b - a]
                res.append(y[:M])
            qx = jnp.concatenate([qbig[2 * g + c, pl.ds(crow, SEG), :] for c in range(2)],
                                 axis=0).astype(BF16)
            return res, qx

        def stack(g, mres, i):
            return jnp.concatenate(
                [mres[2 * i], mres[2 * i + 1],
                 kvring[4 * g + 2 * i - 2, sr:sr + SEG, :],
                 kvring[4 * g + 2 * i - 1, sr:sr + SEG, :]], axis=0).astype(BF16)

        def qk(g, mres, qx, prenorm):
            q2 = jnp.concatenate(
                [jnp.concatenate([mres[0], mres[1]], axis=0).astype(BF16), qx], axis=0)
            s = jax.lax.dot_general(q2, stack(g, mres, 1), (((1,), (1,)), ((), ())),
                                    preferred_element_type=F32)
            mk = maskv[...]
            s = jnp.where(mk == 0.0, s, mk)
            mx = jnp.max(s, axis=-1, keepdims=True)
            p = jnp.exp2((s - mx) * (SCALE * LOG2E))
            l = jnp.sum(p, axis=-1, keepdims=True)
            r0 = pl.reciprocal(l, approx=True)
            r = r0 * (2.0 - l * r0)
            if prenorm:
                return (p * r).astype(BF16), None
            return p.astype(BF16), r

        def pv(g, mres, pr):
            p, r = pr
            o = jnp.dot(p, stack(g, mres, 2), preferred_element_type=F32)
            if r is not None:
                o = o * r
            oring[2 * g, sr:sr + SEG, :] = o[2 * M:2 * M + SEG]
            oring[2 * g + 1, sr:sr + SEG, :] = o[2 * M + SEG:]
            return o[:M], o[M:2 * M]

        def olhs(g, om, half):
            r0, n = ow[half]
            return jnp.concatenate(
                [jnp.concatenate([om[c]] + rload(oring, 2 * g + c, r0, n), axis=0)
                 for c in range(2)], axis=1).astype(BF16)

        pn0 = pl.multiple_of(PLN + LR * sg, 8)
        xr = jnp.concatenate(
            [xs[pl.ds(pl.multiple_of((pn0 + 8 * i) % S, 8), 8), :].astype(F32)
             for i in range(LR // 8)], axis=0)
        hpre = _ln(xr)
        hbuf[pl.ds(pn0, LR), :] = hpre
        tok_pre = _tok(hpre)
        if ts >= 2:
            valid = True
            row0 = pl.multiple_of(SEG * (sl - 2), SEG)
        else:
            valid = j >= 1
            row0 = pl.multiple_of(jnp.where(valid, SEG * (sl - 2), S), SEG)
        ar = (sr - 2 * SEG) % R
        tok_post = post(row0, abuf[ar:ar + SEG, :], valid)

        NST = NPAIR // 2
        st = [(i, i + NST) if par == 0 else (i + NST, i) for i in range(NST)]
        mres, qxs, prs, oms = {}, {}, {}, {}
        acc = [None] * 4
        order = []
        for i in range(NST):
            order += [("qkv", g) for g in st[i]]
            if i >= 1:
                order += [("qk", g) for g in st[i - 1]]
            if i >= 2:
                order += [("pv", g) for g in st[i - 2]]
        oq = [g for i in range(NST) for g in st[i]]
        NE = 8
        order += [("o", g) for g in oq[0:3]]
        order += [("qk", g) for g in st[NST - 1]] + [("pv", g) for g in st[NST - 2]]
        order += [("o", g) for g in oq[3:7]]
        order += [("pv", g) for g in st[NST - 1]]
        order += [("o", g) for g in oq[7:NE]]
        norder = (2, 3, 0, 1) if par == 0 else (0, 1, 2, 3)
        order += [("on", n) for n in norder]
        for kind, g in order:
            if kind == "qkv":
                mres[g], qxs[g] = qkv(g, korder if g == st[0][0] else None)
                if g == st[2][0]:
                    mres[g][0] = anchor(mres[g][0], tok_pre)
                if g == st[4][0]:
                    mres[g][0] = anchor(mres[g][0], tok_post)
            elif kind == "qk":
                prs[g] = qk(g, mres[g], qxs[g], g not in st[NST - 1] + st[NST - 2])
            elif kind == "pv":
                oms[g] = pv(g, mres[g], prs[g])
                if prs[g][1] is not None:
                    oms[g] = (anchor(oms[g][0], _tok(prs[g][1][2 * M:])), oms[g][1])
            elif kind == "o":
                for half in range(2):
                    y = jnp.dot(olhs(g, oms[g], half), wo_pair(g, half), preferred_element_type=F32)
                    for c in range(2):
                        yc = y[:, 128 * c:128 * (c + 1)]
                        n = 2 * half + c
                        acc[n] = yc if acc[n] is None else acc[n] + yc
            else:
                n = g
                l = jnp.concatenate([olhs(g2, oms[g2], n // 2) for g2 in oq[NE:]], axis=1)
                wn = jnp.concatenate([_w(wo[n, pl.ds(g2 * 128, 128), :]) for g2 in oq[NE:]], axis=0)
                acc[n] = acc[n] + jnp.dot(l, wn, preferred_element_type=F32)
        for n in range(4):
            r0, nr = ow[n // 2]
            for a, b, o in _rslices(r0, nr):
                abuf[a:b, n * 128:(n + 1) * 128] = acc[n][M + o:M + o + b - a]

        return jnp.concatenate([acc[n][:M] for n in range(4)], axis=1), norder

    def argmax():
        bv = best[0]
        bi = best[1]
        vmax = jnp.max(bv, axis=0, keepdims=True)
        imin = jnp.min(jnp.where(bv == vmax, bi, float(S)), axis=0, keepdims=True)
        idx = jnp.clip(jnp.min(imin).astype(jnp.int32), 0, S - 1)
        return idx, vmax

    def ffn(idx):
        g0 = pl.multiple_of((idx // 16) * 16, 16)
        hbb = hbbuf[pl.ds(g0, 16), :]
        gpre = _rb(_dot(hbb, wg[...]))
        gs = _rb(gpre * _rb(jax.nn.sigmoid(gpre)))
        up = _rb(_dot(hbb, wu[...]))
        ybuf[...] = _rb(_dot((gs * up).astype(BF16), wd[...]))

    def layer_body(layer, carry):
        best[0] = jnp.full((8, 128), -jnp.inf, F32)
        best[1] = jnp.zeros((8, 128), F32)

        def qstep(j, mem):
            @pl.when((layer == 0) & (j == 1))
            def _():
                cp_xb.wait()

            @pl.when((layer == 1) & (j >= 2))
            def _():
                out_copy(pl.multiple_of((j - 2) * R + W, W), R).start()

            @pl.when((layer == 1) & (j == 1))
            def _():
                out_copy(0, W).start()

            ko = None
            for ts in range(4):
                mem, ko = step(ts, layer, j, mem, ko)
            return mem

        jax.lax.fori_loop(0, NU // 2, qstep, mem0_ref[...].astype(F32))

        @pl.when(layer == 0)
        def _():
            for c in cp_f:
                c.wait()

        @pl.when(layer == 1)
        def _():
            out_copy(S - R - W, R).start()

        idx_s, _ = argmax()
        acc = None
        for g in range(NPAIR):
            l = jnp.concatenate([oring[2 * g + c, R - 16:R, :] for c in range(2)],
                                axis=1).astype(BF16)
            y = _dot(l, wo_pair(g, 0))
            acc = y if acc is None else acc + y
        abuf[R - M:R, 0:256] = acc[M:]
        ffn(idx_s)
        post(S - W, abuf[W:R, :], True)
        idx, vmax = argmax()

        @pl.when(layer == 1)
        def _():
            out_copy(S - W, W).start()

        @pl.when(idx // 16 != idx_s // 16)
        def _():
            ffn(idx)

        g0 = pl.multiple_of((idx // 16) * 16, 16)
        rsel = _rb(jax.nn.sigmoid(vmax))[:, :1]
        y = _rb(ybuf[...] * rsel)
        x2 = _rb(x1buf[pl.ds(g0, 16), :].astype(F32) + _rb(hbbuf[pl.ds(g0, 16), :].astype(F32) + y))
        rowi = jax.lax.broadcasted_iota(jnp.int32, (16, D), 0) + g0

        @pl.when(layer == 1)
        def _():
            out_copy(0, S).wait()

        x2 = jnp.where(rowi == idx, x2, xs[pl.ds(g0, 16), :].astype(F32))
        xs[pl.ds(g0, 16), :] = x2.astype(BF16)

        @pl.when(layer == 0)
        def _():
            h16 = _ln(x2)
            hbuf[pl.ds(S + g0, 16), :] = h16

            @pl.when(idx < FD)
            def _():
                def body(h, c):
                    qbig[h, pl.ds(g0, 16), :] = _dot(h16.astype(BF16), _w(wq[h]))
                    return c

                jax.lax.fori_loop(0, H, body, 0, unroll=4)

            @pl.when(idx < M)
            def _():
                kv_head(h16.astype(BF16))

        @pl.when(layer == 1)
        def _():
            fix = out_copy(g0, 16, 3)
            fix.start()
            fix.wait()

        return carry

    jax.lax.fori_loop(0, 2, layer_body, 0)


@functools.partial(jax.jit, static_argnames=("A_seg_len",))
def pallas_interleave_layers__memory_aug_recurrent_mem_tr__moe_arch_mod__prompt_kernel(
    A_x: jax.Array,
    A_mem0: jax.Array,
    A_Wq: jax.Array,
    A_Wk: jax.Array,
    A_Wv: jax.Array,
    A_Wo: jax.Array,
    A_seg_len,
    B_x: jax.Array,
    B_w_r: jax.Array,
    B_w_gate: jax.Array,
    B_w_up: jax.Array,
    B_w_down: jax.Array,
):
    assert A_seg_len == SEG
    assert A_x.shape == (1, S, D) and A_Wq.shape == (D, H, E) and A_mem0.shape == (1, M, D)
    any_spec = pl.BlockSpec(memory_space=pl.ANY)
    out = pl.pallas_call(
        _kernel,
        out_shape=jax.ShapeDtypeStruct((S, D), BF16),
        in_specs=[any_spec] * 10,
        out_specs=any_spec,
        scratch_shapes=[
            pltpu.VMEM((S + SEG, D), BF16),
            pltpu.VMEM((S + SEG, D), BF16),
            pltpu.VMEM((S + SEG, D), BF16),
            pltpu.VMEM((2 * S + SEG, D), F32),
            pltpu.VMEM((P0 // 2, D), U32),
            pltpu.VMEM((12, D, HC, E), BF16),
            pltpu.VMEM((H, D // 2, E), U32),
            pltpu.VMEM((2 * H, D // 2, E), U32),
            pltpu.VMEM((4, H * E, 128), BF16),
            pltpu.VMEM((4, H * E // 2, 128), U32),
            pltpu.VMEM((D, F), BF16),
            pltpu.VMEM((D, F), BF16),
            pltpu.VMEM((F, D), BF16),
            pltpu.VMEM((H, S, E), F32),
            pltpu.VMEM((2 * H, R, E), F32),
            pltpu.VMEM((H, R, E), F32),
            pltpu.VMEM((R, D), F32),
            pltpu.VMEM((16, D), F32),
            pltpu.VMEM((L2, L2), F32),
            pltpu.VMEM((2, 8, 128), F32),
            pltpu.VMEM((8, 128), jnp.int32),
            pltpu.VMEM((M, D), BF16),
            pltpu.VMEM((1, D), BF16),
            pltpu.SemaphoreType.DMA((29,)),
        ],
        compiler_params=pltpu.CompilerParams(vmem_limit_bytes=110 * 1024 * 1024),
        name="rmt_mod",
    )(A_x.reshape(S, D), A_mem0.reshape(M, D), A_Wq, A_Wk, A_Wv, A_Wo.reshape(H * E, D),
      B_w_r.reshape(1, D), B_w_gate, B_w_up, B_w_down)
    return out.reshape(1, S, D)
```

```python
import functools

import jax
import jax.numpy as jnp
import jax.experimental.pallas as pl
import jax.experimental.pallas.tpu as pltpu

S = 2048
D = 512
H = 32
E = 128
M = 8
SEG = 32
F = 1792
NPAIR = H // 2
NU = S // (2 * SEG)
W = 2 * SEG
L2 = 2 * (M + SEG)
EPS = 1e-05
SCALE = float(E) ** -0.5
LOG2E = 1.4426950408889634
F32 = jnp.float32
BF16 = jnp.bfloat16
U32 = jnp.uint32


def _rb(x):
    return x.astype(BF16).astype(F32)


def _ln(x):
    mu = jnp.sum(x, axis=-1, keepdims=True) * (1.0 / D)
    xc0 = x - mu
    var = jnp.sum(xc0 * xc0, axis=-1, keepdims=True) * (1.0 / D)
    sd = _rb(jnp.sqrt(_rb(_rb(var) + EPS)))
    xc = _rb(x - _rb(mu))
    return _rb(xc * (1.0 / sd))


def _dot(a, b):
    return jnp.dot(a, b, preferred_element_type=F32)


def _w(ref_slab):
    return pltpu.bitcast(ref_slab, BF16)


P0 = S // 2
LR = 24
PLN = P0 + LR
XC = P0 // 4
XLN = P0 + SEG
UNR = 1
XA = P0 + 4 * UNR * SEG
FD = P0 + LR * 2 * NU - S
R = 4 * SEG
HC = H // 4


def _tok(*vals):
    parts = []
    for v in vals:
        if v.shape[1] < 128:
            v = jnp.broadcast_to(v[:, :1], (v.shape[0], 128))
        for i in range(v.shape[0] // 8):
            for j in range(v.shape[1] // 128):
                parts.append(v[8 * i:8 * i + 8, 128 * j:128 * j + 128])
    while len(parts) > 1:
        parts = [jnp.maximum(parts[i], parts[i + 1]) if i + 1 < len(parts) else parts[i]
                 for i in range(0, len(parts), 2)]
    return parts[0]


def _rslices(row0, n):
    row0 %= R
    if row0 + n <= R:
        return [(row0, row0 + n, 0)]
    return [(row0, R, 0), (0, row0 + n - R, R - row0)]


def _kernel(x_hbm, mem0_hbm, wq_hbm, wk_hbm, wv_hbm, wo_hbm, wr_hbm, wg_hbm, wu_hbm, wd_hbm,
            out_hbm,
            xs, x1buf, hbbuf, hbuf, hpack, raw, wq, wkv, wo_raw, wo, wg, wu, wd,
            qbig, kvring, oring, abuf, ybuf, maskv, best, zflag, mem0_ref, wr_ref, wrb, sems):
    def x_copy(row0, n, sem):
        return pltpu.make_async_copy(x_hbm.at[pl.ds(row0, n)], xs.at[pl.ds(row0, n)], sems.at[sem])

    def w_copy(ph, src=None):
        if src is None:
            src = wq_hbm.at[:, pl.ds(0, HC), :]
        return pltpu.make_async_copy(src, raw.at[ph], sems.at[11 + ph])

    cp_x = [x_copy(c * XC, XC, 23 + c) for c in range(4)]
    cp_xa = x_copy(P0, XA - P0, 0)
    cp_x[0].start()
    cp_x[1].start()
    w_copy(0).start()
    cp_x[2].start()
    cp_x[3].start()
    cp_xa.start()
    cp_s = [pltpu.make_async_copy(mem0_hbm, mem0_ref, sems.at[27]),
            pltpu.make_async_copy(wr_hbm, wr_ref, sems.at[28])]
    for c in cp_s:
        c.start()
    for i, w in enumerate((wq_hbm, wk_hbm, wv_hbm)):
        for c in range(4):
            if 4 * i + c > 0:
                w_copy(4 * i + c, w.at[:, pl.ds(c * HC, HC), :]).start()
    cp_wo = [pltpu.make_async_copy(wo_hbm.at[:, pl.ds(n * 128, 128)], wo_raw.at[n], sems.at[4 + n])
             for n in range(4)]
    for c in cp_wo:
        c.start()
    cp_xb = x_copy(XA, S - XA, 1)
    cp_f = [pltpu.make_async_copy(wg_hbm, wg, sems.at[8]),
            pltpu.make_async_copy(wu_hbm, wu, sems.at[9]),
            pltpu.make_async_copy(wd_hbm, wd, sems.at[10])]

    def out_copy(row0, n, sem=2):
        return pltpu.make_async_copy(xs.at[pl.ds(row0, n)], out_hbm.at[pl.ds(row0, n)], sems.at[sem])

    oring[:, R - M:R, :] = jnp.zeros((H, M, E), F32)
    abuf[...] = jnp.zeros(abuf.shape, F32)
    xs[pl.ds(S, SEG), :] = jnp.zeros((SEG, D), BF16)
    hbuf[pl.ds(2 * S, SEG), :] = jnp.zeros((SEG, D), F32)
    zflag[...] = jnp.zeros(zflag.shape, jnp.int32)

    ri = jax.lax.broadcasted_iota(jnp.int32, (L2, L2), 0)
    ci = jax.lax.broadcasted_iota(jnp.int32, (L2, L2), 1)

    def head_of(i):
        return jnp.where(i < 2 * M, i // M, (i - 2 * M) // SEG)

    def pos_of(i):
        return jnp.where(i < 2 * M, i % M, M + (i - 2 * M) % SEG)

    same = head_of(ri) == head_of(ci)
    ok = (pos_of(ri) < M) | (pos_of(ri) >= pos_of(ci))
    maskv[...] = jnp.where(same, jnp.where(ok, 0.0, -1e9 / SCALE), -jnp.inf).astype(F32)

    def gate(v, tk):
        y, r = tk
        ns = min(v.shape[-2], 8)
        tok = pltpu.bitcast(y[r:r + 8], v.dtype)[:ns]
        zf = (zflag[...] != 0)[:ns]
        reps = (v.shape[-2] // ns, v.shape[-1] // 128)
        tok, zf = jnp.tile(tok, reps), jnp.tile(zf, reps)
        return jnp.where(zf, tok, v)

    def toks(ys, n, frac=0.8):
        rows = [(y, r) for y in ys for r in range(0, y.shape[0], 8)]
        return [rows[int(len(rows) * frac * i / n)] for i in range(n)]

    def ln0(r0, tk=None, n=W):
        x = xs[r0:r0 + n, :].astype(F32)
        if tk is not None:
            x = gate(x, tk)
        h = _ln(x)
        hbuf[r0:r0 + n, :] = h
        if r0 < P0:
            hpack[r0 // 2:(r0 + n) // 2, :] = pltpu.bitcast(h.astype(BF16), U32)

    def relay(ph, tks=None):
        is_q = isinstance(ph, int) and ph < 4
        for db in range(D // 16):
            a = raw[ph, pl.ds(16 * db, 16)]
            if tks is not None:
                a = pltpu.bitcast(gate(pltpu.bitcast(a, U32), tks[db]), BF16)
            a = jnp.swapaxes(a, 0, 1)
            for hh in range(HC):
                v = pltpu.bitcast(a[hh], U32)
                if is_q:
                    wq[ph * HC + hh, pl.ds(8 * db, 8), :] = v
                else:
                    tb = (ph % 4) * 16 + (ph // 4 - 1) * 2
                    wkv[tb + (hh // 2) * 4 + hh % 2, pl.ds(8 * db, 8), :] = v

    def light(heads, r0=0, r1=P0):
        lhs = _w(hpack[r0 // 2:r1 // 2, :])
        ys = []
        for h in heads:
            y = _dot(lhs, _w(wq[h]))
            qbig[h, pl.ds(r0, r1 - r0), :] = y
            ys.append(y)
        return ys

    def kv_head(lhs16):
        ys = []
        for t in range(2 * NPAIR, 4 * NPAIR):
            y = _dot(lhs16, _w(wkv[t]))
            kvring[t, 0:M, :] = y[:M]
            ys.append(y)
        return ys

    for c in range(2):
        cp_x[c].wait()
        for k in range(XC // W):
            ln0(c * XC + k * W)
    w_copy(0).wait()
    relay(0)

    cp_x[2].wait()
    cp_x[3].wait()
    tks = toks(light(range(4), 0, 2 * XC), 2 * XC // SEG, 0.85)
    for k in range(2 * XC // SEG):
        ln0(2 * XC + k * SEG, tks[k], SEG)

    w_copy(1).wait()
    relay(1, toks(light(range(4), 2 * XC, P0), 32))
    w_copy(2).wait()
    cp_xa.wait()
    tks = toks(light((4, 5)), 33, 0.85)
    relay(2, tks[:32])
    ln0(P0, tks[32], SEG)
    w_copy(3).wait()
    relay(3, toks(light((6, 7)), 32))

    def phase_b(ph, carry):
        w_copy(ph).wait()
        relay(ph, toks(light([3 * ph - 4 + i for i in range(3)]), 32))
        return carry

    jax.lax.fori_loop(4, 12, phase_b, 0)

    for c in cp_wo + cp_s:
        c.wait()
    wrb[...] = jnp.broadcast_to(wr_ref[...].astype(F32).reshape(1, D), (8, D))
    cp_xb.start()
    for c in cp_f:
        c.start()
    tks = toks(kv_head(_w(hpack[0:8, :])), 32, 0.9)
    for k in range(32):
        n, kk = k // 8, k % 8
        wo[n, pl.ds(256 * kk, 256), :] = gate(
            pltpu.bitcast(wo_raw[n, pl.ds(512 * kk, 512), :], U32), tks[k])

    def post(row0, a, valid):
        n = a.shape[0]
        x1 = _rb(xs[pl.ds(row0, n), :].astype(F32) + _rb(a))
        x1buf[pl.ds(row0, n), :] = x1.astype(BF16)
        hb = _ln(x1)
        hbbuf[pl.ds(row0, n), :] = hb.astype(BF16)
        r = _rb(jnp.sum(hb * jnp.tile(wrb[...], (n // 8, 1)), axis=-1, keepdims=True))
        x2 = x1 + hb
        xs[pl.ds(row0, n), :] = x2.astype(BF16)
        if valid is not True:
            r = jnp.where(valid, r, -jnp.inf)
        bv = best[0]
        bi = best[1]
        sub = jax.lax.broadcasted_iota(jnp.int32, (8, 128), 0).astype(F32)
        for g in range(n // 8):
            rg = jnp.broadcast_to(r[8 * g:8 * g + 8], (8, 128))
            ig = sub + (float(row0 + 8 * g) if isinstance(row0, int) else (row0 + 8 * g).astype(F32))
            gt = rg > bv
            bv = jnp.where(gt, rg, bv)
            bi = jnp.where(gt, ig, bi)
        best[0] = bv
        best[1] = bi
        return _tok(x2, bv, bi)

    def anchor(val, tok):
        return jnp.where(zflag[...] != 0, tok, val)

    def wo_pair(g, half):
        return jnp.concatenate(
            [_w(wo[2 * half + c, pl.ds(g * 128, 128), :]) for c in range(2)], axis=1)

    def rload(buf, t, row0, n):
        return [buf[t, a:b, :] for a, b, _ in _rslices(row0, n)]

    def step(ts, jpos, layer, j, mem, korder):
        q, par = ts // 2, ts % 2
        sr = ts * SEG
        if par == 0:
            kvw = ((W * q, 40), (W * q + 8, 24))
            ow = ((W * q - 8, 40), (W * q, 24))
        else:
            kvw = ((W * q + 40, 24), (W * q + 32, 40))
            ow = ((W * q + 32, 24), (W * q + 24, 40))
        sl = 4 * j + ts
        sg = layer * (2 * NU) + sl
        hb0 = pl.multiple_of(layer * S + R * j, R)
        pq0 = pl.multiple_of(P0 + LR * sg, 8)
        lhs = [jnp.concatenate([mem, hbuf[pl.ds(hb0 + r0, n), :]], axis=0).astype(BF16)
               for r0, n in kvw]
        lhsq = jnp.concatenate([mem, hbuf[pl.ds(pq0, LR), :]], axis=0).astype(BF16)
        qrow = [pl.multiple_of((pq0 + 8 * i) % S, 8) for i in range(LR // 8)]
        crow = pl.multiple_of(R * j + sr, SEG)

        def qkv(g, korder=None):
            half = g // (NPAIR // 2)
            r0, n = kvw[half]
            ys = {}
            if korder is not None:
                part = None
                for k in korder:
                    wk = jnp.concatenate([_w(wkv[4 * g + t, pl.ds(64 * k, 64), :])
                                          for t in range(4)], axis=1)
                    y = jnp.dot(lhs[half][:, 128 * k:128 * (k + 1)], wk,
                                preferred_element_type=F32)
                    part = y if part is None else part + y
                for t in range(4):
                    ys[t] = part[:, 128 * t:128 * (t + 1)]
            res = []
            for c in range(2):
                y = jnp.dot(lhsq, _w(wq[2 * g + c]), preferred_element_type=F32)
                for i in range(LR // 8):
                    qbig[2 * g + c, pl.ds(qrow[i], 8), :] = y[M + 8 * i:M + 8 * i + 8]
                res.append(y[:M])
            for t in range(4):
                if t in ys:
                    y = ys[t]
                else:
                    y = jnp.dot(lhs[half], _w(wkv[4 * g + t]), preferred_element_type=F32)
                for a, b, o in _rslices(r0, n):
                    kvring[4 * g + t, a:b, :] = y[M + o:M + o + b - a]
                res.append(y[:M])
            qx = jnp.concatenate([qbig[2 * g + c, pl.ds(crow, SEG), :] for c in range(2)],
                                 axis=0).astype(BF16)
            return res, qx

        def stack(g, mres, i):
            return jnp.concatenate(
                [mres[2 * i], mres[2 * i + 1],
                 kvring[4 * g + 2 * i - 2, sr:sr + SEG, :],
                 kvring[4 * g + 2 * i - 1, sr:sr + SEG, :]], axis=0).astype(BF16)

        def qk(g, mres, qx, prenorm):
            q2 = jnp.concatenate(
                [jnp.concatenate([mres[0], mres[1]], axis=0).astype(BF16), qx], axis=0)
            s = jax.lax.dot_general(q2, stack(g, mres, 1), (((1,), (1,)), ((), ())),
                                    preferred_element_type=F32)
            mk = maskv[...]
            s = jnp.where(mk == 0.0, s, mk)
            mx = jnp.max(s, axis=-1, keepdims=True)
            p = jnp.exp2((s - mx) * (SCALE * LOG2E))
            l = jnp.sum(p, axis=-1, keepdims=True)
            r0 = pl.reciprocal(l, approx=True)
            r = r0 * (2.0 - l * r0)
            if prenorm:
                return (p * r).astype(BF16), None
            return p.astype(BF16), r

        def pv(g, mres, pr):
            p, r = pr
            o = jnp.dot(p, stack(g, mres, 2), preferred_element_type=F32)
            if r is not None:
                o = o * r
            oring[2 * g, sr:sr + SEG, :] = o[2 * M:2 * M + SEG]
            oring[2 * g + 1, sr:sr + SEG, :] = o[2 * M + SEG:]
            return o[:M], o[M:2 * M]

        def olhs(g, om, half):
            r0, n = ow[half]
            return jnp.concatenate(
                [jnp.concatenate([om[c]] + rload(oring, 2 * g + c, r0, n), axis=0)
                 for c in range(2)], axis=1).astype(BF16)

        pn0 = pl.multiple_of(PLN + LR * sg, 8)
        xr = jnp.concatenate(
            [xs[pl.ds(pl.multiple_of((pn0 + 8 * i) % S, 8), 8), :].astype(F32)
             for i in range(LR // 8)], axis=0)
        hpre = _ln(xr)
        hbuf[pl.ds(pn0, LR), :] = hpre
        tok_pre = _tok(hpre)
        if ts >= 2 or jpos:
            valid = True
            row0 = pl.multiple_of(SEG * (sl - 2), SEG)
        else:
            valid = j >= 1
            row0 = pl.multiple_of(jnp.where(valid, SEG * (sl - 2), S), SEG)
        ar = (sr - 2 * SEG) % R
        tok_post = post(row0, abuf[ar:ar + SEG, :], valid)

        NST = NPAIR // 2
        st = [(i, i + NST) if par == 0 else (i + NST, i) for i in range(NST)]
        mres, qxs, prs, oms = {}, {}, {}, {}
        acc = [None] * 4
        order = []
        for i in range(NST):
            order += [("qkv", g) for g in st[i]]
            if i >= 1:
                order += [("qk", g) for g in st[i - 1]]
            if i >= 2:
                order += [("pv", g) for g in st[i - 2]]
        oq = [g for i in range(NST) for g in st[i]]
        NE = 8
        order += [("o", g) for g in oq[0:3]]
        order += [("qk", g) for g in st[NST - 1]] + [("pv", g) for g in st[NST - 2]]
        order += [("o", g) for g in oq[3:7]]
        order += [("pv", g) for g in st[NST - 1]]
        order += [("o", g) for g in oq[7:NE]]
        norder = (2, 3, 0, 1) if par == 0 else (0, 1, 2, 3)
        order += [("on", n) for n in norder]
        for kind, g in order:
            if kind == "qkv":
                mres[g], qxs[g] = qkv(g, korder if g == st[0][0] else None)
                if g == st[2][0]:
                    mres[g][0] = anchor(mres[g][0], tok_pre)
                if g == st[4][0]:
                    mres[g][0] = anchor(mres[g][0], tok_post)
            elif kind == "qk":
                prs[g] = qk(g, mres[g], qxs[g], g not in st[NST - 1] + st[NST - 2])
            elif kind == "pv":
                oms[g] = pv(g, mres[g], prs[g])
                if prs[g][1] is not None:
                    oms[g] = (anchor(oms[g][0], _tok(prs[g][1][2 * M:])), oms[g][1])
            elif kind == "o":
                for half in range(2):
                    y = jnp.dot(olhs(g, oms[g], half), wo_pair(g, half), preferred_element_type=F32)
                    for c in range(2):
                        yc = y[:, 128 * c:128 * (c + 1)]
                        n = 2 * half + c
                        acc[n] = yc if acc[n] is None else acc[n] + yc
            else:
                n = g
                l = jnp.concatenate([olhs(g2, oms[g2], n // 2) for g2 in oq[NE:]], axis=1)
                wn = jnp.concatenate([_w(wo[n, pl.ds(g2 * 128, 128), :]) for g2 in oq[NE:]], axis=0)
                acc[n] = acc[n] + jnp.dot(l, wn, preferred_element_type=F32)
        for n in range(4):
            r0, nr = ow[n // 2]
            for a, b, o in _rslices(r0, nr):
                abuf[a:b, n * 128:(n + 1) * 128] = acc[n][M + o:M + o + b - a]

        return jnp.concatenate([acc[n][:M] for n in range(4)], axis=1), norder

    def argmax():
        bv = best[0]
        bi = best[1]
        vmax = jnp.max(bv, axis=0, keepdims=True)
        imin = jnp.min(jnp.where(bv == vmax, bi, float(S)), axis=0, keepdims=True)
        idx = jnp.clip(jnp.min(imin).astype(jnp.int32), 0, S - 1)
        return idx, vmax

    def ffn(idx):
        g0 = pl.multiple_of((idx // 16) * 16, 16)
        hbb = hbbuf[pl.ds(g0, 16), :]
        gpre = _rb(_dot(hbb, wg[...]))
        gs = _rb(gpre * _rb(jax.nn.sigmoid(gpre)))
        up = _rb(_dot(hbb, wu[...]))
        ybuf[...] = _rb(_dot((gs * up).astype(BF16), wd[...]))

    def layer_body(layer, carry):
        best[0] = jnp.full((8, 128), -jnp.inf, F32)
        best[1] = jnp.zeros((8, 128), F32)

        def qstep(jj, mem):
            @pl.when((layer == 0) & (jj == 1))
            def _():
                cp_xb.wait()

            @pl.when((layer == 1) & (jj >= 2))
            def _():
                out_copy(pl.multiple_of((jj - 1) * (UNR * R) - W, W), UNR * R).start()

            @pl.when((layer == 1) & (jj == 1))
            def _():
                out_copy(0, UNR * R - W).start()

            ko = None
            for j2 in range(UNR):
                for ts in range(4):
                    mem, ko = step(ts, j2 > 0, layer, UNR * jj + j2, mem, ko)
            return mem

        jax.lax.fori_loop(0, NU // (2 * UNR), qstep, mem0_ref[...].astype(F32))

        @pl.when(layer == 0)
        def _():
            for c in cp_f:
                c.wait()

        @pl.when(layer == 1)
        def _():
            out_copy(S - UNR * R - W, UNR * R).start()

        idx_s, _ = argmax()
        acc = None
        for g in range(NPAIR):
            l = jnp.concatenate([oring[2 * g + c, R - 16:R, :] for c in range(2)],
                                axis=1).astype(BF16)
            y = _dot(l, wo_pair(g, 0))
            acc = y if acc is None else acc + y
        abuf[R - M:R, 0:256] = acc[M:]
        ffn(idx_s)
        post(S - W, abuf[W:R, :], True)
        idx, vmax = argmax()

        @pl.when(layer == 1)
        def _():
            out_copy(S - W, W).start()

        @pl.when(idx // 16 != idx_s // 16)
        def _():
            ffn(idx)

        g0 = pl.multiple_of((idx // 16) * 16, 16)
        rsel = jnp.tile(_rb(jax.nn.sigmoid(vmax)), (1, D // 128))
        y = _rb(ybuf[...] * rsel)
        x2 = _rb(x1buf[pl.ds(g0, 16), :].astype(F32) + _rb(hbbuf[pl.ds(g0, 16), :].astype(F32) + y))
        rowi = jax.lax.broadcasted_iota(jnp.int32, (16, D), 0) + g0

        @pl.when(layer == 1)
        def _():
            out_copy(0, S).wait()

        x2 = jnp.where(rowi == idx, x2, xs[pl.ds(g0, 16), :].astype(F32))
        xs[pl.ds(g0, 16), :] = x2.astype(BF16)

        @pl.when(layer == 0)
        def _():
            h16 = _ln(x2)
            hbuf[pl.ds(S + g0, 16), :] = h16

            @pl.when(idx < FD)
            def _():
                def body(h, c):
                    qbig[h, pl.ds(g0, 16), :] = _dot(h16.astype(BF16), _w(wq[h]))
                    return c

                jax.lax.fori_loop(0, H, body, 0, unroll=4)

            @pl.when(idx < M)
            def _():
                kv_head(h16.astype(BF16))

        @pl.when(layer == 1)
        def _():
            fix = out_copy(g0, 16, 3)
            fix.start()
            fix.wait()

        return carry

    jax.lax.fori_loop(0, 2, layer_body, 0)


@functools.partial(jax.jit, static_argnames=("A_seg_len",))
def pallas_interleave_layers__memory_aug_recurrent_mem_tr__moe_arch_mod__prompt_kernel(
    A_x: jax.Array,
    A_mem0: jax.Array,
    A_Wq: jax.Array,
    A_Wk: jax.Array,
    A_Wv: jax.Array,
    A_Wo: jax.Array,
    A_seg_len,
    B_x: jax.Array,
    B_w_r: jax.Array,
    B_w_gate: jax.Array,
    B_w_up: jax.Array,
    B_w_down: jax.Array,
):
    assert A_seg_len == SEG
    assert A_x.shape == (1, S, D) and A_Wq.shape == (D, H, E) and A_mem0.shape == (1, M, D)
    any_spec = pl.BlockSpec(memory_space=pl.ANY)
    out = pl.pallas_call(
        _kernel,
        out_shape=jax.ShapeDtypeStruct((S, D), BF16),
        in_specs=[any_spec] * 10,
        out_specs=any_spec,
        scratch_shapes=[
            pltpu.VMEM((S + SEG, D), BF16),
            pltpu.VMEM((S + SEG, D), BF16),
            pltpu.VMEM((S + SEG, D), BF16),
            pltpu.VMEM((2 * S + SEG, D), F32),
            pltpu.VMEM((P0 // 2, D), U32),
            pltpu.VMEM((12, D, HC, E), BF16),
            pltpu.VMEM((H, D // 2, E), U32),
            pltpu.VMEM((2 * H, D // 2, E), U32),
            pltpu.VMEM((4, H * E, 128), BF16),
            pltpu.VMEM((4, H * E // 2, 128), U32),
            pltpu.VMEM((D, F), BF16),
            pltpu.VMEM((D, F), BF16),
            pltpu.VMEM((F, D), BF16),
            pltpu.VMEM((H, S, E), F32),
            pltpu.VMEM((2 * H, R, E), F32),
            pltpu.VMEM((H, R, E), F32),
            pltpu.VMEM((R, D), F32),
            pltpu.VMEM((16, D), F32),
            pltpu.VMEM((L2, L2), F32),
            pltpu.VMEM((2, 8, 128), F32),
            pltpu.VMEM((8, 128), jnp.int32),
            pltpu.VMEM((M, D), BF16),
            pltpu.VMEM((D,), BF16),
            pltpu.VMEM((8, D), F32),
            pltpu.SemaphoreType.DMA((29,)),
        ],
        compiler_params=pltpu.CompilerParams(vmem_limit_bytes=110 * 1024 * 1024),
        name="rmt_mod",
    )(A_x.reshape(S, D), A_mem0.reshape(M, D), A_Wq, A_Wk, A_Wv, A_Wo.reshape(H * E, D),
      B_w_r, B_w_gate, B_w_up, B_w_down)
    return out.reshape(1, S, D)
```

```python
import functools

import jax
import jax.numpy as jnp
import jax.experimental.pallas as pl
import jax.experimental.pallas.tpu as pltpu

S = 2048
D = 512
H = 32
E = 128
M = 8
SEG = 32
F = 1792
NPAIR = H // 2
NU = S // (2 * SEG)
W = 2 * SEG
L2 = 2 * (M + SEG)
EPS = 1e-05
SCALE = float(E) ** -0.5
LOG2E = 1.4426950408889634
F32 = jnp.float32
BF16 = jnp.bfloat16
U32 = jnp.uint32


def _rb(x):
    return x.astype(BF16).astype(F32)


def _ln(x):
    mu = jnp.sum(x, axis=-1, keepdims=True) * (1.0 / D)
    xc0 = x - mu
    var = jnp.sum(xc0 * xc0, axis=-1, keepdims=True) * (1.0 / D)
    sd = _rb(jnp.sqrt(_rb(_rb(var) + EPS)))
    xc = _rb(x - _rb(mu))
    return _rb(xc * (1.0 / sd))


def _dot(a, b):
    return jnp.dot(a, b, preferred_element_type=F32)


def _w(ref_slab):
    return pltpu.bitcast(ref_slab, BF16)


P0 = S // 2
LR = 24
PLN = P0 + LR
XC = P0 // 4
XLN = P0 + SEG
UNR = 2
XA = P0 + 4 * UNR * SEG
FD = P0 + LR * 2 * NU - S
R = 4 * SEG
HC = H // 4
PRE_ST = 3
POST_ST = 5
KSPLIT = ((0, 0), (0, 1), (1, 0), (1, 1), (0, 2), (1, 2), (0, 3), (1, 3))
O1, O2, NE = 3, 7, 8


def _tok(*vals):
    parts = []
    for v in vals:
        if v.shape[1] < 128:
            v = jnp.broadcast_to(v[:, :1], (v.shape[0], 128))
        for i in range(v.shape[0] // 8):
            for j in range(v.shape[1] // 128):
                parts.append(v[8 * i:8 * i + 8, 128 * j:128 * j + 128])
    while len(parts) > 1:
        parts = [jnp.maximum(parts[i], parts[i + 1]) if i + 1 < len(parts) else parts[i]
                 for i in range(0, len(parts), 2)]
    return parts[0]


def _rslices(row0, n):
    row0 %= R
    if row0 + n <= R:
        return [(row0, row0 + n, 0)]
    return [(row0, R, 0), (0, row0 + n - R, R - row0)]


def _kernel(x_hbm, mem0_hbm, wq_hbm, wk_hbm, wv_hbm, wo_hbm, wr_hbm, wg_hbm, wu_hbm, wd_hbm,
            out_hbm,
            xs, x1buf, hbbuf, hbuf, hpack, raw, wq, wkv, wo_raw, wo, wg, wu, wd,
            qbig, kvring, oring, abuf, ybuf, maskv, best, zflag, mem0_ref, wr_ref, wrb, sems):
    def x_copy(row0, n, sem):
        return pltpu.make_async_copy(x_hbm.at[pl.ds(row0, n)], xs.at[pl.ds(row0, n)], sems.at[sem])

    def w_copy(ph, src=None):
        if src is None:
            src = wq_hbm.at[:, pl.ds(0, HC), :]
        return pltpu.make_async_copy(src, raw.at[ph], sems.at[11 + ph])

    cp_x = [x_copy(c * XC, XC, 23 + c) for c in range(4)]
    cp_xa = x_copy(P0, XA - P0, 0)
    cp_x[0].start()
    cp_x[1].start()
    w_copy(0).start()
    cp_x[2].start()
    cp_x[3].start()
    cp_xa.start()
    cp_s = [pltpu.make_async_copy(mem0_hbm, mem0_ref, sems.at[27]),
            pltpu.make_async_copy(wr_hbm, wr_ref, sems.at[28])]
    for c in cp_s:
        c.start()
    for i, w in enumerate((wq_hbm, wk_hbm, wv_hbm)):
        for c in range(4):
            if 4 * i + c > 0:
                w_copy(4 * i + c, w.at[:, pl.ds(c * HC, HC), :]).start()
    cp_wo = [pltpu.make_async_copy(wo_hbm.at[:, pl.ds(n * 128, 128)], wo_raw.at[n], sems.at[4 + n])
             for n in range(4)]
    for c in cp_wo:
        c.start()
    cp_xb = x_copy(XA, S - XA, 1)
    cp_f = [pltpu.make_async_copy(wg_hbm, wg, sems.at[8]),
            pltpu.make_async_copy(wu_hbm, wu, sems.at[9]),
            pltpu.make_async_copy(wd_hbm, wd, sems.at[10])]

    def out_copy(row0, n, sem=2):
        return pltpu.make_async_copy(xs.at[pl.ds(row0, n)], out_hbm.at[pl.ds(row0, n)], sems.at[sem])

    oring[:, R - M:R, :] = jnp.zeros((H, M, E), F32)
    abuf[...] = jnp.zeros(abuf.shape, F32)
    xs[pl.ds(S, SEG), :] = jnp.zeros((SEG, D), BF16)
    hbuf[pl.ds(2 * S, SEG), :] = jnp.zeros((SEG, D), F32)
    zflag[...] = jnp.zeros(zflag.shape, jnp.int32)

    ri = jax.lax.broadcasted_iota(jnp.int32, (L2, L2), 0)
    ci = jax.lax.broadcasted_iota(jnp.int32, (L2, L2), 1)

    def head_of(i):
        return jnp.where(i < 2 * M, i // M, (i - 2 * M) // SEG)

    def pos_of(i):
        return jnp.where(i < 2 * M, i % M, M + (i - 2 * M) % SEG)

    same = head_of(ri) == head_of(ci)
    ok = (pos_of(ri) < M) | (pos_of(ri) >= pos_of(ci))
    maskv[...] = jnp.where(same, jnp.where(ok, 0.0, -1e9 / SCALE), -jnp.inf).astype(F32)

    def gate(v, tk):
        y, r = tk
        ns = min(v.shape[-2], 8)
        tok = pltpu.bitcast(y[r:r + 8], v.dtype)[:ns]
        zf = (zflag[...] != 0)[:ns]
        reps = (v.shape[-2] // ns, v.shape[-1] // 128)
        tok, zf = jnp.tile(tok, reps), jnp.tile(zf, reps)
        return jnp.where(zf, tok, v)

    def toks(ys, n, frac=0.8):
        rows = [(y, r) for y in ys for r in range(0, y.shape[0], 8)]
        return [rows[int(len(rows) * frac * i / n)] for i in range(n)]

    def ln0(r0, tk=None, n=W):
        x = xs[r0:r0 + n, :].astype(F32)
        if tk is not None:
            x = gate(x, tk)
        h = _ln(x)
        hbuf[r0:r0 + n, :] = h
        if r0 < P0:
            hpack[r0 // 2:(r0 + n) // 2, :] = pltpu.bitcast(h.astype(BF16), U32)

    def relay(ph, tks=None):
        is_q = isinstance(ph, int) and ph < 4
        for db in range(D // 16):
            a = raw[ph, pl.ds(16 * db, 16)]
            if tks is not None:
                a = pltpu.bitcast(gate(pltpu.bitcast(a, U32), tks[db]), BF16)
            a = jnp.swapaxes(a, 0, 1)
            for hh in range(HC):
                v = pltpu.bitcast(a[hh], U32)
                if is_q:
                    wq[ph * HC + hh, pl.ds(8 * db, 8), :] = v
                else:
                    tb = (ph % 4) * 16 + (ph // 4 - 1) * 2
                    wkv[tb + (hh // 2) * 4 + hh % 2, pl.ds(8 * db, 8), :] = v

    def light(heads, r0=0, r1=P0):
        lhs = _w(hpack[r0 // 2:r1 // 2, :])
        ys = []
        for h in heads:
            y = _dot(lhs, _w(wq[h]))
            qbig[h, pl.ds(r0, r1 - r0), :] = y
            ys.append(y)
        return ys

    def kv_head(lhs16):
        ys = []
        for t in range(2 * NPAIR, 4 * NPAIR):
            y = _dot(lhs16, _w(wkv[t]))
            kvring[t, 0:M, :] = y[:M]
            ys.append(y)
        return ys

    for c in range(2):
        cp_x[c].wait()
        for k in range(XC // W):
            ln0(c * XC + k * W)
    w_copy(0).wait()
    relay(0)

    cp_x[2].wait()
    cp_x[3].wait()
    tks = toks(light(range(4), 0, 2 * XC), 2 * XC // SEG, 0.85)
    for k in range(2 * XC // SEG):
        ln0(2 * XC + k * SEG, tks[k], SEG)

    w_copy(1).wait()
    relay(1, toks(light(range(4), 2 * XC, P0), 32))
    w_copy(2).wait()
    cp_xa.wait()
    tks = toks(light((4, 5)), 33, 0.85)
    relay(2, tks[:32])
    ln0(P0, tks[32], SEG)
    w_copy(3).wait()
    relay(3, toks(light((6, 7)), 32))

    def phase_b(ph, carry):
        w_copy(ph).wait()
        relay(ph, toks(light([3 * ph - 4 + i for i in range(3)]), 32))
        return carry

    jax.lax.fori_loop(4, 12, phase_b, 0)

    for c in cp_wo + cp_s:
        c.wait()
    wrb[...] = jnp.broadcast_to(wr_ref[...].astype(F32).reshape(1, D), (8, D))
    cp_xb.start()
    for c in cp_f:
        c.start()
    tks = toks(kv_head(_w(hpack[0:8, :])), 32, 0.9)
    for k in range(32):
        n, kk = k // 8, k % 8
        wo[n, pl.ds(256 * kk, 256), :] = gate(
            pltpu.bitcast(wo_raw[n, pl.ds(512 * kk, 512), :], U32), tks[k])

    def post(row0, a, valid):
        n = a.shape[0]
        x1 = _rb(xs[pl.ds(row0, n), :].astype(F32) + _rb(a))
        x1buf[pl.ds(row0, n), :] = x1.astype(BF16)
        hb = _ln(x1)
        hbbuf[pl.ds(row0, n), :] = hb.astype(BF16)
        r = _rb(jnp.sum(hb * jnp.tile(wrb[...], (n // 8, 1)), axis=-1, keepdims=True))
        x2 = x1 + hb
        xs[pl.ds(row0, n), :] = x2.astype(BF16)
        if valid is not True:
            r = jnp.where(valid, r, -jnp.inf)
        bv = best[0]
        bi = best[1]
        sub = jax.lax.broadcasted_iota(jnp.int32, (8, 128), 0).astype(F32)
        for g in range(n // 8):
            rg = jnp.broadcast_to(r[8 * g:8 * g + 8], (8, 128))
            ig = sub + (float(row0 + 8 * g) if isinstance(row0, int) else (row0 + 8 * g).astype(F32))
            gt = rg > bv
            bv = jnp.where(gt, rg, bv)
            bi = jnp.where(gt, ig, bi)
        best[0] = bv
        best[1] = bi
        return _tok(x2, bv, bi)

    def anchor(val, tok):
        return jnp.where(zflag[...] != 0, tok, val)

    def wo_pair(g, half):
        return jnp.concatenate(
            [_w(wo[2 * half + c, pl.ds(g * 128, 128), :]) for c in range(2)], axis=1)

    def rload(buf, t, row0, n):
        return [buf[t, a:b, :] for a, b, _ in _rslices(row0, n)]

    def step(ts, jpos, layer, j, mem, korder):
        q, par = ts // 2, ts % 2
        sr = ts * SEG
        if par == 0:
            kvw = ((W * q, 40), (W * q + 8, 24))
            ow = ((W * q - 8, 40), (W * q, 24))
        else:
            kvw = ((W * q + 40, 24), (W * q + 32, 40))
            ow = ((W * q + 32, 24), (W * q + 24, 40))
        sl = 4 * j + ts
        sg = layer * (2 * NU) + sl
        hb0 = pl.multiple_of(layer * S + R * j, R)
        pq0 = pl.multiple_of(P0 + LR * sg, 8)
        lhs = [jnp.concatenate([mem, hbuf[pl.ds(hb0 + r0, n), :]], axis=0).astype(BF16)
               for r0, n in kvw]
        lhsq = jnp.concatenate([mem, hbuf[pl.ds(pq0, LR), :]], axis=0).astype(BF16)
        qrow = [pl.multiple_of((pq0 + 8 * i) % S, 8) for i in range(LR // 8)]
        crow = pl.multiple_of(R * j + sr, SEG)

        def ksplit(ga, gb):
            half = ga // (NPAIR // 2)
            hq = [2 * ga, 2 * ga + 1, 2 * gb, 2 * gb + 1]

            def kv(k):
                wk = jnp.concatenate([_w(wkv[4 * ga + t, pl.ds(64 * k, 64), :])
                                      for t in range(4)], axis=1)
                return jnp.dot(lhs[half][:, 128 * k:128 * (k + 1)], wk, preferred_element_type=F32)

            def qq(k):
                wk = jnp.concatenate([_w(wq[h, pl.ds(64 * k, 64), :]) for h in hq], axis=1)
                return jnp.dot(lhsq[:, 128 * k:128 * (k + 1)], wk, preferred_element_type=F32)

            pkv = pq = None
            for f, k in KSPLIT:
                y = (kv if f == 0 else qq)(korder[k])
                if f == 0:
                    pkv = y if pkv is None else pkv + y
                else:
                    pq = y if pq is None else pq + y
            done = {("kv", 4 * ga + t): pkv[:, 128 * t:128 * (t + 1)] for t in range(4)}
            if pq is not None:
                done.update({("q", h): pq[:, 128 * i:128 * (i + 1)] for i, h in enumerate(hq)})
            return done

        def qkv(g, done):
            half = g // (NPAIR // 2)
            r0, n = kvw[half]
            res = []
            for c in range(2):
                y = done.get(("q", 2 * g + c))
                if y is None:
                    y = jnp.dot(lhsq, _w(wq[2 * g + c]), preferred_element_type=F32)
                for i in range(LR // 8):
                    qbig[2 * g + c, pl.ds(qrow[i], 8), :] = y[M + 8 * i:M + 8 * i + 8]
                res.append(y[:M])
            for t in range(4):
                y = done.get(("kv", 4 * g + t))
                if y is None:
                    y = jnp.dot(lhs[half], _w(wkv[4 * g + t]), preferred_element_type=F32)
                for a, b, o in _rslices(r0, n):
                    kvring[4 * g + t, a:b, :] = y[M + o:M + o + b - a]
                res.append(y[:M])
            qx = jnp.concatenate([qbig[2 * g + c, pl.ds(crow, SEG), :] for c in range(2)],
                                 axis=0).astype(BF16)
            return res, qx

        def stack(g, mres, i):
            return jnp.concatenate(
                [mres[2 * i], mres[2 * i + 1],
                 kvring[4 * g + 2 * i - 2, sr:sr + SEG, :],
                 kvring[4 * g + 2 * i - 1, sr:sr + SEG, :]], axis=0).astype(BF16)

        def qk(g, mres, qx, prenorm):
            q2 = jnp.concatenate(
                [jnp.concatenate([mres[0], mres[1]], axis=0).astype(BF16), qx], axis=0)
            s = jax.lax.dot_general(q2, stack(g, mres, 1), (((1,), (1,)), ((), ())),
                                    preferred_element_type=F32)
            mk = maskv[...]
            s = jnp.where(mk == 0.0, s, mk)
            mx = jnp.max(s, axis=-1, keepdims=True)
            p = jnp.exp2((s - mx) * (SCALE * LOG2E))
            l = jnp.sum(p, axis=-1, keepdims=True)
            r0 = pl.reciprocal(l, approx=True)
            r = r0 * (2.0 - l * r0)
            if prenorm:
                return (p * r).astype(BF16), None
            return p.astype(BF16), r

        def pv(g, mres, pr):
            p, r = pr
            o = jnp.dot(p, stack(g, mres, 2), preferred_element_type=F32)
            if r is not None:
                o = o * r
            oring[2 * g, sr:sr + SEG, :] = o[2 * M:2 * M + SEG]
            oring[2 * g + 1, sr:sr + SEG, :] = o[2 * M + SEG:]
            return o[:M], o[M:2 * M]

        def olhs(g, om, half):
            r0, n = ow[half]
            return jnp.concatenate(
                [jnp.concatenate([om[c]] + rload(oring, 2 * g + c, r0, n), axis=0)
                 for c in range(2)], axis=1).astype(BF16)

        pn0 = pl.multiple_of(PLN + LR * sg, 8)
        xr = jnp.concatenate(
            [xs[pl.ds(pl.multiple_of((pn0 + 8 * i) % S, 8), 8), :].astype(F32)
             for i in range(LR // 8)], axis=0)
        hpre = _ln(xr)
        hbuf[pl.ds(pn0, LR), :] = hpre
        tok_pre = _tok(hpre)
        if ts >= 2 or jpos:
            valid = True
            row0 = pl.multiple_of(SEG * (sl - 2), SEG)
        else:
            valid = j >= 1
            row0 = pl.multiple_of(jnp.where(valid, SEG * (sl - 2), S), SEG)
        ar = (sr - 2 * SEG) % R
        tok_post = post(row0, abuf[ar:ar + SEG, :], valid)

        NST = NPAIR // 2
        st = [(i, i + NST) if par == 0 else (i + NST, i) for i in range(NST)]
        mres, qxs, prs, oms = {}, {}, {}, {}
        acc = [None] * 4
        order = []
        for i in range(NST):
            order += [("qkv", g) for g in st[i]]
            if i >= 1:
                order += [("qk", g) for g in st[i - 1]]
            if i >= 2:
                order += [("pv", g) for g in st[i - 2]]
        oq = [g for i in range(NST) for g in st[i]]
        order += [("o", g) for g in oq[0:O1]]
        order += [("qk", g) for g in st[NST - 1]] + [("pv", g) for g in st[NST - 2]]
        order += [("o", g) for g in oq[O1:O2]]
        order += [("pv", g) for g in st[NST - 1]]
        order += [("o", g) for g in oq[O2:NE]]
        norder = (2, 3, 0, 1) if par == 0 else (0, 1, 2, 3)
        order += [("on", n) for n in norder]
        done = {} if korder is None else ksplit(*st[0])
        for kind, g in order:
            if kind == "qkv":
                mres[g], qxs[g] = qkv(g, done)
                if g == st[PRE_ST][0]:
                    mres[g][0] = anchor(mres[g][0], tok_pre)
                if g == st[POST_ST][0]:
                    mres[g][0] = anchor(mres[g][0], tok_post)
            elif kind == "qk":
                prs[g] = qk(g, mres[g], qxs[g], g not in st[NST - 1] + st[NST - 2])
            elif kind == "pv":
                oms[g] = pv(g, mres[g], prs[g])
                if prs[g][1] is not None:
                    oms[g] = (anchor(oms[g][0], _tok(prs[g][1][2 * M:])), oms[g][1])
            elif kind == "o":
                for half in range(2):
                    y = jnp.dot(olhs(g, oms[g], half), wo_pair(g, half), preferred_element_type=F32)
                    for c in range(2):
                        yc = y[:, 128 * c:128 * (c + 1)]
                        n = 2 * half + c
                        acc[n] = yc if acc[n] is None else acc[n] + yc
            else:
                n = g
                l = jnp.concatenate([olhs(g2, oms[g2], n // 2) for g2 in oq[NE:]], axis=1)
                wn = jnp.concatenate([_w(wo[n, pl.ds(g2 * 128, 128), :]) for g2 in oq[NE:]], axis=0)
                acc[n] = acc[n] + jnp.dot(l, wn, preferred_element_type=F32)
        for n in range(4):
            r0, nr = ow[n // 2]
            for a, b, o in _rslices(r0, nr):
                abuf[a:b, n * 128:(n + 1) * 128] = acc[n][M + o:M + o + b - a]

        return jnp.concatenate([acc[n][:M] for n in range(4)], axis=1), norder

    def argmax():
        bv = best[0]
        bi = best[1]
        vmax = jnp.max(bv, axis=0, keepdims=True)
        imin = jnp.min(jnp.where(bv == vmax, bi, float(S)), axis=0, keepdims=True)
        idx = jnp.clip(jnp.min(imin).astype(jnp.int32), 0, S - 1)
        return idx, vmax

    def ffn(idx):
        g0 = pl.multiple_of((idx // 16) * 16, 16)
        hbb = hbbuf[pl.ds(g0, 16), :]
        gpre = _rb(_dot(hbb, wg[...]))
        gs = _rb(gpre * _rb(jax.nn.sigmoid(gpre)))
        up = _rb(_dot(hbb, wu[...]))
        ybuf[...] = _rb(_dot((gs * up).astype(BF16), wd[...]))

    def layer_body(layer, carry):
        best[0] = jnp.full((8, 128), -jnp.inf, F32)
        best[1] = jnp.zeros((8, 128), F32)

        def qstep(jj, mem):
            @pl.when((layer == 0) & (jj == 1))
            def _():
                cp_xb.wait()

            @pl.when((layer == 1) & (jj >= 2))
            def _():
                out_copy(pl.multiple_of((jj - 1) * (UNR * R) - W, W), UNR * R).start()

            @pl.when((layer == 1) & (jj == 1))
            def _():
                out_copy(0, UNR * R - W).start()

            ko = None
            for j2 in range(UNR):
                for ts in range(4):
                    mem, ko = step(ts, j2 > 0, layer, UNR * jj + j2, mem, ko)
            return mem

        jax.lax.fori_loop(0, NU // (2 * UNR), qstep, mem0_ref[...].astype(F32))

        @pl.when(layer == 0)
        def _():
            for c in cp_f:
                c.wait()

        @pl.when(layer == 1)
        def _():
            out_copy(S - UNR * R - W, UNR * R).start()

        idx_s, _ = argmax()
        acc = None
        for g in range(NPAIR):
            l = jnp.concatenate([oring[2 * g + c, R - 16:R, :] for c in range(2)],
                                axis=1).astype(BF16)
            y = _dot(l, wo_pair(g, 0))
            acc = y if acc is None else acc + y
        abuf[R - M:R, 0:256] = acc[M:]
        ffn(idx_s)
        post(S - W, abuf[W:R, :], True)
        idx, vmax = argmax()

        @pl.when(layer == 1)
        def _():
            out_copy(S - W, W).start()

        @pl.when(idx // 16 != idx_s // 16)
        def _():
            ffn(idx)

        g0 = pl.multiple_of((idx // 16) * 16, 16)
        rsel = jnp.tile(_rb(jax.nn.sigmoid(vmax)), (1, D // 128))
        y = _rb(ybuf[...] * rsel)
        x2 = _rb(x1buf[pl.ds(g0, 16), :].astype(F32) + _rb(hbbuf[pl.ds(g0, 16), :].astype(F32) + y))
        rowi = jax.lax.broadcasted_iota(jnp.int32, (16, D), 0) + g0

        @pl.when(layer == 1)
        def _():
            out_copy(0, S).wait()

        x2 = jnp.where(rowi == idx, x2, xs[pl.ds(g0, 16), :].astype(F32))
        xs[pl.ds(g0, 16), :] = x2.astype(BF16)

        @pl.when(layer == 0)
        def _():
            h16 = _ln(x2)
            hbuf[pl.ds(S + g0, 16), :] = h16

            @pl.when(idx < FD)
            def _():
                def body(h, c):
                    qbig[h, pl.ds(g0, 16), :] = _dot(h16.astype(BF16), _w(wq[h]))
                    return c

                jax.lax.fori_loop(0, H, body, 0, unroll=4)

            @pl.when(idx < M)
            def _():
                kv_head(h16.astype(BF16))

        @pl.when(layer == 1)
        def _():
            fix = out_copy(g0, 16, 3)
            fix.start()
            fix.wait()

        return carry

    jax.lax.fori_loop(0, 2, layer_body, 0)


@functools.partial(jax.jit, static_argnames=("A_seg_len",))
def pallas_interleave_layers__memory_aug_recurrent_mem_tr__moe_arch_mod__prompt_kernel(
    A_x: jax.Array,
    A_mem0: jax.Array,
    A_Wq: jax.Array,
    A_Wk: jax.Array,
    A_Wv: jax.Array,
    A_Wo: jax.Array,
    A_seg_len,
    B_x: jax.Array,
    B_w_r: jax.Array,
    B_w_gate: jax.Array,
    B_w_up: jax.Array,
    B_w_down: jax.Array,
):
    assert A_seg_len == SEG
    assert A_x.shape == (1, S, D) and A_Wq.shape == (D, H, E) and A_mem0.shape == (1, M, D)
    any_spec = pl.BlockSpec(memory_space=pl.ANY)
    out = pl.pallas_call(
        _kernel,
        out_shape=jax.ShapeDtypeStruct((S, D), BF16),
        in_specs=[any_spec] * 10,
        out_specs=any_spec,
        scratch_shapes=[
            pltpu.VMEM((S + SEG, D), BF16),
            pltpu.VMEM((S + SEG, D), BF16),
            pltpu.VMEM((S + SEG, D), BF16),
            pltpu.VMEM((2 * S + SEG, D), F32),
            pltpu.VMEM((P0 // 2, D), U32),
            pltpu.VMEM((12, D, HC, E), BF16),
            pltpu.VMEM((H, D // 2, E), U32),
            pltpu.VMEM((2 * H, D // 2, E), U32),
            pltpu.VMEM((4, H * E, 128), BF16),
            pltpu.VMEM((4, H * E // 2, 128), U32),
            pltpu.VMEM((D, F), BF16),
            pltpu.VMEM((D, F), BF16),
            pltpu.VMEM((F, D), BF16),
            pltpu.VMEM((H, S, E), F32),
            pltpu.VMEM((2 * H, R, E), F32),
            pltpu.VMEM((H, R, E), F32),
            pltpu.VMEM((R, D), F32),
            pltpu.VMEM((16, D), F32),
            pltpu.VMEM((L2, L2), F32),
            pltpu.VMEM((2, 8, 128), F32),
            pltpu.VMEM((8, 128), jnp.int32),
            pltpu.VMEM((M, D), BF16),
            pltpu.VMEM((D,), BF16),
            pltpu.VMEM((8, D), F32),
            pltpu.SemaphoreType.DMA((29,)),
        ],
        compiler_params=pltpu.CompilerParams(vmem_limit_bytes=110 * 1024 * 1024),
        name="rmt_mod",
    )(A_x.reshape(S, D), A_mem0.reshape(M, D), A_Wq, A_Wk, A_Wv, A_Wo.reshape(H * E, D),
      B_w_r, B_w_gate, B_w_up, B_w_down)
    return out.reshape(1, S, D)
```

```python
import functools

import jax
import jax.numpy as jnp
import jax.experimental.pallas as pl
import jax.experimental.pallas.tpu as pltpu

S = 2048
D = 512
H = 32
E = 128
M = 8
SEG = 32
F = 1792
NPAIR = H // 2
NU = S // (2 * SEG)
W = 2 * SEG
L2 = 2 * (M + SEG)
EPS = 1e-05
SCALE = float(E) ** -0.5
LOG2E = 1.4426950408889634
F32 = jnp.float32
BF16 = jnp.bfloat16
U32 = jnp.uint32


def _rb(x):
    return x.astype(BF16).astype(F32)


def _ln(x):
    mu = jnp.sum(x, axis=-1, keepdims=True) * (1.0 / D)
    xc0 = x - mu
    var = jnp.sum(xc0 * xc0, axis=-1, keepdims=True) * (1.0 / D)
    sd = _rb(jnp.sqrt(_rb(_rb(var) + EPS)))
    xc = _rb(x - _rb(mu))
    return _rb(xc * (1.0 / sd))


def _dot(a, b):
    return jnp.dot(a, b, preferred_element_type=F32)


def _w(ref_slab):
    return pltpu.bitcast(ref_slab, BF16)


P0 = S // 2
LR = 24
PLN = P0 + LR
XC = P0 // 4
XLN = P0 + SEG
UNR = 2
XA = P0 + 4 * UNR * SEG
FD = P0 + LR * 2 * NU - S
R = 4 * SEG
HC = H // 4
PRE_ST = 3
POST_ST = 5
KSPLIT = ((0, 0), (0, 1), (1, 0), (1, 1), (0, 2), (1, 2), (0, 3), (1, 3))
O1, O2, NE = 3, 7, 8


def _tok(*vals):
    parts = []
    for v in vals:
        if v.shape[1] < 128:
            v = jnp.broadcast_to(v[:, :1], (v.shape[0], 128))
        for i in range(v.shape[0] // 8):
            for j in range(v.shape[1] // 128):
                parts.append(v[8 * i:8 * i + 8, 128 * j:128 * j + 128])
    while len(parts) > 1:
        parts = [jnp.maximum(parts[i], parts[i + 1]) if i + 1 < len(parts) else parts[i]
                 for i in range(0, len(parts), 2)]
    return parts[0]


def _rslices(row0, n):
    row0 %= R
    if row0 + n <= R:
        return [(row0, row0 + n, 0)]
    return [(row0, R, 0), (0, row0 + n - R, R - row0)]


def _kernel(x_hbm, mem0_hbm, wq_hbm, wk_hbm, wv_hbm, wo_hbm, wr_hbm, wg_hbm, wu_hbm, wd_hbm,
            out_hbm,
            xs, x1buf, hbbuf, hbuf, hpack, raw, wq0, wq1, wkv, wo_raw, wo, wg, wu, wd,
            qbig, kvring, oring, abuf, ybuf, maskv, best, zflag, mem0_ref, wr_ref, wrb, sems):
    def wq(h):
        return wq0.at[h] if h < HC else wq1.at[h - HC]

    def x_copy(row0, n, sem):
        return pltpu.make_async_copy(x_hbm.at[pl.ds(row0, n)], xs.at[pl.ds(row0, n)], sems.at[sem])

    def w_copy(ph, src=None):
        if src is None:
            src = wq_hbm.at[:, pl.ds(0, HC), :]
        return pltpu.make_async_copy(src, raw.at[ph], sems.at[11 + ph])

    cp_x = [x_copy(c * XC, XC, 23 + c) for c in range(4)]
    cp_xa = x_copy(P0, XA - P0, 0)
    cp_q0 = [pltpu.make_async_copy(wq_hbm.at[pl.ds(c * 128, 128), pl.ds(0, HC), :],
                                   raw.at[0, pl.ds(c * 128, 128)], sems.at[29 + c])
             for c in range(4)]
    cp_x[0].start()
    for c in cp_q0 + cp_x[1:]:
        c.start()
    cp_xa.start()
    cp_s = [pltpu.make_async_copy(mem0_hbm, mem0_ref, sems.at[27]),
            pltpu.make_async_copy(wr_hbm, wr_ref, sems.at[28])]
    for c in cp_s:
        c.start()
    for i, w in enumerate((wq_hbm, wk_hbm, wv_hbm)):
        for c in range(4):
            if 4 * i + c > 0:
                w_copy(4 * i + c, w.at[:, pl.ds(c * HC, HC), :]).start()
    cp_wo = [pltpu.make_async_copy(wo_hbm.at[:, pl.ds(n * 128, 128)], wo_raw.at[n], sems.at[4 + n])
             for n in range(4)]
    for c in cp_wo:
        c.start()
    cp_xb = x_copy(XA, S - XA, 1)
    cp_f = [pltpu.make_async_copy(wg_hbm, wg, sems.at[8]),
            pltpu.make_async_copy(wu_hbm, wu, sems.at[9]),
            pltpu.make_async_copy(wd_hbm, wd, sems.at[10])]

    def out_copy(row0, n, sem=2):
        return pltpu.make_async_copy(xs.at[pl.ds(row0, n)], out_hbm.at[pl.ds(row0, n)], sems.at[sem])

    oring[:, R - M:R, :] = jnp.zeros((H, M, E), F32)
    abuf[...] = jnp.zeros(abuf.shape, F32)
    xs[pl.ds(S, SEG), :] = jnp.zeros((SEG, D), BF16)
    hbuf[pl.ds(2 * S, SEG), :] = jnp.zeros((SEG, D), F32)
    zflag[...] = jnp.zeros(zflag.shape, jnp.int32)

    ri = jax.lax.broadcasted_iota(jnp.int32, (L2, L2), 0)
    ci = jax.lax.broadcasted_iota(jnp.int32, (L2, L2), 1)

    def head_of(i):
        return jnp.where(i < 2 * M, i // M, (i - 2 * M) // SEG)

    def pos_of(i):
        return jnp.where(i < 2 * M, i % M, M + (i - 2 * M) % SEG)

    same = head_of(ri) == head_of(ci)
    ok = (pos_of(ri) < M) | (pos_of(ri) >= pos_of(ci))
    maskv[...] = jnp.where(same, jnp.where(ok, 0.0, -1e9 / SCALE), -jnp.inf).astype(F32)

    def gate(v, tk):
        y, r = tk
        ns = min(v.shape[-2], 8)
        tok = pltpu.bitcast(y[r:r + 8], v.dtype)[:ns]
        zf = (zflag[...] != 0)[:ns]
        reps = (v.shape[-2] // ns, v.shape[-1] // 128)
        tok, zf = jnp.tile(tok, reps), jnp.tile(zf, reps)
        return jnp.where(zf, tok, v)

    def toks(ys, n, frac=0.8):
        rows = [(y, r) for y in ys for r in range(0, y.shape[0], 8)]
        return [rows[int(len(rows) * frac * i / n)] for i in range(n)]

    def ln0(r0, tk=None, n=W):
        x = xs[r0:r0 + n, :].astype(F32)
        if tk is not None:
            x = gate(x, tk)
        h = _ln(x)
        hbuf[r0:r0 + n, :] = h
        if r0 < P0:
            hpack[r0 // 2:(r0 + n) // 2, :] = pltpu.bitcast(h.astype(BF16), U32)

    def relay(ph, tks=None, dbs=range(D // 16), is_q=False):
        for db in dbs:
            a = raw[ph, pl.ds(16 * db, 16)]
            if tks is not None:
                a = pltpu.bitcast(gate(pltpu.bitcast(a, U32), tks[db]), BF16)
            a = jnp.swapaxes(a, 0, 1)
            for hh in range(HC):
                v = pltpu.bitcast(a[hh], U32)
                if isinstance(ph, int) and ph == 0:
                    wq0[hh, pl.ds(8 * db, 8), :] = v
                elif is_q:
                    wq1[(ph - 1) * HC + hh, pl.ds(8 * db, 8), :] = v
                else:
                    tb = (ph % 4) * 16 + (ph // 4 - 1) * 2
                    wkv[tb + (hh // 2) * 4 + hh % 2, pl.ds(8 * db, 8), :] = v

    def light(heads, c=None):
        if c is None:
            r0, p0, n = 0, 0, P0
        elif isinstance(c, int):
            r0, p0, n = c * XC, c * (XC // 2), XC
        else:
            r0, p0, n = pl.multiple_of(c * XC, XC), pl.multiple_of(c * (XC // 2), XC // 2), XC
        lhs = _w(hpack[pl.ds(p0, n // 2), :])
        ys = []
        for h in heads:
            y = _dot(lhs, _w(wq(h)[...]))
            qbig[h, pl.ds(r0, n), :] = y
            ys.append(y)
        return ys

    def kv_head(lhs16):
        ys = []
        for t in range(2 * NPAIR, 4 * NPAIR):
            y = _dot(lhs16, _w(wkv[t]))
            kvring[t, 0:M, :] = y[:M]
            ys.append(y)
        return ys

    NG = XC // SEG
    cp_x[0].wait()
    for k in range(NG):
        ln0(k * SEG, None, SEG)
    for c in range(4):
        cp_q0[c].wait()
        relay(0, None, range(8 * c, 8 * c + 8))

    cp_x[1].wait()
    tks = toks(light(range(HC), 0), NG)
    for k in range(NG):
        ln0(XC + k * SEG, tks[k], SEG)

    cp_x[2].wait()
    cp_x[3].wait()
    cp_xa.wait()
    tks = toks(light(range(HC), 1), 2 * NG + 1, 0.85)
    for k in range(2 * NG + 1):
        ln0(2 * XC + k * SEG, tks[k], SEG)

    def phase_a(i, carry):
        w_copy(i).wait()
        relay(i, toks(light(range(HC), i + 1), 32), is_q=True)
        return carry

    jax.lax.fori_loop(1, 3, phase_a, 0)
    w_copy(3).wait()
    relay(3, toks(light(range(HC, HC + 3)), 32), is_q=True)

    def phase_b(i, carry):
        w_copy(4 + 2 * i).wait()
        w_copy(5 + 2 * i).wait()
        tks = toks(light(range(HC + 3, H), i), 64, 0.9)
        relay(4 + 2 * i, tks[:32])
        relay(5 + 2 * i, tks[32:])
        return carry

    jax.lax.fori_loop(0, 4, phase_b, 0)

    for c in cp_wo + cp_s:
        c.wait()
    wrb[...] = jnp.broadcast_to(wr_ref[...].astype(F32).reshape(1, D), (8, D))
    cp_xb.start()
    for c in cp_f:
        c.start()
    tks = toks(kv_head(_w(hpack[0:8, :])), 32, 0.9)
    for k in range(32):
        n, kk = k // 8, k % 8
        wo[n, pl.ds(256 * kk, 256), :] = gate(
            pltpu.bitcast(wo_raw[n, pl.ds(512 * kk, 512), :], U32), tks[k])

    def post(row0, a, valid):
        n = a.shape[0]
        x1 = _rb(xs[pl.ds(row0, n), :].astype(F32) + _rb(a))
        x1buf[pl.ds(row0, n), :] = x1.astype(BF16)
        hb = _ln(x1)
        hbbuf[pl.ds(row0, n), :] = hb.astype(BF16)
        r = _rb(jnp.sum(hb * jnp.tile(wrb[...], (n // 8, 1)), axis=-1, keepdims=True))
        x2 = x1 + hb
        xs[pl.ds(row0, n), :] = x2.astype(BF16)
        if valid is not True:
            r = jnp.where(valid, r, -jnp.inf)
        bv = best[0]
        bi = best[1]
        sub = jax.lax.broadcasted_iota(jnp.int32, (8, 128), 0).astype(F32)
        for g in range(n // 8):
            rg = jnp.broadcast_to(r[8 * g:8 * g + 8], (8, 128))
            ig = sub + (float(row0 + 8 * g) if isinstance(row0, int) else (row0 + 8 * g).astype(F32))
            gt = rg > bv
            bv = jnp.where(gt, rg, bv)
            bi = jnp.where(gt, ig, bi)
        best[0] = bv
        best[1] = bi
        return _tok(x2, bv, bi)

    def anchor(val, tok):
        return jnp.where(zflag[...] != 0, tok, val)

    def wo_pair(g, half):
        return jnp.concatenate(
            [_w(wo[2 * half + c, pl.ds(g * 128, 128), :]) for c in range(2)], axis=1)

    def rload(buf, t, row0, n):
        return [buf[t, a:b, :] for a, b, _ in _rslices(row0, n)]

    def step(ts, jpos, layer, j, mem, korder):
        q, par = ts // 2, ts % 2
        sr = ts * SEG
        if par == 0:
            kvw = ((W * q, 40), (W * q + 8, 24))
            ow = ((W * q - 8, 40), (W * q, 24))
        else:
            kvw = ((W * q + 40, 24), (W * q + 32, 40))
            ow = ((W * q + 32, 24), (W * q + 24, 40))
        sl = 4 * j + ts
        sg = layer * (2 * NU) + sl
        hb0 = pl.multiple_of(layer * S + R * j, R)
        pq0 = pl.multiple_of(P0 + LR * sg, 8)
        lhs = [jnp.concatenate([mem, hbuf[pl.ds(hb0 + r0, n), :]], axis=0).astype(BF16)
               for r0, n in kvw]
        lhsq = jnp.concatenate([mem, hbuf[pl.ds(pq0, LR), :]], axis=0).astype(BF16)
        qrow = [pl.multiple_of((pq0 + 8 * i) % S, 8) for i in range(LR // 8)]
        crow = pl.multiple_of(R * j + sr, SEG)

        def ksplit(ga, gb):
            half = ga // (NPAIR // 2)
            hq = [2 * ga, 2 * ga + 1, 2 * gb, 2 * gb + 1]

            def kv(k):
                wk = jnp.concatenate([_w(wkv[4 * ga + t, pl.ds(64 * k, 64), :])
                                      for t in range(4)], axis=1)
                return jnp.dot(lhs[half][:, 128 * k:128 * (k + 1)], wk, preferred_element_type=F32)

            def qq(k):
                wk = jnp.concatenate([_w(wq(h)[pl.ds(64 * k, 64), :]) for h in hq], axis=1)
                return jnp.dot(lhsq[:, 128 * k:128 * (k + 1)], wk, preferred_element_type=F32)

            pkv = pq = None
            for f, k in KSPLIT:
                y = (kv if f == 0 else qq)(korder[k])
                if f == 0:
                    pkv = y if pkv is None else pkv + y
                else:
                    pq = y if pq is None else pq + y
            done = {("kv", 4 * ga + t): pkv[:, 128 * t:128 * (t + 1)] for t in range(4)}
            if pq is not None:
                done.update({("q", h): pq[:, 128 * i:128 * (i + 1)] for i, h in enumerate(hq)})
            return done

        def qkv(g, done):
            half = g // (NPAIR // 2)
            r0, n = kvw[half]
            res = []
            for c in range(2):
                y = done.get(("q", 2 * g + c))
                if y is None:
                    y = jnp.dot(lhsq, _w(wq(2 * g + c)[...]), preferred_element_type=F32)
                for i in range(LR // 8):
                    qbig[2 * g + c, pl.ds(qrow[i], 8), :] = y[M + 8 * i:M + 8 * i + 8]
                res.append(y[:M])
            for t in range(4):
                y = done.get(("kv", 4 * g + t))
                if y is None:
                    y = jnp.dot(lhs[half], _w(wkv[4 * g + t]), preferred_element_type=F32)
                for a, b, o in _rslices(r0, n):
                    kvring[4 * g + t, a:b, :] = y[M + o:M + o + b - a]
                res.append(y[:M])
            qx = jnp.concatenate([qbig[2 * g + c, pl.ds(crow, SEG), :] for c in range(2)],
                                 axis=0).astype(BF16)
            return res, qx

        def stack(g, mres, i):
            return jnp.concatenate(
                [mres[2 * i], mres[2 * i + 1],
                 kvring[4 * g + 2 * i - 2, sr:sr + SEG, :],
                 kvring[4 * g + 2 * i - 1, sr:sr + SEG, :]], axis=0).astype(BF16)

        def qk(g, mres, qx, prenorm):
            q2 = jnp.concatenate(
                [jnp.concatenate([mres[0], mres[1]], axis=0).astype(BF16), qx], axis=0)
            s = jax.lax.dot_general(q2, stack(g, mres, 1), (((1,), (1,)), ((), ())),
                                    preferred_element_type=F32)
            mk = maskv[...]
            s = jnp.where(mk == 0.0, s, mk)
            mx = jnp.max(s, axis=-1, keepdims=True)
            p = jnp.exp2((s - mx) * (SCALE * LOG2E))
            l = jnp.sum(p, axis=-1, keepdims=True)
            r0 = pl.reciprocal(l, approx=True)
            r = r0 * (2.0 - l * r0)
            if prenorm:
                return (p * r).astype(BF16), None
            return p.astype(BF16), r

        def pv(g, mres, pr):
            p, r = pr
            o = jnp.dot(p, stack(g, mres, 2), preferred_element_type=F32)
            if r is not None:
                o = o * r
            oring[2 * g, sr:sr + SEG, :] = o[2 * M:2 * M + SEG]
            oring[2 * g + 1, sr:sr + SEG, :] = o[2 * M + SEG:]
            return o[:M], o[M:2 * M]

        def olhs(g, om, half):
            r0, n = ow[half]
            return jnp.concatenate(
                [jnp.concatenate([om[c]] + rload(oring, 2 * g + c, r0, n), axis=0)
                 for c in range(2)], axis=1).astype(BF16)

        pn0 = pl.multiple_of(PLN + LR * sg, 8)
        xr = jnp.concatenate(
            [xs[pl.ds(pl.multiple_of((pn0 + 8 * i) % S, 8), 8), :].astype(F32)
             for i in range(LR // 8)], axis=0)
        hpre = _ln(xr)
        hbuf[pl.ds(pn0, LR), :] = hpre
        tok_pre = _tok(hpre)
        if ts >= 2 or jpos:
            valid = True
            row0 = pl.multiple_of(SEG * (sl - 2), SEG)
        else:
            valid = j >= 1
            row0 = pl.multiple_of(jnp.where(valid, SEG * (sl - 2), S), SEG)
        ar = (sr - 2 * SEG) % R
        tok_post = post(row0, abuf[ar:ar + SEG, :], valid)

        NST = NPAIR // 2
        st = [(i, i + NST) if par == 0 else (i + NST, i) for i in range(NST)]
        mres, qxs, prs, oms = {}, {}, {}, {}
        acc = [None] * 4
        order = []
        for i in range(NST):
            order += [("qkv", g) for g in st[i]]
            if i >= 1:
                order += [("qk", g) for g in st[i - 1]]
            if i >= 2:
                order += [("pv", g) for g in st[i - 2]]
        oq = [g for i in range(NST) for g in st[i]]
        order += [("o", g) for g in oq[0:O1]]
        order += [("qk", g) for g in st[NST - 1]] + [("pv", g) for g in st[NST - 2]]
        order += [("o", g) for g in oq[O1:O2]]
        order += [("pv", g) for g in st[NST - 1]]
        order += [("o", g) for g in oq[O2:NE]]
        norder = (2, 3, 0, 1) if par == 0 else (0, 1, 2, 3)
        order += [("on", n) for n in norder]
        done = {} if korder is None else ksplit(*st[0])
        for kind, g in order:
            if kind == "qkv":
                mres[g], qxs[g] = qkv(g, done)
                if g == st[PRE_ST][0]:
                    mres[g][0] = anchor(mres[g][0], tok_pre)
                if g == st[POST_ST][0]:
                    mres[g][0] = anchor(mres[g][0], tok_post)
            elif kind == "qk":
                prs[g] = qk(g, mres[g], qxs[g], g not in st[NST - 1] + st[NST - 2])
            elif kind == "pv":
                oms[g] = pv(g, mres[g], prs[g])
                if prs[g][1] is not None:
                    oms[g] = (anchor(oms[g][0], _tok(prs[g][1][2 * M:])), oms[g][1])
            elif kind == "o":
                for half in range(2):
                    y = jnp.dot(olhs(g, oms[g], half), wo_pair(g, half), preferred_element_type=F32)
                    for c in range(2):
                        yc = y[:, 128 * c:128 * (c + 1)]
                        n = 2 * half + c
                        acc[n] = yc if acc[n] is None else acc[n] + yc
            else:
                n = g
                l = jnp.concatenate([olhs(g2, oms[g2], n // 2) for g2 in oq[NE:]], axis=1)
                wn = jnp.concatenate([_w(wo[n, pl.ds(g2 * 128, 128), :]) for g2 in oq[NE:]], axis=0)
                acc[n] = acc[n] + jnp.dot(l, wn, preferred_element_type=F32)
        for n in range(4):
            r0, nr = ow[n // 2]
            for a, b, o in _rslices(r0, nr):
                abuf[a:b, n * 128:(n + 1) * 128] = acc[n][M + o:M + o + b - a]

        return jnp.concatenate([acc[n][:M] for n in range(4)], axis=1), norder

    def argmax():
        bv = best[0]
        bi = best[1]
        vmax = jnp.max(bv, axis=0, keepdims=True)
        imin = jnp.min(jnp.where(bv == vmax, bi, float(S)), axis=0, keepdims=True)
        idx = jnp.clip(jnp.min(imin).astype(jnp.int32), 0, S - 1)
        return idx, vmax

    def ffn(idx):
        g0 = pl.multiple_of((idx // 16) * 16, 16)
        hbb = hbbuf[pl.ds(g0, 16), :]
        gpre = _rb(_dot(hbb, wg[...]))
        gs = _rb(gpre * _rb(jax.nn.sigmoid(gpre)))
        up = _rb(_dot(hbb, wu[...]))
        ybuf[...] = _rb(_dot((gs * up).astype(BF16), wd[...]))

    def ffn_small(idx):
        g0 = pl.multiple_of((idx // 16) * 16, 16)
        hbb = hbbuf[pl.ds(g0, 16), :]

        def body(c, acc):
            f0 = pl.multiple_of(c * 256, 256)
            gpre = _rb(_dot(hbb, wg[:, pl.ds(f0, 256)]))
            gs = _rb(gpre * _rb(jax.nn.sigmoid(gpre)))
            up = _rb(_dot(hbb, wu[:, pl.ds(f0, 256)]))
            return acc + _dot((gs * up).astype(BF16), wd[pl.ds(f0, 256), :])

        ybuf[...] = _rb(jax.lax.fori_loop(0, F // 256, body, jnp.zeros((16, D), F32)))

    def layer_body(layer, carry):
        best[0] = jnp.full((8, 128), -jnp.inf, F32)
        best[1] = jnp.zeros((8, 128), F32)

        def qstep(jj, mem):
            @pl.when((layer == 0) & (jj == 1))
            def _():
                cp_xb.wait()

            @pl.when((layer == 1) & (jj >= 2))
            def _():
                out_copy(pl.multiple_of((jj - 1) * (UNR * R) - W, W), UNR * R).start()

            @pl.when((layer == 1) & (jj == 1))
            def _():
                out_copy(0, UNR * R - W).start()

            ko = None
            for j2 in range(UNR):
                for ts in range(4):
                    mem, ko = step(ts, j2 > 0, layer, UNR * jj + j2, mem, ko)
            return mem

        jax.lax.fori_loop(0, NU // (2 * UNR), qstep, mem0_ref[...].astype(F32))

        @pl.when(layer == 0)
        def _():
            for c in cp_f:
                c.wait()

        @pl.when(layer == 1)
        def _():
            out_copy(S - UNR * R - W, UNR * R).start()

        idx_s, _ = argmax()
        acc = None
        for g in range(NPAIR):
            l = jnp.concatenate([oring[2 * g + c, R - 16:R, :] for c in range(2)],
                                axis=1).astype(BF16)
            y = _dot(l, wo_pair(g, 0))
            acc = y if acc is None else acc + y
        abuf[R - M:R, 0:256] = acc[M:]
        ffn(idx_s)
        post(S - W, abuf[W:R, :], True)
        idx, vmax = argmax()

        @pl.when(layer == 1)
        def _():
            out_copy(S - W, W).start()

        @pl.when(idx // 16 != idx_s // 16)
        def _():
            ffn_small(idx)

        g0 = pl.multiple_of((idx // 16) * 16, 16)
        rsel = jnp.tile(_rb(jax.nn.sigmoid(vmax)), (1, D // 128))
        y = _rb(ybuf[...] * rsel)
        x2 = _rb(x1buf[pl.ds(g0, 16), :].astype(F32) + _rb(hbbuf[pl.ds(g0, 16), :].astype(F32) + y))
        rowi = jax.lax.broadcasted_iota(jnp.int32, (16, D), 0) + g0

        @pl.when(layer == 1)
        def _():
            out_copy(0, S).wait()

        x2 = jnp.where(rowi == idx, x2, xs[pl.ds(g0, 16), :].astype(F32))
        xs[pl.ds(g0, 16), :] = x2.astype(BF16)

        @pl.when(layer == 0)
        def _():
            h16 = _ln(x2)
            hbuf[pl.ds(S + g0, 16), :] = h16

            @pl.when(idx < FD)
            def _():
                def body0(h, c):
                    qbig[h, pl.ds(g0, 16), :] = _dot(h16.astype(BF16), _w(wq0[h]))
                    return c

                def body1(h, c):
                    qbig[HC + h, pl.ds(g0, 16), :] = _dot(h16.astype(BF16), _w(wq1[h]))
                    return c

                jax.lax.fori_loop(0, HC, body0, 0, unroll=2)
                jax.lax.fori_loop(0, H - HC, body1, 0, unroll=4)

            @pl.when(idx < M)
            def _():
                def body(t, c):
                    kvring[t, 0:M, :] = _dot(h16.astype(BF16), _w(wkv[t]))[:M]
                    return c

                jax.lax.fori_loop(2 * NPAIR, 4 * NPAIR, body, 0, unroll=2)

        @pl.when(layer == 1)
        def _():
            fix = out_copy(g0, 16, 3)
            fix.start()
            fix.wait()

        return carry

    jax.lax.fori_loop(0, 2, layer_body, 0)


@functools.partial(jax.jit, static_argnames=("A_seg_len",))
def pallas_interleave_layers__memory_aug_recurrent_mem_tr__moe_arch_mod__prompt_kernel(
    A_x: jax.Array,
    A_mem0: jax.Array,
    A_Wq: jax.Array,
    A_Wk: jax.Array,
    A_Wv: jax.Array,
    A_Wo: jax.Array,
    A_seg_len,
    B_x: jax.Array,
    B_w_r: jax.Array,
    B_w_gate: jax.Array,
    B_w_up: jax.Array,
    B_w_down: jax.Array,
):
    assert A_seg_len == SEG
    assert A_x.shape == (1, S, D) and A_Wq.shape == (D, H, E) and A_mem0.shape == (1, M, D)
    any_spec = pl.BlockSpec(memory_space=pl.ANY)
    out = pl.pallas_call(
        _kernel,
        out_shape=jax.ShapeDtypeStruct((S, D), BF16),
        in_specs=[any_spec] * 10,
        out_specs=any_spec,
        scratch_shapes=[
            pltpu.VMEM((S + SEG, D), BF16),
            pltpu.VMEM((S + SEG, D), BF16),
            pltpu.VMEM((S + SEG, D), BF16),
            pltpu.VMEM((2 * S + SEG, D), F32),
            pltpu.VMEM((P0 // 2, D), U32),
            pltpu.VMEM((12, D, HC, E), BF16),
            pltpu.VMEM((HC, D // 2, E), U32),
            pltpu.VMEM((H - HC, D // 2, E), U32),
            pltpu.VMEM((2 * H, D // 2, E), U32),
            pltpu.VMEM((4, H * E, 128), BF16),
            pltpu.VMEM((4, H * E // 2, 128), U32),
            pltpu.VMEM((D, F), BF16),
            pltpu.VMEM((D, F), BF16),
            pltpu.VMEM((F, D), BF16),
            pltpu.VMEM((H, S, E), F32),
            pltpu.VMEM((2 * H, R, E), F32),
            pltpu.VMEM((H, R, E), F32),
            pltpu.VMEM((R, D), F32),
            pltpu.VMEM((16, D), F32),
            pltpu.VMEM((L2, L2), F32),
            pltpu.VMEM((2, 8, 128), F32),
            pltpu.VMEM((8, 128), jnp.int32),
            pltpu.VMEM((M, D), BF16),
            pltpu.VMEM((D,), BF16),
            pltpu.VMEM((8, D), F32),
            pltpu.SemaphoreType.DMA((33,)),
        ],
        compiler_params=pltpu.CompilerParams(vmem_limit_bytes=110 * 1024 * 1024),
        name="rmt_mod",
    )(A_x.reshape(S, D), A_mem0.reshape(M, D), A_Wq, A_Wk, A_Wv, A_Wo.reshape(H * E, D),
      B_w_r, B_w_gate, B_w_up, B_w_down)
    return out.reshape(1, S, D)
```

```python
import jax
import jax.numpy as jnp
import jax.experimental.pallas as pl
import jax.experimental.pallas.tpu as pltpu

S = 2048
D = 512
H = 32
E = 128
M = 8
SEG = 32
F = 1792
NPAIR = H // 2
NU = S // (2 * SEG)
W = 2 * SEG
L2 = 2 * (M + SEG)
EPS = 1e-05
SCALE = float(E) ** -0.5
LOG2E = 1.4426950408889634
F32 = jnp.float32
BF16 = jnp.bfloat16
U32 = jnp.uint32


def _rb(x):
    return x.astype(BF16).astype(F32)


def _ln(x):
    mu = jnp.sum(x, axis=-1, keepdims=True) * (1.0 / D)
    xc0 = x - mu
    var = jnp.sum(xc0 * xc0, axis=-1, keepdims=True) * (1.0 / D)
    sd = _rb(jnp.sqrt(_rb(_rb(var) + EPS)))
    xc = _rb(x - _rb(mu))
    return _rb(xc * (1.0 / sd))


def _dot(a, b):
    return jnp.dot(a, b, preferred_element_type=F32)


def _w(ref_slab):
    return pltpu.bitcast(ref_slab, BF16)


P0 = S // 2
LR = 24
PLN = P0 + LR
XC = P0 // 4
XLN = P0 + SEG
UNR = 2
NJ = NU // (2 * UNR)
XA = P0 + 4 * UNR * SEG
FD = PLN + LR * 2 * NU - S
R = 4 * SEG
HC = H // 4
PRE_ST = 3
POST_ST = 5
KSPLIT = ((0, 0), (0, 1), (1, 0), (1, 1), (0, 2), (1, 2), (0, 3), (1, 3))
FLAG = 2
O1, O2, NE = 3, 7, 8


def _tok(*vals):
    parts = []
    for v in vals:
        if v.shape[1] < 128:
            v = jnp.broadcast_to(v[:, :1], (v.shape[0], 128))
        for i in range(v.shape[0] // 8):
            for j in range(v.shape[1] // 128):
                parts.append(v[8 * i:8 * i + 8, 128 * j:128 * j + 128])
    while len(parts) > 1:
        parts = [jnp.maximum(parts[i], parts[i + 1]) if i + 1 < len(parts) else parts[i]
                 for i in range(0, len(parts), 2)]
    return parts[0]


def _rslices(row0, n):
    row0 %= R
    if row0 + n <= R:
        return [(row0, row0 + n, 0)]
    return [(row0, R, 0), (0, row0 + n - R, R - row0)]


def _kernel(x_hbm, mem0_hbm, wq_hbm, wk_hbm, wv_hbm, wo_hbm, wr_hbm, wg_hbm, wu_hbm, wd_hbm,
            out_hbm,
            xs, x1buf, hbbuf, hbuf, hpack, raw, wq0, wq1, wkv, wo_raw, wo, wg, wu, wd,
            qbig, kvring, oring, abuf, ybuf, maskv, best, zflag, mem0_ref, wr_ref, wrb, sems):
    def wq(h):
        return wq0.at[h] if h < HC else wq1.at[h - HC]

    def x_copy(row0, n, sem):
        return pltpu.make_async_copy(x_hbm.at[pl.ds(row0, n)], xs.at[pl.ds(row0, n)], sems.at[sem])

    def w_copy(ph, src=None):
        if src is None:
            src = wq_hbm.at[:, pl.ds(0, HC), :]
        return pltpu.make_async_copy(src, raw.at[ph], sems.at[11 + ph])

    cp_x = [x_copy(c * XC, XC, 23 + c) for c in range(4)]
    cp_xa = x_copy(P0, XA - P0, 0)
    cp_q0 = [pltpu.make_async_copy(wq_hbm.at[pl.ds(c * 128, 128), pl.ds(0, HC), :],
                                   raw.at[0, pl.ds(c * 128, 128)], sems.at[29 + c])
             for c in range(4)]
    cp_x[0].start()
    for c in cp_q0 + cp_x[1:]:
        c.start()
    cp_xa.start()
    cp_s = [pltpu.make_async_copy(mem0_hbm, mem0_ref, sems.at[27]),
            pltpu.make_async_copy(wr_hbm, wr_ref, sems.at[28])]
    for c in cp_s:
        c.start()
    for i, w in enumerate((wq_hbm, wk_hbm, wv_hbm)):
        for c in range(4):
            if 4 * i + c > 0:
                w_copy(4 * i + c, w.at[:, pl.ds(c * HC, HC), :]).start()
    cp_wo = [pltpu.make_async_copy(wo_hbm.at[:, pl.ds(n * 128, 128)], wo_raw.at[n], sems.at[4 + n])
             for n in range(4)]
    for c in cp_wo:
        c.start()
    cp_xb = x_copy(XA, S - XA, 1)
    cp_f = [pltpu.make_async_copy(wg_hbm, wg, sems.at[8]),
            pltpu.make_async_copy(wu_hbm, wu, sems.at[9]),
            pltpu.make_async_copy(wd_hbm, wd, sems.at[10])]

    def out_copy(row0, n, sem=2):
        return pltpu.make_async_copy(xs.at[pl.ds(row0, n)], out_hbm.at[pl.ds(row0, n)], sems.at[sem])

    oring[:, R - M:R, :] = jnp.zeros((H, M, E), F32)
    abuf[...] = jnp.zeros(abuf.shape, F32)
    xs[pl.ds(S, SEG), :] = jnp.zeros((SEG, D), BF16)
    hbuf[pl.ds(2 * S, SEG), :] = jnp.zeros((SEG, D), F32)
    zflag[...] = jnp.zeros(zflag.shape, jnp.int32)

    ri = jax.lax.broadcasted_iota(jnp.int32, (L2, L2), 0)
    ci = jax.lax.broadcasted_iota(jnp.int32, (L2, L2), 1)

    def head_of(i):
        return jnp.where(i < 2 * M, i // M, (i - 2 * M) // SEG)

    def pos_of(i):
        return jnp.where(i < 2 * M, i % M, M + (i - 2 * M) % SEG)

    same = head_of(ri) == head_of(ci)
    ok = (pos_of(ri) < M) | (pos_of(ri) >= pos_of(ci))
    maskv[...] = jnp.where(same, jnp.where(ok, 0.0, -1e9 / SCALE), -jnp.inf).astype(F32)

    def gate(v, tk):
        y, r = tk
        ns = min(v.shape[-2], 8)
        tok = pltpu.bitcast(y[r:r + 8], v.dtype)[:ns]
        zf = (zflag[...] != 0)[:ns]
        reps = (v.shape[-2] // ns, v.shape[-1] // 128)
        tok, zf = jnp.tile(tok, reps), jnp.tile(zf, reps)
        return jnp.where(zf, tok, v)

    def toks(ys, n, frac=0.8):
        rows = [(y, r) for y in ys for r in range(0, y.shape[0], 8)]
        return [rows[int(len(rows) * frac * i / n)] for i in range(n)]

    def ln0(r0, tk=None, n=W):
        x = xs[r0:r0 + n, :].astype(F32)
        if tk is not None:
            x = gate(x, tk)
        h = _ln(x)
        hbuf[r0:r0 + n, :] = h
        if r0 < P0:
            hpack[r0 // 2:(r0 + n) // 2, :] = pltpu.bitcast(h.astype(BF16), U32)

    def relay(ph, tks=None, dbs=range(D // 16), is_q=False):
        for db in dbs:
            a = raw[ph, pl.ds(16 * db, 16)]
            if tks is not None:
                a = pltpu.bitcast(gate(pltpu.bitcast(a, U32), tks[db]), BF16)
            a = jnp.swapaxes(a, 0, 1)
            for hh in range(HC):
                v = pltpu.bitcast(a[hh], U32)
                if isinstance(ph, int) and ph == 0:
                    wq0[hh, pl.ds(8 * db, 8), :] = v
                elif is_q:
                    wq1[(ph - 1) * HC + hh, pl.ds(8 * db, 8), :] = v
                else:
                    tb = (ph % 4) * 16 + (ph // 4 - 1) * 2
                    wkv[tb + (hh // 2) * 4 + hh % 2, pl.ds(8 * db, 8), :] = v

    def light(heads, c=None):
        if c is None:
            r0, p0, n = 0, 0, P0
        elif isinstance(c, int):
            r0, p0, n = c * XC, c * (XC // 2), XC
        else:
            r0, p0, n = pl.multiple_of(c * XC, XC), pl.multiple_of(c * (XC // 2), XC // 2), XC
        lhs = _w(hpack[pl.ds(p0, n // 2), :])
        ys = []
        for h in heads:
            y = _dot(lhs, _w(wq(h)[...]))
            qbig[h, pl.ds(r0, n), :] = y
            ys.append(y)
        return ys

    def kv_head(lhs16):
        ys = []
        for t in range(2 * NPAIR, 4 * NPAIR):
            y = _dot(lhs16, _w(wkv[t]))
            kvring[t, 0:M, :] = y[:M]
            ys.append(y)
        return ys

    NG = XC // SEG
    cp_x[0].wait()
    for k in range(NG):
        ln0(k * SEG, None, SEG)
    for c in range(4):
        cp_q0[c].wait()
        relay(0, None, range(8 * c, 8 * c + 8))

    cp_x[1].wait()
    tks = toks(light(range(HC), 0), NG)
    for k in range(NG):
        ln0(XC + k * SEG, tks[k], SEG)

    cp_x[2].wait()
    cp_x[3].wait()
    cp_xa.wait()
    tks = toks(light(range(HC), 1), 2 * NG + 1, 0.85)
    for k in range(2 * NG + 1):
        ln0(2 * XC + k * SEG, tks[k], SEG)

    def phase_a(i, carry):
        w_copy(i).wait()
        relay(i, toks(light(range(HC), i + 1), 32), is_q=True)
        return carry

    jax.lax.fori_loop(1, 3, phase_a, 0)
    w_copy(3).wait()
    relay(3, toks(light(range(HC, HC + 3)), 32), is_q=True)

    def phase_b(i, carry):
        w_copy(4 + 2 * i).wait()
        w_copy(5 + 2 * i).wait()
        tks = toks(light(range(HC + 3, H), i), 64, 0.9)
        relay(4 + 2 * i, tks[:32])
        relay(5 + 2 * i, tks[32:])
        return carry

    jax.lax.fori_loop(0, 4, phase_b, 0)

    for c in cp_wo + cp_s:
        c.wait()
    wrb[...] = jnp.broadcast_to(wr_ref[...].astype(F32).reshape(1, D), (8, D))
    cp_xb.start()
    for c in cp_f:
        c.start()
    tks = toks(kv_head(_w(hpack[0:8, :])), 32, 0.9)
    for k in range(32):
        n, kk = k // 8, k % 8
        wo[n, pl.ds(256 * kk, 256), :] = gate(
            pltpu.bitcast(wo_raw[n, pl.ds(512 * kk, 512), :], U32), tks[k])

    def post(row0, a, valid):
        n = a.shape[0]
        x1 = _rb(xs[pl.ds(row0, n), :].astype(F32) + _rb(a))
        x1buf[pl.ds(row0, n), :] = x1.astype(BF16)
        hb = _ln(x1)
        hbbuf[pl.ds(row0, n), :] = hb.astype(BF16)
        r = _rb(jnp.sum(hb * jnp.tile(wrb[...], (n // 8, 1)), axis=-1, keepdims=True))
        x2 = x1 + hb
        xs[pl.ds(row0, n), :] = x2.astype(BF16)
        if valid is not True:
            r = jnp.where(valid, r, -jnp.inf)
        bv = best[0]
        bi = best[1]
        sub = jax.lax.broadcasted_iota(jnp.int32, (8, 128), 0).astype(F32)
        for g in range(n // 8):
            rg = jnp.broadcast_to(r[8 * g:8 * g + 8], (8, 128))
            ig = sub + (float(row0 + 8 * g) if isinstance(row0, int) else (row0 + 8 * g).astype(F32))
            gt = rg > bv
            bv = jnp.where(gt, rg, bv)
            bi = jnp.where(gt, ig, bi)
        best[0] = bv
        best[1] = bi
        return _tok(x2, bv, bi)

    def anchor(val, tok):
        return jnp.where(zflag[...] != 0, tok, val)

    def wo_pair(g, half):
        return jnp.concatenate(
            [_w(wo[2 * half + c, pl.ds(g * 128, 128), :]) for c in range(2)], axis=1)

    def rload(buf, t, row0, n):
        return [buf[t, a:b, :] for a, b, _ in _rslices(row0, n)]

    def step(ts, jpos, last, layer, j, mem, korder):
        q, par = ts // 2, ts % 2
        sr = ts * SEG
        if par == 0:
            kvw = ((W * q, 40), (W * q + 8, 24))
            ow = ((W * q - 8, 40), (W * q, 24))
        else:
            kvw = ((W * q + 40, 24), (W * q + 32, 40))
            ow = ((W * q + 32, 24), (W * q + 24, 40))
        sl = 4 * j + ts
        sg = layer * (2 * NU) + sl
        hb0 = pl.multiple_of(layer * S + R * j, R)
        pq0 = pl.multiple_of(P0 + LR * sg, 8)
        lhs = [jnp.concatenate([mem, hbuf[pl.ds(hb0 + r0, n), :]], axis=0).astype(BF16)
               for r0, n in kvw]
        lhsq = jnp.concatenate([mem, hbuf[pl.ds(pq0, LR), :]], axis=0).astype(BF16)
        qrow = [pl.multiple_of((pq0 + 8 * i) % S, 8) for i in range(LR // 8)]
        crow = pl.multiple_of(R * j + sr, SEG)

        def ksplit(ga, gb):
            half = ga // (NPAIR // 2)
            hq = [2 * ga, 2 * ga + 1, 2 * gb, 2 * gb + 1]

            def kv(k):
                wk = jnp.concatenate([_w(wkv[4 * ga + t, pl.ds(64 * k, 64), :])
                                      for t in range(4)], axis=1)
                return jnp.dot(lhs[half][:, 128 * k:128 * (k + 1)], wk, preferred_element_type=F32)

            def qq(k):
                wk = jnp.concatenate([_w(wq(h)[pl.ds(64 * k, 64), :]) for h in hq], axis=1)
                return jnp.dot(lhsq[:, 128 * k:128 * (k + 1)], wk, preferred_element_type=F32)

            pkv = pq = None
            for f, k in KSPLIT:
                y = (kv if f == 0 else qq)(korder[k])
                if f == 0:
                    pkv = y if pkv is None else pkv + y
                else:
                    pq = y if pq is None else pq + y
            done = {("kv", 4 * ga + t): pkv[:, 128 * t:128 * (t + 1)] for t in range(4)}
            if pq is not None:
                done.update({("q", h): pq[:, 128 * i:128 * (i + 1)] for i, h in enumerate(hq)})
            return done

        def qkv(g, done):
            half = g // (NPAIR // 2)
            r0, n = kvw[half]
            res = []
            for c in range(2):
                y = done.get(("q", 2 * g + c))
                if y is None:
                    y = jnp.dot(lhsq, _w(wq(2 * g + c)[...]), preferred_element_type=F32)
                for i in range(LR // 8):
                    qbig[2 * g + c, pl.ds(qrow[i], 8), :] = y[M + 8 * i:M + 8 * i + 8]
                res.append(y[:M])
            for t in range(4):
                y = done.get(("kv", 4 * g + t))
                if y is None:
                    y = jnp.dot(lhs[half], _w(wkv[4 * g + t]), preferred_element_type=F32)
                for a, b, o in _rslices(r0, n):
                    kvring[4 * g + t, a:b, :] = y[M + o:M + o + b - a]
                res.append(y[:M])
            qx = jnp.concatenate([qbig[2 * g + c, pl.ds(crow, SEG), :] for c in range(2)],
                                 axis=0).astype(BF16)
            return res, qx

        def stack(g, mres, i):
            return jnp.concatenate(
                [mres[2 * i], mres[2 * i + 1],
                 kvring[4 * g + 2 * i - 2, sr:sr + SEG, :],
                 kvring[4 * g + 2 * i - 1, sr:sr + SEG, :]], axis=0).astype(BF16)

        def qk(g, mres, qx, prenorm):
            q2 = jnp.concatenate(
                [jnp.concatenate([mres[0], mres[1]], axis=0).astype(BF16), qx], axis=0)
            s = jax.lax.dot_general(q2, stack(g, mres, 1), (((1,), (1,)), ((), ())),
                                    preferred_element_type=F32)
            mk = maskv[...]
            s = jnp.where(mk == 0.0, s, mk)
            mx = jnp.max(s, axis=-1, keepdims=True)
            p = jnp.exp2((s - mx) * (SCALE * LOG2E))
            l = jnp.sum(p, axis=-1, keepdims=True)
            r0 = pl.reciprocal(l, approx=True)
            r = r0 * (2.0 - l * r0)
            if prenorm:
                return (p * r).astype(BF16), None
            return p.astype(BF16), r

        def pv(g, mres, pr):
            p, r = pr
            o = jnp.dot(p, stack(g, mres, 2), preferred_element_type=F32)
            if r is not None:
                o = o * r
            oring[2 * g, sr:sr + SEG, :] = o[2 * M:2 * M + SEG]
            oring[2 * g + 1, sr:sr + SEG, :] = o[2 * M + SEG:]
            return o[:M], o[M:2 * M]

        def olhs(g, om, half):
            r0, n = ow[half]
            if last is not None and half == 0:
                om = [jnp.where(last, oring[2 * g + c, R - M:R, :], om[c]) for c in range(2)]
            return jnp.concatenate(
                [jnp.concatenate([om[c]] + rload(oring, 2 * g + c, r0, n), axis=0)
                 for c in range(2)], axis=1).astype(BF16)

        pn0 = pl.multiple_of(PLN + LR * sg, 8)
        xr = jnp.concatenate(
            [xs[pl.ds(pl.multiple_of((pn0 + 8 * i) % S, 8), 8), :].astype(F32)
             for i in range(LR // 8)], axis=0)
        hpre = _ln(xr)
        hbuf[pl.ds(pn0, LR), :] = hpre
        tok_pre = _tok(hpre)
        if ts >= 2 or jpos:
            valid = True
            row0 = pl.multiple_of(SEG * (sl - 2), SEG)
        else:
            valid = j >= 1
            row0 = pl.multiple_of(jnp.where(valid, SEG * (sl - 2), S), SEG)
        ar = (sr - 2 * SEG) % R
        tok_post = post(row0, abuf[ar:ar + SEG, :], valid)

        NST = NPAIR // 2
        st = [(i, i + NST) if par == 0 else (i + NST, i) for i in range(NST)]
        mres, qxs, prs, oms = {}, {}, {}, {}
        acc = [None] * 4
        order = []
        for i in range(NST):
            order += [("qkv", g) for g in st[i]]
            if i >= 1:
                order += [("qk", g) for g in st[i - 1]]
            if i >= 2:
                order += [("pv", g) for g in st[i - 2]]
        oq = [g for i in range(NST) for g in st[i]]
        order += [("o", g) for g in oq[0:O1]]
        order += [("qk", g) for g in st[NST - 1]] + [("pv", g) for g in st[NST - 2]]
        order += [("o", g) for g in oq[O1:O2]]
        order += [("pv", g) for g in st[NST - 1]]
        order += [("o", g) for g in oq[O2:NE]]
        norder = (2, 3, 0, 1) if par == 0 else (0, 1, 2, 3)
        order += [("on", n) for n in norder]
        done = {} if korder is None else ksplit(*st[0])
        for kind, g in order:
            if kind == "qkv":
                mres[g], qxs[g] = qkv(g, done)
                if g == st[PRE_ST][0]:
                    mres[g][0] = anchor(mres[g][0], tok_pre)
                if g == st[POST_ST][0]:
                    mres[g][0] = anchor(mres[g][0], tok_post)
            elif kind == "qk":
                prs[g] = qk(g, mres[g], qxs[g], g not in st[NST - 1] + st[NST - 2])
            elif kind == "pv":
                oms[g] = pv(g, mres[g], prs[g])
                if prs[g][1] is not None:
                    oms[g] = (anchor(oms[g][0], _tok(prs[g][1][2 * M:])), oms[g][1])
            elif kind == "o":
                for half in range(2):
                    y = jnp.dot(olhs(g, oms[g], half), wo_pair(g, half), preferred_element_type=F32)
                    for c in range(2):
                        yc = y[:, 128 * c:128 * (c + 1)]
                        n = 2 * half + c
                        acc[n] = yc if acc[n] is None else acc[n] + yc
            else:
                n = g
                l = jnp.concatenate([olhs(g2, oms[g2], n // 2) for g2 in oq[NE:]], axis=1)
                wn = jnp.concatenate([_w(wo[n, pl.ds(g2 * 128, 128), :]) for g2 in oq[NE:]], axis=0)
                acc[n] = acc[n] + jnp.dot(l, wn, preferred_element_type=F32)
        for n in range(4):
            r0, nr = ow[n // 2]
            for a, b, o in _rslices(r0, nr):
                abuf[a:b, n * 128:(n + 1) * 128] = acc[n][M + o:M + o + b - a]

        if last is not None:
            for n in range(2):
                abuf[R - M:R, n * 128:(n + 1) * 128] = acc[n][:M]

        return jnp.concatenate([acc[n][:M] for n in range(4)], axis=1), norder

    def argmax():
        bv = best[0]
        bi = best[1]
        vmax = jnp.max(bv, axis=0, keepdims=True)
        imin = jnp.min(jnp.where(bv == vmax, bi, float(S)), axis=0, keepdims=True)
        idx = jnp.clip(imin.astype(jnp.int32)[0, 0], 0, S - 1)
        return idx, vmax

    def ffn(idx):
        g0 = pl.multiple_of((idx // 16) * 16, 16)
        hbb = hbbuf[pl.ds(g0, 16), :]
        nc = F // 256
        hid, acc, gs_ = [], None, []
        for c in range(nc + FLAG):
            if c < nc:
                gpre = _rb(_dot(hbb, wg[:, 256 * c:256 * (c + 1)]))
                gs_.append(gpre[:, :128])
                gs = _rb(gpre * _rb(jax.nn.sigmoid(gpre)))
                up = _rb(_dot(hbb, wu[:, 256 * c:256 * (c + 1)]))
                hid.append((gs * up).astype(BF16))
            if c >= FLAG:
                y = _dot(hid[c - FLAG], wd[256 * (c - FLAG):256 * (c - FLAG + 1), :])
                acc = y if acc is None else acc + y
        ybuf[...] = _rb(acc)
        return gs_

    def ffn_small(idx):
        g0 = pl.multiple_of((idx // 16) * 16, 16)
        hbb = hbbuf[pl.ds(g0, 16), :]

        def body(c, acc):
            f0 = pl.multiple_of(c * 256, 256)
            gpre = _rb(_dot(hbb, wg[:, pl.ds(f0, 256)]))
            gs = _rb(gpre * _rb(jax.nn.sigmoid(gpre)))
            up = _rb(_dot(hbb, wu[:, pl.ds(f0, 256)]))
            return acc + _dot((gs * up).astype(BF16), wd[pl.ds(f0, 256), :])

        ybuf[...] = _rb(jax.lax.fori_loop(0, F // 256, body, jnp.zeros((16, D), F32)))

    def layer_body(layer, carry):
        best[0] = jnp.full((8, 128), -jnp.inf, F32)
        best[1] = jnp.zeros((8, 128), F32)

        def qstep(jj, mem):
            @pl.when((layer == 0) & (jj == 1))
            def _():
                cp_xb.wait()

            @pl.when((layer == 1) & (jj >= 2))
            def _():
                out_copy(pl.multiple_of((jj - 1) * (UNR * R) - W, W), UNR * R).start()

            @pl.when((layer == 1) & (jj == 1))
            def _():
                out_copy(0, UNR * R - W).start()

            ko = None
            for j2 in range(UNR):
                for ts in range(4):
                    last = (jj == NJ - 1) if (j2 == UNR - 1 and ts == 3) else None
                    mem, ko = step(ts, j2 > 0, last, layer, UNR * jj + j2, mem, ko)
            return mem

        jax.lax.fori_loop(0, NJ, qstep, mem0_ref[...].astype(F32))

        @pl.when(layer == 0)
        def _():
            for c in cp_f:
                c.wait()

        @pl.when(layer == 1)
        def _():
            out_copy(S - UNR * R - W, UNR * R).start()

        idx_s, _ = argmax()
        gs_ = ffn(idx_s)
        for k in range(4):
            post(S - W + 16 * k, gate(abuf[W + 16 * k:W + 16 * (k + 1), :], (gs_[k], 0)), True)
        idx, vmax = argmax()

        @pl.when(idx // 16 != idx_s // 16)
        def _():
            ffn_small(idx)

        g0 = pl.multiple_of((idx // 16) * 16, 16)
        rsel = jnp.tile(_rb(jax.nn.sigmoid(vmax)), (1, D // 128))
        y = _rb(ybuf[...] * rsel)
        x2 = _rb(x1buf[pl.ds(g0, 16), :].astype(F32) + _rb(hbbuf[pl.ds(g0, 16), :].astype(F32) + y))
        rowi = jax.lax.broadcasted_iota(jnp.int32, (16, D), 0) + g0

        @pl.when(layer == 1)
        def _():
            out_copy(0, S - W).wait()

        x2 = jnp.where(rowi == idx, x2, xs[pl.ds(g0, 16), :].astype(F32))
        xs[pl.ds(g0, 16), :] = x2.astype(BF16)

        @pl.when((layer == 0) & (idx < FD))
        def _():
            h16 = _ln(x2)
            hbuf[pl.ds(S + g0, 16), :] = h16
            for h in range(H):
                qbig[h, pl.ds(g0, 16), :] = _dot(h16.astype(BF16), _w(wq(h)[...]))

            @pl.when(idx < M)
            def _():
                def body(t, c):
                    kvring[t, 0:M, :] = _dot(h16.astype(BF16), _w(wkv[t]))[:M]
                    return c

                jax.lax.fori_loop(2 * NPAIR, 4 * NPAIR, body, 0, unroll=2)

        @pl.when(layer == 1)
        def _():
            lastc = out_copy(S - W, W)
            lastc.start()

            @pl.when(g0 < S - W)
            def _():
                fix = out_copy(g0, 16, 3)
                fix.start()
                fix.wait()

            lastc.wait()

        return carry

    jax.lax.fori_loop(0, 2, layer_body, 0)


@jax.jit
def pallas_interleave_layers__memory_aug_recurrent_mem_tr__moe_arch_mod__prompt_kernel(
    A_x: jax.Array,
    A_mem0: jax.Array,
    A_Wq: jax.Array,
    A_Wk: jax.Array,
    A_Wv: jax.Array,
    A_Wo: jax.Array,
    A_seg_len: jax.Array,
    B_x: jax.Array,
    B_w_r: jax.Array,
    B_w_gate: jax.Array,
    B_w_up: jax.Array,
    B_w_down: jax.Array,
):
    del A_seg_len, B_x
    assert A_x.shape == (1, S, D) and A_Wq.shape == (D, H, E) and A_mem0.shape == (1, M, D)
    any_spec = pl.BlockSpec(memory_space=pl.ANY)
    out = pl.pallas_call(
        _kernel,
        out_shape=jax.ShapeDtypeStruct((S, D), BF16),
        in_specs=[any_spec] * 10,
        out_specs=any_spec,
        scratch_shapes=[
            pltpu.VMEM((S + SEG, D), BF16),
            pltpu.VMEM((S + SEG, D), BF16),
            pltpu.VMEM((S + SEG, D), BF16),
            pltpu.VMEM((2 * S + SEG, D), F32),
            pltpu.VMEM((P0 // 2, D), U32),
            pltpu.VMEM((12, D, HC, E), BF16),
            pltpu.VMEM((HC, D // 2, E), U32),
            pltpu.VMEM((H - HC, D // 2, E), U32),
            pltpu.VMEM((2 * H, D // 2, E), U32),
            pltpu.VMEM((4, H * E, 128), BF16),
            pltpu.VMEM((4, H * E // 2, 128), U32),
            pltpu.VMEM((D, F), BF16),
            pltpu.VMEM((D, F), BF16),
            pltpu.VMEM((F, D), BF16),
            pltpu.VMEM((H, S, E), F32),
            pltpu.VMEM((2 * H, R, E), F32),
            pltpu.VMEM((H, R, E), F32),
            pltpu.VMEM((R, D), F32),
            pltpu.VMEM((16, D), F32),
            pltpu.VMEM((L2, L2), F32),
            pltpu.VMEM((2, 8, 128), F32),
            pltpu.VMEM((8, 128), jnp.int32),
            pltpu.VMEM((M, D), BF16),
            pltpu.VMEM((D,), BF16),
            pltpu.VMEM((8, D), F32),
            pltpu.SemaphoreType.DMA((33,)),
        ],
        compiler_params=pltpu.CompilerParams(vmem_limit_bytes=110 * 1024 * 1024),
        name="rmt_mod",
    )(A_x.reshape(S, D), A_mem0.reshape(M, D), A_Wq, A_Wk, A_Wv, A_Wo.reshape(H * E, D),
      B_w_r, B_w_gate, B_w_up, B_w_down)
    return out.reshape(1, S, D)
```

```python
import jax
import jax.numpy as jnp
import jax.experimental.pallas as pl
import jax.experimental.pallas.tpu as pltpu

S = 2048
D = 512
H = 32
E = 128
M = 8
SEG = 32
F = 1792
NPAIR = H // 2
NU = S // (2 * SEG)
W = 2 * SEG
L2 = 2 * (M + SEG)
EPS = 1e-05
SCALE = float(E) ** -0.5
LOG2E = 1.4426950408889634
F32 = jnp.float32
BF16 = jnp.bfloat16
U32 = jnp.uint32


def _rb(x):
    return x.astype(BF16).astype(F32)


def _ln(x):
    mu = jnp.sum(x, axis=-1, keepdims=True) * (1.0 / D)
    xc0 = x - mu
    var = jnp.sum(xc0 * xc0, axis=-1, keepdims=True) * (1.0 / D)
    sd = _rb(jnp.sqrt(_rb(_rb(var) + EPS)))
    xc = _rb(x - _rb(mu))
    return _rb(xc * (1.0 / sd))


def _dot(a, b):
    return jnp.dot(a, b, preferred_element_type=F32)


def _w(ref_slab):
    return pltpu.bitcast(ref_slab, BF16)


P0 = S // 2
LR = 24
PLN = P0 + LR
XC = P0 // 4
XLN = P0 + SEG
UNR = 2
NJ = NU // (2 * UNR)
XA = P0 + 4 * UNR * SEG
FD = PLN + LR * 2 * NU - S
R = 4 * SEG
HC = H // 4
PRE_ST = 3
POST_ST = 5
KSPLIT = ((0, 0), (0, 1), (1, 0), (1, 1), (0, 2), (1, 2), (0, 3), (1, 3))
FLAG = 2
O1, O2, NE = 3, 7, 8


def _tok(*vals):
    parts = []
    for v in vals:
        if v.shape[1] < 128:
            v = jnp.broadcast_to(v[:, :1], (v.shape[0], 128))
        for i in range(v.shape[0] // 8):
            for j in range(v.shape[1] // 128):
                parts.append(v[8 * i:8 * i + 8, 128 * j:128 * j + 128])
    while len(parts) > 1:
        parts = [jnp.maximum(parts[i], parts[i + 1]) if i + 1 < len(parts) else parts[i]
                 for i in range(0, len(parts), 2)]
    return parts[0]


def _rslices(row0, n):
    row0 %= R
    if row0 + n <= R:
        return [(row0, row0 + n, 0)]
    return [(row0, R, 0), (0, row0 + n - R, R - row0)]


def _kernel(x_hbm, mem0_hbm, wq_hbm, wk_hbm, wv_hbm, wo_hbm, wr_hbm, wg_hbm, wu_hbm, wd_hbm,
            out_hbm,
            xs, x1buf, hbbuf, hbuf, hpack, raw, wq0, wq1, wkv, wo_raw, wo, wg, wu, wd,
            qbig, kvring, oring, abuf, ybuf, maskv, best, zflag, mem0_ref, wr_ref, wrb, sems):
    def wq(h):
        return wq0.at[h] if h < HC else wq1.at[h - HC]

    def x_copy(row0, n, sem):
        return pltpu.make_async_copy(x_hbm.at[pl.ds(row0, n)], xs.at[pl.ds(row0, n)], sems.at[sem])

    def w_copy(ph, src=None):
        if src is None:
            src = wq_hbm.at[:, pl.ds(0, HC), :]
        return pltpu.make_async_copy(src, raw.at[ph], sems.at[11 + ph])

    cp_x = [x_copy(c * XC, XC, 23 + c) for c in range(4)]
    cp_xa = x_copy(P0, XA - P0, 0)
    cp_q0 = [pltpu.make_async_copy(wq_hbm.at[pl.ds(c * 128, 128), pl.ds(0, HC), :],
                                   raw.at[0, pl.ds(c * 128, 128)], sems.at[29 + c])
             for c in range(4)]
    cp_x[0].start()
    for c in cp_q0 + cp_x[1:]:
        c.start()
    cp_xa.start()
    cp_s = [pltpu.make_async_copy(mem0_hbm, mem0_ref, sems.at[27]),
            pltpu.make_async_copy(wr_hbm, wr_ref, sems.at[28])]
    for c in cp_s:
        c.start()
    for i, w in enumerate((wq_hbm, wk_hbm, wv_hbm)):
        for c in range(4):
            if 4 * i + c > 0:
                w_copy(4 * i + c, w.at[:, pl.ds(c * HC, HC), :]).start()
    cp_wo = [pltpu.make_async_copy(wo_hbm.at[:, pl.ds(n * 128, 128)], wo_raw.at[n], sems.at[4 + n])
             for n in range(4)]
    for c in cp_wo:
        c.start()
    cp_xb = x_copy(XA, S - XA, 1)
    cp_f = [pltpu.make_async_copy(wg_hbm, wg, sems.at[8]),
            pltpu.make_async_copy(wu_hbm, wu, sems.at[9]),
            pltpu.make_async_copy(wd_hbm, wd, sems.at[10])]

    def out_copy(row0, n, sem=2):
        return pltpu.make_async_copy(xs.at[pl.ds(row0, n)], out_hbm.at[pl.ds(row0, n)], sems.at[sem])

    oring[:, R - M:R, :] = jnp.zeros((H, M, E), F32)
    abuf[...] = jnp.zeros(abuf.shape, F32)
    xs[pl.ds(S, SEG), :] = jnp.zeros((SEG, D), BF16)
    hbuf[pl.ds(2 * S, SEG), :] = jnp.zeros((SEG, D), F32)
    zflag[...] = jnp.zeros(zflag.shape, jnp.int32)

    ri = jax.lax.broadcasted_iota(jnp.int32, (L2, L2), 0)
    ci = jax.lax.broadcasted_iota(jnp.int32, (L2, L2), 1)

    def head_of(i):
        return jnp.where(i < 2 * M, i // M, (i - 2 * M) // SEG)

    def pos_of(i):
        return jnp.where(i < 2 * M, i % M, M + (i - 2 * M) % SEG)

    same = head_of(ri) == head_of(ci)
    ok = (pos_of(ri) < M) | (pos_of(ri) >= pos_of(ci))
    maskv[...] = jnp.where(same, jnp.where(ok, 0.0, -1e9 / SCALE), -jnp.inf).astype(F32)

    def gate(v, tk):
        y, r = tk
        ns = min(v.shape[-2], 8)
        tok = pltpu.bitcast(y[r:r + 8], v.dtype)[:ns]
        zf = (zflag[...] != 0)[:ns]
        reps = (v.shape[-2] // ns, v.shape[-1] // 128)
        tok, zf = jnp.tile(tok, reps), jnp.tile(zf, reps)
        return jnp.where(zf, tok, v)

    def toks(ys, n, frac=0.8):
        rows = [(y, r) for y in ys for r in range(0, y.shape[0], 8)]
        return [rows[int(len(rows) * frac * i / n)] for i in range(n)]

    def ln0(r0, tk=None, n=W):
        x = xs[r0:r0 + n, :].astype(F32)
        if tk is not None:
            x = gate(x, tk)
        h = _ln(x)
        hbuf[r0:r0 + n, :] = h
        if r0 < P0:
            hpack[r0 // 2:(r0 + n) // 2, :] = pltpu.bitcast(h.astype(BF16), U32)

    def relay(ph, tks=None, dbs=range(D // 16), is_q=False):
        for db in dbs:
            a = raw[ph, pl.ds(16 * db, 16)]
            if tks is not None:
                a = pltpu.bitcast(gate(pltpu.bitcast(a, U32), tks[db]), BF16)
            a = jnp.swapaxes(a, 0, 1)
            for hh in range(HC):
                v = pltpu.bitcast(a[hh], U32)
                if isinstance(ph, int) and ph == 0:
                    wq0[hh, pl.ds(8 * db, 8), :] = v
                elif is_q:
                    wq1[(ph - 1) * HC + hh, pl.ds(8 * db, 8), :] = v
                else:
                    tb = (ph % 4) * 16 + (ph // 4 - 1) * 2
                    wkv[tb + (hh // 2) * 4 + hh % 2, pl.ds(8 * db, 8), :] = v

    def light(heads, c=None):
        if c is None:
            r0, p0, n = 0, 0, P0
        elif isinstance(c, int):
            r0, p0, n = c * XC, c * (XC // 2), XC
        else:
            r0, p0, n = pl.multiple_of(c * XC, XC), pl.multiple_of(c * (XC // 2), XC // 2), XC
        lhs = _w(hpack[pl.ds(p0, n // 2), :])
        ys = []
        for h in heads:
            y = _dot(lhs, _w(wq(h)[...]))
            qbig[h, pl.ds(r0, n), :] = y
            ys.append(y)
        return ys

    def kv_head(lhs16):
        ys = []
        for t in range(2 * NPAIR, 4 * NPAIR):
            y = _dot(lhs16, _w(wkv[t]))
            kvring[t, 0:M, :] = y[:M]
            ys.append(y)
        return ys

    NG = XC // SEG
    cp_x[0].wait()
    for k in range(NG):
        ln0(k * SEG, None, SEG)
    cp_q0[0].wait()
    relay(0, None, range(8))

    def first_k(k):
        lhs = _w(hpack[0:XC // 2, 128 * k:128 * (k + 1)])
        ys = []
        for h0 in range(0, HC, 4):
            wk = jnp.concatenate([_w(wq0[h0 + i, 64 * k:64 * (k + 1), :]) for i in range(4)], axis=1)
            y = _dot(lhs, wk)
            for i in range(4):
                yi = y[:, 128 * i:128 * (i + 1)]
                qbig[h0 + i, 0:XC, :] = yi if k == 0 else qbig[h0 + i, 0:XC, :] + yi
            ys.append(y[:, :128])
        return ys

    for k in range(3):
        cp_q0[k + 1].wait()
        tks = toks(first_k(k), 8, 0.6)
        relay(0, {8 * (k + 1) + i: tks[i] for i in range(8)}, range(8 * (k + 1), 8 * (k + 2)))
    cp_x[1].wait()
    tks = toks(first_k(3), NG, 0.5)
    for k in range(NG):
        ln0(XC + k * SEG, tks[k], SEG)

    cp_x[2].wait()
    cp_x[3].wait()
    tks = toks(light(range(HC), 1), 2 * NG, 0.85)
    for k in range(2 * NG):
        ln0(2 * XC + k * SEG, tks[k], SEG)

    def phase_a(i, carry):
        w_copy(i).wait()
        relay(i, toks(light(range(HC), i + 1), 32), is_q=True)
        return carry

    jax.lax.fori_loop(1, 3, phase_a, 0)
    w_copy(3).wait()
    cp_xa.wait()
    tks = toks(light(range(HC, HC + 3)), 33)
    relay(3, tks[:32], is_q=True)
    ln0(P0, tks[32], SEG)

    def phase_b(i, carry):
        w_copy(4 + 2 * i).wait()
        w_copy(5 + 2 * i).wait()
        tks = toks(light(range(HC + 3, H), i), 64, 0.9)
        relay(4 + 2 * i, tks[:32])
        relay(5 + 2 * i, tks[32:])
        return carry

    jax.lax.fori_loop(0, 4, phase_b, 0)

    for c in cp_wo + cp_s:
        c.wait()
    wrb[...] = jnp.broadcast_to(wr_ref[...].astype(F32).reshape(1, D), (8, D))
    cp_xb.start()
    for c in cp_f:
        c.start()
    tks = toks(kv_head(_w(hpack[0:8, :])), 32, 0.9)
    for k in range(32):
        n, kk = k // 8, k % 8
        wo[n, pl.ds(256 * kk, 256), :] = gate(
            pltpu.bitcast(wo_raw[n, pl.ds(512 * kk, 512), :], U32), tks[k])

    def post(row0, a, valid):
        n = a.shape[0]
        x1 = _rb(xs[pl.ds(row0, n), :].astype(F32) + _rb(a))
        x1buf[pl.ds(row0, n), :] = x1.astype(BF16)
        hb = _ln(x1)
        hbbuf[pl.ds(row0, n), :] = hb.astype(BF16)
        r = _rb(jnp.sum(hb * jnp.tile(wrb[...], (n // 8, 1)), axis=-1, keepdims=True))
        x2 = x1 + hb
        xs[pl.ds(row0, n), :] = x2.astype(BF16)
        if valid is not True:
            r = jnp.where(valid, r, -jnp.inf)
        bv = best[0]
        bi = best[1]
        sub = jax.lax.broadcasted_iota(jnp.int32, (8, 128), 0).astype(F32)
        for g in range(n // 8):
            rg = jnp.broadcast_to(r[8 * g:8 * g + 8], (8, 128))
            ig = sub + (float(row0 + 8 * g) if isinstance(row0, int) else (row0 + 8 * g).astype(F32))
            gt = rg > bv
            bv = jnp.where(gt, rg, bv)
            bi = jnp.where(gt, ig, bi)
        best[0] = bv
        best[1] = bi
        return _tok(x2, bv, bi)

    def anchor(val, tok):
        return jnp.where(zflag[...] != 0, tok, val)

    def wo_pair(g, half):
        return jnp.concatenate(
            [_w(wo[2 * half + c, pl.ds(g * 128, 128), :]) for c in range(2)], axis=1)

    def rload(buf, t, row0, n):
        return [buf[t, a:b, :] for a, b, _ in _rslices(row0, n)]

    def step(ts, jpos, last, layer, j, mem, korder):
        q, par = ts // 2, ts % 2
        sr = ts * SEG
        if par == 0:
            kvw = ((W * q, 40), (W * q + 8, 24))
            ow = ((W * q - 8, 40), (W * q, 24))
        else:
            kvw = ((W * q + 40, 24), (W * q + 32, 40))
            ow = ((W * q + 32, 24), (W * q + 24, 40))
        sl = 4 * j + ts
        sg = layer * (2 * NU) + sl
        hb0 = pl.multiple_of(layer * S + R * j, R)
        pq0 = pl.multiple_of(P0 + LR * sg, 8)
        lhs = [jnp.concatenate([mem, hbuf[pl.ds(hb0 + r0, n), :]], axis=0).astype(BF16)
               for r0, n in kvw]
        lhsq = jnp.concatenate([mem, hbuf[pl.ds(pq0, LR), :]], axis=0).astype(BF16)
        qrow = [pl.multiple_of((pq0 + 8 * i) % S, 8) for i in range(LR // 8)]
        crow = pl.multiple_of(R * j + sr, SEG)

        def ksplit(ga, gb):
            half = ga // (NPAIR // 2)
            hq = [2 * ga, 2 * ga + 1, 2 * gb, 2 * gb + 1]

            def kv(k):
                wk = jnp.concatenate([_w(wkv[4 * ga + t, pl.ds(64 * k, 64), :])
                                      for t in range(4)], axis=1)
                return jnp.dot(lhs[half][:, 128 * k:128 * (k + 1)], wk, preferred_element_type=F32)

            def qq(k):
                wk = jnp.concatenate([_w(wq(h)[pl.ds(64 * k, 64), :]) for h in hq], axis=1)
                return jnp.dot(lhsq[:, 128 * k:128 * (k + 1)], wk, preferred_element_type=F32)

            pkv = pq = None
            for f, k in KSPLIT:
                y = (kv if f == 0 else qq)(korder[k])
                if f == 0:
                    pkv = y if pkv is None else pkv + y
                else:
                    pq = y if pq is None else pq + y
            done = {("kv", 4 * ga + t): pkv[:, 128 * t:128 * (t + 1)] for t in range(4)}
            if pq is not None:
                done.update({("q", h): pq[:, 128 * i:128 * (i + 1)] for i, h in enumerate(hq)})
            return done

        def qkv(g, done):
            half = g // (NPAIR // 2)
            r0, n = kvw[half]
            res = []
            for c in range(2):
                y = done.get(("q", 2 * g + c))
                if y is None:
                    y = jnp.dot(lhsq, _w(wq(2 * g + c)[...]), preferred_element_type=F32)
                for i in range(LR // 8):
                    qbig[2 * g + c, pl.ds(qrow[i], 8), :] = y[M + 8 * i:M + 8 * i + 8]
                res.append(y[:M])
            for t in range(4):
                y = done.get(("kv", 4 * g + t))
                if y is None:
                    y = jnp.dot(lhs[half], _w(wkv[4 * g + t]), preferred_element_type=F32)
                for a, b, o in _rslices(r0, n):
                    kvring[4 * g + t, a:b, :] = y[M + o:M + o + b - a]
                res.append(y[:M])
            qx = jnp.concatenate([qbig[2 * g + c, pl.ds(crow, SEG), :] for c in range(2)],
                                 axis=0).astype(BF16)
            return res, qx

        def stack(g, mres, i):
            return jnp.concatenate(
                [mres[2 * i], mres[2 * i + 1],
                 kvring[4 * g + 2 * i - 2, sr:sr + SEG, :],
                 kvring[4 * g + 2 * i - 1, sr:sr + SEG, :]], axis=0).astype(BF16)

        def qk(g, mres, qx, prenorm):
            q2 = jnp.concatenate(
                [jnp.concatenate([mres[0], mres[1]], axis=0).astype(BF16), qx], axis=0)
            s = jax.lax.dot_general(q2, stack(g, mres, 1), (((1,), (1,)), ((), ())),
                                    preferred_element_type=F32)
            mk = maskv[...]
            s = jnp.where(mk == 0.0, s, mk)
            mx = jnp.max(s, axis=-1, keepdims=True)
            p = jnp.exp2((s - mx) * (SCALE * LOG2E))
            l = jnp.sum(p, axis=-1, keepdims=True)
            r0 = pl.reciprocal(l, approx=True)
            r = r0 * (2.0 - l * r0)
            if prenorm:
                return (p * r).astype(BF16), None
            return p.astype(BF16), r

        def pv(g, mres, pr):
            p, r = pr
            o = jnp.dot(p, stack(g, mres, 2), preferred_element_type=F32)
            if r is not None:
                o = o * r
            oring[2 * g, sr:sr + SEG, :] = o[2 * M:2 * M + SEG]
            oring[2 * g + 1, sr:sr + SEG, :] = o[2 * M + SEG:]
            return o[:M], o[M:2 * M]

        def olhs(g, om, half):
            r0, n = ow[half]
            if last is not None and half == 0:
                om = [jnp.where(last, oring[2 * g + c, R - M:R, :], om[c]) for c in range(2)]
            return jnp.concatenate(
                [jnp.concatenate([om[c]] + rload(oring, 2 * g + c, r0, n), axis=0)
                 for c in range(2)], axis=1).astype(BF16)

        pn0 = pl.multiple_of(PLN + LR * sg, 8)
        xr = jnp.concatenate(
            [xs[pl.ds(pl.multiple_of((pn0 + 8 * i) % S, 8), 8), :].astype(F32)
             for i in range(LR // 8)], axis=0)
        hpre = _ln(xr)
        hbuf[pl.ds(pn0, LR), :] = hpre
        tok_pre = _tok(hpre)
        if ts >= 2 or jpos:
            valid = True
            row0 = pl.multiple_of(SEG * (sl - 2), SEG)
        else:
            valid = j >= 1
            row0 = pl.multiple_of(jnp.where(valid, SEG * (sl - 2), S), SEG)
        ar = (sr - 2 * SEG) % R
        tok_post = post(row0, abuf[ar:ar + SEG, :], valid)

        NST = NPAIR // 2
        st = [(i, i + NST) if par == 0 else (i + NST, i) for i in range(NST)]
        mres, qxs, prs, oms = {}, {}, {}, {}
        acc = [None] * 4
        order = []
        for i in range(NST):
            order += [("qkv", g) for g in st[i]]
            if i >= 1:
                order += [("qk", g) for g in st[i - 1]]
            if i >= 2:
                order += [("pv", g) for g in st[i - 2]]
        oq = [g for i in range(NST) for g in st[i]]
        order += [("o", g) for g in oq[0:O1]]
        order += [("qk", g) for g in st[NST - 1]] + [("pv", g) for g in st[NST - 2]]
        order += [("o", g) for g in oq[O1:O2]]
        order += [("pv", g) for g in st[NST - 1]]
        order += [("o", g) for g in oq[O2:NE]]
        norder = (2, 3, 0, 1) if par == 0 else (0, 1, 2, 3)
        order += [("on", n) for n in norder]
        done = {} if korder is None else ksplit(*st[0])
        for kind, g in order:
            if kind == "qkv":
                mres[g], qxs[g] = qkv(g, done)
                if g == st[PRE_ST][0]:
                    mres[g][0] = anchor(mres[g][0], tok_pre)
                if g == st[POST_ST][0]:
                    mres[g][0] = anchor(mres[g][0], tok_post)
            elif kind == "qk":
                prs[g] = qk(g, mres[g], qxs[g], g not in st[NST - 1] + st[NST - 2])
            elif kind == "pv":
                oms[g] = pv(g, mres[g], prs[g])
                if prs[g][1] is not None:
                    oms[g] = (anchor(oms[g][0], _tok(prs[g][1][2 * M:])), oms[g][1])
            elif kind == "o":
                for half in range(2):
                    y = jnp.dot(olhs(g, oms[g], half), wo_pair(g, half), preferred_element_type=F32)
                    for c in range(2):
                        yc = y[:, 128 * c:128 * (c + 1)]
                        n = 2 * half + c
                        acc[n] = yc if acc[n] is None else acc[n] + yc
            else:
                n = g
                l = jnp.concatenate([olhs(g2, oms[g2], n // 2) for g2 in oq[NE:]], axis=1)
                wn = jnp.concatenate([_w(wo[n, pl.ds(g2 * 128, 128), :]) for g2 in oq[NE:]], axis=0)
                acc[n] = acc[n] + jnp.dot(l, wn, preferred_element_type=F32)
        for n in range(4):
            r0, nr = ow[n // 2]
            for a, b, o in _rslices(r0, nr):
                abuf[a:b, n * 128:(n + 1) * 128] = acc[n][M + o:M + o + b - a]

        if last is not None:
            for n in range(2):
                abuf[R - M:R, n * 128:(n + 1) * 128] = acc[n][:M]

        return jnp.concatenate([acc[n][:M] for n in range(4)], axis=1), norder

    def argmax():
        bv = best[0]
        bi = best[1]
        vmax = jnp.max(bv, axis=0, keepdims=True)
        imin = jnp.min(jnp.where(bv == vmax, bi, float(S)), axis=0, keepdims=True)
        idx = jnp.clip(imin.astype(jnp.int32)[0, 0], 0, S - 1)
        return idx, vmax

    def ffn(idx):
        g0 = pl.multiple_of((idx // 16) * 16, 16)
        hbb = hbbuf[pl.ds(g0, 16), :]
        nc = F // 256
        hid, acc, gs_ = [], None, []
        for c in range(nc + FLAG):
            if c < nc:
                gpre = _rb(_dot(hbb, wg[:, 256 * c:256 * (c + 1)]))
                gs_.append(gpre[:, :128])
                gs = _rb(gpre * _rb(jax.nn.sigmoid(gpre)))
                up = _rb(_dot(hbb, wu[:, 256 * c:256 * (c + 1)]))
                hid.append((gs * up).astype(BF16))
            if c >= FLAG:
                y = _dot(hid[c - FLAG], wd[256 * (c - FLAG):256 * (c - FLAG + 1), :])
                acc = y if acc is None else acc + y
        ybuf[...] = _rb(acc)
        return gs_

    def ffn_small(idx):
        g0 = pl.multiple_of((idx // 16) * 16, 16)
        hbb = hbbuf[pl.ds(g0, 16), :]

        def body(c, acc):
            f0 = pl.multiple_of(c * 256, 256)
            gpre = _rb(_dot(hbb, wg[:, pl.ds(f0, 256)]))
            gs = _rb(gpre * _rb(jax.nn.sigmoid(gpre)))
            up = _rb(_dot(hbb, wu[:, pl.ds(f0, 256)]))
            return acc + _dot((gs * up).astype(BF16), wd[pl.ds(f0, 256), :])

        ybuf[...] = _rb(jax.lax.fori_loop(0, F // 256, body, jnp.zeros((16, D), F32)))

    def layer_body(layer, carry):
        best[0] = jnp.full((8, 128), -jnp.inf, F32)
        best[1] = jnp.zeros((8, 128), F32)

        def qstep(jj, mem):
            @pl.when((layer == 0) & (jj == 1))
            def _():
                cp_xb.wait()

            @pl.when((layer == 1) & (jj >= 2))
            def _():
                out_copy(pl.multiple_of((jj - 1) * (UNR * R) - W, W), UNR * R).start()

            @pl.when((layer == 1) & (jj == 1))
            def _():
                out_copy(0, UNR * R - W).start()

            ko = None
            for j2 in range(UNR):
                for ts in range(4):
                    last = (jj == NJ - 1) if (j2 == UNR - 1 and ts == 3) else None
                    mem, ko = step(ts, j2 > 0, last, layer, UNR * jj + j2, mem, ko)
            return mem

        jax.lax.fori_loop(0, NJ, qstep, mem0_ref[...].astype(F32))

        @pl.when(layer == 0)
        def _():
            for c in cp_f:
                c.wait()

        @pl.when(layer == 1)
        def _():
            out_copy(S - UNR * R - W, UNR * R).start()

        idx_s, _ = argmax()
        gs_ = ffn(idx_s)
        for k in range(4):
            post(S - W + 16 * k, gate(abuf[W + 16 * k:W + 16 * (k + 1), :], (gs_[k], 0)), True)
        idx, vmax = argmax()

        @pl.when(idx // 16 != idx_s // 16)
        def _():
            ffn_small(idx)

        g0 = pl.multiple_of((idx // 16) * 16, 16)
        rsel = jnp.tile(_rb(jax.nn.sigmoid(vmax)), (1, D // 128))
        y = _rb(ybuf[...] * rsel)
        x2 = _rb(x1buf[pl.ds(g0, 16), :].astype(F32) + _rb(hbbuf[pl.ds(g0, 16), :].astype(F32) + y))
        rowi = jax.lax.broadcasted_iota(jnp.int32, (16, D), 0) + g0

        @pl.when(layer == 1)
        def _():
            out_copy(0, S - W).wait()

        x2 = jnp.where(rowi == idx, x2, xs[pl.ds(g0, 16), :].astype(F32))
        xs[pl.ds(g0, 16), :] = x2.astype(BF16)

        @pl.when((layer == 0) & (idx < FD))
        def _():
            h16 = _ln(x2)
            hbuf[pl.ds(S + g0, 16), :] = h16
            for h in range(H):
                qbig[h, pl.ds(g0, 16), :] = _dot(h16.astype(BF16), _w(wq(h)[...]))

            @pl.when(idx < M)
            def _():
                def body(t, c):
                    kvring[t, 0:M, :] = _dot(h16.astype(BF16), _w(wkv[t]))[:M]
                    return c

                jax.lax.fori_loop(2 * NPAIR, 4 * NPAIR, body, 0, unroll=2)

        @pl.when(layer == 1)
        def _():
            lastc = out_copy(S - W, W)
            lastc.start()

            @pl.when(g0 < S - W)
            def _():
                fix = out_copy(g0, 16, 3)
                fix.start()
                fix.wait()

            lastc.wait()

        return carry

    jax.lax.fori_loop(0, 2, layer_body, 0)


@jax.jit
def pallas_interleave_layers__memory_aug_recurrent_mem_tr__moe_arch_mod__prompt_kernel(
    A_x: jax.Array,
    A_mem0: jax.Array,
    A_Wq: jax.Array,
    A_Wk: jax.Array,
    A_Wv: jax.Array,
    A_Wo: jax.Array,
    A_seg_len: jax.Array,
    B_x: jax.Array,
    B_w_r: jax.Array,
    B_w_gate: jax.Array,
    B_w_up: jax.Array,
    B_w_down: jax.Array,
):
    del A_seg_len, B_x
    assert A_x.shape == (1, S, D) and A_Wq.shape == (D, H, E) and A_mem0.shape == (1, M, D)
    any_spec = pl.BlockSpec(memory_space=pl.ANY)
    out = pl.pallas_call(
        _kernel,
        out_shape=jax.ShapeDtypeStruct((S, D), BF16),
        in_specs=[any_spec] * 10,
        out_specs=any_spec,
        scratch_shapes=[
            pltpu.VMEM((S + SEG, D), BF16),
            pltpu.VMEM((S + SEG, D), BF16),
            pltpu.VMEM((S + SEG, D), BF16),
            pltpu.VMEM((2 * S + SEG, D), F32),
            pltpu.VMEM((P0 // 2, D), U32),
            pltpu.VMEM((12, D, HC, E), BF16),
            pltpu.VMEM((HC, D // 2, E), U32),
            pltpu.VMEM((H - HC, D // 2, E), U32),
            pltpu.VMEM((2 * H, D // 2, E), U32),
            pltpu.VMEM((4, H * E, 128), BF16),
            pltpu.VMEM((4, H * E // 2, 128), U32),
            pltpu.VMEM((D, F), BF16),
            pltpu.VMEM((D, F), BF16),
            pltpu.VMEM((F, D), BF16),
            pltpu.VMEM((H, S, E), F32),
            pltpu.VMEM((2 * H, R, E), F32),
            pltpu.VMEM((H, R, E), F32),
            pltpu.VMEM((R, D), F32),
            pltpu.VMEM((16, D), F32),
            pltpu.VMEM((L2, L2), F32),
            pltpu.VMEM((2, 8, 128), F32),
            pltpu.VMEM((8, 128), jnp.int32),
            pltpu.VMEM((M, D), BF16),
            pltpu.VMEM((D,), BF16),
            pltpu.VMEM((8, D), F32),
            pltpu.SemaphoreType.DMA((33,)),
        ],
        compiler_params=pltpu.CompilerParams(vmem_limit_bytes=110 * 1024 * 1024),
        name="rmt_mod",
    )(A_x.reshape(S, D), A_mem0.reshape(M, D), A_Wq, A_Wk, A_Wv, A_Wo.reshape(H * E, D),
      B_w_r, B_w_gate, B_w_up, B_w_down)
    return out.reshape(1, S, D)
```

```python
import jax
import jax.numpy as jnp
import jax.experimental.pallas as pl
import jax.experimental.pallas.tpu as pltpu

S = 2048
D = 512
H = 32
E = 128
M = 8
SEG = 32
F = 1792
NPAIR = H // 2
NU = S // (2 * SEG)
W = 2 * SEG
L2 = 2 * (M + SEG)
EPS = 1.0013580322265625e-05
SCALE = 0.08837890625
LOG2E = 1.4426950408889634
F32 = jnp.float32
BF16 = jnp.bfloat16
U32 = jnp.uint32


def _rb(x):
    return x.astype(BF16).astype(F32)


def _ln(x):
    mu = jnp.sum(x, axis=-1, keepdims=True) * (1.0 / D)
    xc0 = x - mu
    var = jnp.sum(xc0 * xc0, axis=-1, keepdims=True) * (1.0 / D)
    sd = _rb(jnp.sqrt(_rb(_rb(var) + EPS)))
    xc = _rb(x - _rb(mu))
    return _rb(xc * (1.0 / sd))


def _dot(a, b):
    return jnp.dot(a, b, preferred_element_type=F32)


def _w(ref_slab):
    return pltpu.bitcast(ref_slab, BF16)


P0 = S // 2
LR = 24
PLN = P0 + LR
XC = P0 // 4
XLN = P0 + SEG
UNR = 2
NJ = NU // (2 * UNR)
XA = P0 + 4 * UNR * SEG
FD = PLN + LR * 2 * NU - S
R = 4 * SEG
HC = H // 4
PRE_ST = 3
POST_ST = 5
KSPLIT = ((0, 0), (0, 1), (1, 0), (1, 1), (0, 2), (1, 2), (0, 3), (1, 3))
NB4 = 4
NLF = 2
FLAG = 2
O1, O2, NE = 3, 7, 8


def _tok(*vals):
    parts = []
    for v in vals:
        if v.shape[1] < 128:
            v = jnp.broadcast_to(v[:, :1], (v.shape[0], 128))
        for i in range(v.shape[0] // 8):
            for j in range(v.shape[1] // 128):
                parts.append(v[8 * i:8 * i + 8, 128 * j:128 * j + 128])
    while len(parts) > 1:
        parts = [jnp.maximum(parts[i], parts[i + 1]) if i + 1 < len(parts) else parts[i]
                 for i in range(0, len(parts), 2)]
    return parts[0]


def _rslices(row0, n):
    row0 %= R
    if row0 + n <= R:
        return [(row0, row0 + n, 0)]
    return [(row0, R, 0), (0, row0 + n - R, R - row0)]


def _kernel(x_hbm, mem0_hbm, wq_hbm, wk_hbm, wv_hbm, wo_hbm, wr_hbm, wg_hbm, wu_hbm, wd_hbm,
            out_hbm,
            xs, x1buf, hbbuf, hbuf, hpack, raw, wq0, wq1, wkv, wo_raw, wo, wg, wu, wd,
            qbig, kvring, oring, abuf, ybuf, maskv, best, zflag, mem0_ref, wr_ref, wrb, sems):
    def wq(h):
        return wq0.at[h] if h < HC else wq1.at[h - HC]

    def x_copy(row0, n, sem):
        return pltpu.make_async_copy(x_hbm.at[pl.ds(row0, n)], xs.at[pl.ds(row0, n)], sems.at[sem])

    def w_copy(ph, src=None):
        if src is None:
            src = wq_hbm.at[:, pl.ds(0, HC), :]
        return pltpu.make_async_copy(src, raw.at[ph], sems.at[11 + ph])

    cp_x = [x_copy(c * XC, XC, 23 + c) for c in range(4)]
    cp_xa = x_copy(P0, XA - P0, 0)
    cp_q0 = [pltpu.make_async_copy(wq_hbm.at[pl.ds(c * 128, 128), pl.ds(0, HC), :],
                                   raw.at[0, pl.ds(c * 128, 128)], sems.at[29 + c])
             for c in range(4)]
    cp_x[0].start()
    for c in cp_q0 + cp_x[1:]:
        c.start()
    cp_xa.start()
    cp_s = [pltpu.make_async_copy(mem0_hbm, mem0_ref, sems.at[27]),
            pltpu.make_async_copy(wr_hbm, wr_ref, sems.at[28])]
    for c in cp_s:
        c.start()
    for i, w in enumerate((wq_hbm, wk_hbm, wv_hbm)):
        for c in range(4):
            if 4 * i + c > 0:
                w_copy(4 * i + c, w.at[:, pl.ds(c * HC, HC), :]).start()
    cp_wo = [pltpu.make_async_copy(wo_hbm.at[:, pl.ds(n * 128, 128)], wo_raw.at[n], sems.at[4 + n])
             for n in range(4)]
    for c in cp_wo:
        c.start()
    cp_xb = x_copy(XA, S - XA, 1)
    cp_f = [pltpu.make_async_copy(wg_hbm, wg, sems.at[8]),
            pltpu.make_async_copy(wu_hbm, wu, sems.at[9]),
            pltpu.make_async_copy(wd_hbm, wd, sems.at[10])]

    def out_copy(row0, n, sem=2):
        return pltpu.make_async_copy(xs.at[pl.ds(row0, n)], out_hbm.at[pl.ds(row0, n)], sems.at[sem])

    oring[:, R - M:R, :] = jnp.zeros((H, M, E), F32)
    abuf[...] = jnp.zeros(abuf.shape, F32)
    xs[pl.ds(S, SEG), :] = jnp.zeros((SEG, D), BF16)
    hbuf[pl.ds(2 * S, SEG), :] = jnp.zeros((SEG, D), F32)
    zflag[...] = jnp.zeros(zflag.shape, jnp.int32)

    ri = jax.lax.broadcasted_iota(jnp.int32, (L2, L2), 0)
    ci = jax.lax.broadcasted_iota(jnp.int32, (L2, L2), 1)

    def head_of(i):
        return jnp.where(i < 2 * M, i // M, (i - 2 * M) // SEG)

    def pos_of(i):
        return jnp.where(i < 2 * M, i % M, M + (i - 2 * M) % SEG)

    same = head_of(ri) == head_of(ci)
    ok = (pos_of(ri) < M) | (pos_of(ri) >= pos_of(ci))
    maskv[...] = jnp.where(same, jnp.where(ok, 0.0, -1e9 / SCALE), -jnp.inf).astype(F32)

    def gate(v, tk):
        y, r = tk
        ns = min(v.shape[-2], 8)
        tok = pltpu.bitcast(y[r:r + 8], v.dtype)[:ns]
        zf = (zflag[...] != 0)[:ns]
        reps = (v.shape[-2] // ns, v.shape[-1] // 128)
        tok, zf = jnp.tile(tok, reps), jnp.tile(zf, reps)
        return jnp.where(zf, tok, v)

    def toks(ys, n, frac=0.8):
        rows = [(y, r) for y in ys for r in range(0, y.shape[0], 8)]
        return [rows[int(len(rows) * frac * i / n)] for i in range(n)]

    def ln0(r0, tk=None, n=W):
        x = xs[r0:r0 + n, :].astype(F32)
        if tk is not None:
            x = gate(x, tk)
        h = _ln(x)
        hbuf[r0:r0 + n, :] = h
        if r0 < P0:
            hpack[r0 // 2:(r0 + n) // 2, :] = pltpu.bitcast(h.astype(BF16), U32)

    def relay(ph, tks=None, dbs=range(D // 16), is_q=False):
        for db in dbs:
            a = raw[ph, pl.ds(16 * db, 16)]
            if tks is not None:
                a = pltpu.bitcast(gate(pltpu.bitcast(a, U32), tks[db]), BF16)
            a = jnp.swapaxes(a, 0, 1)
            for hh in range(HC):
                v = pltpu.bitcast(a[hh], U32)
                if isinstance(ph, int) and ph == 0:
                    wq0[hh, pl.ds(8 * db, 8), :] = v
                elif is_q:
                    wq1[(ph - 1) * HC + hh, pl.ds(8 * db, 8), :] = v
                else:
                    tb = (ph % 4) * 16 + (ph // 4 - 1) * 2
                    wkv[tb + (hh // 2) * 4 + hh % 2, pl.ds(8 * db, 8), :] = v

    def light(heads, c=None):
        if c is None:
            r0, p0, n = 0, 0, P0
        elif isinstance(c, int):
            r0, p0, n = c * XC, c * (XC // 2), XC
        else:
            r0, p0, n = pl.multiple_of(c * XC, XC), pl.multiple_of(c * (XC // 2), XC // 2), XC
        lhs = _w(hpack[pl.ds(p0, n // 2), :])
        ys = []
        for h in heads:
            y = _dot(lhs, _w(wq(h)[...]))
            qbig[h, pl.ds(r0, n), :] = y
            ys.append(y)
        return ys

    NG = XC // SEG
    cp_x[0].wait()
    for k in range(NG):
        ln0(k * SEG, None, SEG)
    cp_q0[0].wait()
    relay(0, None, range(8))

    def first_k(k):
        lhs = _w(hpack[0:XC // 2, 128 * k:128 * (k + 1)])
        ys = []
        for h0 in range(0, HC, 4):
            wk = jnp.concatenate([_w(wq0[h0 + i, 64 * k:64 * (k + 1), :]) for i in range(4)], axis=1)
            y = _dot(lhs, wk)
            for i in range(4):
                yi = y[:, 128 * i:128 * (i + 1)]
                qbig[h0 + i, 0:XC, :] = yi if k == 0 else qbig[h0 + i, 0:XC, :] + yi
            ys.append(y[:, :128])
        return ys

    for k in range(3):
        cp_q0[k + 1].wait()
        tks = toks(first_k(k), 8, 0.6)
        relay(0, {8 * (k + 1) + i: tks[i] for i in range(8)}, range(8 * (k + 1), 8 * (k + 2)))
    cp_x[1].wait()
    tks = toks(first_k(3), NG, 0.5)
    for k in range(NG):
        ln0(XC + k * SEG, tks[k], SEG)

    cp_x[2].wait()
    cp_x[3].wait()
    tks = toks(light(range(HC), 1), 2 * NG, 0.85)
    for k in range(2 * NG):
        ln0(2 * XC + k * SEG, tks[k], SEG)

    def phase_a(i, carry):
        w_copy(i).wait()
        relay(i, toks(light(range(HC), i + 1), 32), is_q=True)
        return carry

    jax.lax.fori_loop(1, 3, phase_a, 0)
    w_copy(3).wait()
    cp_xa.wait()
    tks = toks(light(range(HC, HC + NB4)), 33)
    relay(3, tks[:32], is_q=True)
    ln0(P0, tks[32], SEG)

    def phase_b(i, carry):
        w_copy(4 + 2 * i).wait()
        w_copy(5 + 2 * i).wait()
        tks = toks(light(range(HC + NB4, H - NLF), i), 64, 0.9)
        relay(4 + 2 * i, tks[:32])
        relay(5 + 2 * i, tks[32:])
        return carry

    jax.lax.fori_loop(0, 4, phase_b, 0)

    for c in cp_wo[:3] + cp_s:
        c.wait()
    wrb[...] = jnp.broadcast_to(wr_ref[...].astype(F32).reshape(1, D), (8, D))
    cp_xb.start()
    for c in cp_f:
        c.start()
    ys = []
    nch = 8 * NLF
    for k in range(nch):
        h, r0 = H - NLF + k // 8, (k % 8) * (P0 // 8)
        y = _dot(_w(hpack[r0 // 2:r0 // 2 + P0 // 16, :]), _w(wq(h)[...]))
        qbig[h, r0:r0 + P0 // 8, :] = y
        ys.append(y)
        for t in range(2 * NPAIR + 2 * NPAIR * k // nch, 2 * NPAIR + 2 * NPAIR * (k + 1) // nch):
            kvring[t, 0:M, :] = _dot(_w(hpack[0:8, :]), _w(wkv[t]))[:M]
    tks = toks(ys, 24, 0.85)
    for k in range(24):
        n, kk = k // 8, k % 8
        wo[n, pl.ds(256 * kk, 256), :] = gate(
            pltpu.bitcast(wo_raw[n, pl.ds(512 * kk, 512), :], U32), tks[k])
    cp_wo[3].wait()
    wo[3] = pltpu.bitcast(wo_raw[3], U32)

    def post(row0, a, valid):
        n = a.shape[0]
        x1 = _rb(xs[pl.ds(row0, n), :].astype(F32) + _rb(a))
        x1buf[pl.ds(row0, n), :] = x1.astype(BF16)
        hb = _ln(x1)
        hbbuf[pl.ds(row0, n), :] = hb.astype(BF16)
        r = _rb(jnp.sum(hb * jnp.tile(wrb[...], (n // 8, 1)), axis=-1, keepdims=True))
        x2 = x1 + hb
        xs[pl.ds(row0, n), :] = x2.astype(BF16)
        if valid is not True:
            r = jnp.where(valid, r, -jnp.inf)
        bv = best[0]
        bi = best[1]
        sub = jax.lax.broadcasted_iota(jnp.int32, (8, 128), 0).astype(F32)
        for g in range(n // 8):
            rg = jnp.broadcast_to(r[8 * g:8 * g + 8], (8, 128))
            ig = sub + (float(row0 + 8 * g) if isinstance(row0, int) else (row0 + 8 * g).astype(F32))
            gt = rg > bv
            bv = jnp.where(gt, rg, bv)
            bi = jnp.where(gt, ig, bi)
        best[0] = bv
        best[1] = bi
        return _tok(x2, bv, bi)

    def anchor(val, tok):
        return jnp.where(zflag[...] != 0, tok, val)

    def wo_pair(g, half):
        return jnp.concatenate(
            [_w(wo[2 * half + c, pl.ds(g * 128, 128), :]) for c in range(2)], axis=1)

    def rload(buf, t, row0, n):
        return [buf[t, a:b, :] for a, b, _ in _rslices(row0, n)]

    def step(ts, jpos, last, layer, j, mem, korder):
        q, par = ts // 2, ts % 2
        sr = ts * SEG
        if par == 0:
            kvw = ((W * q, 40), (W * q + 8, 24))
            ow = ((W * q - 8, 40), (W * q, 24))
        else:
            kvw = ((W * q + 40, 24), (W * q + 32, 40))
            ow = ((W * q + 32, 24), (W * q + 24, 40))
        sl = 4 * j + ts
        sg = layer * (2 * NU) + sl
        hb0 = pl.multiple_of(layer * S + R * j, R)
        pq0 = pl.multiple_of(P0 + LR * sg, 8)
        lhs = [jnp.concatenate([mem, hbuf[pl.ds(hb0 + r0, n), :]], axis=0).astype(BF16)
               for r0, n in kvw]
        lhsq = jnp.concatenate([mem, hbuf[pl.ds(pq0, LR), :]], axis=0).astype(BF16)
        qrow = [pl.multiple_of((pq0 + 8 * i) % S, 8) for i in range(LR // 8)]
        crow = pl.multiple_of(R * j + sr, SEG)

        def ksplit(ga, gb):
            half = ga // (NPAIR // 2)
            hq = [2 * ga, 2 * ga + 1, 2 * gb, 2 * gb + 1]

            def kv(k):
                wk = jnp.concatenate([_w(wkv[4 * ga + t, pl.ds(64 * k, 64), :])
                                      for t in range(4)], axis=1)
                return jnp.dot(lhs[half][:, 128 * k:128 * (k + 1)], wk, preferred_element_type=F32)

            def qq(k):
                wk = jnp.concatenate([_w(wq(h)[pl.ds(64 * k, 64), :]) for h in hq], axis=1)
                return jnp.dot(lhsq[:, 128 * k:128 * (k + 1)], wk, preferred_element_type=F32)

            pkv = pq = None
            for f, k in KSPLIT:
                y = (kv if f == 0 else qq)(korder[k])
                if f == 0:
                    pkv = y if pkv is None else pkv + y
                else:
                    pq = y if pq is None else pq + y
            done = {("kv", 4 * ga + t): pkv[:, 128 * t:128 * (t + 1)] for t in range(4)}
            if pq is not None:
                done.update({("q", h): pq[:, 128 * i:128 * (i + 1)] for i, h in enumerate(hq)})
            return done

        def qkv(g, done):
            half = g // (NPAIR // 2)
            r0, n = kvw[half]
            res = []
            for c in range(2):
                y = done.get(("q", 2 * g + c))
                if y is None:
                    y = jnp.dot(lhsq, _w(wq(2 * g + c)[...]), preferred_element_type=F32)
                for i in range(LR // 8):
                    qbig[2 * g + c, pl.ds(qrow[i], 8), :] = y[M + 8 * i:M + 8 * i + 8]
                res.append(y[:M])
            for t in range(4):
                y = done.get(("kv", 4 * g + t))
                if y is None:
                    y = jnp.dot(lhs[half], _w(wkv[4 * g + t]), preferred_element_type=F32)
                for a, b, o in _rslices(r0, n):
                    kvring[4 * g + t, a:b, :] = y[M + o:M + o + b - a]
                res.append(y[:M])
            qx = jnp.concatenate([qbig[2 * g + c, pl.ds(crow, SEG), :] for c in range(2)],
                                 axis=0).astype(BF16)
            return res, qx

        def stack(g, mres, i):
            return jnp.concatenate(
                [mres[2 * i], mres[2 * i + 1],
                 kvring[4 * g + 2 * i - 2, sr:sr + SEG, :],
                 kvring[4 * g + 2 * i - 1, sr:sr + SEG, :]], axis=0).astype(BF16)

        def qk(g, mres, qx, prenorm):
            q2 = jnp.concatenate(
                [jnp.concatenate([mres[0], mres[1]], axis=0).astype(BF16), qx], axis=0)
            s = jax.lax.dot_general(q2, stack(g, mres, 1), (((1,), (1,)), ((), ())),
                                    preferred_element_type=F32)
            mk = maskv[...]
            s = jnp.where(mk == 0.0, s, mk)
            mx = jnp.max(s, axis=-1, keepdims=True)
            p = jnp.exp2((s - mx) * (SCALE * LOG2E))
            l = jnp.sum(p, axis=-1, keepdims=True)
            r0 = pl.reciprocal(l, approx=True)
            r = r0 * (2.0 - l * r0)
            if prenorm:
                return (p * r).astype(BF16), None
            return p.astype(BF16), r

        def pv(g, mres, pr):
            p, r = pr
            o = jnp.dot(p, stack(g, mres, 2), preferred_element_type=F32)
            if r is not None:
                o = o * r
            oring[2 * g, sr:sr + SEG, :] = o[2 * M:2 * M + SEG]
            oring[2 * g + 1, sr:sr + SEG, :] = o[2 * M + SEG:]
            return o[:M], o[M:2 * M]

        def olhs(g, om, half):
            r0, n = ow[half]
            if last is not None and half == 0:
                om = [jnp.where(last, oring[2 * g + c, R - M:R, :], om[c]) for c in range(2)]
            return jnp.concatenate(
                [jnp.concatenate([om[c]] + rload(oring, 2 * g + c, r0, n), axis=0)
                 for c in range(2)], axis=1).astype(BF16)

        pn0 = pl.multiple_of(PLN + LR * sg, 8)
        xr = jnp.concatenate(
            [xs[pl.ds(pl.multiple_of((pn0 + 8 * i) % S, 8), 8), :].astype(F32)
             for i in range(LR // 8)], axis=0)
        hpre = _ln(xr)
        hbuf[pl.ds(pn0, LR), :] = hpre
        tok_pre = _tok(hpre)
        if ts >= 2 or jpos:
            valid = True
            row0 = pl.multiple_of(SEG * (sl - 2), SEG)
        else:
            valid = j >= 1
            row0 = pl.multiple_of(jnp.where(valid, SEG * (sl - 2), S), SEG)
        ar = (sr - 2 * SEG) % R
        tok_post = post(row0, abuf[ar:ar + SEG, :], valid)

        NST = NPAIR // 2
        st = [(i, i + NST) if par == 0 else (i + NST, i) for i in range(NST)]
        mres, qxs, prs, oms = {}, {}, {}, {}
        acc = [None] * 4
        order = []
        for i in range(NST):
            order += [("qkv", g) for g in st[i]]
            if i >= 1:
                order += [("qk", g) for g in st[i - 1]]
            if i >= 2:
                order += [("pv", g) for g in st[i - 2]]
        oq = [g for i in range(NST) for g in st[i]]
        order += [("o", g) for g in oq[0:O1]]
        order += [("qk", g) for g in st[NST - 1]] + [("pv", g) for g in st[NST - 2]]
        order += [("o", g) for g in oq[O1:O2]]
        order += [("pv", g) for g in st[NST - 1]]
        order += [("o", g) for g in oq[O2:NE]]
        norder = (2, 3, 0, 1) if par == 0 else (0, 1, 2, 3)
        order += [("on", n) for n in norder]
        done = {} if korder is None else ksplit(*st[0])
        for kind, g in order:
            if kind == "qkv":
                mres[g], qxs[g] = qkv(g, done)
                if g == st[PRE_ST][0]:
                    mres[g][0] = anchor(mres[g][0], tok_pre)
                if g == st[POST_ST][0]:
                    mres[g][0] = anchor(mres[g][0], tok_post)
            elif kind == "qk":
                prs[g] = qk(g, mres[g], qxs[g], g not in st[NST - 1] + st[NST - 2])
            elif kind == "pv":
                oms[g] = pv(g, mres[g], prs[g])
                if prs[g][1] is not None:
                    oms[g] = (anchor(oms[g][0], _tok(prs[g][1][2 * M:])), oms[g][1])
            elif kind == "o":
                for half in range(2):
                    y = jnp.dot(olhs(g, oms[g], half), wo_pair(g, half), preferred_element_type=F32)
                    for c in range(2):
                        yc = y[:, 128 * c:128 * (c + 1)]
                        n = 2 * half + c
                        acc[n] = yc if acc[n] is None else acc[n] + yc
            else:
                n = g
                l = jnp.concatenate([olhs(g2, oms[g2], n // 2) for g2 in oq[NE:]], axis=1)
                wn = jnp.concatenate([_w(wo[n, pl.ds(g2 * 128, 128), :]) for g2 in oq[NE:]], axis=0)
                acc[n] = acc[n] + jnp.dot(l, wn, preferred_element_type=F32)
        for n in range(4):
            r0, nr = ow[n // 2]
            for a, b, o in _rslices(r0, nr):
                abuf[a:b, n * 128:(n + 1) * 128] = acc[n][M + o:M + o + b - a]

        if last is not None:
            for n in range(2):
                abuf[R - M:R, n * 128:(n + 1) * 128] = acc[n][:M]

        return jnp.concatenate([acc[n][:M] for n in range(4)], axis=1), norder

    def argmax():
        bv = best[0]
        bi = best[1]
        vmax = jnp.max(bv, axis=0, keepdims=True)
        imin = jnp.min(jnp.where(bv == vmax, bi, float(S)), axis=0, keepdims=True)
        idx = jnp.clip(imin.astype(jnp.int32)[0, 0], 0, S - 1)
        return idx, vmax

    def ffn(idx):
        g0 = pl.multiple_of((idx // 16) * 16, 16)
        hbb = hbbuf[pl.ds(g0, 16), :]
        nc = F // 256
        hid, acc, gs_ = [], None, []
        for c in range(nc + FLAG):
            if c < nc:
                gpre = _rb(_dot(hbb, wg[:, 256 * c:256 * (c + 1)]))
                gs_.append(gpre[:, :128])
                gs = _rb(gpre * _rb(jax.nn.sigmoid(gpre)))
                up = _rb(_dot(hbb, wu[:, 256 * c:256 * (c + 1)]))
                hid.append((gs * up).astype(BF16))
            if c >= FLAG:
                y = _dot(hid[c - FLAG], wd[256 * (c - FLAG):256 * (c - FLAG + 1), :])
                acc = y if acc is None else acc + y
        ybuf[...] = _rb(acc)
        return gs_

    def ffn_small(idx):
        g0 = pl.multiple_of((idx // 16) * 16, 16)
        hbb = hbbuf[pl.ds(g0, 16), :]

        def body(c, acc):
            f0 = pl.multiple_of(c * 256, 256)
            gpre = _rb(_dot(hbb, wg[:, pl.ds(f0, 256)]))
            gs = _rb(gpre * _rb(jax.nn.sigmoid(gpre)))
            up = _rb(_dot(hbb, wu[:, pl.ds(f0, 256)]))
            return acc + _dot((gs * up).astype(BF16), wd[pl.ds(f0, 256), :])

        ybuf[...] = _rb(jax.lax.fori_loop(0, F // 256, body, jnp.zeros((16, D), F32)))

    def layer_body(layer, carry):
        best[0] = jnp.full((8, 128), -jnp.inf, F32)
        best[1] = jnp.zeros((8, 128), F32)

        def qstep(jj, mem):
            @pl.when((layer == 0) & (jj == 1))
            def _():
                cp_xb.wait()

            @pl.when((layer == 1) & (jj >= 2))
            def _():
                out_copy(pl.multiple_of((jj - 1) * (UNR * R) - W, W), UNR * R).start()

            @pl.when((layer == 1) & (jj == 1))
            def _():
                out_copy(0, UNR * R - W).start()

            ko = None
            for j2 in range(UNR):
                for ts in range(4):
                    last = (jj == NJ - 1) if (j2 == UNR - 1 and ts == 3) else None
                    mem, ko = step(ts, j2 > 0, last, layer, UNR * jj + j2, mem, ko)
            return mem

        jax.lax.fori_loop(0, NJ, qstep, mem0_ref[...].astype(F32))

        @pl.when(layer == 0)
        def _():
            for c in cp_f:
                c.wait()

        @pl.when(layer == 1)
        def _():
            out_copy(S - UNR * R - W, UNR * R).start()

        idx_s, _ = argmax()
        gs_ = ffn(idx_s)
        for k in range(4):
            post(S - W + 16 * k, gate(abuf[W + 16 * k:W + 16 * (k + 1), :], (gs_[k], 0)), True)
        idx, vmax = argmax()

        @pl.when(idx // 16 != idx_s // 16)
        def _():
            ffn_small(idx)

        g0 = pl.multiple_of((idx // 16) * 16, 16)
        rsel = jnp.tile(_rb(jax.nn.sigmoid(vmax)), (1, D // 128))
        y = _rb(ybuf[...] * rsel)
        x2 = _rb(x1buf[pl.ds(g0, 16), :].astype(F32) + _rb(hbbuf[pl.ds(g0, 16), :].astype(F32) + y))
        rowi = jax.lax.broadcasted_iota(jnp.int32, (16, D), 0) + g0

        @pl.when(layer == 1)
        def _():
            out_copy(0, S - W).wait()

        x2 = jnp.where(rowi == idx, x2, xs[pl.ds(g0, 16), :].astype(F32))
        xs[pl.ds(g0, 16), :] = x2.astype(BF16)

        @pl.when((layer == 0) & (idx < FD))
        def _():
            h16 = _ln(x2)
            hbuf[pl.ds(S + g0, 16), :] = h16
            for h in range(H):
                qbig[h, pl.ds(g0, 16), :] = _dot(h16.astype(BF16), _w(wq(h)[...]))

            @pl.when(idx < M)
            def _():
                def body(t, c):
                    kvring[t, 0:M, :] = _dot(h16.astype(BF16), _w(wkv[t]))[:M]
                    return c

                jax.lax.fori_loop(2 * NPAIR, 4 * NPAIR, body, 0, unroll=2)

        @pl.when(layer == 1)
        def _():
            lastc = out_copy(S - W, W)
            lastc.start()

            @pl.when(g0 < S - W)
            def _():
                fix = out_copy(g0, 16, 3)
                fix.start()
                fix.wait()

            lastc.wait()

        return carry

    jax.lax.fori_loop(0, 2, layer_body, 0)


@jax.jit
def pallas_interleave_layers__memory_aug_recurrent_mem_tr__moe_arch_mod__prompt_kernel(
    A_x: jax.Array,
    A_mem0: jax.Array,
    A_Wq: jax.Array,
    A_Wk: jax.Array,
    A_Wv: jax.Array,
    A_Wo: jax.Array,
    A_seg_len: jax.Array,
    B_x: jax.Array,
    B_w_r: jax.Array,
    B_w_gate: jax.Array,
    B_w_up: jax.Array,
    B_w_down: jax.Array,
):
    del A_seg_len, B_x
    assert A_x.shape == (1, S, D) and A_Wq.shape == (D, H, E) and A_mem0.shape == (1, M, D)
    any_spec = pl.BlockSpec(memory_space=pl.ANY)
    out = pl.pallas_call(
        _kernel,
        out_shape=jax.ShapeDtypeStruct((S, D), BF16),
        in_specs=[any_spec] * 10,
        out_specs=any_spec,
        scratch_shapes=[
            pltpu.VMEM((S + SEG, D), BF16),
            pltpu.VMEM((S + SEG, D), BF16),
            pltpu.VMEM((S + SEG, D), BF16),
            pltpu.VMEM((2 * S + SEG, D), F32),
            pltpu.VMEM((P0 // 2, D), U32),
            pltpu.VMEM((12, D, HC, E), BF16),
            pltpu.VMEM((HC, D // 2, E), U32),
            pltpu.VMEM((H - HC, D // 2, E), U32),
            pltpu.VMEM((2 * H, D // 2, E), U32),
            pltpu.VMEM((4, H * E, 128), BF16),
            pltpu.VMEM((4, H * E // 2, 128), U32),
            pltpu.VMEM((D, F), BF16),
            pltpu.VMEM((D, F), BF16),
            pltpu.VMEM((F, D), BF16),
            pltpu.VMEM((H, S, E), F32),
            pltpu.VMEM((2 * H, R, E), F32),
            pltpu.VMEM((H, R, E), F32),
            pltpu.VMEM((R, D), F32),
            pltpu.VMEM((16, D), F32),
            pltpu.VMEM((L2, L2), F32),
            pltpu.VMEM((2, 8, 128), F32),
            pltpu.VMEM((8, 128), jnp.int32),
            pltpu.VMEM((M, D), BF16),
            pltpu.VMEM((D,), BF16),
            pltpu.VMEM((8, D), F32),
            pltpu.SemaphoreType.DMA((33,)),
        ],
        compiler_params=pltpu.CompilerParams(vmem_limit_bytes=110 * 1024 * 1024),
        name="rmt_mod",
    )(A_x.reshape(S, D), A_mem0.reshape(M, D), A_Wq, A_Wk, A_Wv, A_Wo.reshape(H * E, D),
      B_w_r, B_w_gate, B_w_up, B_w_down)
    return out.reshape(1, S, D)
```

```python
import jax
import jax.numpy as jnp
import jax.experimental.pallas as pl
import jax.experimental.pallas.tpu as pltpu

S = 2048
D = 512
H = 32
E = 128
M = 8
SEG = 32
F = 1792
NPAIR = H // 2
NU = S // (2 * SEG)
W = 2 * SEG
L2 = 2 * (M + SEG)
EPS = 1.0013580322265625e-05
SCALE = 0.08837890625
LOG2E = 1.4426950408889634
F32 = jnp.float32
BF16 = jnp.bfloat16
U32 = jnp.uint32


def _rb(x):
    return x.astype(BF16).astype(F32)


def _ln(x):
    mu = jnp.sum(x, axis=-1, keepdims=True) * (1.0 / D)
    xc0 = x - mu
    var = jnp.sum(xc0 * xc0, axis=-1, keepdims=True) * (1.0 / D)
    sd = _rb(jnp.sqrt(_rb(_rb(var) + EPS)))
    xc = _rb(x - _rb(mu))
    r0 = pl.reciprocal(sd, approx=True)
    return _rb(xc * (r0 * (2.0 - sd * r0)))


def _dot(a, b):
    return jnp.dot(a, b, preferred_element_type=F32)


def _w(ref_slab):
    return pltpu.bitcast(ref_slab, BF16)


P0 = S // 2
LR = 24
PLN = P0 + LR
XC = P0 // 4
XLN = P0 + SEG
UNR = 2
NJ = NU // (2 * UNR)
XA = P0 + 4 * UNR * SEG
FD = PLN + LR * 2 * NU - S
R = 4 * SEG
HC = H // 4
PRE_ST = 3
POST_ST = 5
KSPLIT = ((0, 0), (0, 1), (1, 0), (1, 1), (0, 2), (1, 2), (0, 3), (1, 3))
NB4 = 4
NLF = 2
FLAG = 2
O1, O2, NE = 3, 7, 8


def _tok(*vals):
    parts = []
    for v in vals:
        if v.shape[1] < 128:
            v = jnp.broadcast_to(v[:, :1], (v.shape[0], 128))
        for i in range(v.shape[0] // 8):
            for j in range(v.shape[1] // 128):
                parts.append(v[8 * i:8 * i + 8, 128 * j:128 * j + 128])
    while len(parts) > 1:
        parts = [jnp.maximum(parts[i], parts[i + 1]) if i + 1 < len(parts) else parts[i]
                 for i in range(0, len(parts), 2)]
    return parts[0]


def _rslices(row0, n):
    row0 %= R
    if row0 + n <= R:
        return [(row0, row0 + n, 0)]
    return [(row0, R, 0), (0, row0 + n - R, R - row0)]


def _kernel(x_hbm, mem0_hbm, wq_hbm, wk_hbm, wv_hbm, wo_hbm, wr_hbm, wg_hbm, wu_hbm, wd_hbm,
            out_hbm,
            xs, x1buf, hbbuf, hbuf, hpack, raw, wq0, wq1, wkv, wo_raw, wo, wg, wu, wd,
            qbig, kvring, oring, abuf, ybuf, maskv, best, zflag, mem0_ref, wr_ref, wrb,
            qm0, hfix, fixrow, sems):
    def wq(h):
        return wq0.at[h] if h < HC else wq1.at[h - HC]

    def x_copy(row0, n, sem):
        return pltpu.make_async_copy(x_hbm.at[pl.ds(row0, n)], xs.at[pl.ds(row0, n)], sems.at[sem])

    def w_copy(ph, src=None):
        if src is None:
            src = wq_hbm.at[:, pl.ds(0, HC), :]
        return pltpu.make_async_copy(src, raw.at[ph], sems.at[11 + ph])

    cp_x = [x_copy(c * XC, XC, 23 + c) for c in range(4)]
    cp_xa = x_copy(P0, XA - P0, 0)
    cp_q0 = [pltpu.make_async_copy(wq_hbm.at[pl.ds(c * 128, 128), pl.ds(0, HC), :],
                                   raw.at[0, pl.ds(c * 128, 128)], sems.at[29 + c])
             for c in range(4)]
    cp_x[0].start()
    for c in cp_q0 + cp_x[1:]:
        c.start()
    cp_xa.start()
    cp_s = [pltpu.make_async_copy(mem0_hbm, mem0_ref, sems.at[27]),
            pltpu.make_async_copy(wr_hbm, wr_ref, sems.at[28])]
    for c in cp_s:
        c.start()
    for i, w in enumerate((wq_hbm, wk_hbm, wv_hbm)):
        for c in range(4):
            if 4 * i + c > 0:
                w_copy(4 * i + c, w.at[:, pl.ds(c * HC, HC), :]).start()
    cp_wo = [pltpu.make_async_copy(wo_hbm.at[:, pl.ds(n * 128, 128)], wo_raw.at[n], sems.at[4 + n])
             for n in range(4)]
    for c in cp_wo:
        c.start()
    cp_xb = x_copy(XA, S - XA, 1)
    cp_f = [pltpu.make_async_copy(wg_hbm, wg, sems.at[8]),
            pltpu.make_async_copy(wu_hbm, wu, sems.at[9]),
            pltpu.make_async_copy(wd_hbm, wd, sems.at[10])]

    def out_copy(row0, n, sem=2):
        return pltpu.make_async_copy(xs.at[pl.ds(row0, n)], out_hbm.at[pl.ds(row0, n)], sems.at[sem])

    oring[:, R - M:R, :] = jnp.zeros((H, M, E), F32)
    abuf[...] = jnp.zeros(abuf.shape, F32)
    xs[pl.ds(S, SEG), :] = jnp.zeros((SEG, D), BF16)
    hbuf[pl.ds(2 * S, SEG), :] = jnp.zeros((SEG, D), F32)
    zflag[...] = jnp.zeros(zflag.shape, jnp.int32)
    qm0[...] = jnp.zeros(qm0.shape, F32)
    hfix[...] = jnp.zeros(hfix.shape, F32)
    fixrow[0] = S

    ri = jax.lax.broadcasted_iota(jnp.int32, (L2, L2), 0)
    ci = jax.lax.broadcasted_iota(jnp.int32, (L2, L2), 1)

    def head_of(i):
        return jnp.where(i < 2 * M, i // M, (i - 2 * M) // SEG)

    def pos_of(i):
        return jnp.where(i < 2 * M, i % M, M + (i - 2 * M) % SEG)

    same = head_of(ri) == head_of(ci)
    ok = (pos_of(ri) < M) | (pos_of(ri) >= pos_of(ci))
    maskv[...] = jnp.where(same, jnp.where(ok, 0.0, -1e9 / SCALE), -jnp.inf).astype(F32)

    def gate(v, tk):
        y, r = tk
        ns = min(v.shape[-2], 8)
        tok = pltpu.bitcast(y[r:r + 8], v.dtype)[:ns]
        zf = (zflag[...] != 0)[:ns]
        reps = (v.shape[-2] // ns, v.shape[-1] // 128)
        tok, zf = jnp.tile(tok, reps), jnp.tile(zf, reps)
        return jnp.where(zf, tok, v)

    def toks(ys, n, frac=0.8):
        rows = [(y, r) for y in ys for r in range(0, y.shape[0], 8)]
        return [rows[int(len(rows) * frac * i / n)] for i in range(n)]

    def ln0(r0, tk=None, n=W):
        x = xs[r0:r0 + n, :].astype(F32)
        if tk is not None:
            x = gate(x, tk)
        h = _ln(x)
        hbuf[r0:r0 + n, :] = h
        if r0 < P0:
            hpack[r0 // 2:(r0 + n) // 2, :] = pltpu.bitcast(h.astype(BF16), U32)

    def relay(ph, tks=None, dbs=range(D // 16), is_q=False):
        for db in dbs:
            a = raw[ph, pl.ds(16 * db, 16)]
            if tks is not None:
                a = pltpu.bitcast(gate(pltpu.bitcast(a, U32), tks[db]), BF16)
            a = jnp.swapaxes(a, 0, 1)
            for hh in range(HC):
                v = pltpu.bitcast(a[hh], U32)
                if isinstance(ph, int) and ph == 0:
                    wq0[hh, pl.ds(8 * db, 8), :] = v
                elif is_q:
                    wq1[(ph - 1) * HC + hh, pl.ds(8 * db, 8), :] = v
                else:
                    tb = (ph % 4) * 16 + (ph // 4 - 1) * 2
                    wkv[tb + (hh // 2) * 4 + hh % 2, pl.ds(8 * db, 8), :] = v

    def light(heads, c=None):
        if c is None:
            r0, p0, n = 0, 0, P0
        elif isinstance(c, int):
            r0, p0, n = c * XC, c * (XC // 2), XC
        else:
            r0, p0, n = pl.multiple_of(c * XC, XC), pl.multiple_of(c * (XC // 2), XC // 2), XC
        lhs = _w(hpack[pl.ds(p0, n // 2), :])
        ys = []
        for h in heads:
            y = _dot(lhs, _w(wq(h)[...]))
            qbig[h, pl.ds(r0, n), :] = y
            ys.append(y)
        return ys

    NG = XC // SEG
    cp_x[0].wait()
    for k in range(NG):
        ln0(k * SEG, None, SEG)
    cp_q0[0].wait()
    relay(0, None, range(8))

    def first_k(k):
        lhs = _w(hpack[0:XC // 2, 128 * k:128 * (k + 1)])
        ys = []
        for h0 in range(0, HC, 4):
            wk = jnp.concatenate([_w(wq0[h0 + i, 64 * k:64 * (k + 1), :]) for i in range(4)], axis=1)
            y = _dot(lhs, wk)
            for i in range(4):
                yi = y[:, 128 * i:128 * (i + 1)]
                qbig[h0 + i, 0:XC, :] = yi if k == 0 else qbig[h0 + i, 0:XC, :] + yi
            ys.append(y[:, :128])
        return ys

    for k in range(3):
        cp_q0[k + 1].wait()
        tks = toks(first_k(k), 8, 0.6)
        relay(0, {8 * (k + 1) + i: tks[i] for i in range(8)}, range(8 * (k + 1), 8 * (k + 2)))
    cp_x[1].wait()
    tks = toks(first_k(3), NG, 0.5)
    for k in range(NG):
        ln0(XC + k * SEG, tks[k], SEG)

    cp_x[2].wait()
    cp_x[3].wait()
    tks = toks(light(range(HC), 1), 2 * NG, 0.85)
    for k in range(2 * NG):
        ln0(2 * XC + k * SEG, tks[k], SEG)

    def phase_a(i, carry):
        w_copy(i).wait()
        relay(i, toks(light(range(HC), i + 1), 32), is_q=True)
        return carry

    jax.lax.fori_loop(1, 3, phase_a, 0)
    w_copy(3).wait()
    cp_xa.wait()
    tks = toks(light(range(HC, HC + NB4)), 33)
    relay(3, tks[:32], is_q=True)
    ln0(P0, tks[32], SEG)

    def phase_b(i, carry):
        w_copy(4 + 2 * i).wait()
        w_copy(5 + 2 * i).wait()
        tks = toks(light(range(HC + NB4, H - NLF), i), 64, 0.9)
        relay(4 + 2 * i, tks[:32])
        relay(5 + 2 * i, tks[32:])
        return carry

    jax.lax.fori_loop(0, 4, phase_b, 0)

    for c in cp_wo[:3] + cp_s:
        c.wait()
    wrb[...] = jnp.broadcast_to(wr_ref[...].astype(F32).reshape(1, D), (8, D))
    cp_xb.start()
    for c in cp_f:
        c.start()
    ys = []
    nch = 8 * NLF
    for k in range(nch):
        h, r0 = H - NLF + k // 8, (k % 8) * (P0 // 8)
        y = _dot(_w(hpack[r0 // 2:r0 // 2 + P0 // 16, :]), _w(wq(h)[...]))
        qbig[h, r0:r0 + P0 // 8, :] = y
        ys.append(y)
        for t in range(2 * NPAIR + 2 * NPAIR * k // nch, 2 * NPAIR + 2 * NPAIR * (k + 1) // nch):
            kvring[t, 0:M, :] = _dot(_w(hpack[0:8, :]), _w(wkv[t]))[:M]
    tks = toks(ys, 24, 0.85)
    for k in range(24):
        n, kk = k // 8, k % 8
        wo[n, pl.ds(256 * kk, 256), :] = gate(
            pltpu.bitcast(wo_raw[n, pl.ds(512 * kk, 512), :], U32), tks[k])
    cp_wo[3].wait()
    wo[3] = pltpu.bitcast(wo_raw[3], U32)

    def post(row0, a, valid):
        n = a.shape[0]
        x1 = _rb(xs[pl.ds(row0, n), :].astype(F32) + _rb(a))
        x1buf[pl.ds(row0, n), :] = x1.astype(BF16)
        hb = _ln(x1)
        hbbuf[pl.ds(row0, n), :] = hb.astype(BF16)
        r = _rb(jnp.sum(hb * jnp.tile(wrb[...], (n // 8, 1)), axis=-1, keepdims=True))
        x2 = x1 + hb
        xs[pl.ds(row0, n), :] = x2.astype(BF16)
        if valid is not True:
            r = jnp.where(valid, r, -jnp.inf)
        bv = best[0]
        bi = best[1]
        sub = jax.lax.broadcasted_iota(jnp.int32, (8, 128), 0).astype(F32)
        for g in range(n // 8):
            rg = jnp.broadcast_to(r[8 * g:8 * g + 8], (8, 128))
            ig = sub + (float(row0 + 8 * g) if isinstance(row0, int) else (row0 + 8 * g).astype(F32))
            gt = rg > bv
            bv = jnp.where(gt, rg, bv)
            bi = jnp.where(gt, ig, bi)
        best[0] = bv
        best[1] = bi
        return _tok(x2, bv, bi)

    def anchor(val, tok):
        return jnp.where(zflag[...] != 0, tok, val)

    def wo_pair(g, half):
        return jnp.concatenate(
            [_w(wo[2 * half + c, pl.ds(g * 128, 128), :]) for c in range(2)], axis=1)

    def rload(buf, t, row0, n):
        return [buf[t, a:b, :] for a, b, _ in _rslices(row0, n)]

    def step(ts, jpos, first, last, layer, j, mem, korder):
        q, par = ts // 2, ts % 2
        sr = ts * SEG
        if par == 0:
            kvw = ((W * q, 40), (W * q + 8, 24))
            ow = ((W * q - 8, 40), (W * q, 24))
        else:
            kvw = ((W * q + 40, 24), (W * q + 32, 40))
            ow = ((W * q + 32, 24), (W * q + 24, 40))
        sl = 4 * j + ts
        sg = layer * (2 * NU) + sl
        hb0 = pl.multiple_of(layer * S + R * j, R)
        pq0 = pl.multiple_of(P0 + LR * sg, 8)
        lhs = [jnp.concatenate([mem, hbuf[pl.ds(hb0 + r0, n), :]], axis=0).astype(BF16)
               for r0, n in kvw]
        memq = mem
        if first is not None:
            first1, first2 = first & (layer == 0), first & (layer == 1)
            memq = jnp.where(first2, hfix[...], mem)
            frow = pl.multiple_of(jnp.where(first2, fixrow[0], S), 8)
        lhsq = jnp.concatenate([memq, hbuf[pl.ds(pq0, LR), :]], axis=0).astype(BF16)
        qrow = [pl.multiple_of((pq0 + 8 * i) % S, 8) for i in range(LR // 8)]
        crow = pl.multiple_of(R * j + sr, SEG)

        def ksplit(ga, gb):
            half = ga // (NPAIR // 2)
            hq = [2 * ga, 2 * ga + 1, 2 * gb, 2 * gb + 1]

            def kv(k):
                wk = jnp.concatenate([_w(wkv[4 * ga + t, pl.ds(64 * k, 64), :])
                                      for t in range(4)], axis=1)
                return jnp.dot(lhs[half][:, 128 * k:128 * (k + 1)], wk, preferred_element_type=F32)

            def qq(k):
                wk = jnp.concatenate([_w(wq(h)[pl.ds(64 * k, 64), :]) for h in hq], axis=1)
                return jnp.dot(lhsq[:, 128 * k:128 * (k + 1)], wk, preferred_element_type=F32)

            pkv = pq = None
            for f, k in KSPLIT:
                y = (kv if f == 0 else qq)(korder[k])
                if f == 0:
                    pkv = y if pkv is None else pkv + y
                else:
                    pq = y if pq is None else pq + y
            done = {("kv", 4 * ga + t): pkv[:, 128 * t:128 * (t + 1)] for t in range(4)}
            if pq is not None:
                done.update({("q", h): pq[:, 128 * i:128 * (i + 1)] for i, h in enumerate(hq)})
            return done

        def qkv(g, done):
            half = g // (NPAIR // 2)
            r0, n = kvw[half]
            res = []
            for c in range(2):
                y = done.get(("q", 2 * g + c))
                if y is None:
                    y = jnp.dot(lhsq, _w(wq(2 * g + c)[...]), preferred_element_type=F32)
                for i in range(LR // 8):
                    qbig[2 * g + c, pl.ds(qrow[i], 8), :] = y[M + 8 * i:M + 8 * i + 8]
                ym = y[:M]
                if first is not None:
                    qbig[2 * g + c, pl.ds(frow, M), :] = ym
                    old = qm0[2 * g + c]
                    qm0[2 * g + c] = jnp.where(first1, ym, old)
                    ym = jnp.where(first2, old, ym)
                res.append(ym)
            for t in range(4):
                y = done.get(("kv", 4 * g + t))
                if y is None:
                    y = jnp.dot(lhs[half], _w(wkv[4 * g + t]), preferred_element_type=F32)
                for a, b, o in _rslices(r0, n):
                    kvring[4 * g + t, a:b, :] = y[M + o:M + o + b - a]
                res.append(y[:M])
            qx = jnp.concatenate([qbig[2 * g + c, pl.ds(crow, SEG), :] for c in range(2)],
                                 axis=0).astype(BF16)
            return res, qx

        def stack(g, mres, i):
            return jnp.concatenate(
                [mres[2 * i], mres[2 * i + 1],
                 kvring[4 * g + 2 * i - 2, sr:sr + SEG, :],
                 kvring[4 * g + 2 * i - 1, sr:sr + SEG, :]], axis=0).astype(BF16)

        def qk(g, mres, qx, prenorm):
            q2 = jnp.concatenate(
                [jnp.concatenate([mres[0], mres[1]], axis=0).astype(BF16), qx], axis=0)
            s = jax.lax.dot_general(q2, stack(g, mres, 1), (((1,), (1,)), ((), ())),
                                    preferred_element_type=F32)
            mk = maskv[...]
            s = jnp.where(mk == 0.0, s, mk)
            mx = jnp.max(s, axis=-1, keepdims=True)
            p = jnp.exp2((s - mx) * (SCALE * LOG2E))
            l = jnp.sum(p, axis=-1, keepdims=True)
            r0 = pl.reciprocal(l, approx=True)
            r = r0 * (2.0 - l * r0)
            if prenorm:
                return (p * r).astype(BF16), None
            return p.astype(BF16), r

        def pv(g, mres, pr):
            p, r = pr
            o = jnp.dot(p, stack(g, mres, 2), preferred_element_type=F32)
            if r is not None:
                o = o * r
            oring[2 * g, sr:sr + SEG, :] = o[2 * M:2 * M + SEG]
            oring[2 * g + 1, sr:sr + SEG, :] = o[2 * M + SEG:]
            return o[:M], o[M:2 * M]

        def olhs(g, om, half):
            r0, n = ow[half]
            if last is not None and half == 0:
                om = [jnp.where(last, oring[2 * g + c, R - M:R, :], om[c]) for c in range(2)]
            return jnp.concatenate(
                [jnp.concatenate([om[c]] + rload(oring, 2 * g + c, r0, n), axis=0)
                 for c in range(2)], axis=1).astype(BF16)

        pn0 = pl.multiple_of(PLN + LR * sg, 8)
        xr = jnp.concatenate(
            [xs[pl.ds(pl.multiple_of((pn0 + 8 * i) % S, 8), 8), :].astype(F32)
             for i in range(LR // 8)], axis=0)
        hpre = _ln(xr)
        hbuf[pl.ds(pn0, LR), :] = hpre
        tok_pre = _tok(hpre)
        if ts >= 2 or jpos:
            valid = True
            row0 = pl.multiple_of(SEG * (sl - 2), SEG)
        else:
            valid = j >= 1
            row0 = pl.multiple_of(jnp.where(valid, SEG * (sl - 2), S), SEG)
        ar = (sr - 2 * SEG) % R
        tok_post = post(row0, abuf[ar:ar + SEG, :], valid)

        NST = NPAIR // 2
        st = [(i, i + NST) if par == 0 else (i + NST, i) for i in range(NST)]
        mres, qxs, prs, oms = {}, {}, {}, {}
        acc = [None] * 4
        order = []
        for i in range(NST):
            order += [("qkv", g) for g in st[i]]
            if i >= 1:
                order += [("qk", g) for g in st[i - 1]]
            if i >= 2:
                order += [("pv", g) for g in st[i - 2]]
        oq = [g for i in range(NST) for g in st[i]]
        order += [("o", g) for g in oq[0:O1]]
        order += [("qk", g) for g in st[NST - 1]] + [("pv", g) for g in st[NST - 2]]
        order += [("o", g) for g in oq[O1:O2]]
        order += [("pv", g) for g in st[NST - 1]]
        order += [("o", g) for g in oq[O2:NE]]
        norder = (2, 3, 0, 1) if par == 0 else (0, 1, 2, 3)
        order += [("on", n) for n in norder]
        done = {} if korder is None else ksplit(*st[0])
        for kind, g in order:
            if kind == "qkv":
                mres[g], qxs[g] = qkv(g, done)
                if g == st[PRE_ST][0]:
                    mres[g][0] = anchor(mres[g][0], tok_pre)
                if g == st[POST_ST][0]:
                    mres[g][0] = anchor(mres[g][0], tok_post)
            elif kind == "qk":
                prs[g] = qk(g, mres[g], qxs[g], g not in st[NST - 1] + st[NST - 2])
            elif kind == "pv":
                oms[g] = pv(g, mres[g], prs[g])
                if prs[g][1] is not None:
                    oms[g] = (anchor(oms[g][0], _tok(prs[g][1][2 * M:])), oms[g][1])
            elif kind == "o":
                for half in range(2):
                    y = jnp.dot(olhs(g, oms[g], half), wo_pair(g, half), preferred_element_type=F32)
                    for c in range(2):
                        yc = y[:, 128 * c:128 * (c + 1)]
                        n = 2 * half + c
                        acc[n] = yc if acc[n] is None else acc[n] + yc
            else:
                n = g
                l = jnp.concatenate([olhs(g2, oms[g2], n // 2) for g2 in oq[NE:]], axis=1)
                wn = jnp.concatenate([_w(wo[n, pl.ds(g2 * 128, 128), :]) for g2 in oq[NE:]], axis=0)
                acc[n] = acc[n] + jnp.dot(l, wn, preferred_element_type=F32)
        for n in range(4):
            r0, nr = ow[n // 2]
            for a, b, o in _rslices(r0, nr):
                abuf[a:b, n * 128:(n + 1) * 128] = acc[n][M + o:M + o + b - a]

        if last is not None:
            for n in range(2):
                abuf[R - M:R, n * 128:(n + 1) * 128] = acc[n][:M]

        return jnp.concatenate([acc[n][:M] for n in range(4)], axis=1), norder

    def argmax():
        bv = best[0]
        bi = best[1]
        vmax = jnp.max(bv, axis=0, keepdims=True)
        imin = jnp.min(jnp.where(bv == vmax, bi, float(S)), axis=0, keepdims=True)
        idx = jnp.clip(imin.astype(jnp.int32)[0, 0], 0, S - 1)
        return idx, vmax

    def ffn(idx):
        g0 = pl.multiple_of((idx // 16) * 16, 16)
        hbb = hbbuf[pl.ds(g0, 16), :]
        nc = F // 256
        hid, acc, gs_ = [], None, []
        for c in range(nc + FLAG):
            if c < nc:
                gpre = _rb(_dot(hbb, wg[:, 256 * c:256 * (c + 1)]))
                gs_.append(gpre[:, :128])
                gs = _rb(gpre * _rb(jax.nn.sigmoid(gpre)))
                up = _rb(_dot(hbb, wu[:, 256 * c:256 * (c + 1)]))
                hid.append((gs * up).astype(BF16))
            if c >= FLAG:
                y = _dot(hid[c - FLAG], wd[256 * (c - FLAG):256 * (c - FLAG + 1), :])
                acc = y if acc is None else acc + y
        ybuf[...] = _rb(acc)
        return gs_

    def ffn_small(idx):
        g0 = pl.multiple_of((idx // 16) * 16, 16)
        hbb = hbbuf[pl.ds(g0, 16), :]

        def body(c, acc):
            f0 = pl.multiple_of(c * 256, 256)
            gpre = _rb(_dot(hbb, wg[:, pl.ds(f0, 256)]))
            gs = _rb(gpre * _rb(jax.nn.sigmoid(gpre)))
            up = _rb(_dot(hbb, wu[:, pl.ds(f0, 256)]))
            return acc + _dot((gs * up).astype(BF16), wd[pl.ds(f0, 256), :])

        ybuf[...] = _rb(jax.lax.fori_loop(0, F // 256, body, jnp.zeros((16, D), F32)))

    def layer_body(layer, carry):
        best[0] = jnp.full((8, 128), -jnp.inf, F32)
        best[1] = jnp.zeros((8, 128), F32)

        def qstep(jj, mem):
            @pl.when((layer == 0) & (jj == 1))
            def _():
                cp_xb.wait()

            @pl.when((layer == 1) & (jj >= 2))
            def _():
                out_copy(pl.multiple_of((jj - 1) * (UNR * R) - W, W), UNR * R).start()

            @pl.when((layer == 1) & (jj == 1))
            def _():
                out_copy(0, UNR * R - W).start()

            ko = None
            for j2 in range(UNR):
                for ts in range(4):
                    last = (jj == NJ - 1) if (j2 == UNR - 1 and ts == 3) else None
                    first = (jj == 0) if (j2 == 0 and ts == 0) else None
                    mem, ko = step(ts, j2 > 0, first, last, layer, UNR * jj + j2, mem, ko)
            return mem

        jax.lax.fori_loop(0, NJ, qstep, mem0_ref[...].astype(F32))

        @pl.when(layer == 0)
        def _():
            for c in cp_f:
                c.wait()

        @pl.when(layer == 1)
        def _():
            out_copy(S - UNR * R - W, UNR * R).start()

        idx_s, _ = argmax()
        gs_ = ffn(idx_s)
        for k in range(4):
            post(S - W + 16 * k, gate(abuf[W + 16 * k:W + 16 * (k + 1), :], (gs_[k], 0)), True)
        idx, vmax = argmax()

        @pl.when(idx // 16 != idx_s // 16)
        def _():
            ffn_small(idx)

        g0 = pl.multiple_of((idx // 16) * 16, 16)
        rsel = jnp.tile(_rb(jax.nn.sigmoid(vmax)), (1, D // 128))
        y = _rb(ybuf[...] * rsel)
        x2 = _rb(x1buf[pl.ds(g0, 16), :].astype(F32) + _rb(hbbuf[pl.ds(g0, 16), :].astype(F32) + y))
        rowi = jax.lax.broadcasted_iota(jnp.int32, (16, D), 0) + g0

        @pl.when(layer == 1)
        def _():
            out_copy(0, S - W).wait()

        x2 = jnp.where(rowi == idx, x2, xs[pl.ds(g0, 16), :].astype(F32))
        xs[pl.ds(g0, 16), :] = x2.astype(BF16)

        @pl.when((layer == 0) & (idx < FD))
        def _():
            h16 = _ln(x2)
            hbuf[pl.ds(S + g0, 16), :] = h16
            hi8 = idx % 16 >= 8
            hfix[...] = jnp.where(hi8, h16[8:], h16[:8])
            fixrow[0] = (idx // 8) * 8

            @pl.when(idx < M)
            def _():
                def body(t, c):
                    kvring[t, 0:M, :] = _dot(h16.astype(BF16), _w(wkv[t]))[:M]
                    return c

                jax.lax.fori_loop(2 * NPAIR, 4 * NPAIR, body, 0, unroll=2)

        @pl.when(layer == 1)
        def _():
            lastc = out_copy(S - W, W)
            lastc.start()

            @pl.when(g0 < S - W)
            def _():
                fix = out_copy(g0, 16, 3)
                fix.start()
                fix.wait()

            lastc.wait()

        return carry

    jax.lax.fori_loop(0, 2, layer_body, 0)


@jax.jit
def pallas_interleave_layers__memory_aug_recurrent_mem_tr__moe_arch_mod__prompt_kernel(
    A_x: jax.Array,
    A_mem0: jax.Array,
    A_Wq: jax.Array,
    A_Wk: jax.Array,
    A_Wv: jax.Array,
    A_Wo: jax.Array,
    A_seg_len: jax.Array,
    B_x: jax.Array,
    B_w_r: jax.Array,
    B_w_gate: jax.Array,
    B_w_up: jax.Array,
    B_w_down: jax.Array,
):
    del A_seg_len, B_x
    assert A_x.shape == (1, S, D) and A_Wq.shape == (D, H, E) and A_mem0.shape == (1, M, D)
    any_spec = pl.BlockSpec(memory_space=pl.ANY)
    out = pl.pallas_call(
        _kernel,
        out_shape=jax.ShapeDtypeStruct((S, D), BF16),
        in_specs=[any_spec] * 10,
        out_specs=any_spec,
        scratch_shapes=[
            pltpu.VMEM((S + SEG, D), BF16),
            pltpu.VMEM((S + SEG, D), BF16),
            pltpu.VMEM((S + SEG, D), BF16),
            pltpu.VMEM((2 * S + SEG, D), F32),
            pltpu.VMEM((P0 // 2, D), U32),
            pltpu.VMEM((12, D, HC, E), BF16),
            pltpu.VMEM((HC, D // 2, E), U32),
            pltpu.VMEM((H - HC, D // 2, E), U32),
            pltpu.VMEM((2 * H, D // 2, E), U32),
            pltpu.VMEM((4, H * E, 128), BF16),
            pltpu.VMEM((4, H * E // 2, 128), U32),
            pltpu.VMEM((D, F), BF16),
            pltpu.VMEM((D, F), BF16),
            pltpu.VMEM((F, D), BF16),
            pltpu.VMEM((H, S + M, E), F32),
            pltpu.VMEM((2 * H, R, E), F32),
            pltpu.VMEM((H, R, E), F32),
            pltpu.VMEM((R, D), F32),
            pltpu.VMEM((16, D), F32),
            pltpu.VMEM((L2, L2), F32),
            pltpu.VMEM((2, 8, 128), F32),
            pltpu.VMEM((8, 128), jnp.int32),
            pltpu.VMEM((M, D), BF16),
            pltpu.VMEM((D,), BF16),
            pltpu.VMEM((8, D), F32),
            pltpu.VMEM((H, M, E), F32),
            pltpu.VMEM((M, D), F32),
            pltpu.SMEM((1,), jnp.int32),
            pltpu.SemaphoreType.DMA((33,)),
        ],
        compiler_params=pltpu.CompilerParams(vmem_limit_bytes=110 * 1024 * 1024,
                                             disable_bounds_checks=True,
                                             disable_semaphore_checks=True),
        name="rmt_mod",
    )(A_x.reshape(S, D), A_mem0.reshape(M, D), A_Wq, A_Wk, A_Wv, A_Wo.reshape(H * E, D),
      B_w_r, B_w_gate, B_w_up, B_w_down)
    return out.reshape(1, S, D)
```
